```python
import jax
import jax.numpy as jnp

def _softmax(x, axis=-1):
    return jax.nn.softmax(x, axis=axis)

def _gelu(x):
    return jax.nn.gelu(x, approximate=True)

def _silu(x):
    return jax.nn.silu(x)

def _sigmoid(x):
    return jax.nn.sigmoid(x)

def _layernorm(x, axis=-1, eps=1e-05):
    m = jnp.mean(x, axis=axis, keepdims=True)
    v = jnp.var(x, axis=axis, keepdims=True)
    return (x - m) / jnp.sqrt(v + eps)

def _scatter_add(tgt, idx, src, axis=0):
    return tgt.at[idx].add(src)

def _segment_sum(src, seg, n):
    return jax.ops.segment_sum(src, seg, n)

class _Rng:

    def __init__(self, key):
        self._k = key

    def _next(self):
        self._k, sub = jax.random.split(self._k)
        return sub

    def normal(self, shape):
        return jax.random.normal(self._next(), shape, dtype=jnp.bfloat16)

    def randint(self, lo, hi, shape):
        return jax.random.randint(self._next(), shape, lo, hi, dtype=jnp.int32)

    def uniform(self, shape, lo=0.0, hi=1.0):
        return jax.random.uniform(self._next(), shape, jnp.bfloat16, lo, hi)

    def permutation(self, n):
        return jax.random.permutation(self._next(), n)
kernel_name = 'adaLN_cond__sliding_local_dilated__glu_gated_swiglu__prompt'

def setup_inputs():
    _rng = _Rng(jax.random.key(int.from_bytes(__import__("os").urandom(4), "little")))
    _w = lambda a: (lambda t: t.astype(jnp.bfloat16) if jnp.issubdtype(t.dtype, jnp.floating) else t)(jnp.asarray(a))

    def _A_setup():
        B, S, D = (1, 2048, 1024)
        return {'x': _w((lambda *s: _rng.normal(s) * 0.05)(B, S, D)), 'wqkv': _w((lambda *s: _rng.normal(s) * 0.05)(D, 3 * D)), 'wo': _w((lambda *s: _rng.normal(s) * 0.05)(D, D))}
    _A_in = _A_setup()

    def _B_setup():
        B, S, D, F = (1, 2048, 1024, 3584)
        return {'x': _w((lambda *s: _rng.normal(s) * 0.05)(B, S, D)), 'w1': _w((lambda *s: _rng.normal(s) * 0.05)(D, F) * (2.0 / D) ** 0.5), 'w3': _w((lambda *s: _rng.normal(s) * 0.05)(D, F) * (2.0 / D) ** 0.5), 'w2': _w((lambda *s: _rng.normal(s) * 0.05)(F, D) * (2.0 / F) ** 0.5)}
    _B_in = _B_setup()
    return {'A_x': _A_in['x'], 'A_wqkv': _A_in['wqkv'], 'A_wo': _A_in['wo'], 'B_x': _B_in['x'], 'B_w1': _B_in['w1'], 'B_w3': _B_in['w3'], 'B_w2': _B_in['w2'], 'c': _w((lambda *s: _rng.normal(s) * 0.05)(1, 1024)), 'w_mod': _w((lambda *s: _rng.normal(s) * 0.05)(1024, 6 * 1024) * 1024 ** (-0.5))}

def reference(A_x, A_wqkv, A_wo, B_x, B_w1, B_w3, B_w2, c, w_mod):

    def _A_ref(x, wqkv, wo):
        B, S, D = x.shape
        H = 32
        Dh = D // H
        W, dil = (8, 2)
        qkv = (lambda x, *d: x.transpose(*d))((x @ wqkv).reshape(B, S, 3, H, Dh), 2, 0, 3, 1, 4)
        q, k, v = (qkv[0], qkv[1], qkv[2])
        scale = Dh ** (-0.5)
        pos = jnp.arange(S)
        off = jnp.arange(W) * dil
        idx = pos[:, None] - off[None, :]
        mask = idx >= 0
        idx_c = jnp.where(mask, idx, 0).reshape(-1)
        kg = k[:, :, idx_c, :].reshape(B, H, S, W, Dh)
        vg = v[:, :, idx_c, :].reshape(B, H, S, W, Dh)
        logits = jnp.einsum('bhsd,bhswd->bhsw', q, kg) * scale
        logits = jnp.where(mask[None, None, :, :], logits, -1000000000.0)
        attn = _softmax(logits, axis=-1)
        o = jnp.einsum('bhsw,bhswd->bhsd', attn, vg)
        return (lambda x, *d: x.transpose(*d))(o, 0, 2, 1, 3).reshape(B, S, D) @ wo

    def _B_ref(x, w1, w3, w2):
        gate = jnp.einsum('bsd,df->bsf', x, w1)
        up = jnp.einsum('bsd,df->bsf', x, w3)
        h = _silu(gate) * up
        out = jnp.einsum('bsf,fd->bsd', h, w2)
        return out
    x = A_x
    mod = (_silu(c) @ w_mod).reshape(c.shape[0], 6, 1, -1)
    sa, ca, ga, sb, cb, gb = (mod[:, 0].copy(), mod[:, 1].copy(), mod[:, 2].copy(), mod[:, 3].copy(), mod[:, 4].copy(), mod[:, 5].copy())
    h = _layernorm(x, axis=-1) * (1 + ca) + sa
    x = x + ga * _A_ref(h, A_wqkv, A_wo)
    h = _layernorm(x, axis=-1) * (1 + cb) + sb
    x = x + gb * _B_ref(h, B_w1, B_w3, B_w2)
    return x
```

```python
import functools
import math

import jax
import jax.numpy as jnp
import jax.experimental.pallas as pl
import jax.experimental.pallas.tpu as pltpu

S = 2048
D = 1024
F = 3584
H = 32
DH = D // H
WIN = 8
DIL = 2
NC = D // 128
HALO = 16
EPS = 1e-5
NEG = -1000000000.0
SM_SCALE = DH ** -0.5
LOG2E = math.log2(math.e)

F32 = jnp.float32
BF16 = jnp.bfloat16
U32 = jnp.uint32


def _build(TM=256, RG=8, LG=16, FC=512, QN=1024):
    NB = S // TM

    def kernel(x_hbm, wqkv_hbm, wo_hbm, w1_hbm, w3_hbm, w2_hbm, c_ref, wmod_hbm,
               out_hbm,
               x_v, wqkv_v, wo_raw, wo_tmp, wo_p, w1_v, w3_v, w2_v, wmod_v, mod_v,
               h1a, h1b, qa, ka, va, qb, kb, vb, oa, ob, x1_v, h2_v, act_v, obuf,
               sem_x, sem_w, sem_o):
        bufs = {
            "a": (h1a, qa, ka, va, oa),
            "b": (h1b, qb, kb, vb, ob),
        }

        def cp_x(i):
            return pltpu.make_async_copy(x_hbm.at[0, pl.ds(i * TM, TM), :],
                                         x_v.at[pl.ds(i * TM, TM), :], sem_x.at[i])

        def cp_mod(j):
            return pltpu.make_async_copy(wmod_hbm.at[:, pl.ds(j * D, D)],
                                         wmod_v.at[:, pl.ds(j * D, D)], sem_w.at[j])

        def cp_qkv(g):
            return pltpu.make_async_copy(wqkv_hbm.at[:, pl.ds(g * D, D)],
                                         wqkv_v.at[:, pl.ds(g * D, D)], sem_w.at[6 + g])

        def cp_wo():
            return pltpu.make_async_copy(wo_hbm, wo_raw, sem_w.at[9])

        def cp_w1():
            return pltpu.make_async_copy(w1_hbm, w1_v, sem_w.at[10])

        def cp_w3():
            return pltpu.make_async_copy(w3_hbm, w3_v, sem_w.at[11])

        def cp_w2():
            return pltpu.make_async_copy(w2_hbm, w2_v, sem_w.at[12])

        def cp_out(j, slot):
            return pltpu.make_async_copy(obuf.at[slot],
                                         out_hbm.at[0, pl.ds(j * TM, TM), :], sem_o.at[slot])

        lane = jax.lax.broadcasted_iota(jnp.int32, (8, 128), 1)

        def lane_bit_clear(bit, rows):
            l = jax.lax.broadcasted_iota(jnp.int32, (rows, 128), 1)
            return ((l >> bit) & 1) == 0

        def mod_row(j):
            return mod_v[j, 0:1, :]

        def compute_mod(j, add_one):
            cf = c_ref[...].astype(F32)
            sc = (cf * jax.nn.sigmoid(cf)).astype(BF16)
            lhs = jnp.broadcast_to(sc, (16, D))
            r = jnp.dot(lhs, wmod_v[:, j * D:(j + 1) * D], preferred_element_type=F32)
            r = r[0:8]
            if add_one:
                r = r + 1.0
            mod_v[j] = r

        def permute_qkv_rows(g, r0, nrows):
            vals = [pltpu.bitcast(wqkv_v[pl.ds(r0, nrows), g * D + c * 128: g * D + (c + 1) * 128], U32)
                    for c in range(NC)]
            for cb, lb in ((2, 3), (1, 2), (0, 1)):
                s = 1 << lb
                m = lane_bit_clear(lb, nrows // 2)
                for c in range(NC):
                    if c & (1 << cb):
                        continue
                    a, b = vals[c], vals[c | (1 << cb)]
                    vals[c] = jnp.where(m, a, pltpu.roll(b, s, 1))
                    vals[c | (1 << cb)] = jnp.where(m, pltpu.roll(a, 128 - s, 1), b)
            for c in range(NC):
                wqkv_v[pl.ds(r0, nrows), g * D + c * 128: g * D + (c + 1) * 128] = pltpu.bitcast(vals[c], BF16)

        def permute_qkv_group(g):
            def body(i, carry):
                permute_qkv_rows(g, pl.multiple_of(i * 64, 64), 64)
                return carry
            jax.lax.fori_loop(0, D // 64, body, 0)

        def permute_wo():
            for c in range(NC):
                for r in range(0, D, 128):
                    wo_tmp[c, r // 2:r // 2 + 64, :] = pltpu.bitcast(
                        wo_raw[r:r + 128, c * 128:(c + 1) * 128], U32)
            for c in range(NC):
                for G in range(64):
                    base = (G & 7) * 8 + (G >> 3)
                    t = wo_tmp[c, pl.ds(base, 8, stride=64), :]
                    wo_p[G * 16:(G + 1) * 16, c * 128:(c + 1) * 128] = pltpu.bitcast(t, BF16)

        def layernorm_mod(xf, scale_row, shift_row):
            mu = jnp.mean(xf, axis=-1, keepdims=True)
            d = xf - mu
            var = jnp.mean(d * d, axis=-1, keepdims=True)
            return d * jax.lax.rsqrt(var + EPS) * scale_row + shift_row

        def ln1(row0, buf):
            h1 = bufs[buf][0]
            sc, sh = mod_row(1), mod_row(0)
            for r in range(0, TM, LG):
                xf = x_v[pl.ds(row0 + r, LG), :].astype(F32)
                h1[r:r + LG, :] = layernorm_mod(xf, sc, sh).astype(BF16)

        def qkv(buf, prev, first):
            h1, q, k, v, _ = bufs[buf]
            dst = (q, k, v)
            if not first:
                _, _, kp, vp, _ = bufs[prev]
                for c in range(NC):
                    k[c, 0:HALO, :] = kp[c, TM:TM + HALO, :]
                    v[c, 0:HALO, :] = vp[c, TM:TM + HALO, :]
            lhs = h1[...]
            for n0 in range(0, 3 * D, QN):
                res = jnp.dot(lhs, wqkv_v[:, n0:n0 + QN], preferred_element_type=F32)
                for cc in range(QN // 128):
                    col = n0 + cc * 128
                    g, c = col // D, (col % D) // 128
                    off = 0 if g == 0 else HALO
                    dst[g][c, off:off + TM, :] = res[:, cc * 128:(cc + 1) * 128]
            if first:
                for c in range(NC):
                    k[c, 0:HALO, :] = jnp.zeros((HALO, 128), F32)
                    v[c, 0:HALO, :] = jnp.broadcast_to(v[c, HALO:HALO + 1, :], (HALO, 128))

        def attn(buf, first):
            _, q, k, v, o = bufs[buf]
            m0 = lane_bit_clear(0, RG)
            m4 = lane_bit_clear(4, RG)
            for r in range(0, TM, RG):
                qs = [q[c, r:r + RG, :] for c in range(NC)]
                ss = []
                for w in range(WIN):
                    st = HALO + r - DIL * w
                    s = qs[0] * k[0, st:st + RG, :]
                    for c in range(1, NC):
                        s = s + qs[c] * k[c, st:st + RG, :]
                    s = s + jnp.where(m0, pltpu.roll(s, 127, 1), pltpu.roll(s, 1, 1))
                    s = s + jnp.where(m4, pltpu.roll(s, 112, 1), pltpu.roll(s, 16, 1))
                    if first and r < DIL * w:
                        pos = r + jax.lax.broadcasted_iota(jnp.int32, (RG, 128), 0)
                        s = jnp.where(pos >= DIL * w, s, NEG / SM_SCALE)
                    ss.append(s)
                m = ss[0]
                for w in range(1, WIN):
                    m = jnp.maximum(m, ss[w])
                ps = [jnp.exp2((ss[w] - m) * (SM_SCALE * LOG2E)) for w in range(WIN)]
                den = ps[0]
                for w in range(1, WIN):
                    den = den + ps[w]
                inv = 1.0 / den
                ps = [p * inv for p in ps]
                for c in range(NC):
                    acc = ps[0] * v[c, HALO + r:HALO + r + RG, :]
                    for w in range(1, WIN):
                        st = HALO + r - DIL * w
                        acc = acc + ps[w] * v[c, st:st + RG, :]
                    o[c, r:r + RG, :] = acc

        def wo_ln2(buf, row0):
            o = bufs[buf][4]
            lhs = jnp.concatenate([o[c].astype(BF16) for c in range(NC)], axis=-1)
            y = jnp.dot(lhs, wo_p[...], preferred_element_type=F32)
            ga, sc, sh = mod_row(2), mod_row(4), mod_row(3)
            for r in range(0, TM, LG):
                x1 = x_v[pl.ds(row0 + r, LG), :].astype(F32) + ga * y[r:r + LG, :]
                x1_v[pl.ds(row0 + r, LG), :] = x1
                h2_v[pl.ds(row0 + r, LG), :] = layernorm_mod(x1, sc, sh).astype(BF16)

        def ffn(row0, slot):
            h = h2_v[pl.ds(row0, TM), :]
            for f0 in range(0, F, FC):
                g = jnp.dot(h, w1_v[:, f0:f0 + FC], preferred_element_type=F32)
                u = jnp.dot(h, w3_v[:, f0:f0 + FC], preferred_element_type=F32)
                act_v[:, f0:f0 + FC] = (g * jax.nn.sigmoid(g) * u).astype(BF16)
            y = jnp.dot(act_v[...], w2_v[...], preferred_element_type=F32)
            obuf[slot] = (x1_v[pl.ds(row0, TM), :] + mod_row(5) * y).astype(BF16)

        cp_x(0).start()
        cp_mod(1).start()
        cp_mod(0).start()
        cp_qkv(0).start()
        cp_qkv(1).start()
        cp_qkv(2).start()
        cp_x(1).start()
        cp_wo().start()
        cp_mod(2).start()
        cp_mod(4).start()
        cp_mod(3).start()
        for i in range(2, NB):
            cp_x(i).start()
        cp_mod(5).start()
        cp_w1().start()
        cp_w3().start()
        cp_w2().start()

        cp_mod(1).wait()
        compute_mod(1, True)
        cp_mod(0).wait()
        compute_mod(0, False)
        cp_x(0).wait()
        ln1(0, "a")
        for g in range(3):
            cp_qkv(g).wait()
            permute_qkv_group(g)
        cp_x(1).wait()
        cp_wo().wait()
        cp_mod(2).wait()
        cp_mod(4).wait()
        cp_mod(3).wait()
        cp_x(2).wait()

        qkv("a", None, True)
        permute_wo()
        compute_mod(2, False)
        compute_mod(4, True)
        compute_mod(3, False)
        ln1(TM, "b")
        qkv("b", "a", False)
        attn("a", True)
        wo_ln2("a", 0)
        ln1(2 * TM, "a")

        for i in range(3, NB):
            cp_x(i).wait()

        def a_step(s, carry):
            ra = pl.multiple_of(2 * s * TM, TM)
            qkv("a", "b", False)
            attn("b", False)
            wo_ln2("b", ra - TM)
            ln1(ra + TM, "b")
            qkv("b", "a", False)
            attn("a", False)
            wo_ln2("a", ra)
            nxt = pl.multiple_of(jnp.minimum(ra + 2 * TM, S - TM), TM)
            ln1(nxt, "a")
            return carry

        jax.lax.fori_loop(1, NB // 2, a_step, 0)

        cp_mod(5).wait()
        cp_w1().wait()
        cp_w3().wait()
        cp_w2().wait()

        compute_mod(5, False)
        attn("b", False)
        wo_ln2("b", S - TM)
        ffn(0, 0)
        cp_out(0, 0).start()

        def b_step(j, carry):
            slot = j % 2

            @pl.when(j >= 2)
            def _():
                cp_out(j - 2, slot).wait()

            ffn(pl.multiple_of(j * TM, TM), slot)
            cp_out(j, slot).start()
            return carry

        jax.lax.fori_loop(1, NB, b_step, 0)
        cp_out(NB - 2, (NB - 2) % 2).wait()
        cp_out(NB - 1, (NB - 1) % 2).wait()

    any_spec = pl.BlockSpec(memory_space=pl.ANY)
    kv_shape = (NC, HALO + TM, 128)
    scratch = [
        pltpu.VMEM((S, D), BF16),
        pltpu.VMEM((D, 3 * D), BF16),
        pltpu.VMEM((D, D), BF16),
        pltpu.VMEM((NC, D // 2, 128), U32),
        pltpu.VMEM((D, D), BF16),
        pltpu.VMEM((D, F), BF16),
        pltpu.VMEM((D, F), BF16),
        pltpu.VMEM((F, D), BF16),
        pltpu.VMEM((D, 6 * D), BF16),
        pltpu.VMEM((6, 8, D), F32),
        pltpu.VMEM((TM, D), BF16),
        pltpu.VMEM((TM, D), BF16),
        pltpu.VMEM((NC, TM, 128), F32),
        pltpu.VMEM(kv_shape, F32),
        pltpu.VMEM(kv_shape, F32),
        pltpu.VMEM((NC, TM, 128), F32),
        pltpu.VMEM(kv_shape, F32),
        pltpu.VMEM(kv_shape, F32),
        pltpu.VMEM((NC, TM, 128), F32),
        pltpu.VMEM((NC, TM, 128), F32),
        pltpu.VMEM((S, D), F32),
        pltpu.VMEM((S, D), BF16),
        pltpu.VMEM((TM, F), BF16),
        pltpu.VMEM((2, TM, D), BF16),
        pltpu.SemaphoreType.DMA((NB,)),
        pltpu.SemaphoreType.DMA((13,)),
        pltpu.SemaphoreType.DMA((2,)),
    ]

    def call(A_x, A_wqkv, A_wo, B_w1, B_w3, B_w2, c, w_mod):
        return pl.pallas_call(
            kernel,
            out_shape=jax.ShapeDtypeStruct((1, S, D), BF16),
            in_specs=[any_spec] * 6 + [pl.BlockSpec(memory_space=pltpu.VMEM), any_spec],
            out_specs=any_spec,
            scratch_shapes=scratch,
            compiler_params=pltpu.CompilerParams(vmem_limit_bytes=120 * 1024 * 1024),
        )(A_x, A_wqkv, A_wo, B_w1, B_w3, B_w2, c, w_mod)

    return call


@jax.jit
def pallas_adaLN_cond__sliding_local_dilated__glu_gated_swiglu__prompt_kernel(
    A_x: jax.Array,
    A_wqkv: jax.Array,
    A_wo: jax.Array,
    B_x: jax.Array,
    B_w1: jax.Array,
    B_w3: jax.Array,
    B_w2: jax.Array,
    c: jax.Array,
    w_mod: jax.Array,
):
    del B_x
    return _build()(A_x, A_wqkv, A_wo, B_w1, B_w3, B_w2, c, w_mod)
```

```python
import functools
import math

import jax
import jax.numpy as jnp
import jax.experimental.pallas as pl
import jax.experimental.pallas.tpu as pltpu

S = 2048
D = 1024
F = 3584
H = 32
DH = D // H
WIN = 8
DIL = 2
NC = D // 128
HALO = 16
EPS = 1e-5
NEG = -1000000000.0
SM_SCALE = DH ** -0.5
LOG2E = math.log2(math.e)

TM = 128
NB = S // TM
KV = HALO + TM
RG = 8
LG = 16
KH = 512

F32 = jnp.float32
BF16 = jnp.bfloat16
U32 = jnp.uint32


def _tree(op, xs):
    xs = list(xs)
    while len(xs) > 1:
        xs = [op(xs[i], xs[i + 1]) if i + 1 < len(xs) else xs[i] for i in range(0, len(xs), 2)]
    return xs[0]


def _add(a, b):
    return a + b


def _build(TMB=128, FC=512, DL=4, CH=2, GATE=True, SKIP_FFN=False):
    NBB = S // TMB

    def kernel(x_hbm, wqkv_hbm, wo_hbm, w1_hbm, w3_hbm, w2_hbm, c_ref, wmod_hbm,
               out_hbm,
               x_v, wqkv_v, wqkv_p, wo_v, wo_tmp, wo_p, w1_v, w3_v, w2_v, wmod_v, cb_v, modp_v, mod_v,
               h1a, h1b, qka, vpa, qkb, vpb, oa, ob, otmp, y_v, h2_v, act_v, obuf,
               zs, sem_x, sem_w, sem_o):
        bufs = {"a": (h1a, qka, vpa, oa), "b": (h1b, qkb, vpb, ob)}

        def cp_x(i, n=1):
            return pltpu.make_async_copy(x_hbm.at[0, pl.ds(i * TM, n * TM), :],
                                         x_v.at[pl.ds(i * TM, n * TM), :], sem_x.at[(i + 1) // 2])

        def cp_mod(j, n=1):
            return pltpu.make_async_copy(wmod_hbm.at[:, pl.ds(j * D, n * D)],
                                         wmod_v.at[pl.ds(0, D), pl.ds(j * D, n * D)], sem_w.at[j])

        def cp_qkv(g):
            return pltpu.make_async_copy(wqkv_hbm.at[:, pl.ds(g * D, D)],
                                         wqkv_v.at[pl.ds(0, D), pl.ds(g * D, D)], sem_w.at[4 + g])

        def cp_wo():
            return pltpu.make_async_copy(wo_hbm, wo_v.at[pl.ds(0, D), :], sem_w.at[7])

        def cp_ffn(k):
            src, dst = ((w1_hbm, w1_v), (w3_hbm, w3_v), (w2_hbm, w2_v.at[pl.ds(0, F), :]))[k]
            return pltpu.make_async_copy(src, dst, sem_w.at[8 + k])

        def cp_out(j, slot):
            return pltpu.make_async_copy(obuf.at[slot],
                                         out_hbm.at[0, pl.ds(j * TMB, TMB), :], sem_o.at[slot])

        st = {"z": None, "clock": 0, "pend": {}, "sched": {}}

        def begin(sched):
            st.update(z=zs[0], clock=0, pend={}, sched=sched)

        def poke(ref, tok):
            if not GATE:
                return
            z = st["z"]
            if len(ref.shape) == 3:
                ref[0, pl.ds(pl.multiple_of(KV + z, 8), 8), :] = tok
            elif ref.dtype == BF16:
                r = ref.shape[0] - 16
                ref[pl.ds(pl.multiple_of(r + z, 16), 16), 0:128] = pltpu.bitcast(tok, BF16)
            else:
                r = ref.shape[0] - 8
                t = tok if ref.dtype == F32 else pltpu.bitcast(tok, ref.dtype)
                ref[pl.ds(pl.multiple_of(r + z, 8), 8), 0:128] = t

        def unit(w_ref, load_w, lhs, acc):
            for tok in st["pend"].pop(st["clock"], []):
                poke(w_ref, tok)
            r = jnp.dot(lhs, load_w(), preferred_element_type=F32)
            return r if acc is None else acc + r

        def release(tok):
            for refs, fn in st["sched"].pop(st["clock"], []):
                for ref in refs:
                    poke(ref, tok)
                t = fn()
                if t is not None:
                    st["pend"].setdefault(st["clock"] + DL, []).append(t)
            st["clock"] += 1

        def place(sched, items, units):
            for i, it in enumerate(items):
                sched.setdefault(units[(i * len(units)) // len(items)], []).append(it)

        def matmul(lhs_fn, w_ref, w_fn, nk, cols, sink):
            for n0 in cols:
                r = None
                for k in range(nk):
                    r = unit(w_ref, functools.partial(w_fn, k, n0), lhs_fn(k), r)
                    if k == nk - 1:
                        sink(n0, r)
                    release(r[0:8])

        def lane_iota(rows):
            return jax.lax.broadcasted_iota(jnp.int32, (rows, 128), 1)

        def ld16(ref, r0, n, c0, c1):
            return pltpu.bitcast(ref[r0 // 2:(r0 + n) // 2, c0:c1], BF16)

        def silu_c():
            cf = c_ref[...].astype(F32)
            return (cf * jax.nn.sigmoid(cf)).astype(BF16)

        def mod_mxu(j, add_one):
            lhs = jnp.broadcast_to(silu_c(), (16, D))
            r = jnp.dot(lhs, wmod_v[0:D, j * D:(j + 1) * D], preferred_element_type=F32)[0:8]
            mod_v[j] = r + 1.0 if add_one else r

        def mod_items(col0, ntiles, nsub=4):
            items, acc = [], {}

            def one(t, s):
                rows = D // nsub
                c0 = pl.multiple_of(col0 + t * 128, 128)
                w = wmod_v[s * rows:(s + 1) * rows, pl.ds(c0, 128)].astype(F32)
                p = (w * cb_v[s * rows:(s + 1) * rows, :]).reshape(rows // 8, 8, 128)
                p = _tree(_add, [p[i] for i in range(rows // 8)])
                acc[t] = p if s == 0 else acc[t] + p
                if s == nsub - 1:
                    modp_v[:, pl.ds(c0, 128)] = acc.pop(t)
            for t in range(ntiles):
                for s in range(nsub):
                    items.append(((wmod_v, cb_v), functools.partial(one, t, s)))
            return items

        def perm_qkv(g, i, nrows):
            n = nrows // 2
            r0, p0 = i * nrows, i * n
            if not isinstance(i, int):
                r0, p0 = pl.multiple_of(r0, nrows), pl.multiple_of(p0, n)
            l = lane_iota(n)
            vals = [pltpu.bitcast(wqkv_v[pl.ds(r0, nrows), g * D + c * 128: g * D + (c + 1) * 128], U32)
                    for c in range(NC)]
            for b in range(3):
                m = ((l >> (2 + b)) & 1) == 0
                for c in range(NC):
                    if c & (1 << b):
                        continue
                    lo, hi = vals[c], vals[c | (1 << b)]
                    vals[c] = jnp.where(m, lo, hi)
                    vals[c | (1 << b)] = jnp.where(m, hi, lo)
            for j in range(NC):
                idx = ((((l >> 1) & 3) << 5) | ((((l >> 3) & 7) ^ j) << 2)
                       | ((l >> 6) << 1) | (l & 1))
                t = jnp.take_along_axis(vals[j], idx, axis=1, mode="promise_in_bounds")
                wqkv_p[pl.ds(p0, n), g * D + j * 128: g * D + (j + 1) * 128] = t

        def perm_qkv_items(g, nrows=64):
            return [((wqkv_v,), functools.partial(perm_qkv, g, i, nrows)) for i in range(D // nrows)]

        def perm_wo_items():
            low = jax.lax.broadcasted_iota(jnp.int32, (8, 128), 0) < 4

            def one(c):
                for r in range(0, D, 128):
                    wo_tmp[c, r // 2:r // 2 + 64, :] = pltpu.bitcast(
                        wo_v[r:r + 128, c * 128:(c + 1) * 128], U32)
                for G in range(64):
                    j, e, ch = G >> 3, (G >> 2) & 1, G & 3
                    dd = (((2 * ch) ^ j) << 1) | e
                    ta = wo_tmp[c, pl.ds(ch * 128 + dd, 8, stride=16), :]
                    tb = wo_tmp[c, pl.ds(ch * 128 + (dd ^ 2), 8, stride=16), :]
                    wo_p[G * 8:(G + 1) * 8, c * 128:(c + 1) * 128] = jnp.where(low, ta, tb)
            return [((wo_v,), functools.partial(one, c)) for c in range(NC)]

        def ln_items(load, refs, dst, nrows, j_scale, j_shift):
            stat = {}

            def s_mean(r):
                stat[r] = jnp.mean(load(r), axis=-1, keepdims=True)

            def s_var(r):
                d = load(r) - stat[r]
                stat[r] = (stat[r], jax.lax.rsqrt(jnp.mean(d * d, axis=-1, keepdims=True) + EPS))

            def s_out(r):
                mu, rs = stat.pop(r)
                y = ((load(r) - mu) * rs).reshape(LG // 8, 8, D) * mod_v[j_scale][None] + mod_v[j_shift][None]
                dst[r // 2:(r + LG) // 2, :] = pltpu.bitcast(y.reshape(LG, D).astype(BF16), U32)
                return _tree(_add, [y[i, :, D - 128:] for i in range(LG // 8)])
            rows = list(range(0, nrows, LG))
            items = []
            for i in range(len(rows) + 2):
                for lag, fn in ((2, s_out), (1, s_var), (0, s_mean)):
                    if 0 <= i - lag < len(rows):
                        items.append((refs, functools.partial(fn, rows[i - lag])))
            return items

        def ln1_items(row0, buf):
            return ln_items(lambda r: x_v[pl.ds(row0 + r, LG), :].astype(F32), (x_v,),
                            bufs[buf][0], TM, 1, 0)

        def x1_rows(row, n, c0, c1):
            xf = x_v[pl.ds(row, n), c0:c1].astype(F32).reshape(n // 8, 8, c1 - c0)
            y = y_v[pl.ds(row, n), c0:c1].reshape(n // 8, 8, c1 - c0)
            return (xf + mod_v[2, :, c0:c1][None] * y).reshape(n, c1 - c0)

        def post_items(row0):
            return ln_items(lambda r: x1_rows(row0 + r, LG, 0, D), (x_v, y_v), h2_v, TMB, 4, 3)

        def logit_items(buf, first):
            _, qk, vp, _ = bufs[buf]
            swap = lane_iota(RG) ^ 1

            def one(r):
                qs = [qk[c, HALO + r:HALO + r + RG, :] for c in range(NC)]
                ss = []
                for w in range(WIN):
                    k0 = HALO + r - DIL * w
                    s = _tree(_add, [qs[c] * qk[NC + c, k0:k0 + RG, :] for c in range(NC)])
                    if CH and w % CH == CH - 1 and w < WIN - 1:
                        poke(qk, s)
                    s = s + pltpu.roll(s, 64, 1)
                    s = s + jnp.take_along_axis(s, swap, axis=1, mode="promise_in_bounds")
                    if first and r < DIL * w:
                        pos = r + jax.lax.broadcasted_iota(jnp.int32, (RG, 128), 0)
                        s = jnp.where(pos >= DIL * w, s, NEG / SM_SCALE)
                    ss.append(s)
                m = _tree(jnp.maximum, ss)
                ps = [jnp.exp2((s - m) * (SM_SCALE * LOG2E)) for s in ss]
                inv = 1.0 / _tree(_add, ps)
                for w in range(WIN):
                    vp[NC + w, r:r + RG, :] = ps[w] * inv
                return inv
            return [((qk,), functools.partial(one, r)) for r in range(0, TM, RG)]

        def pv_items(buf):
            _, _, vp, o = bufs[buf]

            def one(r):
                ps = [vp[NC + w, r:r + RG, :] for w in range(WIN)]
                for c in range(NC):
                    acc = _tree(_add, [ps[w] * vp[c, HALO + r - DIL * w:HALO + r - DIL * w + RG, :]
                                       for w in range(WIN)])
                    if CH and c % CH == CH - 1 and c < NC - 1:
                        poke(vp, acc)
                    if (r // RG) % 2 == 0:
                        otmp[c] = acc
                    else:
                        both = jnp.concatenate([otmp[c], acc], axis=0).astype(BF16)
                        o[(r - RG) // 2:(r + RG) // 2, c * 128:(c + 1) * 128] = pltpu.bitcast(both, U32)
            return [((vp,), functools.partial(one, r)) for r in range(0, TM, RG)]

        def halo(buf, prev, part):
            _, qk, vp, _ = bufs[buf]
            for c in range(NC):
                if part == 1:
                    qk[NC + c, 0:HALO, :] = (jnp.zeros((HALO, 128), F32) if prev is None
                                             else bufs[prev][1][NC + c, TM:TM + HALO, :])
                else:
                    vp[c, 0:HALO, :] = (jnp.broadcast_to(vp[c, HALO:HALO + 1, :], (HALO, 128)) if prev is None
                                        else bufs[prev][2][c, TM:TM + HALO, :])

        def qkv_part(buf, part):
            h1, qk, vp, _ = bufs[buf]

            def sink(n0, r):
                ch = n0 // 128
                dst, ci = (qk, ch) if ch < 2 * NC else (vp, ch - 2 * NC)
                dst[ci, HALO:HALO + TM, :] = r
            matmul(lambda k: ld16(h1, 0, TM, k * KH, (k + 1) * KH), wqkv_p,
                   lambda k, n0: ld16(wqkv_p, k * KH, KH, n0, n0 + 128),
                   D // KH, range(part * D, (part + 1) * D, 128), sink)

        def wo_mm(buf, row0):
            o = bufs[buf][3]

            def sink(n0, r):
                y_v[pl.ds(row0, TM), n0:n0 + 128] = r
            matmul(lambda k: ld16(o, 0, TM, k * KH, (k + 1) * KH), wo_p,
                   lambda k, n0: ld16(wo_p, k * KH, KH, n0, n0 + 128),
                   D // KH, range(0, D, 128), sink)

        UP = NC * (D // KH)

        def run_now(items):
            for _, fn in items:
                fn()

        def ffn(row0, slot, nxt_row):
            h = ld16(h2_v, 0, TMB, 0, D)
            for f0 in range(0, F, FC):
                g = jnp.dot(h, w1_v[:, f0:f0 + FC], preferred_element_type=F32)
                u = jnp.dot(h, w3_v[:, f0:f0 + FC], preferred_element_type=F32)
                act_v[:, f0:f0 + FC] = pltpu.bitcast((g * jax.nn.sigmoid(g) * u).astype(BF16), U32)
            nk = F // KH
            sched = {}
            place(sched, post_items(nxt_row), list(range(0, NC * nk - DL - 1)))
            begin(sched)

            def sink(n0, r):
                z = (mod_v[5, :, n0:n0 + 128][None] * r.reshape(TMB // 8, 8, 128)).reshape(TMB, 128)
                obuf[slot, :, n0:n0 + 128] = (x1_rows(row0, TMB, n0, n0 + 128) + z).astype(BF16)
            matmul(lambda k: ld16(act_v, 0, TMB, k * KH, (k + 1) * KH), w2_v,
                   lambda k, n0: w2_v[k * KH:(k + 1) * KH, n0:n0 + 128],
                   nk, range(0, D, 128), sink)

        with jax.named_scope("prologue"):
            zs[0] = 0
            cp_x(0, 2).start()
            cp_qkv(0).start()
            cp_mod(1).start()
            cb_v[0:D, :] = jnp.broadcast_to(silu_c().astype(F32), (128, D)).T
            cp_x(0, 2).wait()
            cp_mod(0).start()
            cp_qkv(0).wait()
            cp_qkv(1).start()

            def perm_body(i, carry):
                perm_qkv(0, i, 128)
                return carry
            jax.lax.fori_loop(0, D // 128, perm_body, 0)
            cp_mod(1).wait()
            cp_qkv(2).start()
            mod_mxu(1, True)
            cp_mod(0).wait()
            cp_x(2).start()
            cp_wo().start()
            mod_mxu(0, False)
            run_now(ln1_items(0, "a"))
            run_now(ln1_items(TM, "b"))
            halo("a", None, 1)

        with jax.named_scope("step0"):
            begin({})
            qkv_part("a", 0)
            cp_qkv(1).wait()
            cp_x(3, 2).start()
            sched = {}
            place(sched, perm_qkv_items(1), list(range(0, UP - 2)))
            begin(sched)
            qkv_part("b", 0)
            qkv_part("a", 1)
            cp_qkv(2).wait()
            cp_mod(2).start()
            sched = {}
            place(sched, perm_qkv_items(2), list(range(0, UP - 2)))
            place(sched, logit_items("a", True), list(range(UP, 2 * UP - DL)))
            begin(sched)
            halo("b", "a", 1)
            qkv_part("b", 1)
            qkv_part("a", 2)
            halo("a", None, 2)
            cp_x(2).wait()
            cp_wo().wait()
            cp_x(5, NB - 5).start()
            sched = {}
            place(sched, pv_items("a"), list(range(0, UP - 3)))
            place(sched, perm_wo_items(), list(range(0, UP - 3)))
            place(sched, logit_items("b", False), list(range(UP - 2, 2 * UP - DL)))
            place(sched, ln1_items(2 * TM, "a"), list(range(UP - 2, 2 * UP - DL)))
            begin(sched)
            halo("b", "a", 2)
            qkv_part("b", 2)
            wo_mm("a", 0)
            cp_x(3, 2).wait()
            cp_mod(3, 3).start()

        MT = 6

        def half(X, Y, u0, sched, row_ln1, row_wo, extra):
            place(sched, pv_items(Y), list(range(u0, u0 + 2 * UP, 2)))
            place(sched, logit_items(X, False), list(range(u0 + 2 * UP + 1, u0 + 4 * UP - DL)))
            place(sched, ln1_items(row_ln1, Y) + extra, list(range(u0 + 1, u0 + 4 * UP - DL, 2)))

            def run():
                halo(X, Y, 1)
                halo(X, Y, 2)
                for part in range(3):
                    qkv_part(X, part)
                wo_mm(Y, row_wo)
            return run

        def a_step(s, carry):
            @pl.when(s == 2)
            def _():
                cp_mod(2).wait()
                cp_x(5, NB - 5).wait()
                cp_ffn(0).start()
                cp_ffn(1).start()

            @pl.when(s == 3)
            def _():
                cp_mod(3, 3).wait()
                cp_ffn(2).start()

            ra = pl.multiple_of(2 * s * TM, TM)
            nxt = pl.multiple_of(jnp.minimum(ra + 2 * TM, S - TM), TM)
            col0 = pl.multiple_of(jnp.minimum(2 * D + (s - 2) * (MT * 128), 6 * D - MT * 128), 128)
            mi = mod_items(col0, MT)
            sched = {}
            run_a = half("a", "b", 0, sched, ra + TM, ra - TM, mi[:len(mi) // 2])
            run_b = half("b", "a", 4 * UP, sched, nxt, ra, mi[len(mi) // 2:])
            begin(sched)
            run_a()
            run_b()
            return carry

        with jax.named_scope("aloop"):
            jax.lax.fori_loop(1, NB // 2, a_step, 0)

        with jax.named_scope("atail"):
            for j in range(4):
                r = jnp.sum(modp_v[:, (2 + j) * D:(3 + j) * D], axis=0, keepdims=True)
                mod_v[2 + j] = jnp.broadcast_to(r + 1.0 if j == 2 else r, (8, D))
            begin({})
            run_now(pv_items("b"))
            sched = {}
            place(sched, post_items(0), list(range(0, UP - 2)))
            begin(sched)
            wo_mm("b", S - TM)
            for k in range(3):
                cp_ffn(k).wait()

        def b_step(j, carry):
            slot = j % 2

            @pl.when(j >= 2)
            def _():
                cp_out(j - 2, slot).wait()

            row0 = pl.multiple_of(j * TMB, TMB)
            nxt = pl.multiple_of(jnp.minimum(row0 + TMB, S - TMB), TMB)
            if SKIP_FFN:
                obuf[slot] = x1_rows(row0, TMB, 0, D).astype(BF16)
            else:
                ffn(row0, slot, nxt)
            cp_out(j, slot).start()
            return carry

        with jax.named_scope("bloop"):
            jax.lax.fori_loop(0, NBB, b_step, 0)
        with jax.named_scope("tail"):
            cp_out(NBB - 2, (NBB - 2) % 2).wait()
            cp_out(NBB - 1, (NBB - 1) % 2).wait()

    any_spec = pl.BlockSpec(memory_space=pl.ANY)
    scratch = [
        pltpu.VMEM((S + 16, D), BF16),
        pltpu.VMEM((D + 16, 3 * D), BF16),
        pltpu.VMEM((D // 2 + 8, 3 * D), U32),
        pltpu.VMEM((D + 16, D), BF16),
        pltpu.VMEM((NC, D // 2, 128), U32),
        pltpu.VMEM((D // 2 + 8, D), U32),
        pltpu.VMEM((D, F), BF16),
        pltpu.VMEM((D, F), BF16),
        pltpu.VMEM((F + 16, D), BF16),
        pltpu.VMEM((D + 16, 6 * D), BF16),
        pltpu.VMEM((D + 8, 128), F32),
        pltpu.VMEM((8, 6 * D), F32),
        pltpu.VMEM((6, 8, D), F32),
        pltpu.VMEM((TM // 2, D), U32),
        pltpu.VMEM((TM // 2, D), U32),
        pltpu.VMEM((2 * NC, KV + 8, 128), F32),
        pltpu.VMEM((2 * NC, KV + 8, 128), F32),
        pltpu.VMEM((2 * NC, KV + 8, 128), F32),
        pltpu.VMEM((2 * NC, KV + 8, 128), F32),
        pltpu.VMEM((TM // 2, D), U32),
        pltpu.VMEM((TM // 2, D), U32),
        pltpu.VMEM((NC, RG, 128), F32),
        pltpu.VMEM((S + 8, D), F32),
        pltpu.VMEM((TMB // 2, D), U32),
        pltpu.VMEM((TMB // 2, F), U32),
        pltpu.VMEM((2, TMB, D), BF16),
        pltpu.SMEM((1,), jnp.int32),
        pltpu.SemaphoreType.DMA((4,)),
        pltpu.SemaphoreType.DMA((11,)),
        pltpu.SemaphoreType.DMA((2,)),
    ]

    def call(A_x, A_wqkv, A_wo, B_w1, B_w3, B_w2, c, w_mod):
        return pl.pallas_call(
            kernel,
            out_shape=jax.ShapeDtypeStruct((1, S, D), BF16),
            in_specs=[any_spec] * 6 + [pl.BlockSpec(memory_space=pltpu.VMEM), any_spec],
            out_specs=any_spec,
            scratch_shapes=scratch,
            compiler_params=pltpu.CompilerParams(vmem_limit_bytes=120 * 1024 * 1024),
        )(A_x, A_wqkv, A_wo, B_w1, B_w3, B_w2, c, w_mod)

    return call


@jax.jit
def pallas_adaLN_cond__sliding_local_dilated__glu_gated_swiglu__prompt_kernel(
    A_x: jax.Array,
    A_wqkv: jax.Array,
    A_wo: jax.Array,
    B_x: jax.Array,
    B_w1: jax.Array,
    B_w3: jax.Array,
    B_w2: jax.Array,
    c: jax.Array,
    w_mod: jax.Array,
):
    del B_x
    return _build()(A_x, A_wqkv, A_wo, B_w1, B_w3, B_w2, c, w_mod)
```

```python
import functools
import math

import jax
import jax.numpy as jnp
import jax.experimental.pallas as pl
import jax.experimental.pallas.tpu as pltpu

S = 2048
D = 1024
F = 3584
H = 32
DH = D // H
WIN = 8
DIL = 2
NC = D // 128
HALO = 16
EPS = 1e-5
NEG = -1000000000.0
SM_SCALE = DH ** -0.5
LOG2E = math.log2(math.e)

TM = 128
NB = S // TM
KV = HALO + TM
RG = 8
LG = 16
KH = 512

F32 = jnp.float32
BF16 = jnp.bfloat16
U32 = jnp.uint32


def _tree(op, xs):
    xs = list(xs)
    while len(xs) > 1:
        xs = [op(xs[i], xs[i + 1]) if i + 1 < len(xs) else xs[i] for i in range(0, len(xs), 2)]
    return xs[0]


def _add(a, b):
    return a + b


def _build(TMB=128, FC=512, GATE=True, SKIP_FFN=False, SKIP_A=False,
           SCH=0, MT=6, NSUB=8, PB1=5, L0=1, L1=4, SPREAD=128, RELOAD=True,
           LS=16, LE=24, P0=0, P1=16, N0=1, N1=30):
    NBB = S // TMB

    def kernel(x_hbm, wqkv_hbm, wo_hbm, w1_hbm, w3_hbm, w2_hbm, c_ref, wmod_hbm,
               out_hbm,
               x_v, wqkv_v, wqkv_p, wo_v, wo_tmp, wo_p, w1_v, w3_v, w2_v, wmod_v, cb_v, modp_v, mod_v,
               h1a, h1b, qka, va, pa, qkb, vb, pb_, oa, ob, otmp, y_v, x1n, h2_v, act_v, obuf,
               zs, sem_x, sem_w, sem_o):
        bufs = {"a": (h1a, qka, va, oa, pa), "b": (h1b, qkb, vb, ob, pb_)}

        def cp_x(i, n=1):
            return pltpu.make_async_copy(x_hbm.at[0, pl.ds(i * TM, n * TM), :],
                                         x_v.at[pl.ds(i * TM, n * TM), :], sem_x.at[(i + 1) // 2])

        def cp_mod(j, n=1):
            return pltpu.make_async_copy(wmod_hbm.at[:, pl.ds(j * D, n * D)],
                                         wmod_v.at[pl.ds(0, D), pl.ds(j * D, n * D)], sem_w.at[j])

        def cp_qkv(g):
            return pltpu.make_async_copy(wqkv_hbm.at[:, pl.ds(g * D, D)],
                                         wqkv_v.at[pl.ds(0, D), pl.ds(g * D, D)], sem_w.at[4 + g])

        def cp_wo():
            return pltpu.make_async_copy(wo_hbm, wo_v.at[pl.ds(0, D), :], sem_w.at[7])

        def cp_ffn(k):
            src, dst = ((w1_hbm, w1_v), (w3_hbm, w3_v), (w2_hbm, w2_v.at[pl.ds(0, F), :]))[k]
            return pltpu.make_async_copy(src, dst, sem_w.at[8 + k])

        def cp_out(j, slot):
            return pltpu.make_async_copy(obuf.at[slot],
                                         out_hbm.at[0, pl.ds(j * TMB, TMB), :], sem_o.at[slot])

        st = {"z": None, "never": None, "clock": 0, "sched": {}, "tok": None}

        def begin(sched):
            z = zs[0]
            st.update(z=z, never=jnp.full((8, 128), z, jnp.int32) != 0, clock=0, sched=sched, tok=None)

        def gate(val, i, n):
            r = st["tok"]
            if r is None or not GATE:
                return val
            row = (i * SPREAD // n) // 8 * 8
            t = r[row:row + 8]
            return jnp.where(st["never"], t if val.dtype == F32 else pltpu.bitcast(t, val.dtype), val)

        def place(sched, items, units):
            units = list(units)
            for i, it in enumerate(items):
                sched.setdefault(units[(i * len(units)) // len(items)], []).append(it)

        def matmul(lhs_fn, w_fn, nk, cols, sink):
            for n0 in cols:
                r = None
                for k in range(nk):
                    d = jnp.dot(lhs_fn(k), w_fn(k, n0), preferred_element_type=F32)
                    r = d if r is None else r + d
                    if k == nk - 1:
                        sink(n0, r)
                    st["tok"] = r
                    for fn in st["sched"].pop(st["clock"], []):
                        fn()
                    st["tok"] = None
                    st["clock"] += 1

        def finish():
            assert not st["sched"]

        def lane_iota(rows):
            return jax.lax.broadcasted_iota(jnp.int32, (rows, 128), 1)

        def ld16(ref, r0, n, c0, c1):
            return pltpu.bitcast(ref[r0 // 2:(r0 + n) // 2, c0:c1], BF16)

        def silu_c():
            cf = c_ref[...].astype(F32)
            return (cf * jax.nn.sigmoid(cf)).astype(BF16)

        def mod_mxu(j, add_one):
            lhs = jnp.broadcast_to(silu_c(), (16, D))
            r = jnp.dot(lhs, wmod_v[0:D, j * D:(j + 1) * D], preferred_element_type=F32)[0:8]
            mod_v[j] = r + 1.0 if add_one else r

        def mod_items(col0, ntiles):
            rows = D // NSUB

            def one(t, i):
                c0 = pl.multiple_of(col0 + t * 128, 128)
                w = wmod_v[i * rows:(i + 1) * rows, pl.ds(c0, 128)].astype(F32)
                p = (w * cb_v[i * rows:(i + 1) * rows, :]).reshape(rows // 8, 8, 128)
                modp_v[i, :, pl.ds(c0, 128)] = gate(_tree(_add, [p[k] for k in range(rows // 8)]), 1, 2)
            return [functools.partial(one, t, i) for t in range(ntiles) for i in range(NSUB)]

        def perm_qkv(g, i, nrows):
            n = nrows // 2
            r0, p0 = i * nrows, i * n
            if not isinstance(i, int):
                r0, p0 = pl.multiple_of(r0, nrows), pl.multiple_of(p0, n)
            l = lane_iota(n)
            vals = [pltpu.bitcast(wqkv_v[pl.ds(r0, nrows), g * D + c * 128: g * D + (c + 1) * 128], U32)
                    for c in range(NC)]
            for b in range(3):
                m = ((l >> (2 + b)) & 1) == 0
                for c in range(NC):
                    if c & (1 << b):
                        continue
                    lo, hi = vals[c], vals[c | (1 << b)]
                    vals[c] = jnp.where(m, lo, hi)
                    vals[c | (1 << b)] = jnp.where(m, hi, lo)
            for j in range(NC):
                idx = ((((l >> 1) & 3) << 5) | ((((l >> 3) & 7) ^ j) << 2)
                       | ((l >> 6) << 1) | (l & 1))
                v = jnp.concatenate([gate(vals[j][q:q + 8], j, NC) for q in range(0, n, 8)], axis=0)
                t = jnp.take_along_axis(v, idx, axis=1, mode="promise_in_bounds")
                wqkv_p[pl.ds(p0, n), g * D + j * 128: g * D + (j + 1) * 128] = t

        def perm_qkv_items(g, nrows=64):
            return [functools.partial(perm_qkv, g, i, nrows) for i in range(D // nrows)]

        def perm_wo_items():
            low = jax.lax.broadcasted_iota(jnp.int32, (8, 128), 0) < 4

            def one(c):
                for r in range(0, D // 2, 8):
                    wo_tmp[c, r:r + 8, :] = gate(pltpu.bitcast(
                        wo_v[2 * r:2 * r + 16, c * 128:(c + 1) * 128], U32), r, D // 2)
                for G in range(64):
                    j, e, ch = G >> 3, (G >> 2) & 1, G & 3
                    dd = (((2 * ch) ^ j) << 1) | e
                    ta = wo_tmp[c, pl.ds(ch * 128 + dd, 8, stride=16), :]
                    tb = wo_tmp[c, pl.ds(ch * 128 + (dd ^ 2), 8, stride=16), :]
                    wo_p[G * 8:(G + 1) * 8, c * 128:(c + 1) * 128] = jnp.where(low, ta, tb)
            return [functools.partial(one, c) for c in range(NC)]

        def row_mean(x, gated):
            part = _tree(_add, [x[:, c * 128:(c + 1) * 128] for c in range(NC)])
            if gated:
                part = jnp.concatenate([gate(part[q:q + 8], q, LG) for q in range(0, LG, 8)], axis=0)
            return jnp.sum(part, axis=-1, keepdims=True) * (1.0 / D)

        def ln_items(load, dst, nrows, j_scale, j_shift):
            def one(r):
                mu = row_mean(load(r, 0), True)
                d = load(r, 1) - mu
                rs = jax.lax.rsqrt(row_mean(d * d, False) + EPS)
                y = ((load(r, 2) - mu) * rs).reshape(LG // 8, 8, D) * mod_v[j_scale][None] + mod_v[j_shift][None]
                dst[r // 2:(r + LG) // 2, :] = pltpu.bitcast(y.reshape(LG, D).astype(BF16), U32)
            return [functools.partial(one, r) for r in range(0, nrows, LG)]

        def opaque_row(row, k):
            return row if k == 0 or not RELOAD else pl.multiple_of(row + k * st["z"], LG)

        def ln1_items(row0, buf):
            return ln_items(lambda r, k: x_v[pl.ds(opaque_row(row0 + r, k), LG), :].astype(F32),
                            bufs[buf][0], TM, 1, 0)

        def x1_rows(row, n, c0, c1):
            xf = x_v[pl.ds(row, n), c0:c1].astype(F32).reshape(n // 8, 8, c1 - c0)
            y = y_v[pl.ds(row, n), c0:c1].reshape(n // 8, 8, c1 - c0)
            return (xf + mod_v[2, :, c0:c1][None] * y).reshape(n, c1 - c0)

        def post_items(row0):
            def load(r, k):
                if k:
                    return x1n[pl.ds(opaque_row(r, k), LG), :]
                x1 = x1_rows(row0 + r, LG, 0, D)
                x1n[r:r + LG, :] = x1
                return x1
            return ln_items(load, h2_v, TMB, 4, 3)

        def logit_items(buf, first):
            _, qk, _, _, pb = bufs[buf]
            swap = lane_iota(RG) ^ 1

            def one(r):
                qs = [qk[c, HALO + r:HALO + r + RG, :] for c in range(NC)]
                ss = []
                for w in range(WIN):
                    k0 = HALO + r - DIL * w
                    s = _tree(_add, [qs[c] * qk[NC + c, k0:k0 + RG, :] for c in range(NC)])
                    s = gate(s, w, WIN)
                    s = s + pltpu.roll(s, 64, 1)
                    s = s + jnp.take_along_axis(s, swap, axis=1, mode="promise_in_bounds")
                    if first and r < DIL * w:
                        pos = r + jax.lax.broadcasted_iota(jnp.int32, (RG, 128), 0)
                        s = jnp.where(pos >= DIL * w, s, NEG / SM_SCALE)
                    ss.append(s)
                m = _tree(jnp.maximum, ss)
                ps = [jnp.exp2((s - m) * (SM_SCALE * LOG2E)) for s in ss]
                inv = 1.0 / _tree(_add, ps)
                for w in range(WIN):
                    pb[w, r:r + RG, :] = ps[w] * inv
            return [functools.partial(one, r) for r in range(0, TM, RG)]

        def pv_items(buf):
            _, _, vp, o, pb = bufs[buf]

            def one(r):
                ps = [pb[w, r:r + RG, :] for w in range(WIN)]
                for c in range(NC):
                    acc = _tree(_add, [ps[w] * vp[c, HALO + r - DIL * w:HALO + r - DIL * w + RG, :]
                                       for w in range(WIN)])
                    acc = gate(acc, c, NC)
                    if (r // RG) % 2 == 0:
                        otmp[c, pl.ds(pl.multiple_of(st["z"], 8), RG), :] = acc
                    else:
                        both = jnp.concatenate([otmp[c], acc], axis=0).astype(BF16)
                        o[(r - RG) // 2:(r + RG) // 2, c * 128:(c + 1) * 128] = pltpu.bitcast(both, U32)
            return [functools.partial(one, r) for r in range(0, TM, RG)]

        def halo(buf, prev, part):
            _, qk, vp, _, _ = bufs[buf]
            for c in range(NC):
                if part == 1:
                    qk[NC + c, 0:HALO, :] = (jnp.zeros((HALO, 128), F32) if prev is None
                                             else bufs[prev][1][NC + c, TM:TM + HALO, :])
                else:
                    vp[c, 0:HALO, :] = (jnp.broadcast_to(vp[c, HALO:HALO + 1, :], (HALO, 128)) if prev is None
                                        else bufs[prev][2][c, TM:TM + HALO, :])

        def qkv_part(buf, part):
            h1, qk, vp, _, _ = bufs[buf]

            def sink(n0, r):
                ch = n0 // 128
                dst, ci = (qk, ch) if ch < 2 * NC else (vp, ch - 2 * NC)
                dst[ci, HALO:HALO + TM, :] = r
            matmul(lambda k: ld16(h1, 0, TM, k * KH, (k + 1) * KH),
                   lambda k, n0: ld16(wqkv_p, k * KH, KH, n0, n0 + 128),
                   D // KH, range(part * D, (part + 1) * D, 128), sink)

        def wo_mm(buf, row0):
            o = bufs[buf][3]

            def sink(n0, r):
                y_v[pl.ds(row0, TM), n0:n0 + 128] = r
            matmul(lambda k: ld16(o, 0, TM, k * KH, (k + 1) * KH),
                   lambda k, n0: ld16(wo_p, k * KH, KH, n0, n0 + 128),
                   D // KH, range(0, D, 128), sink)

        UP = NC * (D // KH)

        def run_now(items):
            for fn in items:
                fn()

        def ffn(row0, slot, nxt_row):
            h = ld16(h2_v, 0, TMB, 0, D)
            for f0 in range(0, F, FC):
                g = jnp.dot(h, w1_v[:, f0:f0 + FC], preferred_element_type=F32)
                u = jnp.dot(h, w3_v[:, f0:f0 + FC], preferred_element_type=F32)
                act_v[:, f0:f0 + FC] = pltpu.bitcast((g * jax.nn.sigmoid(g) * u).astype(BF16), U32)
            nk = F // KH
            sched = {}
            place(sched, post_items(nxt_row), range(0, NC * nk - PB1))
            begin(sched)

            def sink(n0, r):
                z = (mod_v[5, :, n0:n0 + 128][None] * r.reshape(TMB // 8, 8, 128)).reshape(TMB, 128)
                obuf[slot, :, n0:n0 + 128] = (x1_rows(row0, TMB, n0, n0 + 128) + z).astype(BF16)
            matmul(lambda k: ld16(act_v, 0, TMB, k * KH, (k + 1) * KH),
                   lambda k, n0: w2_v[k * KH:(k + 1) * KH, n0:n0 + 128],
                   nk, range(0, D, 128), sink)

        with jax.named_scope("prologue"):
            zs[0] = 0
            begin({})
            cp_x(0, 2).start()
            cp_qkv(0).start()
            cp_mod(1).start()
            cb_v[0:D, :] = jnp.broadcast_to(silu_c().astype(F32), (128, D)).T
            cp_x(0, 2).wait()
            cp_mod(0).start()
            cp_qkv(0).wait()
            cp_qkv(1).start()

            def perm_body(i, carry):
                perm_qkv(0, i, 128)
                return carry
            jax.lax.fori_loop(0, D // 128, perm_body, 0)
            cp_mod(1).wait()
            cp_qkv(2).start()
            mod_mxu(1, True)
            cp_mod(0).wait()
            cp_x(2).start()
            cp_wo().start()
            mod_mxu(0, False)
            run_now(ln1_items(0, "a"))
            run_now(ln1_items(TM, "b"))
            halo("a", None, 1)

        with jax.named_scope("step0"):
            begin({})
            qkv_part("a", 0)
            cp_qkv(1).wait()
            cp_x(3, 2).start()
            sched = {}
            place(sched, perm_qkv_items(1), range(0, UP - 2))
            begin(sched)
            qkv_part("b", 0)
            qkv_part("a", 1)
            cp_qkv(2).wait()
            cp_mod(2).start()
            sched = {}
            place(sched, perm_qkv_items(2), range(0, UP - 2))
            place(sched, logit_items("a", True), range(UP - 2, 2 * UP - L1))
            begin(sched)
            halo("b", "a", 1)
            qkv_part("b", 1)
            qkv_part("a", 2)
            finish()
            halo("a", None, 2)
            cp_x(2).wait()
            cp_wo().wait()
            cp_x(5, NB - 5).start()
            sched = {}
            place(sched, pv_items("a"), range(0, UP - 2))
            place(sched, perm_wo_items(), range(0, UP - 2))
            place(sched, ln1_items(2 * TM, "a"), range(0, UP + 4))
            place(sched, logit_items("b", False)[:LS], range(UP - 2, 2 * UP - L1))
            begin(sched)
            halo("b", "a", 2)
            qkv_part("b", 2)
            wo_mm("a", 0)
            finish()
            cp_x(3, 2).wait()
            cp_mod(3, 3).start()


        def half(X, Y, u0, sched, row_ln1, row_wo, extra):
            lx, ly = logit_items(X, False), logit_items(Y, False)
            if LS < len(ly):
                place(sched, ly[LS:], range(u0, u0 + LE))
            place(sched, pv_items(Y), range(u0 + P0, u0 + 3 * UP - P1))
            place(sched, lx[:LS], range(u0 + 2 * UP + L0, u0 + 4 * UP - L1))
            place(sched, ln1_items(row_ln1, Y), range(u0 + N0, u0 + N1))
            if extra:
                place(sched, extra, range(u0, u0 + 4 * UP - 1))

            def run():
                halo(X, Y, 1)
                halo(X, Y, 2)
                for part in range(3):
                    qkv_part(X, part)
                wo_mm(Y, row_wo)
            return run

        def a_step(s, carry):
            @pl.when(s == 2)
            def _():
                cp_mod(2).wait()
                cp_x(5, NB - 5).wait()
                cp_ffn(0).start()
                cp_ffn(1).start()

            @pl.when(s == 3)
            def _():
                cp_mod(3, 3).wait()
                cp_ffn(2).start()

            ra = pl.multiple_of(2 * s * TM, TM)
            nxt = pl.multiple_of(jnp.minimum(ra + 2 * TM, S - TM), TM)
            col0 = pl.multiple_of(jnp.minimum(2 * D + (s - 2) * (MT * 128), 6 * D - MT * 128), 128)
            mi = mod_items(col0, MT)
            sched = {}
            run_a = half("a", "b", 0, sched, ra + TM, ra - TM, mi[:len(mi) // 2])
            run_b = half("b", "a", 4 * UP, sched, nxt, ra, mi[len(mi) // 2:])
            begin(sched)
            run_a()
            run_b()
            finish()
            return carry

        with jax.named_scope("aloop"):
            if SKIP_A:
                cp_mod(2).wait()
                cp_x(5, NB - 5).wait()
                cp_mod(3, 3).wait()
                for k in range(3):
                    cp_ffn(k).start()
            else:
                jax.lax.fori_loop(1, NB // 2, a_step, 0)

        with jax.named_scope("atail"):
            for j in range(4):
                r = _tree(_add, [modp_v[i, :, (2 + j) * D:(3 + j) * D] for i in range(NSUB)])
                r = jnp.sum(r, axis=0, keepdims=True)
                mod_v[2 + j] = jnp.broadcast_to(r + 1.0 if j == 2 else r, (8, D))
            begin({})
            run_now(logit_items("b", False)[LS:])
            run_now(pv_items("b"))
            sched = {}
            place(sched, post_items(0), range(0, UP - 2))
            begin(sched)
            wo_mm("b", S - TM)
            finish()
            for k in range(3):
                cp_ffn(k).wait()

        def b_step(j, carry):
            slot = j % 2

            @pl.when(j >= 2)
            def _():
                cp_out(j - 2, slot).wait()

            row0 = pl.multiple_of(j * TMB, TMB)
            nxt = pl.multiple_of(jnp.minimum(row0 + TMB, S - TMB), TMB)
            if SKIP_FFN:
                obuf[slot] = x1_rows(row0, TMB, 0, D).astype(BF16)
            else:
                ffn(row0, slot, nxt)
            cp_out(j, slot).start()
            return carry

        with jax.named_scope("bloop"):
            jax.lax.fori_loop(0, NBB, b_step, 0)
        with jax.named_scope("tail"):
            cp_out(NBB - 2, (NBB - 2) % 2).wait()
            cp_out(NBB - 1, (NBB - 1) % 2).wait()

    any_spec = pl.BlockSpec(memory_space=pl.ANY)
    scratch = [
        pltpu.VMEM((S, D), BF16),
        pltpu.VMEM((D, 3 * D), BF16),
        pltpu.VMEM((D // 2, 3 * D), U32),
        pltpu.VMEM((D, D), BF16),
        pltpu.VMEM((NC, D // 2, 128), U32),
        pltpu.VMEM((D // 2, D), U32),
        pltpu.VMEM((D, F), BF16),
        pltpu.VMEM((D, F), BF16),
        pltpu.VMEM((F, D), BF16),
        pltpu.VMEM((D, 6 * D), BF16),
        pltpu.VMEM((D, 128), F32),
        pltpu.VMEM((NSUB, 8, 6 * D), F32),
        pltpu.VMEM((6, 8, D), F32),
        pltpu.VMEM((TM // 2, D), U32),
        pltpu.VMEM((TM // 2, D), U32),
        pltpu.VMEM((2 * NC, KV, 128), F32),
        pltpu.VMEM((NC, KV, 128), F32),
        pltpu.VMEM((WIN, TM, 128), F32),
        pltpu.VMEM((2 * NC, KV, 128), F32),
        pltpu.VMEM((NC, KV, 128), F32),
        pltpu.VMEM((WIN, TM, 128), F32),
        pltpu.VMEM((TM // 2, D), U32),
        pltpu.VMEM((TM // 2, D), U32),
        pltpu.VMEM((NC, RG, 128), F32),
        pltpu.VMEM((S, D), F32),
        pltpu.VMEM((TMB, D), F32),
        pltpu.VMEM((TMB // 2, D), U32),
        pltpu.VMEM((TMB // 2, F), U32),
        pltpu.VMEM((2, TMB, D), BF16),
        pltpu.SMEM((1,), jnp.int32),
        pltpu.SemaphoreType.DMA((4,)),
        pltpu.SemaphoreType.DMA((11,)),
        pltpu.SemaphoreType.DMA((2,)),
    ]

    def call(A_x, A_wqkv, A_wo, B_w1, B_w3, B_w2, c, w_mod):
        return pl.pallas_call(
            kernel,
            out_shape=jax.ShapeDtypeStruct((1, S, D), BF16),
            in_specs=[any_spec] * 6 + [pl.BlockSpec(memory_space=pltpu.VMEM), any_spec],
            out_specs=any_spec,
            scratch_shapes=scratch,
            compiler_params=pltpu.CompilerParams(vmem_limit_bytes=120 * 1024 * 1024),
        )(A_x, A_wqkv, A_wo, B_w1, B_w3, B_w2, c, w_mod)

    return call


@jax.jit
def pallas_adaLN_cond__sliding_local_dilated__glu_gated_swiglu__prompt_kernel(
    A_x: jax.Array,
    A_wqkv: jax.Array,
    A_wo: jax.Array,
    B_x: jax.Array,
    B_w1: jax.Array,
    B_w3: jax.Array,
    B_w2: jax.Array,
    c: jax.Array,
    w_mod: jax.Array,
):
    del B_x
    return _build()(A_x, A_wqkv, A_wo, B_w1, B_w3, B_w2, c, w_mod)
```

```python
import functools
import math

import jax
import jax.numpy as jnp
import jax.experimental.pallas as pl
import jax.experimental.pallas.tpu as pltpu

S = 2048
D = 1024
F = 3584
H = 32
DH = D // H
WIN = 8
DIL = 2
NC = D // 128
HALO = 16
EPS = 1e-5
NEG = -1000000000.0
SM_SCALE = DH ** -0.5
LOG2E = math.log2(math.e)

TM = 128
NB = S // TM
KV = HALO + TM
RG = 8
LG = 16
KH = 512

F32 = jnp.float32
BF16 = jnp.bfloat16
U32 = jnp.uint32


def _tree(op, xs):
    xs = list(xs)
    while len(xs) > 1:
        xs = [op(xs[i], xs[i + 1]) if i + 1 < len(xs) else xs[i] for i in range(0, len(xs), 2)]
    return xs[0]


def _add(a, b):
    return a + b


def _build(TMB=128, FC=512, GATE=True, SKIP_FFN=False, SKIP_A=False,
           SCH=0, MT=6, NSUB=16, PB1=5, L0=0, L1=1, SPREAD=128, LLAG=3,
           P0=0, P1=16, N0=1, N1=30):
    NBB = S // TMB

    def kernel(x_hbm, wqkv_hbm, wo_hbm, w1_hbm, w3_hbm, w2_hbm, c_ref, wmod_hbm,
               out_hbm,
               x_v, wqkv_v, wqkv_p, wo_v, wo_tmp, wo_p, w1_v, w3_v, w2_v, wmod_v, cb_v, modp_v, mod_v,
               h1a, h1b, qka, va, pa, qkb, vb, pb_, oa, ob, otmp, sl0, sl1, sl2, stat1, stat2, y_v, x1n, h2_v, act_v, obuf,
               zs, sem_x, sem_w, sem_o):
        bufs = {"a": (h1a, qka, va, oa, pa), "b": (h1b, qkb, vb, ob, pb_)}

        sls = (sl0, sl1, sl2)

        def cp_x(i, n=1):
            return pltpu.make_async_copy(x_hbm.at[0, pl.ds(i * TM, n * TM), :],
                                         x_v.at[pl.ds(i * TM, n * TM), :], sem_x.at[(i + 1) // 2])

        def cp_mod(j, n=1):
            return pltpu.make_async_copy(wmod_hbm.at[:, pl.ds(j * D, n * D)],
                                         wmod_v.at[pl.ds(0, D), pl.ds(j * D, n * D)], sem_w.at[j])

        def cp_qkv(g):
            return pltpu.make_async_copy(wqkv_hbm.at[:, pl.ds(g * D, D)],
                                         wqkv_v.at[pl.ds(0, D), pl.ds(g * D, D)], sem_w.at[4 + g])

        def cp_wo():
            return pltpu.make_async_copy(wo_hbm, wo_v.at[pl.ds(0, D), :], sem_w.at[7])

        def cp_ffn(k):
            src, dst = ((w1_hbm, w1_v), (w3_hbm, w3_v), (w2_hbm, w2_v.at[pl.ds(0, F), :]))[k]
            return pltpu.make_async_copy(src, dst, sem_w.at[8 + k])

        def cp_out(j, slot):
            return pltpu.make_async_copy(obuf.at[slot],
                                         out_hbm.at[0, pl.ds(j * TMB, TMB), :], sem_o.at[slot])

        st = {"z": None, "never": None, "clock": 0, "sched": {}, "tok": None}

        def begin(sched):
            z = zs[0]
            st.update(z=z, never=jnp.full((8, 128), z, jnp.int32) != 0, clock=0, sched=sched, tok=None)

        def gate(val, i, n):
            r = st["tok"]
            if r is None or not GATE:
                return val
            row = (i * SPREAD // n) // 8 * 8
            t = r[row:row + 8]
            return jnp.where(st["never"], t if val.dtype == F32 else pltpu.bitcast(t, val.dtype), val)

        def place(sched, items, units):
            units = list(units)
            for i, it in enumerate(items):
                sched.setdefault(units[(i * len(units)) // len(items)], []).append(it)

        def matmul(lhs_fn, w_fn, nk, cols, sink):
            for n0 in cols:
                r = None
                for k in range(nk):
                    d = jnp.dot(lhs_fn(k), w_fn(k, n0), preferred_element_type=F32)
                    r = d if r is None else r + d
                    if k == nk - 1:
                        sink(n0, r)
                    st["tok"] = r
                    for fn in st["sched"].pop(st["clock"], []):
                        fn()
                    st["tok"] = None
                    st["clock"] += 1

        def finish():
            assert not st["sched"]

        def lane_iota(rows):
            return jax.lax.broadcasted_iota(jnp.int32, (rows, 128), 1)

        def ld16(ref, r0, n, c0, c1):
            return pltpu.bitcast(ref[r0 // 2:(r0 + n) // 2, c0:c1], BF16)

        def silu_c():
            cf = c_ref[...].astype(F32)
            return (cf * jax.nn.sigmoid(cf)).astype(BF16)

        def mod_mxu(j, add_one):
            lhs = jnp.broadcast_to(silu_c(), (16, D))
            r = jnp.dot(lhs, wmod_v[0:D, j * D:(j + 1) * D], preferred_element_type=F32)[0:8]
            mod_v[j] = r + 1.0 if add_one else r

        def mod_items(col0, ntiles):
            rows = D // NSUB

            def one(t, i):
                c0 = pl.multiple_of(col0 + t * 128, 128)
                w = wmod_v[i * rows:(i + 1) * rows, pl.ds(c0, 128)].astype(F32)
                p = (w * cb_v[i * rows:(i + 1) * rows, :]).reshape(rows // 8, 8, 128)
                modp_v[i, :, pl.ds(c0, 128)] = gate(_tree(_add, [p[k] for k in range(rows // 8)]), 1, 2)
            return [functools.partial(one, t, i) for t in range(ntiles) for i in range(NSUB)]

        def perm_qkv(g, i, nrows):
            n = nrows // 2
            r0, p0 = i * nrows, i * n
            if not isinstance(i, int):
                r0, p0 = pl.multiple_of(r0, nrows), pl.multiple_of(p0, n)
            l = lane_iota(n)
            vals = [pltpu.bitcast(wqkv_v[pl.ds(r0, nrows), g * D + c * 128: g * D + (c + 1) * 128], U32)
                    for c in range(NC)]
            for b in range(3):
                m = ((l >> (2 + b)) & 1) == 0
                for c in range(NC):
                    if c & (1 << b):
                        continue
                    lo, hi = vals[c], vals[c | (1 << b)]
                    vals[c] = jnp.where(m, lo, hi)
                    vals[c | (1 << b)] = jnp.where(m, hi, lo)
            for j in range(NC):
                idx = ((((l >> 1) & 3) << 5) | ((((l >> 3) & 7) ^ j) << 2)
                       | ((l >> 6) << 1) | (l & 1))
                v = jnp.concatenate([gate(vals[j][q:q + 8], j, NC) for q in range(0, n, 8)], axis=0)
                t = jnp.take_along_axis(v, idx, axis=1, mode="promise_in_bounds")
                wqkv_p[pl.ds(p0, n), g * D + j * 128: g * D + (j + 1) * 128] = t

        def perm_qkv_items(g, nrows=64):
            return [functools.partial(perm_qkv, g, i, nrows) for i in range(D // nrows)]

        def perm_wo_items():
            low = jax.lax.broadcasted_iota(jnp.int32, (8, 128), 0) < 4

            def one(c):
                for r in range(0, D // 2, 8):
                    wo_tmp[c, r:r + 8, :] = gate(pltpu.bitcast(
                        wo_v[2 * r:2 * r + 16, c * 128:(c + 1) * 128], U32), r, D // 2)
                for G in range(64):
                    j, e, ch = G >> 3, (G >> 2) & 1, G & 3
                    dd = (((2 * ch) ^ j) << 1) | e
                    ta = wo_tmp[c, pl.ds(ch * 128 + dd, 8, stride=16), :]
                    tb = wo_tmp[c, pl.ds(ch * 128 + (dd ^ 2), 8, stride=16), :]
                    wo_p[G * 8:(G + 1) * 8, c * 128:(c + 1) * 128] = jnp.where(low, ta, tb)
            return [functools.partial(one, c) for c in range(NC)]

        def zrow(row, k=1):
            return row + k * st["z"]

        def gate16(v, i, n):
            return jnp.concatenate([gate(v[q:q + 8], i, n) for q in range(0, LG, 8)], axis=0)

        def staged(stages, n, lag):
            items = []
            for t in range(n + lag * (len(stages) - 1)):
                for k in reversed(range(len(stages))):
                    if 0 <= t - k * lag < n:
                        items.append(functools.partial(stages[k], t - k * lag))
            return items

        def ln_items(load, stat, dst, nrows, j_scale, j_shift):
            def chunks(x):
                return [x[:, c * 128:(c + 1) * 128] for c in range(NC)]

            def put(j, r, part, fn):
                m = jnp.sum(part, axis=-1, keepdims=True) * (1.0 / D)
                stat[j, pl.ds(pl.multiple_of(zrow(r), LG), LG), :] = jnp.broadcast_to(fn(m), (LG, 128))

            def s_mean(i):
                put(0, i * LG, gate16(_tree(_add, chunks(load(i * LG, 0))), 1, 2), lambda m: m)

            def s_var(i):
                r = i * LG
                mu = gate16(stat[0, r:r + LG, :], 0, 1)
                put(1, r, _tree(_add, [(x - mu) * (x - mu) for x in chunks(load(r, 1))]),
                    lambda m: jax.lax.rsqrt(m + EPS))

            def s_out(i):
                r = i * LG
                mu, rs = stat[0, r:r + LG, :], stat[1, r:r + LG, :]
                for c, x in enumerate(chunks(load(r, 2))):
                    cs = slice(c * 128, (c + 1) * 128)
                    if c % (NC // 2) == 0:
                        rg = gate16(rs, c, NC)
                    y = ((x - mu) * rg).reshape(LG // 8, 8, 128) * mod_v[j_scale, :, cs][None] + mod_v[j_shift, :, cs][None]
                    dst[r // 2:(r + LG) // 2, cs] = pltpu.bitcast(y.reshape(LG, 128).astype(BF16), U32)
            return staged((s_mean, s_var, s_out), nrows // LG, 1)

        def ln1_items(row0, buf):
            return ln_items(lambda r, k: x_v[pl.ds(pl.multiple_of(zrow(row0 + r, k), LG), LG), :].astype(F32),
                            stat1, bufs[buf][0], TM, 1, 0)

        def x1_rows(row, n, c0, c1):
            xf = x_v[pl.ds(row, n), c0:c1].astype(F32).reshape(n // 8, 8, c1 - c0)
            y = y_v[pl.ds(row, n), c0:c1].reshape(n // 8, 8, c1 - c0)
            return (xf + mod_v[2, :, c0:c1][None] * y).reshape(n, c1 - c0)

        def post_items(row0):
            def load(r, k):
                if k:
                    return x1n[pl.ds(pl.multiple_of(zrow(r, k), LG), LG), :]
                x1 = x1_rows(row0 + r, LG, 0, D)
                x1n[r:r + LG, :] = x1
                return x1
            return ln_items(load, stat2, h2_v, TMB, 4, 3)

        def logit_items(buf, first):
            _, qk, _, _, pb = bufs[buf]
            swap = lane_iota(RG) ^ 1

            def s_logit(g):
                r = g * RG
                qs = [qk[c, HALO + r:HALO + r + RG, :] for c in range(NC)]
                for w in range(WIN):
                    k0 = HALO + r - DIL * w
                    if w >= WIN // 2:
                        k0 = zrow(k0)
                    s = _tree(_add, [qs[c] * qk[NC + c, pl.ds(k0, RG), :] for c in range(NC)])
                    s = gate(s, w, WIN)
                    s = s + pltpu.roll(s, 64, 1)
                    s = s + jnp.take_along_axis(s, swap, axis=1, mode="promise_in_bounds")
                    if first and r < DIL * w:
                        pos = r + jax.lax.broadcasted_iota(jnp.int32, (RG, 128), 0)
                        s = jnp.where(pos >= DIL * w, s, NEG * LOG2E)
                    sls[g % len(sls)][w, pl.ds(pl.multiple_of(zrow(0), RG), RG), :] = s

            def s_soft(g):
                r = g * RG
                ss = [sls[g % len(sls)][w] for w in range(WIN)]
                m = gate(_tree(jnp.maximum, ss), 0, 1)
                es = [jnp.exp2(s - m) for s in ss]
                for w in range(WIN):
                    pb[w, r:r + RG, :] = es[w]
                den = _tree(_add, es)
                inv = pl.reciprocal(den, approx=True)
                pb[WIN, r:r + RG, :] = inv * (2.0 - den * inv)
            return staged((s_logit, s_soft), TM // RG, LLAG)

        def pv_items(buf):
            _, _, vp, o, pb = bufs[buf]

            def one(r):
                ps = [pb[w, r:r + RG, :] for w in range(WIN + 1)]
                for c in range(NC):
                    ks = [HALO + r - DIL * w if w < WIN // 2 else zrow(HALO + r - DIL * w) for w in range(WIN)]
                    acc = _tree(_add, [ps[w] * vp[c, pl.ds(ks[w], RG), :] for w in range(WIN)])
                    acc = gate(acc * ps[WIN], c, NC)
                    if (r // RG) % 2 == 0:
                        otmp[c, pl.ds(pl.multiple_of(zrow(0), 8), RG), :] = acc
                    else:
                        both = jnp.concatenate([otmp[c], acc], axis=0).astype(BF16)
                        o[(r - RG) // 2:(r + RG) // 2, c * 128:(c + 1) * 128] = pltpu.bitcast(both, U32)
            return [functools.partial(one, r) for r in range(0, TM, RG)]

        def halo(buf, prev, part):
            _, qk, vp, _, _ = bufs[buf]
            for c in range(NC):
                if part == 1:
                    qk[NC + c, 0:HALO, :] = (jnp.zeros((HALO, 128), F32) if prev is None
                                             else bufs[prev][1][NC + c, TM:TM + HALO, :])
                else:
                    vp[c, 0:HALO, :] = (jnp.broadcast_to(vp[c, HALO:HALO + 1, :], (HALO, 128)) if prev is None
                                        else bufs[prev][2][c, TM:TM + HALO, :])

        def qkv_part(buf, part):
            h1, qk, vp, _, _ = bufs[buf]

            def sink(n0, r):
                ch = n0 // 128
                dst, ci = (qk, ch) if ch < 2 * NC else (vp, ch - 2 * NC)
                dst[ci, HALO:HALO + TM, :] = r * (SM_SCALE * LOG2E) if ch < NC else r
            matmul(lambda k: ld16(h1, 0, TM, k * KH, (k + 1) * KH),
                   lambda k, n0: ld16(wqkv_p, k * KH, KH, n0, n0 + 128),
                   D // KH, range(part * D, (part + 1) * D, 128), sink)

        def wo_mm(buf, row0):
            o = bufs[buf][3]

            def sink(n0, r):
                y_v[pl.ds(row0, TM), n0:n0 + 128] = r
            matmul(lambda k: ld16(o, 0, TM, k * KH, (k + 1) * KH),
                   lambda k, n0: ld16(wo_p, k * KH, KH, n0, n0 + 128),
                   D // KH, range(0, D, 128), sink)

        UP = NC * (D // KH)

        def run_now(items):
            for fn in items:
                fn()

        def ffn(row0, slot, nxt_row):
            h = ld16(h2_v, 0, TMB, 0, D)
            for f0 in range(0, F, FC):
                g = jnp.dot(h, w1_v[:, f0:f0 + FC], preferred_element_type=F32)
                u = jnp.dot(h, w3_v[:, f0:f0 + FC], preferred_element_type=F32)
                act_v[:, f0:f0 + FC] = pltpu.bitcast((g * jax.nn.sigmoid(g) * u).astype(BF16), U32)
            nk = F // KH
            sched = {}
            place(sched, post_items(nxt_row), range(0, NC * nk - PB1))
            begin(sched)

            def sink(n0, r):
                z = (mod_v[5, :, n0:n0 + 128][None] * r.reshape(TMB // 8, 8, 128)).reshape(TMB, 128)
                obuf[slot, :, n0:n0 + 128] = (x1_rows(row0, TMB, n0, n0 + 128) + z).astype(BF16)
            matmul(lambda k: ld16(act_v, 0, TMB, k * KH, (k + 1) * KH),
                   lambda k, n0: w2_v[k * KH:(k + 1) * KH, n0:n0 + 128],
                   nk, range(0, D, 128), sink)

        with jax.named_scope("prologue"):
            zs[0] = 0
            begin({})
            cp_x(0, 2).start()
            cp_qkv(0).start()
            cp_mod(1).start()
            cb_v[0:D, :] = jnp.broadcast_to(silu_c().astype(F32), (128, D)).T
            cp_x(0, 2).wait()
            cp_mod(0).start()
            cp_qkv(0).wait()
            cp_qkv(1).start()

            def perm_body(i, carry):
                perm_qkv(0, i, 128)
                return carry
            jax.lax.fori_loop(0, D // 128, perm_body, 0)
            cp_mod(1).wait()
            cp_qkv(2).start()
            mod_mxu(1, True)
            cp_mod(0).wait()
            cp_x(2).start()
            cp_wo().start()
            mod_mxu(0, False)
            run_now(ln1_items(0, "a"))
            run_now(ln1_items(TM, "b"))
            halo("a", None, 1)

        with jax.named_scope("step0"):
            begin({})
            qkv_part("a", 0)
            cp_qkv(1).wait()
            cp_x(3, 2).start()
            sched = {}
            place(sched, perm_qkv_items(1), range(0, UP - 2))
            begin(sched)
            qkv_part("b", 0)
            qkv_part("a", 1)
            cp_qkv(2).wait()
            cp_mod(2).start()
            sched = {}
            place(sched, perm_qkv_items(2), range(0, UP - 2))
            place(sched, logit_items("a", True), range(UP - 2, 2 * UP - L1))
            begin(sched)
            halo("b", "a", 1)
            qkv_part("b", 1)
            qkv_part("a", 2)
            finish()
            halo("a", None, 2)
            cp_x(2).wait()
            cp_wo().wait()
            cp_x(5, NB - 5).start()
            sched = {}
            place(sched, pv_items("a"), range(0, UP - 2))
            place(sched, perm_wo_items(), range(0, UP - 2))
            place(sched, ln1_items(2 * TM, "a"), range(0, UP + 4))
            place(sched, logit_items("b", False), range(UP - 2, 2 * UP - L1))
            begin(sched)
            halo("b", "a", 2)
            qkv_part("b", 2)
            wo_mm("a", 0)
            finish()
            cp_x(3, 2).wait()
            cp_mod(3, 3).start()


        def half(X, Y, u0, sched, row_ln1, row_wo, extra):
            place(sched, pv_items(Y), range(u0 + P0, u0 + 3 * UP - P1))
            place(sched, logit_items(X, False), range(u0 + 2 * UP + L0, u0 + 4 * UP - L1))
            place(sched, ln1_items(row_ln1, Y), range(u0 + N0, u0 + N1))
            if extra:
                place(sched, extra, range(u0, u0 + 4 * UP - 1))

            def run():
                halo(X, Y, 1)
                halo(X, Y, 2)
                for part in range(3):
                    qkv_part(X, part)
                wo_mm(Y, row_wo)
            return run

        def a_step(s, carry):
            @pl.when(s == 2)
            def _():
                cp_mod(2).wait()
                cp_x(5, NB - 5).wait()
                cp_ffn(0).start()
                cp_ffn(1).start()

            @pl.when(s == 3)
            def _():
                cp_mod(3, 3).wait()
                cp_ffn(2).start()

            ra = pl.multiple_of(2 * s * TM, TM)
            nxt = pl.multiple_of(jnp.minimum(ra + 2 * TM, S - TM), TM)
            col0 = pl.multiple_of(jnp.minimum(2 * D + (s - 2) * (MT * 128), 6 * D - MT * 128), 128)
            mi = mod_items(col0, MT)
            sched = {}
            run_a = half("a", "b", 0, sched, ra + TM, ra - TM, mi[:len(mi) // 2])
            run_b = half("b", "a", 4 * UP, sched, nxt, ra, mi[len(mi) // 2:])
            begin(sched)
            run_a()
            run_b()
            finish()
            return carry

        with jax.named_scope("aloop"):
            if SKIP_A:
                cp_mod(2).wait()
                cp_x(5, NB - 5).wait()
                cp_mod(3, 3).wait()
                for k in range(3):
                    cp_ffn(k).start()
            else:
                jax.lax.fori_loop(1, NB // 2, a_step, 0)

        with jax.named_scope("atail"):
            for j in range(4):
                r = _tree(_add, [modp_v[i, :, (2 + j) * D:(3 + j) * D] for i in range(NSUB)])
                r = jnp.sum(r, axis=0, keepdims=True)
                mod_v[2 + j] = jnp.broadcast_to(r + 1.0 if j == 2 else r, (8, D))
            begin({})
            run_now(pv_items("b"))
            sched = {}
            place(sched, post_items(0), range(0, UP - 2))
            begin(sched)
            wo_mm("b", S - TM)
            finish()
            for k in range(3):
                cp_ffn(k).wait()

        def b_step(j, carry):
            slot = j % 2

            @pl.when(j >= 2)
            def _():
                cp_out(j - 2, slot).wait()

            row0 = pl.multiple_of(j * TMB, TMB)
            nxt = pl.multiple_of(jnp.minimum(row0 + TMB, S - TMB), TMB)
            if SKIP_FFN:
                obuf[slot] = x1_rows(row0, TMB, 0, D).astype(BF16)
            else:
                ffn(row0, slot, nxt)
            cp_out(j, slot).start()
            return carry

        with jax.named_scope("bloop"):
            jax.lax.fori_loop(0, NBB, b_step, 0)
        with jax.named_scope("tail"):
            cp_out(NBB - 2, (NBB - 2) % 2).wait()
            cp_out(NBB - 1, (NBB - 1) % 2).wait()

    any_spec = pl.BlockSpec(memory_space=pl.ANY)
    scratch = [
        pltpu.VMEM((S, D), BF16),
        pltpu.VMEM((D, 3 * D), BF16),
        pltpu.VMEM((D // 2, 3 * D), U32),
        pltpu.VMEM((D, D), BF16),
        pltpu.VMEM((NC, D // 2, 128), U32),
        pltpu.VMEM((D // 2, D), U32),
        pltpu.VMEM((D, F), BF16),
        pltpu.VMEM((D, F), BF16),
        pltpu.VMEM((F, D), BF16),
        pltpu.VMEM((D, 6 * D), BF16),
        pltpu.VMEM((D, 128), F32),
        pltpu.VMEM((NSUB, 8, 6 * D), F32),
        pltpu.VMEM((6, 8, D), F32),
        pltpu.VMEM((TM // 2, D), U32),
        pltpu.VMEM((TM // 2, D), U32),
        pltpu.VMEM((2 * NC, KV, 128), F32),
        pltpu.VMEM((NC, KV, 128), F32),
        pltpu.VMEM((WIN + 1, TM, 128), F32),
        pltpu.VMEM((2 * NC, KV, 128), F32),
        pltpu.VMEM((NC, KV, 128), F32),
        pltpu.VMEM((WIN + 1, TM, 128), F32),
        pltpu.VMEM((TM // 2, D), U32),
        pltpu.VMEM((TM // 2, D), U32),
        pltpu.VMEM((NC, RG, 128), F32),
        pltpu.VMEM((WIN, RG, 128), F32),
        pltpu.VMEM((WIN, RG, 128), F32),
        pltpu.VMEM((WIN, RG, 128), F32),
        pltpu.VMEM((2, TM, 128), F32),
        pltpu.VMEM((2, TMB, 128), F32),
        pltpu.VMEM((S, D), F32),
        pltpu.VMEM((TMB, D), F32),
        pltpu.VMEM((TMB // 2, D), U32),
        pltpu.VMEM((TMB // 2, F), U32),
        pltpu.VMEM((2, TMB, D), BF16),
        pltpu.SMEM((1,), jnp.int32),
        pltpu.SemaphoreType.DMA((4,)),
        pltpu.SemaphoreType.DMA((11,)),
        pltpu.SemaphoreType.DMA((2,)),
    ]

    def call(A_x, A_wqkv, A_wo, B_w1, B_w3, B_w2, c, w_mod):
        return pl.pallas_call(
            kernel,
            out_shape=jax.ShapeDtypeStruct((1, S, D), BF16),
            in_specs=[any_spec] * 6 + [pl.BlockSpec(memory_space=pltpu.VMEM), any_spec],
            out_specs=any_spec,
            scratch_shapes=scratch,
            compiler_params=pltpu.CompilerParams(vmem_limit_bytes=120 * 1024 * 1024),
        )(A_x, A_wqkv, A_wo, B_w1, B_w3, B_w2, c, w_mod)

    return call


@jax.jit
def pallas_adaLN_cond__sliding_local_dilated__glu_gated_swiglu__prompt_kernel(
    A_x: jax.Array,
    A_wqkv: jax.Array,
    A_wo: jax.Array,
    B_x: jax.Array,
    B_w1: jax.Array,
    B_w3: jax.Array,
    B_w2: jax.Array,
    c: jax.Array,
    w_mod: jax.Array,
):
    del B_x
    return _build()(A_x, A_wqkv, A_wo, B_w1, B_w3, B_w2, c, w_mod)
```

```python
import functools
import math

import jax
import jax.numpy as jnp
import jax.experimental.pallas as pl
import jax.experimental.pallas.tpu as pltpu

S = 2048
D = 1024
F = 3584
H = 32
DH = D // H
WIN = 8
DIL = 2
NC = D // 128
HALO = 16
EPS = 1e-5
NEG = -1000000000.0
SM_SCALE = DH ** -0.5
LOG2E = math.log2(math.e)

TM = 128
NB = S // TM
KV = HALO + TM
RG = 8
LG = 16
NS = 4
NDMA = 19
KH = 512

F32 = jnp.float32
BF16 = jnp.bfloat16
U32 = jnp.uint32


def _tree(op, xs):
    xs = list(xs)
    while len(xs) > 1:
        xs = [op(xs[i], xs[i + 1]) if i + 1 < len(xs) else xs[i] for i in range(0, len(xs), 2)]
    return xs[0]


def _add(a, b):
    return a + b


def _build(TMB=128, FC=512, GATE=True, SKIP_FFN=False, SKIP_A=False,
           SCH=0, MT=6, NSUB=16, PB1=5, L0=0, L1=1, SPREAD=128, LLAG=3,
           P0=0, P1=16, N0=1, N1=30, PR=64):
    NBB = S // TMB

    def kernel(x_hbm, wqkv_hbm, wo_hbm, w1_hbm, w3_hbm, w2_hbm, c_ref, wmod_hbm,
               out_hbm,
               x_v, wqkv_v, wqkv_p, wo_v, wo_tmp, wo_p, w1_v, w3_v, w2_v, wmod_v, cb_v, modp_v, mod_v,
               h1a, h1b, h1s, part, stats, qka, va, pa, qkb, vb, pb_, oa, ob, otmp, sl0, sl1, sl2, stat1, stat2, y_v, x1n, h2_v, act_v, obuf,
               zs, sem_w, sem_o):
        bufs = {"a": (h1a, qka, va, oa, pa), "b": (h1b, qkb, vb, ob, pb_)}

        sls = (sl0, sl1, sl2)

        dmas = {}

        def add_dma(name, src, dst):
            dmas[name] = (src, dst, len(dmas))

        for name, (b0, b1) in (("x0", (0, NS)), ("x1", (NS, NS + 3)), ("x2", (NS + 3, NB))):
            rows = pl.ds(b0 * TM, (b1 - b0) * TM)
            add_dma(name, x_hbm.at[0, rows, :], x_v.at[rows, :])
        for name, (c0, c1) in (("sa0", (0, KH)), ("sa1", (KH, D)), ("ca0", (D, D + KH)), ("ca1", (D + KH, 2 * D)),
                               ("m2", (2 * D, 3 * D)), ("m3", (3 * D, 6 * D))):
            cols = pl.ds(c0, c1 - c0)
            add_dma(name, wmod_hbm.at[:, cols], wmod_v.at[:, cols])
        for g in range(3):
            for k in range(2):
                rows, cols = pl.ds(k * KH, KH), pl.ds(g * D, D)
                add_dma("qkv"[g] + str(k), wqkv_hbm.at[rows, cols], wqkv_v.at[rows, cols])
        add_dma("wo", wo_hbm, wo_v)
        add_dma("w1", w1_hbm, w1_v)
        add_dma("w3", w3_hbm, w3_v)
        add_dma("w2", w2_hbm, w2_v)
        assert len(dmas) == NDMA

        def cp(name):
            src, dst, i = dmas[name]
            return pltpu.make_async_copy(src, dst, sem_w.at[i])

        def start(*names):
            for n in names:
                cp(n).start()

        def wait(*names):
            for n in names:
                cp(n).wait()

        def cp_out(j, slot):
            return pltpu.make_async_copy(obuf.at[slot],
                                         out_hbm.at[0, pl.ds(j * TMB, TMB), :], sem_o.at[slot])

        st = {"z": None, "never": None, "clock": 0, "sched": {}, "tok": None}

        def begin(sched):
            z = zs[0]
            st.update(z=z, never=jnp.full((8, 128), z, jnp.int32) != 0, clock=0, sched=sched, tok=None)

        def gate(val, i, n):
            r = st["tok"]
            if r is None or not GATE:
                return val
            row = (i * SPREAD // n) // 8 * 8
            t = r[row:row + 8]
            return jnp.where(st["never"], t if val.dtype == F32 else pltpu.bitcast(t, val.dtype), val)

        def place(sched, items, units):
            units = list(units)
            for i, it in enumerate(items):
                sched.setdefault(units[(i * len(units)) // len(items)], []).append(it)

        def matmul(lhs_fn, w_fn, ks, cols, sink):
            for n0 in cols:
                r = None
                for k in ks:
                    d = jnp.dot(lhs_fn(k), w_fn(k, n0), preferred_element_type=F32)
                    r = d if r is None else r + d
                    if k == ks[-1]:
                        sink(n0, r)
                    st["tok"] = r
                    for fn in st["sched"].pop(st["clock"], []):
                        fn()
                    st["tok"] = None
                    st["clock"] += 1

        def finish():
            assert not st["sched"]

        def lane_iota(rows):
            return jax.lax.broadcasted_iota(jnp.int32, (rows, 128), 1)

        def ld16(ref, r0, n, c0, c1):
            return pltpu.bitcast(ref[r0 // 2:(r0 + n) // 2, c0:c1], BF16)

        def silu_c():
            cf = c_ref[...].astype(F32)
            return (cf * jax.nn.sigmoid(cf)).astype(BF16)

        def mod_mxu(j, k):
            cs = slice(k * KH, (k + 1) * KH)
            lhs = jnp.broadcast_to(silu_c(), (16, D))
            r = jnp.dot(lhs, wmod_v[:, j * D + k * KH:j * D + (k + 1) * KH], preferred_element_type=F32)[0:8]
            mod_v[j, :, cs] = r + 1.0 if j in (1, 4) else r

        def mod_finish(j, c0, c1):
            r = _tree(_add, [modp_v[i, :, j * D + c0:j * D + c1] for i in range(NSUB)])
            r = jnp.sum(r, axis=0, keepdims=True)
            mod_v[j, :, c0:c1] = jnp.broadcast_to(r + 1.0 if j in (1, 4) else r, (8, c1 - c0))

        def mod_items(col0, ntiles):
            rows = D // NSUB

            def one(t, i):
                c0 = col0 + t * 128
                c0 = c0 if isinstance(c0, int) else pl.multiple_of(c0, 128)
                w = wmod_v[i * rows:(i + 1) * rows, pl.ds(c0, 128)].astype(F32)
                p = (w * cb_v[i * rows:(i + 1) * rows, :]).reshape(rows // 8, 8, 128)
                modp_v[i, :, pl.ds(c0, 128)] = gate(_tree(_add, [p[k] for k in range(rows // 8)]), 1, 2)
            return [functools.partial(one, t, i) for t in range(ntiles) for i in range(NSUB)]

        def perm_qkv(g, i, nrows):
            n = nrows // 2
            r0, p0 = i * nrows, i * n
            l = lane_iota(n)
            vals = [pltpu.bitcast(wqkv_v[pl.ds(r0, nrows), g * D + c * 128: g * D + (c + 1) * 128], U32)
                    for c in range(NC)]
            for b in range(3):
                m = ((l >> (2 + b)) & 1) == 0
                for c in range(NC):
                    if c & (1 << b):
                        continue
                    lo, hi = vals[c], vals[c | (1 << b)]
                    vals[c] = jnp.where(m, lo, hi)
                    vals[c | (1 << b)] = jnp.where(m, hi, lo)
            for j in range(NC):
                idx = ((((l >> 1) & 3) << 5) | ((((l >> 3) & 7) ^ j) << 2)
                       | ((l >> 6) << 1) | (l & 1))
                v = jnp.concatenate([gate(vals[j][q:q + 8], j, NC) for q in range(0, n, 8)], axis=0)
                t = jnp.take_along_axis(v, idx, axis=1, mode="promise_in_bounds")
                wqkv_p[pl.ds(p0, n), g * D + j * 128: g * D + (j + 1) * 128] = t

        def perm_qkv_items(g, k, nrows=PR):
            n = KH // nrows
            return [functools.partial(perm_qkv, g, i, nrows) for i in range(k * n, (k + 1) * n)]

        def perm_wo_items():
            low = jax.lax.broadcasted_iota(jnp.int32, (8, 128), 0) < 4

            def one(c):
                for r in range(0, D // 2, 8):
                    wo_tmp[c, r:r + 8, :] = gate(pltpu.bitcast(
                        wo_v[2 * r:2 * r + 16, c * 128:(c + 1) * 128], U32), r, D // 2)
                for G in range(64):
                    j, e, ch = G >> 3, (G >> 2) & 1, G & 3
                    dd = (((2 * ch) ^ j) << 1) | e
                    ta = wo_tmp[c, pl.ds(ch * 128 + dd, 8, stride=16), :]
                    tb = wo_tmp[c, pl.ds(ch * 128 + (dd ^ 2), 8, stride=16), :]
                    wo_p[G * 8:(G + 1) * 8, c * 128:(c + 1) * 128] = jnp.where(low, ta, tb)
            return [functools.partial(one, c) for c in range(NC)]

        def zrow(row, k=1):
            return row + k * st["z"]

        def gate16(v, i, n):
            return jnp.concatenate([gate(v[q:q + 8], i, n) for q in range(0, LG, 8)], axis=0)

        def staged(stages, n, lag):
            items = []
            for t in range(n + lag * (len(stages) - 1)):
                for k in reversed(range(len(stages))):
                    if 0 <= t - k * lag < n:
                        items.append(functools.partial(stages[k], t - k * lag))
            return items

        def ln_stages(load, stat, dst, j_scale, j_shift, cols=range(NC)):
            def chunks(x):
                return [x[:, c * 128:(c + 1) * 128] for c in range(NC)]

            def put(j, r, part, fn):
                m = jnp.sum(part, axis=-1, keepdims=True) * (1.0 / D)
                stat[j, pl.ds(pl.multiple_of(zrow(r), LG), LG), :] = jnp.broadcast_to(fn(m), (LG, 128))

            def s_mean(i):
                put(0, i * LG, gate16(_tree(_add, chunks(load(i * LG, 0))), 1, 2), lambda m: m)

            def s_var(i):
                r = i * LG
                mu = gate16(stat[0, r:r + LG, :], 0, 1)
                put(1, r, _tree(_add, [(x - mu) * (x - mu) for x in chunks(load(r, 1))]),
                    lambda m: jax.lax.rsqrt(m + EPS))

            def s_out(i):
                r = i * LG
                mu, rs = stat[0, r:r + LG, :], stat[1, r:r + LG, :]
                xs = chunks(load(r, 2))
                for c in cols:
                    x, cs = xs[c], slice(c * 128, (c + 1) * 128)
                    if c % (NC // 2) == 0:
                        rg = gate16(rs, c - cols[0], NC)
                    y = ((x - mu) * rg).reshape(LG // 8, 8, 128) * mod_v[j_scale, :, cs][None] + mod_v[j_shift, :, cs][None]
                    dst[r // 2:(r + LG) // 2, cs] = pltpu.bitcast(y.reshape(LG, 128).astype(BF16), U32)
            return s_mean, s_var, s_out

        def load_x(row0):
            return lambda r, k: x_v[pl.ds(pl.multiple_of(zrow(row0 + r, k), LG), LG), :].astype(F32)

        def ln1_items(row0, buf):
            return staged(ln_stages(load_x(row0), stat1, bufs[buf][0], 1, 0), TM // LG, 1)

        def ln1_start(b, k):
            return ln_stages(load_x(b * TM), stats.at[:, pl.ds(b * TM, TM), :], h1s.at[b], 1, 0,
                             range(k * NC // 2, (k + 1) * NC // 2))

        def ln1_out_items(b, k):
            return [functools.partial(ln1_start(b, k)[2], i) for i in range(TM // LG)]

        def x1_rows(row, n, c0, c1):
            xf = x_v[pl.ds(row, n), c0:c1].astype(F32).reshape(n // 8, 8, c1 - c0)
            y = y_v[pl.ds(row, n), c0:c1].reshape(n // 8, 8, c1 - c0)
            return (xf + mod_v[2, :, c0:c1][None] * y).reshape(n, c1 - c0)

        def post_items(row0):
            def load(r, k):
                if k:
                    return x1n[pl.ds(pl.multiple_of(zrow(r, k), LG), LG), :]
                x1 = x1_rows(row0 + r, LG, 0, D)
                x1n[r:r + LG, :] = x1
                return x1
            return staged(ln_stages(load, stat2, h2_v, 4, 3), TMB // LG, 1)

        def logit_items(buf, first):
            _, qk, _, _, pb = bufs[buf]
            swap = lane_iota(RG) ^ 1

            def s_logit(g):
                r = g * RG
                qs = [qk[c, HALO + r:HALO + r + RG, :] for c in range(NC)]
                for w in range(WIN):
                    k0 = HALO + r - DIL * w
                    if w >= WIN // 2:
                        k0 = zrow(k0)
                    s = _tree(_add, [qs[c] * qk[NC + c, pl.ds(k0, RG), :] for c in range(NC)])
                    s = gate(s, w, WIN)
                    s = s + pltpu.roll(s, 64, 1)
                    s = s + jnp.take_along_axis(s, swap, axis=1, mode="promise_in_bounds")
                    if first and r < DIL * w:
                        pos = r + jax.lax.broadcasted_iota(jnp.int32, (RG, 128), 0)
                        s = jnp.where(pos >= DIL * w, s, NEG * LOG2E)
                    sls[g % len(sls)][w, pl.ds(pl.multiple_of(zrow(0), RG), RG), :] = s

            def s_soft(g):
                r = g * RG
                ss = [sls[g % len(sls)][w] for w in range(WIN)]
                m = gate(_tree(jnp.maximum, ss), 0, 1)
                es = [jnp.exp2(s - m) for s in ss]
                for w in range(WIN):
                    pb[w, r:r + RG, :] = es[w]
                den = _tree(_add, es)
                inv = pl.reciprocal(den, approx=True)
                pb[WIN, r:r + RG, :] = inv * (2.0 - den * inv)
            return staged((s_logit, s_soft), TM // RG, LLAG)

        def pv_items(buf):
            _, _, vp, o, pb = bufs[buf]

            def one(r):
                ps = [pb[w, r:r + RG, :] for w in range(WIN + 1)]
                for c in range(NC):
                    ks = [HALO + r - DIL * w if w < WIN // 2 else zrow(HALO + r - DIL * w) for w in range(WIN)]
                    acc = _tree(_add, [ps[w] * vp[c, pl.ds(ks[w], RG), :] for w in range(WIN)])
                    acc = gate(acc * ps[WIN], c, NC)
                    if (r // RG) % 2 == 0:
                        otmp[c, pl.ds(pl.multiple_of(zrow(0), 8), RG), :] = acc
                    else:
                        both = jnp.concatenate([otmp[c], acc], axis=0).astype(BF16)
                        o[(r - RG) // 2:(r + RG) // 2, c * 128:(c + 1) * 128] = pltpu.bitcast(both, U32)
            return [functools.partial(one, r) for r in range(0, TM, RG)]

        def halo(buf, prev, part):
            _, qk, vp, _, _ = bufs[buf]
            for c in range(NC):
                if part == 1:
                    qk[NC + c, 0:HALO, :] = (jnp.zeros((HALO, 128), F32) if prev is None
                                             else bufs[prev][1][NC + c, TM:TM + HALO, :])
                else:
                    vp[c, 0:HALO, :] = (jnp.broadcast_to(vp[c, HALO:HALO + 1, :], (HALO, 128)) if prev is None
                                        else bufs[prev][2][c, TM:TM + HALO, :])

        def qkv_part(buf, g, sb=None, k=None):
            h1, qk, vp, _, _ = bufs[buf] if buf else (None,) * 5
            if sb is not None:
                h1 = h1s.at[sb]

            def sink(n0, r):
                ch = n0 // 128
                if k == 0:
                    part[sb, ch] = r
                    return
                if k == 1:
                    r = r + part[sb, ch]
                dst, ci = (qk, ch) if ch < 2 * NC else (vp, ch - 2 * NC)
                dst[ci, HALO:HALO + TM, :] = r * (SM_SCALE * LOG2E) if ch < NC else r
            matmul(lambda kk: ld16(h1, 0, TM, kk * KH, (kk + 1) * KH),
                   lambda kk, n0: ld16(wqkv_p, kk * KH, KH, n0, n0 + 128),
                   (0, 1) if k is None else (k,), range(g * D, (g + 1) * D, 128), sink)

        def wo_mm(buf, row0):
            o = bufs[buf][3]

            def sink(n0, r):
                y_v[pl.ds(row0, TM), n0:n0 + 128] = r
            matmul(lambda k: ld16(o, 0, TM, k * KH, (k + 1) * KH),
                   lambda k, n0: ld16(wo_p, k * KH, KH, n0, n0 + 128),
                   (0, 1), range(0, D, 128), sink)

        UP = NC * (D // KH)

        def run_now(items):
            for fn in items:
                fn()

        def ffn(row0, slot, nxt_row):
            h = ld16(h2_v, 0, TMB, 0, D)
            for f0 in range(0, F, FC):
                g = jnp.dot(h, w1_v[:, f0:f0 + FC], preferred_element_type=F32)
                u = jnp.dot(h, w3_v[:, f0:f0 + FC], preferred_element_type=F32)
                act_v[:, f0:f0 + FC] = pltpu.bitcast((g * jax.nn.sigmoid(g) * u).astype(BF16), U32)
            nk = F // KH
            sched = {}
            place(sched, post_items(nxt_row), range(0, NC * nk - PB1))
            begin(sched)

            def sink(n0, r):
                z = (mod_v[5, :, n0:n0 + 128][None] * r.reshape(TMB // 8, 8, 128)).reshape(TMB, 128)
                obuf[slot, :, n0:n0 + 128] = (x1_rows(row0, TMB, n0, n0 + 128) + z).astype(BF16)
            matmul(lambda k: ld16(act_v, 0, TMB, k * KH, (k + 1) * KH),
                   lambda k, n0: w2_v[k * KH:(k + 1) * KH, n0:n0 + 128],
                   tuple(range(nk)), range(0, D, 128), sink)

        U8 = NC

        def segment(*placements):
            sched = {}
            for items, units in placements:
                place(sched, items, units)
            begin(sched)

        with jax.named_scope("prologue"):
            zs[0] = 0
            begin({})
            start("x0", "ca0")
            cb_v[...] = jnp.broadcast_to(silu_c().astype(F32), (128, D)).T
            wait("x0")
            start("q0")
            for b in range(NS):
                s_mean, s_var, _ = ln1_start(b, 0)
                run_now(staged((s_mean, s_var), TM // LG, 4))
            wait("ca0")
            start("sa0")
            mod_mxu(1, 0)
            wait("q0")
            start("k0")
            run_now(perm_qkv_items(0, 0))
            wait("sa0")
            start("v0")
            mod_mxu(0, 0)
            run_now(ln1_out_items(0, 0))

        with jax.named_scope("pass1"):
            segment((ln1_out_items(1, 0), range(0, U8 - 2)),
                    (ln1_out_items(2, 0) + ln1_out_items(3, 0), range(U8 - 2, 2 * U8)))
            qkv_part(None, 0, 0, 0)
            qkv_part(None, 0, 1, 0)
            wait("k0")
            start("ca1", "sa1")
            segment((perm_qkv_items(1, 0), range(0, 2 * U8 - 2)))
            for g, b in ((0, 2), (0, 3), (1, 0), (1, 1)):
                qkv_part(None, g, b, 0)
            wait("v0", "ca1")
            start("q1", "k1")
            segment((perm_qkv_items(2, 0), range(0, 2 * U8 - 2)),
                    (mod_items(D + KH, 4) + [functools.partial(mod_finish, 1, KH, D)], range(2 * U8 - 2, 4 * U8)))
            for g, b in ((1, 2), (1, 3), (2, 0), (2, 1)):
                qkv_part(None, g, b, 0)
            wait("sa1", "q1")
            start("v1", "wo")
            segment((mod_items(KH, 4) + [functools.partial(mod_finish, 0, KH, D)], range(0, U8 + 2)),
                    (perm_qkv_items(0, 1), range(0, 2 * U8 - 2)),
                    (ln1_out_items(0, 1), range(U8 + 3, 2 * U8 - 1)))
            qkv_part(None, 2, 2, 0)
            qkv_part(None, 2, 3, 0)

        with jax.named_scope("pass2"):
            wait("k1")
            start("x1")
            segment((perm_qkv_items(1, 1), range(0, U8 - 2)),
                    (ln1_out_items(1, 1), range(0, U8)))
            halo("a", None, 1)
            qkv_part("a", 0, 0, 1)
            wait("v1")
            start("m2")
            la = logit_items("a", True)
            segment((perm_qkv_items(2, 1), range(0, U8 - 2)),
                    (la, range(U8, 3 * U8 + 4)),
                    (pv_items("a"), range(2 * U8 + 4, 4 * U8)),
                    (ln1_out_items(2, 1) + ln1_out_items(3, 1), range(U8, 4 * U8)))
            qkv_part("a", 1, 0, 1)
            qkv_part("a", 2, 0, 1)
            halo("a", None, 2)
            halo("b", "a", 1)
            halo("b", "a", 2)
            qkv_part("b", 0, 1, 1)
            qkv_part("b", 1, 1, 1)
            wait("wo", "x1")
            start("x2")
            segment((perm_wo_items(), range(0, U8 - 1)),
                    (logit_items("b", False), range(0, 3 * U8 + 4)),
                    (pv_items("b"), range(3 * U8 + 2, 6 * U8 - 1)),
                    (logit_items("a", False), range(5 * U8, 8 * U8 + 4)),
                    (pv_items("a"), range(8 * U8 + 2, 11 * U8 - 1)),
                    (ln1_items(NS * TM, "a"), range(8 * U8 + 4, 10 * U8)),
                    (logit_items("b", False), range(10 * U8, 13 * U8 - L1)))
            qkv_part("b", 2, 1, 1)
            wo_mm("a", 0)
            for X, Y, b in (("a", "b", 2), ("b", "a", 3)):
                halo(X, Y, 1)
                halo(X, Y, 2)
                for g in range(3):
                    qkv_part(X, g, b, 1)
                wo_mm(Y, (b - 1) * TM)
            finish()
            wait("m2")
            start("m3")


        def half(X, Y, u0, sched, row_ln1, row_wo, extra):
            place(sched, pv_items(Y), range(u0 + P0, u0 + 3 * UP - P1))
            place(sched, logit_items(X, False), range(u0 + 2 * UP + L0, u0 + 4 * UP - L1))
            place(sched, ln1_items(row_ln1, Y), range(u0 + N0, u0 + N1))
            if extra:
                place(sched, extra, range(u0, u0 + 4 * UP - 1))

            def run():
                halo(X, Y, 1)
                halo(X, Y, 2)
                for g in range(3):
                    qkv_part(X, g)
                wo_mm(Y, row_wo)
            return run

        def a_step(s, carry):
            @pl.when(s == 2)
            def _():
                start("w1")

            @pl.when(s == 3)
            def _():
                wait("x2", "m3")
                start("w3")

            @pl.when(s == 4)
            def _():
                start("w2")

            ra = pl.multiple_of(2 * s * TM, TM)
            nxt = pl.multiple_of(jnp.minimum(ra + 2 * TM, S - TM), TM)
            col0 = pl.multiple_of(jnp.minimum(2 * D + (s - 2) * (MT * 128), 6 * D - MT * 128), 128)
            mi = mod_items(col0, MT)
            sched = {}
            run_a = half("a", "b", 0, sched, ra + TM, ra - TM, mi[:len(mi) // 2])
            run_b = half("b", "a", 4 * UP, sched, nxt, ra, mi[len(mi) // 2:])
            begin(sched)
            run_a()
            run_b()
            finish()
            return carry

        with jax.named_scope("aloop"):
            if SKIP_A:
                wait("x2", "m3")
                start("w1", "w3", "w2")
            else:
                jax.lax.fori_loop(NS // 2, NB // 2, a_step, 0)

        with jax.named_scope("atail"):
            begin({})
            for j in range(2, 6):
                mod_finish(j, 0, D)
            run_now(pv_items("b"))
            sched = {}
            place(sched, post_items(0), range(0, UP - 2))
            begin(sched)
            wo_mm("b", S - TM)
            finish()
            wait("w1", "w3", "w2")

        def b_step(j, carry):
            slot = j % 2

            @pl.when(j >= 2)
            def _():
                cp_out(j - 2, slot).wait()

            row0 = pl.multiple_of(j * TMB, TMB)
            nxt = pl.multiple_of(jnp.minimum(row0 + TMB, S - TMB), TMB)
            if SKIP_FFN:
                obuf[slot] = x1_rows(row0, TMB, 0, D).astype(BF16)
            else:
                ffn(row0, slot, nxt)
            cp_out(j, slot).start()
            return carry

        with jax.named_scope("bloop"):
            jax.lax.fori_loop(0, NBB, b_step, 0)
        with jax.named_scope("tail"):
            cp_out(NBB - 2, (NBB - 2) % 2).wait()
            cp_out(NBB - 1, (NBB - 1) % 2).wait()

    any_spec = pl.BlockSpec(memory_space=pl.ANY)
    scratch = [
        pltpu.VMEM((S, D), BF16),
        pltpu.VMEM((D, 3 * D), BF16),
        pltpu.VMEM((D // 2, 3 * D), U32),
        pltpu.VMEM((D, D), BF16),
        pltpu.VMEM((NC, D // 2, 128), U32),
        pltpu.VMEM((D // 2, D), U32),
        pltpu.VMEM((D, F), BF16),
        pltpu.VMEM((D, F), BF16),
        pltpu.VMEM((F, D), BF16),
        pltpu.VMEM((D, 6 * D), BF16),
        pltpu.VMEM((D, 128), F32),
        pltpu.VMEM((NSUB, 8, 6 * D), F32),
        pltpu.VMEM((6, 8, D), F32),
        pltpu.VMEM((TM // 2, D), U32),
        pltpu.VMEM((TM // 2, D), U32),
        pltpu.VMEM((NS, TM // 2, D), U32),
        pltpu.VMEM((NS, 3 * NC, TM, 128), F32),
        pltpu.VMEM((2, NS * TM, 128), F32),
        pltpu.VMEM((2 * NC, KV, 128), F32),
        pltpu.VMEM((NC, KV, 128), F32),
        pltpu.VMEM((WIN + 1, TM, 128), F32),
        pltpu.VMEM((2 * NC, KV, 128), F32),
        pltpu.VMEM((NC, KV, 128), F32),
        pltpu.VMEM((WIN + 1, TM, 128), F32),
        pltpu.VMEM((TM // 2, D), U32),
        pltpu.VMEM((TM // 2, D), U32),
        pltpu.VMEM((NC, RG, 128), F32),
        pltpu.VMEM((WIN, RG, 128), F32),
        pltpu.VMEM((WIN, RG, 128), F32),
        pltpu.VMEM((WIN, RG, 128), F32),
        pltpu.VMEM((2, TM, 128), F32),
        pltpu.VMEM((2, TMB, 128), F32),
        pltpu.VMEM((S, D), F32),
        pltpu.VMEM((TMB, D), F32),
        pltpu.VMEM((TMB // 2, D), U32),
        pltpu.VMEM((TMB // 2, F), U32),
        pltpu.VMEM((2, TMB, D), BF16),
        pltpu.SMEM((1,), jnp.int32),
        pltpu.SemaphoreType.DMA((NDMA,)),
        pltpu.SemaphoreType.DMA((2,)),
    ]

    def call(A_x, A_wqkv, A_wo, B_w1, B_w3, B_w2, c, w_mod):
        return pl.pallas_call(
            kernel,
            out_shape=jax.ShapeDtypeStruct((1, S, D), BF16),
            in_specs=[any_spec] * 6 + [pl.BlockSpec(memory_space=pltpu.VMEM), any_spec],
            out_specs=any_spec,
            scratch_shapes=scratch,
            compiler_params=pltpu.CompilerParams(vmem_limit_bytes=120 * 1024 * 1024),
        )(A_x, A_wqkv, A_wo, B_w1, B_w3, B_w2, c, w_mod)

    return call


@jax.jit
def pallas_adaLN_cond__sliding_local_dilated__glu_gated_swiglu__prompt_kernel(
    A_x: jax.Array,
    A_wqkv: jax.Array,
    A_wo: jax.Array,
    B_x: jax.Array,
    B_w1: jax.Array,
    B_w3: jax.Array,
    B_w2: jax.Array,
    c: jax.Array,
    w_mod: jax.Array,
):
    del B_x
    return _build()(A_x, A_wqkv, A_wo, B_w1, B_w3, B_w2, c, w_mod)
```

```python
import functools
import math

import jax
import jax.numpy as jnp
import jax.experimental.pallas as pl
import jax.experimental.pallas.tpu as pltpu

S = 2048
D = 1024
F = 3584
H = 32
DH = D // H
WIN = 8
DIL = 2
NC = D // 128
HALO = 16
EPS = 1e-5
NEG = -1000000000.0
SM_SCALE = DH ** -0.5
LOG2E = math.log2(math.e)

TM = 128
NB = S // TM
KV = HALO + TM
RG = 8
LG = 16
NS = 4
NDMA = 20
KH = 512

F32 = jnp.float32
BF16 = jnp.bfloat16
U32 = jnp.uint32


def _tree(op, xs):
    xs = list(xs)
    while len(xs) > 1:
        xs = [op(xs[i], xs[i + 1]) if i + 1 < len(xs) else xs[i] for i in range(0, len(xs), 2)]
    return xs[0]


def _add(a, b):
    return a + b


def _build(TMB=128, FC=512, GATE=True, SKIP_FFN=False, SKIP_A=False,
           SCH=0, MT=6, NSUB=16, PB1=5, L0=0, L1=1, SPREAD=128, LLAG=3,
           P0=0, P1=16, N0=1, N1=30, PR=64, LA=4, LB=4, PADK=0):
    NBB = S // TMB

    def kernel(x_hbm, wqkv_hbm, wo_hbm, w1_hbm, w3_hbm, w2_hbm, c_hbm, wmod_hbm,
               out_hbm,
               x_v, wqkv_v, wtmp, wqkv_p, wo_v, wo_tmp, wo_p, w1_v, w3_v, w2_v, wmod_v, cb_v, modp_v, mod_v,
               h1a, h1b, h1s, part, stats, qka, va, pa, qkb, vb, pb_, qkc, vc, pc, oa, ob, oc, otmp, sl0, sl1, sl2, stat1, stat2, y_v, x1n, h2_v, act_v, obuf, c_ref,
               zs, sem_w, sem_o):
        bufs = {"a": (h1a, qka, va, oa, pa), "b": (h1b, qkb, vb, ob, pb_),
                "c": (None, qkc, vc, oc, pc)}

        sls = (sl0, sl1, sl2)

        dmas = {}

        def add_dma(name, src, dst):
            dmas[name] = (src, dst, len(dmas))

        for name, (b0, b1) in (("x0", (0, NS)), ("x1", (NS, NS + 3)), ("x2", (NS + 3, NB))):
            rows = pl.ds(b0 * TM, (b1 - b0) * TM)
            add_dma(name, x_hbm.at[0, rows, :], x_v.at[rows, :])
        for name, (c0, c1) in (("sa0", (0, KH)), ("sa1", (KH, D)), ("ca0", (D, D + KH)), ("ca1", (D + KH, 2 * D)),
                               ("m2", (2 * D, 3 * D)), ("m3", (3 * D, 6 * D))):
            cols = pl.ds(c0, c1 - c0)
            add_dma(name, wmod_hbm.at[:, cols], wmod_v.at[:, cols])
        for g in range(3):
            for k in range(2):
                rows, cols = pl.ds(k * KH, KH), pl.ds(g * D, D)
                add_dma("qkv"[g] + str(k), wqkv_hbm.at[rows, cols], wqkv_v.at[rows, cols])
        add_dma("c", c_hbm, c_ref)
        add_dma("wo", wo_hbm, wo_v)
        add_dma("w1", w1_hbm, w1_v)
        add_dma("w3", w3_hbm, w3_v)
        add_dma("w2", w2_hbm, w2_v)
        assert len(dmas) == NDMA

        def cp(name):
            src, dst, i = dmas[name]
            return pltpu.make_async_copy(src, dst, sem_w.at[i])

        def start(*names):
            for n in names:
                cp(n).start()

        def wait(*names):
            for n in names:
                cp(n).wait()

        def cp_out(j, slot):
            return pltpu.make_async_copy(obuf.at[slot],
                                         out_hbm.at[0, pl.ds(j * TMB, TMB), :], sem_o.at[slot])

        st = {"z": None, "never": None, "clock": 0, "sched": {}, "tok": None}

        def begin(sched):
            z = zs[0]
            st.update(z=z, never=jnp.full((8, 128), z, jnp.int32) != 0, clock=0, sched=sched, tok=None)

        def gate(val, i, n):
            r = st["tok"]
            if r is None or not GATE:
                return val
            row = (i * SPREAD // n) // 8 * 8
            t = r[row:row + 8]
            return jnp.where(st["never"], t if val.dtype == F32 else pltpu.bitcast(t, val.dtype), val)

        def place(sched, items, units):
            units = list(units)
            for i, it in enumerate(items):
                sched.setdefault(units[(i * len(units)) // len(items)], []).append(it)

        def matmul(lhs_fn, w_fn, ks, cols, sink):
            for n0 in cols:
                r = None
                for k in ks:
                    d = jnp.dot(lhs_fn(k), w_fn(k, n0), preferred_element_type=F32)
                    r = d if r is None else r + d
                    if k == ks[-1]:
                        sink(n0, r)
                    st["tok"] = r
                    for fn in st["sched"].pop(st["clock"], []):
                        fn()
                    st["tok"] = None
                    st["clock"] += 1

        def finish():
            assert not st["sched"]

        def lane_iota(rows):
            return jax.lax.broadcasted_iota(jnp.int32, (rows, 128), 1)

        def ld16(ref, r0, n, c0, c1):
            return pltpu.bitcast(ref[r0 // 2:(r0 + n) // 2, c0:c1], BF16)

        def silu_c():
            cf = c_ref[...].astype(F32)
            return (cf * jax.nn.sigmoid(cf)).astype(BF16)

        def mod_mxu(j, k):
            cs = slice(k * KH, (k + 1) * KH)
            lhs = jnp.broadcast_to(silu_c(), (16, D))
            r = jnp.dot(lhs, wmod_v[:, j * D + k * KH:j * D + (k + 1) * KH], preferred_element_type=F32)[0:8]
            mod_v[j, :, cs] = r + 1.0 if j in (1, 4) else r

        def mod_finish(j, c0, c1):
            r = _tree(_add, [modp_v[i, :, j * D + c0:j * D + c1] for i in range(NSUB)])
            r = jnp.sum(r, axis=0, keepdims=True)
            mod_v[j, :, c0:c1] = jnp.broadcast_to(r + 1.0 if j in (1, 4) else r, (8, c1 - c0))

        def mod_items(col0, ntiles):
            rows = D // NSUB

            def one(t, i):
                c0 = col0 + t * 128
                c0 = c0 if isinstance(c0, int) else pl.multiple_of(c0, 128)
                w = wmod_v[i * rows:(i + 1) * rows, pl.ds(c0, 128)].astype(F32)
                p = (w * cb_v[i * rows:(i + 1) * rows, :]).reshape(rows // 8, 8, 128)
                modp_v[i, :, pl.ds(c0, 128)] = gate(_tree(_add, [p[k] for k in range(rows // 8)]), 1, 2)
            return [functools.partial(one, t, i) for t in range(ntiles) for i in range(NSUB)]

        def perm_mix(g, i, nrows):
            n = nrows // 2
            l = lane_iota(n)
            vals = [pltpu.bitcast(wqkv_v[i * nrows:(i + 1) * nrows, g * D + c * 128: g * D + (c + 1) * 128], U32)
                    for c in range(NC)]
            for b in range(3):
                m = ((l >> (2 + b)) & 1) == 0
                for c in range(NC):
                    if c & (1 << b):
                        continue
                    lo, hi = vals[c], vals[c | (1 << b)]
                    vals[c] = jnp.where(m, lo, hi)
                    vals[c | (1 << b)] = jnp.where(m, hi, lo)
            p0 = (i * n) % (KH // 2)
            for j in range(NC):
                v = jnp.concatenate([gate(vals[j][q:q + 8], j, NC) for q in range(0, n, 8)], axis=0)
                wtmp[j, pl.ds(pl.multiple_of(zrow(p0), 8), n), :] = v

        def perm_gather(g, k, j):
            l = lane_iota(8)
            idx = ((((l >> 1) & 3) << 5) | ((((l >> 3) & 7) ^ j) << 2) | ((l >> 6) << 1) | (l & 1))
            for q in range(0, KH // 2, 8):
                t = jnp.take_along_axis(gate(wtmp[j, q:q + 8, :], q, KH // 2), idx, axis=1,
                                        mode="promise_in_bounds")
                wqkv_p[k * KH // 2 + q:k * KH // 2 + q + 8, g * D + j * 128: g * D + (j + 1) * 128] = t

        def perm_qkv_items(g, k, nrows=PR):
            n = KH // nrows
            return ([functools.partial(perm_mix, g, i, nrows) for i in range(k * n, (k + 1) * n)]
                    + [functools.partial(perm_gather, g, k, j) for j in range(NC)])

        def perm_wo_items():
            low = jax.lax.broadcasted_iota(jnp.int32, (8, 128), 0) < 4

            def spread(c):
                for r in range(0, D // 2, 8):
                    wo_tmp[c, pl.ds(zrow(r + r // 16), 8), :] = gate(pltpu.bitcast(
                        wo_v[2 * r:2 * r + 16, c * 128:(c + 1) * 128], U32), r, D // 2)

            def gather(c):
                for G in range(64):
                    j, e, ch = G >> 3, (G >> 2) & 1, G & 3
                    dd = (((2 * ch) ^ j) << 1) | e
                    ta = wo_tmp[c, pl.ds(ch * 136 + dd, 8, stride=17), :]
                    tb = wo_tmp[c, pl.ds(ch * 136 + (dd ^ 2), 8, stride=17), :]
                    wo_p[pl.ds(pl.multiple_of(zrow(G * 8), 8), 8), c * 128:(c + 1) * 128] = gate(
                        jnp.where(low, ta, tb), G, 64)
            return staged((spread, gather), NC, 1)

        def zrow(row, k=1):
            return row + k * st["z"]

        def gate16(v, i, n):
            return jnp.concatenate([gate(v[q:q + 8], i, n) for q in range(0, LG, 8)], axis=0)

        def staged(stages, n, lag):
            items = []
            for t in range(n + lag * (len(stages) - 1)):
                for k in reversed(range(len(stages))):
                    if 0 <= t - k * lag < n:
                        items.append(functools.partial(stages[k], t - k * lag))
            return items

        def ln_stages(load, stat, dst, j_scale, j_shift, cols=range(NC)):
            def chunks(x):
                return [x[:, c * 128:(c + 1) * 128] for c in range(NC)]

            def put(j, r, part, fn):
                m = jnp.sum(part, axis=-1, keepdims=True) * (1.0 / D)
                stat[j, pl.ds(pl.multiple_of(zrow(r), LG), LG), :] = jnp.broadcast_to(fn(m), (LG, 128))

            def s_mean(i):
                put(0, i * LG, gate16(_tree(_add, chunks(load(i * LG, 0))), 1, 2), lambda m: m)

            def s_var(i):
                r = i * LG
                mu = gate16(stat[0, r:r + LG, :], 0, 1)
                put(1, r, _tree(_add, [(x - mu) * (x - mu) for x in chunks(load(r, 1))]),
                    lambda m: jax.lax.rsqrt(m + EPS))

            def s_out(i):
                r = i * LG
                mu, rs = stat[0, r:r + LG, :], stat[1, r:r + LG, :]
                xs = chunks(load(r, 2))
                for c in cols:
                    x, cs = xs[c], slice(c * 128, (c + 1) * 128)
                    if c % (NC // 2) == 0:
                        rg = gate16(rs, c - cols[0], NC)
                    y = ((x - mu) * rg).reshape(LG // 8, 8, 128) * mod_v[j_scale, :, cs][None] + mod_v[j_shift, :, cs][None]
                    dst[r // 2:(r + LG) // 2, cs] = pltpu.bitcast(y.reshape(LG, 128).astype(BF16), U32)
            return s_mean, s_var, s_out

        def load_x(row0):
            return lambda r, k: x_v[pl.ds(pl.multiple_of(zrow(row0 + r, k), LG), LG), :].astype(F32)

        def ln1_items(row0, buf):
            return staged(ln_stages(load_x(row0), stat1, bufs[buf][0], 1, 0), TM // LG, 1)

        def ln1_start(b, k):
            return ln_stages(load_x(b * TM), stats.at[:, pl.ds(b * TM, TM), :], h1s.at[b], 1, 0,
                             range(k * NC // 2, (k + 1) * NC // 2))

        def ln1_out_items(b, k):
            return [functools.partial(ln1_start(b, k)[2], i) for i in range(TM // LG)]

        def x1_rows(row, n, c0, c1):
            xf = x_v[pl.ds(row, n), c0:c1].astype(F32).reshape(n // 8, 8, c1 - c0)
            y = y_v[pl.ds(row, n), c0:c1].reshape(n // 8, 8, c1 - c0)
            return (xf + mod_v[2, :, c0:c1][None] * y).reshape(n, c1 - c0)

        def post_items(row0):
            def load(r, k):
                if k:
                    return x1n[pl.ds(pl.multiple_of(zrow(r, k), LG), LG), :]
                x1 = x1_rows(row0 + r, LG, 0, D)
                x1n[r:r + LG, :] = x1
                return x1
            return staged(ln_stages(load, stat2, h2_v, 4, 3), TMB // LG, 1)

        def logit_items(buf, first):
            _, qk, _, _, pb = bufs[buf]
            swap = lane_iota(RG) ^ 1

            def s_logit(g):
                r = g * RG
                qs = [qk[c, HALO + r:HALO + r + RG, :] for c in range(NC)]
                for w in range(WIN):
                    k0 = HALO + r - DIL * w
                    if w >= WIN // 2:
                        k0 = zrow(k0)
                    s = _tree(_add, [qs[c] * qk[NC + c, pl.ds(k0, RG), :] for c in range(NC)])
                    s = gate(s, w, WIN)
                    s = s + pltpu.roll(s, 64, 1)
                    s = s + jnp.take_along_axis(s, swap, axis=1, mode="promise_in_bounds")
                    if first and r < DIL * w:
                        pos = r + jax.lax.broadcasted_iota(jnp.int32, (RG, 128), 0)
                        s = jnp.where(pos >= DIL * w, s, NEG * LOG2E)
                    sls[g % len(sls)][w, pl.ds(pl.multiple_of(zrow(0), RG), RG), :] = s

            def s_soft(g):
                r = g * RG
                ss = [sls[g % len(sls)][w] for w in range(WIN)]
                m = gate(_tree(jnp.maximum, ss), 0, 1)
                es = [jnp.exp2(s - m) for s in ss]
                for w in range(WIN):
                    pb[w, r:r + RG, :] = es[w]
                den = _tree(_add, es)
                inv = pl.reciprocal(den, approx=True)
                pb[WIN, r:r + RG, :] = inv * (2.0 - den * inv)
            return staged((s_logit, s_soft), TM // RG, LLAG)

        def pv_items(buf):
            _, _, vp, o, pb = bufs[buf]

            def one(r):
                ps = [pb[w, r:r + RG, :] for w in range(WIN + 1)]
                for c in range(NC):
                    ks = [HALO + r - DIL * w if w < WIN // 2 else zrow(HALO + r - DIL * w) for w in range(WIN)]
                    acc = _tree(_add, [ps[w] * vp[c, pl.ds(ks[w], RG), :] for w in range(WIN)])
                    acc = gate(acc * ps[WIN], c, NC)
                    if (r // RG) % 2 == 0:
                        otmp[c, pl.ds(pl.multiple_of(zrow(0), 8), RG), :] = acc
                    else:
                        both = jnp.concatenate([otmp[c], acc], axis=0).astype(BF16)
                        o[(r - RG) // 2:(r + RG) // 2, c * 128:(c + 1) * 128] = pltpu.bitcast(both, U32)
            return [functools.partial(one, r) for r in range(0, TM, RG)]

        def halo(buf, prev, part):
            _, qk, vp, _, _ = bufs[buf]
            for c in range(NC):
                if part == 1:
                    qk[NC + c, 0:HALO, :] = (jnp.zeros((HALO, 128), F32) if prev is None
                                             else bufs[prev][1][NC + c, TM:TM + HALO, :])
                else:
                    vp[c, 0:HALO, :] = (jnp.broadcast_to(vp[c, HALO:HALO + 1, :], (HALO, 128)) if prev is None
                                        else bufs[prev][2][c, TM:TM + HALO, :])

        def qkv_part(buf, g, sb=None, k=None):
            h1, qk, vp, _, _ = bufs[buf] if buf else (None,) * 5
            if sb is not None:
                h1 = h1s.at[sb]

            def sink(n0, r):
                ch = n0 // 128
                if k == 0:
                    part[sb, ch] = r
                    return
                if k == 1:
                    r = r + part[sb, ch]
                dst, ci = (qk, ch) if ch < 2 * NC else (vp, ch - 2 * NC)
                dst[ci, HALO:HALO + TM, :] = r * (SM_SCALE * LOG2E) if ch < NC else r
            matmul(lambda kk: ld16(h1, 0, TM, kk * KH, (kk + 1) * KH),
                   lambda kk, n0: ld16(wqkv_p, kk * KH, KH, n0, n0 + 128),
                   (0, 1) if k is None else (k,), range(g * D, (g + 1) * D, 128), sink)

        def wo_mm(buf, row0):
            o = bufs[buf][3]

            def sink(n0, r):
                y_v[pl.ds(row0, TM), n0:n0 + 128] = r
            matmul(lambda k: ld16(o, 0, TM, k * KH, (k + 1) * KH),
                   lambda k, n0: ld16(wo_p, k * KH, KH, n0, n0 + 128),
                   (0, 1), range(0, D, 128), sink)

        UP = NC * (D // KH)

        def run_now(items):
            for fn in items:
                fn()

        def ffn(row0, slot, nxt_row):
            h = ld16(h2_v, 0, TMB, 0, D)
            for f0 in range(0, F, FC):
                g = jnp.dot(h, w1_v[:, f0:f0 + FC], preferred_element_type=F32)
                u = jnp.dot(h, w3_v[:, f0:f0 + FC], preferred_element_type=F32)
                act_v[:, f0:f0 + FC] = pltpu.bitcast((g * jax.nn.sigmoid(g) * u).astype(BF16), U32)
            nk = F // KH
            sched = {}
            place(sched, post_items(nxt_row), range(0, NC * nk - PB1))
            begin(sched)

            def sink(n0, r):
                z = (mod_v[5, :, n0:n0 + 128][None] * r.reshape(TMB // 8, 8, 128)).reshape(TMB, 128)
                obuf[slot, :, n0:n0 + 128] = (x1_rows(row0, TMB, n0, n0 + 128) + z).astype(BF16)
            matmul(lambda k: ld16(act_v, 0, TMB, k * KH, (k + 1) * KH),
                   lambda k, n0: w2_v[k * KH:(k + 1) * KH, n0:n0 + 128],
                   tuple(range(nk)), range(0, D, 128), sink)

        U8 = NC

        def segment(*placements):
            sched = {}
            for items, units in placements:
                place(sched, items, units)
            begin(sched)

        with jax.named_scope("prologue"):
            zs[0] = 0
            begin({})
            start("c", "x0", "ca0", "q0", "sa0", "k0", "v0", "ca1", "sa1", "q1", "k1", "v1", "wo",
                  "x1", "m2", "x2")
            wait("c")
            cb_v[...] = jnp.broadcast_to(silu_c().astype(F32), (128, D)).T
            wait("x0")
            for r in range(0, NS * TM, LG):
                xf = x_v[r:r + LG, :].astype(F32)
                mu = jnp.mean(xf, axis=-1, keepdims=True)
                d = xf - mu
                rs = jax.lax.rsqrt(jnp.mean(d * d, axis=-1, keepdims=True) + EPS)
                stats[0, r:r + LG, :] = jnp.broadcast_to(mu, (LG, 128))
                stats[1, r:r + LG, :] = jnp.broadcast_to(rs, (LG, 128))
            wait("ca0")
            mod_mxu(1, 0)
            wait("q0")
            run_now(perm_qkv_items(0, 0))
            wait("sa0")
            mod_mxu(0, 0)
            run_now(ln1_out_items(0, 0))

        with jax.named_scope("pass1"):
            segment((ln1_out_items(1, 0), range(0, U8 - 2)),
                    (ln1_out_items(2, 0) + ln1_out_items(3, 0), range(U8 - 2, 2 * U8)))
            qkv_part(None, 0, 0, 0)
            qkv_part(None, 0, 1, 0)
            wait("k0")
            segment((perm_qkv_items(1, 0), range(0, 2 * U8 - 2)))
            for g, b in ((0, 2), (0, 3), (1, 0), (1, 1)):
                qkv_part(None, g, b, 0)
            wait("v0", "ca1")
            segment((perm_qkv_items(2, 0), range(0, 2 * U8 - 2)),
                    (mod_items(D + KH, 4) + [functools.partial(mod_finish, 1, KH, D)], range(2 * U8 - 2, 4 * U8)))
            for g, b in ((1, 2), (1, 3), (2, 0), (2, 1)):
                qkv_part(None, g, b, 0)
            wait("sa1", "q1")
            segment((mod_items(KH, 4) + [functools.partial(mod_finish, 0, KH, D)], range(0, U8 + 2)),
                    (perm_qkv_items(0, 1), range(0, 2 * U8 - 2)),
                    (ln1_out_items(0, 1), range(U8 + 3, 2 * U8 - 1)))
            qkv_part(None, 2, 2, 0)
            qkv_part(None, 2, 3, 0)

        with jax.named_scope("pass2"):
            wait("k1")
            segment((perm_qkv_items(1, 1), range(0, 2 * U8 - 2)),
                    (ln1_out_items(1, 1), range(0, U8 - 2)),
                    (ln1_out_items(2, 1), range(U8 - 2, 2 * U8)))
            halo("b", None, 1)
            qkv_part("b", 0, 0, 1)
            qkv_part("c", 0, 1, 1)
            wait("v1")
            l1 = logit_items("c", False)
            segment((perm_qkv_items(2, 1), range(0, 2 * U8 - 2)),
                    (ln1_out_items(3, 1), range(0, U8)),
                    (logit_items("b", True), range(U8, 4 * U8 - LA)),
                    (l1[:LB], range(4 * U8 - LA, 4 * U8)))
            qkv_part("b", 1, 0, 1)
            halo("c", "b", 1)
            qkv_part("c", 1, 1, 1)
            qkv_part("b", 2, 0, 1)
            halo("b", None, 2)
            halo("c", "b", 2)
            qkv_part("c", 2, 1, 1)
            wait("wo", "x1")
            segment((perm_wo_items(), range(0, 3 * U8 - 2)),
                    (pv_items("b"), range(0, 3 * U8 - 1)),
                    (l1[LB:], range(0, 2 * U8 + 2)),
                    (logit_items("a", False), range(2 * U8 + 2, 5 * U8 + 4)),
                    (pv_items("c"), range(3 * U8, 7 * U8)),
                    (ln1_items(NS * TM, "a"), range(5 * U8 + 4, 7 * U8)),
                    (pv_items("a"), range(7 * U8, 10 * U8 - 1)),
                    (logit_items("b", False), range(7 * U8, 12 * U8 - L1)))
            halo("a", "c", 1)
            halo("a", "c", 2)
            for g in range(3):
                qkv_part("a", g, 2, 1)
            wo_mm("b", 0)
            halo("b", "a", 1)
            halo("b", "a", 2)
            for g in range(3):
                qkv_part("b", g, 3, 1)
            wo_mm("c", TM)
            wo_mm("a", 2 * TM)
            finish()
            wait("m2")
            start("m3", "w1", "w3", "w2")


        def half(X, Y, u0, sched, row_ln1, row_wo, extra):
            place(sched, pv_items(Y), range(u0 + P0, u0 + 3 * UP - P1))
            place(sched, logit_items(X, False), range(u0 + 2 * UP + L0, u0 + 4 * UP - L1))
            place(sched, ln1_items(row_ln1, Y), range(u0 + N0, u0 + N1))
            if extra:
                place(sched, extra, range(u0, u0 + 4 * UP - 1))

            def run():
                halo(X, Y, 1)
                halo(X, Y, 2)
                for g in range(3):
                    qkv_part(X, g)
                wo_mm(Y, row_wo)
            return run

        def a_step(s, carry):
            @pl.when(s == 3)
            def _():
                wait("x2", "m3")

            ra = pl.multiple_of(2 * s * TM, TM)
            nxt = pl.multiple_of(jnp.minimum(ra + 2 * TM, S - TM), TM)
            col0 = pl.multiple_of(jnp.minimum(2 * D + (s - 2) * (MT * 128), 6 * D - MT * 128), 128)
            mi = mod_items(col0, MT)
            sched = {}
            run_a = half("a", "b", 0, sched, ra + TM, ra - TM, mi[:len(mi) // 2])
            run_b = half("b", "a", 4 * UP, sched, nxt, ra, mi[len(mi) // 2:])
            begin(sched)
            run_a()
            run_b()
            finish()
            return carry

        with jax.named_scope("aloop"):
            if SKIP_A:
                wait("x2", "m3")
            else:
                jax.lax.fori_loop(NS // 2, NB // 2, a_step, 0)

        with jax.named_scope("atail"):
            begin({})
            for j in range(2, 6):
                mod_finish(j, 0, D)
            run_now(pv_items("b"))
            sched = {}
            place(sched, post_items(0), range(0, UP - 2))
            begin(sched)
            wo_mm("b", S - TM)
            finish()
            wait("w1", "w3", "w2")

        def b_step(j, carry):
            slot = j % 2

            @pl.when(j >= 2)
            def _():
                cp_out(j - 2, slot).wait()

            row0 = pl.multiple_of(j * TMB, TMB)
            nxt = pl.multiple_of(jnp.minimum(row0 + TMB, S - TMB), TMB)
            if SKIP_FFN:
                obuf[slot] = x1_rows(row0, TMB, 0, D).astype(BF16)
            else:
                ffn(row0, slot, nxt)
            cp_out(j, slot).start()
            return carry

        with jax.named_scope("bloop"):
            jax.lax.fori_loop(0, NBB, b_step, 0)
        with jax.named_scope("tail"):
            cp_out(NBB - 2, (NBB - 2) % 2).wait()
            cp_out(NBB - 1, (NBB - 1) % 2).wait()

    any_spec = pl.BlockSpec(memory_space=pl.ANY)
    scratch = [
        pltpu.VMEM((S, D), BF16),
        pltpu.VMEM((D, 3 * D), BF16),
        pltpu.VMEM((NC, KH // 2, 128), U32),
        pltpu.VMEM((D // 2, 3 * D), U32),
        pltpu.VMEM((D, D), BF16),
        pltpu.VMEM((NC, D // 32 * 17, 128), U32),
        pltpu.VMEM((D // 2, D), U32),
        pltpu.VMEM((D, F), BF16),
        pltpu.VMEM((D, F), BF16),
        pltpu.VMEM((F, D), BF16),
        pltpu.VMEM((D, 6 * D), BF16),
        pltpu.VMEM((D, 128), F32),
        pltpu.VMEM((NSUB, 8, 6 * D), F32),
        pltpu.VMEM((6, 8, D), F32),
        pltpu.VMEM((TM // 2, D), U32),
        pltpu.VMEM((TM // 2, D), U32),
        pltpu.VMEM((NS, TM // 2, D), U32),
        pltpu.VMEM((NS, 3 * NC, TM, 128), F32),
        pltpu.VMEM((2, NS * TM, 128), F32),
        pltpu.VMEM((2 * NC, KV + PADK, 128), F32),
        pltpu.VMEM((NC, KV + PADK, 128), F32),
        pltpu.VMEM((WIN + 1, TM, 128), F32),
        pltpu.VMEM((2 * NC, KV + PADK, 128), F32),
        pltpu.VMEM((NC, KV + PADK, 128), F32),
        pltpu.VMEM((WIN + 1, TM, 128), F32),
        pltpu.VMEM((2 * NC, KV + PADK, 128), F32),
        pltpu.VMEM((NC, KV + PADK, 128), F32),
        pltpu.VMEM((WIN + 1, TM, 128), F32),
        pltpu.VMEM((TM // 2, D), U32),
        pltpu.VMEM((TM // 2, D), U32),
        pltpu.VMEM((TM // 2, D), U32),
        pltpu.VMEM((NC, RG, 128), F32),
        pltpu.VMEM((WIN, RG, 128), F32),
        pltpu.VMEM((WIN, RG, 128), F32),
        pltpu.VMEM((WIN, RG, 128), F32),
        pltpu.VMEM((2, TM, 128), F32),
        pltpu.VMEM((2, TMB, 128), F32),
        pltpu.VMEM((S, D), F32),
        pltpu.VMEM((TMB, D), F32),
        pltpu.VMEM((TMB // 2, D), U32),
        pltpu.VMEM((TMB // 2, F), U32),
        pltpu.VMEM((2, TMB, D), BF16),
        pltpu.VMEM((1, D), BF16),
        pltpu.SMEM((1,), jnp.int32),
        pltpu.SemaphoreType.DMA((NDMA,)),
        pltpu.SemaphoreType.DMA((2,)),
    ]

    def call(A_x, A_wqkv, A_wo, B_w1, B_w3, B_w2, c, w_mod):
        return pl.pallas_call(
            kernel,
            out_shape=jax.ShapeDtypeStruct((1, S, D), BF16),
            in_specs=[any_spec] * 8,
            out_specs=any_spec,
            scratch_shapes=scratch,
            compiler_params=pltpu.CompilerParams(vmem_limit_bytes=120 * 1024 * 1024),
        )(A_x, A_wqkv, A_wo, B_w1, B_w3, B_w2, c, w_mod)

    return call


@jax.jit
def pallas_adaLN_cond__sliding_local_dilated__glu_gated_swiglu__prompt_kernel(
    A_x: jax.Array,
    A_wqkv: jax.Array,
    A_wo: jax.Array,
    B_x: jax.Array,
    B_w1: jax.Array,
    B_w3: jax.Array,
    B_w2: jax.Array,
    c: jax.Array,
    w_mod: jax.Array,
):
    del B_x
    return _build()(A_x, A_wqkv, A_wo, B_w1, B_w3, B_w2, c, w_mod)
```

```python
import functools
import math

import jax
import jax.numpy as jnp
import jax.experimental.pallas as pl
import jax.experimental.pallas.tpu as pltpu

S = 2048
D = 1024
F = 3584
H = 32
DH = D // H
WIN = 8
DIL = 2
NC = D // 128
HALO = 16
EPS = 1e-5
NEG = -1000000000.0
SM_SCALE = DH ** -0.5
LOG2E = math.log2(math.e)

TM = 128
NB = S // TM
KV = HALO + TM
RG = 8
LG = 16
NS = 4
NDMA = 21
KH = 512

F32 = jnp.float32
BF16 = jnp.bfloat16
U32 = jnp.uint32


def _tree(op, xs):
    xs = list(xs)
    while len(xs) > 1:
        xs = [op(xs[i], xs[i + 1]) if i + 1 < len(xs) else xs[i] for i in range(0, len(xs), 2)]
    return xs[0]


def _add(a, b):
    return a + b


def _build(TMB=128, FC=512, GATE=True, SKIP_FFN=False, SKIP_A=False,
           SCH=0, MT=6, NSUB=16, PB1=5, L0=0, L1=1, SPREAD=128, LLAG=3,
           P0=0, P1=16, N0=1, N1=30, PR=64, B0=15, B1=30, LB=15, PADK=0, C0=12, C1=40, C2=68):
    NBB = S // TMB

    def kernel(x_hbm, wqkv_hbm, wo_hbm, w1_hbm, w3_hbm, w2_hbm, c_hbm, wmod_hbm,
               out_hbm,
               x_v, wqkv_v, wtmp, wqkv_p, wo_v, wo_tmp, wo_p, w1_v, w3_v, w2_v, wmod_v, cb_v, modp_v, mod_v,
               h1a, h1b, h1s, part, stats, qka, va, pa, qkb, vb, pb_, qkc, vc, pc, oa, ob, oc, ota, otb, otc, sl0, sl1, sl2, stat1, stat2, y_v, x1n, h2_v, act_v, obuf, c_ref,
               zs, sem_w, sem_o):
        bufs = {"a": (h1a, qka, va, oa, pa), "b": (h1b, qkb, vb, ob, pb_),
                "c": (None, qkc, vc, oc, pc)}

        sls = (sl0, sl1, sl2)
        otmps = {"a": ota, "b": otb, "c": otc}

        dmas = {}

        def add_dma(name, src, dst):
            dmas[name] = (src, dst, len(dmas))

        for name, (b0, b1) in (("x0", (0, NS)), ("x4", (NS, NS + 1)), ("x1", (NS + 1, NS + 3)), ("x2", (NS + 3, NB))):
            rows = pl.ds(b0 * TM, (b1 - b0) * TM)
            add_dma(name, x_hbm.at[0, rows, :], x_v.at[rows, :])
        for name, (c0, c1) in (("sa0", (0, KH)), ("sa1", (KH, D)), ("ca0", (D, D + KH)), ("ca1", (D + KH, 2 * D)),
                               ("m2", (2 * D, 3 * D)), ("m3", (3 * D, 6 * D))):
            cols = pl.ds(c0, c1 - c0)
            add_dma(name, wmod_hbm.at[:, cols], wmod_v.at[:, cols])
        for g in range(3):
            for k in range(2):
                rows, cols = pl.ds(k * KH, KH), pl.ds(g * D, D)
                add_dma("qkv"[g] + str(k), wqkv_hbm.at[rows, cols], wqkv_v.at[rows, cols])
        add_dma("c", c_hbm, c_ref)
        add_dma("wo", wo_hbm, wo_v)
        add_dma("w1", w1_hbm, w1_v)
        add_dma("w3", w3_hbm, w3_v)
        add_dma("w2", w2_hbm, w2_v)
        assert len(dmas) == NDMA

        def cp(name):
            src, dst, i = dmas[name]
            return pltpu.make_async_copy(src, dst, sem_w.at[i])

        def start(*names):
            for n in names:
                cp(n).start()

        def wait(*names):
            for n in names:
                cp(n).wait()

        def cp_out(j, slot):
            return pltpu.make_async_copy(obuf.at[slot],
                                         out_hbm.at[0, pl.ds(j * TMB, TMB), :], sem_o.at[slot])

        st = {"z": None, "never": None, "clock": 0, "sched": {}, "tok": None}

        have = set()

        def need(*keys):
            assert all(k in have for k in keys), keys

        def begin(sched):
            z = zs[0]
            st.update(z=z, never=jnp.full((8, 128), z, jnp.int32) != 0, clock=0, sched=sched, tok=None)

        def gate(val, i, n):
            r = st["tok"]
            if r is None or not GATE:
                return val
            row = (i * SPREAD // n) // 8 * 8
            t = r[row:row + 8]
            return jnp.where(st["never"], t if val.dtype == F32 else pltpu.bitcast(t, val.dtype), val)

        def place(sched, items, units):
            units = list(units)
            for i, it in enumerate(items):
                sched.setdefault(units[(i * len(units)) // len(items)], []).append(it)

        def matmul(lhs_fn, w_fn, ks, cols, sink, gives=None):
            for n0 in cols:
                r = None
                for k in ks:
                    d = jnp.dot(lhs_fn(k), w_fn(k, n0), preferred_element_type=F32)
                    r = d if r is None else r + d
                    if k == ks[-1]:
                        sink(n0, r)
                    if n0 == cols[-1] and k == ks[-1]:
                        have.add(gives)
                    st["tok"] = r
                    for fn in st["sched"].pop(st["clock"], []):
                        fn()
                    st["tok"] = None
                    st["clock"] += 1

        def finish():
            assert not st["sched"]

        def lane_iota(rows):
            return jax.lax.broadcasted_iota(jnp.int32, (rows, 128), 1)

        def ld16(ref, r0, n, c0, c1):
            return pltpu.bitcast(ref[r0 // 2:(r0 + n) // 2, c0:c1], BF16)

        def silu_c():
            cf = c_ref[...].astype(F32)
            return (cf * jax.nn.sigmoid(cf)).astype(BF16)

        def mod_mxu(j, k):
            cs = slice(k * KH, (k + 1) * KH)
            lhs = jnp.broadcast_to(silu_c(), (16, D))
            r = jnp.dot(lhs, wmod_v[:, j * D + k * KH:j * D + (k + 1) * KH], preferred_element_type=F32)[0:8]
            mod_v[j, :, cs] = r + 1.0 if j in (1, 4) else r

        def mod_finish(j, c0, c1):
            r = _tree(_add, [modp_v[i, :, j * D + c0:j * D + c1] for i in range(NSUB)])
            r = jnp.sum(r, axis=0, keepdims=True)
            mod_v[j, :, c0:c1] = jnp.broadcast_to(r + 1.0 if j in (1, 4) else r, (8, c1 - c0))

        def mod_items(col0, ntiles):
            rows = D // NSUB

            def one(t, i):
                c0 = col0 + t * 128
                c0 = c0 if isinstance(c0, int) else pl.multiple_of(c0, 128)
                w = wmod_v[i * rows:(i + 1) * rows, pl.ds(c0, 128)].astype(F32)
                p = (w * cb_v[i * rows:(i + 1) * rows, :]).reshape(rows // 8, 8, 128)
                modp_v[i, :, pl.ds(c0, 128)] = gate(_tree(_add, [p[k] for k in range(rows // 8)]), 1, 2)
            return [functools.partial(one, t, i) for t in range(ntiles) for i in range(NSUB)]

        def perm_mix(g, i, nrows):
            n = nrows // 2
            l = lane_iota(n)
            vals = [pltpu.bitcast(wqkv_v[i * nrows:(i + 1) * nrows, g * D + c * 128: g * D + (c + 1) * 128], U32)
                    for c in range(NC)]
            for b in range(3):
                m = ((l >> (2 + b)) & 1) == 0
                for c in range(NC):
                    if c & (1 << b):
                        continue
                    lo, hi = vals[c], vals[c | (1 << b)]
                    vals[c] = jnp.where(m, lo, hi)
                    vals[c | (1 << b)] = jnp.where(m, hi, lo)
            p0 = (i * n) % (KH // 2)
            for j in range(NC):
                v = jnp.concatenate([gate(vals[j][q:q + 8], j, NC) for q in range(0, n, 8)], axis=0)
                wtmp[j, pl.ds(pl.multiple_of(zrow(p0), 8), n), :] = v

        def perm_gather(g, k, j):
            have.add(("w", g, k, j))
            l = lane_iota(8)
            idx = ((((l >> 1) & 3) << 5) | ((((l >> 3) & 7) ^ j) << 2) | ((l >> 6) << 1) | (l & 1))
            for q in range(0, KH // 2, 8):
                t = jnp.take_along_axis(gate(wtmp[j, q:q + 8, :], q, KH // 2), idx, axis=1,
                                        mode="promise_in_bounds")
                wqkv_p[k * KH // 2 + q:k * KH // 2 + q + 8, g * D + j * 128: g * D + (j + 1) * 128] = t

        def perm_qkv_items(g, k, nrows=PR):
            n = KH // nrows
            return ([functools.partial(perm_mix, g, i, nrows) for i in range(k * n, (k + 1) * n)]
                    + [functools.partial(perm_gather, g, k, j) for j in range(NC)])

        def perm_wo_items():
            low = jax.lax.broadcasted_iota(jnp.int32, (8, 128), 0) < 4

            def spread(c, h):
                for r in range(h * 256, h * 256 + 256, 8):
                    wo_tmp[c, pl.ds(zrow(r + r // 16), 8), :] = gate(pltpu.bitcast(
                        wo_v[2 * r:2 * r + 16, c * 128:(c + 1) * 128], U32), r % 256, 256)

            def gather(c, h):
                for G in range(h * 32, h * 32 + 32):
                    j, e, ch = G >> 3, (G >> 2) & 1, G & 3
                    dd = (((2 * ch) ^ j) << 1) | e
                    ta = wo_tmp[c, pl.ds(ch * 136 + dd, 8, stride=17), :]
                    tb = wo_tmp[c, pl.ds(ch * 136 + (dd ^ 2), 8, stride=17), :]
                    wo_p[G * 8:G * 8 + 8, c * 128:(c + 1) * 128] = jnp.where(low, ta, tb)
            return [functools.partial(fn, c, h) for fn in (spread, gather) for c in range(NC) for h in range(2)]

        def zrow(row, k=1):
            return row + k * st["z"]

        def gate16(v, i, n):
            return jnp.concatenate([gate(v[q:q + 8], i, n) for q in range(0, LG, 8)], axis=0)

        def staged(stages, n, lag):
            items = []
            for t in range(n + lag * (len(stages) - 1)):
                for k in reversed(range(len(stages))):
                    if 0 <= t - k * lag < n:
                        items.append(functools.partial(stages[k], t - k * lag))
            return items

        def ln_stages(load, stat, dst, j_scale, j_shift, cols=range(NC)):
            def chunks(x):
                return [x[:, c * 128:(c + 1) * 128] for c in range(NC)]

            def put(j, r, part, fn):
                m = jnp.sum(part, axis=-1, keepdims=True) * (1.0 / D)
                stat[j, pl.ds(pl.multiple_of(zrow(r), LG), LG), :] = jnp.broadcast_to(fn(m), (LG, 128))

            def s_mean(i):
                put(0, i * LG, gate16(_tree(_add, chunks(load(i * LG, 0))), 1, 2), lambda m: m)

            def s_var(i):
                r = i * LG
                mu = gate16(stat[0, r:r + LG, :], 0, 1)
                put(1, r, _tree(_add, [(x - mu) * (x - mu) for x in chunks(load(r, 1))]),
                    lambda m: jax.lax.rsqrt(m + EPS))

            def s_out(i):
                r = i * LG
                mu, rs = stat[0, r:r + LG, :], stat[1, r:r + LG, :]
                xs = chunks(load(r, 2))
                for c in cols:
                    x, cs = xs[c], slice(c * 128, (c + 1) * 128)
                    if c % (NC // 2) == 0:
                        rg = gate16(rs, c - cols[0], NC)
                    y = ((x - mu) * rg).reshape(LG // 8, 8, 128) * mod_v[j_scale, :, cs][None] + mod_v[j_shift, :, cs][None]
                    dst[r // 2:(r + LG) // 2, cs] = pltpu.bitcast(y.reshape(LG, 128).astype(BF16), U32)
            return s_mean, s_var, s_out

        def load_x(row0):
            return lambda r, k: x_v[pl.ds(pl.multiple_of(zrow(row0 + r, k), LG), LG), :].astype(F32)

        def ln1_items(row0, buf):
            return staged(ln_stages(load_x(row0), stat1, bufs[buf][0], 1, 0), TM // LG, 1)

        def ln1_start(b, k):
            return ln_stages(load_x(b * TM), stats.at[:, pl.ds(b * TM, TM), :], h1s.at[b] if b < NS else h1a,
                             1, 0, range(k * NC // 2, (k + 1) * NC // 2))

        def ln1_out_items(b, k):
            def one(i):
                have.add(("h", b, k, i))
                ln1_start(b, k)[2](i)
            return [functools.partial(one, i) for i in range(TM // LG)]

        def x1_rows(row, n, c0, c1):
            xf = x_v[pl.ds(row, n), c0:c1].astype(F32).reshape(n // 8, 8, c1 - c0)
            y = y_v[pl.ds(row, n), c0:c1].reshape(n // 8, 8, c1 - c0)
            return (xf + mod_v[2, :, c0:c1][None] * y).reshape(n, c1 - c0)

        def post_items(row0):
            def load(r, k):
                if k:
                    return x1n[pl.ds(pl.multiple_of(zrow(r, k), LG), LG), :]
                x1 = x1_rows(row0 + r, LG, 0, D)
                x1n[r:r + LG, :] = x1
                return x1
            return staged(ln_stages(load, stat2, h2_v, 4, 3), TMB // LG, 1)

        def logit_items(buf, first):
            _, qk, _, _, pb = bufs[buf]
            swap = lane_iota(RG) ^ 1

            def s_logit(g):
                need(("q", buf), ("k", buf))
                have.add(("l", buf, g))
                r = g * RG
                qs = [qk[c, HALO + r:HALO + r + RG, :] for c in range(NC)]
                for w in range(WIN):
                    k0 = HALO + r - DIL * w
                    if w >= WIN // 2:
                        k0 = zrow(k0)
                    s = _tree(_add, [qs[c] * qk[NC + c, pl.ds(k0, RG), :] for c in range(NC)])
                    s = gate(s, w, WIN)
                    s = s + pltpu.roll(s, 64, 1)
                    s = s + jnp.take_along_axis(s, swap, axis=1, mode="promise_in_bounds")
                    if first and r < DIL * w:
                        pos = r + jax.lax.broadcasted_iota(jnp.int32, (RG, 128), 0)
                        s = jnp.where(pos >= DIL * w, s, NEG * LOG2E)
                    sls[g % len(sls)][w, pl.ds(pl.multiple_of(zrow(0), RG), RG), :] = s

            def s_soft(g):
                assert ("p", buf, g) not in have
                have.add(("p", buf, g))
                r = g * RG
                ss = [sls[g % len(sls)][w] for w in range(WIN)]
                m = gate(_tree(jnp.maximum, ss), 0, 1)
                es = [jnp.exp2(s - m) for s in ss]
                for w in range(WIN):
                    pb[w, r:r + RG, :] = es[w]
                den = _tree(_add, es)
                inv = pl.reciprocal(den, approx=True)
                pb[WIN, r:r + RG, :] = inv * (2.0 - den * inv)
            return staged((s_logit, s_soft), TM // RG, LLAG)

        def pv_items(buf):
            _, _, vp, o, pb = bufs[buf]
            otmp = otmps[buf]

            def one(r):
                need(("v", buf), ("p", buf, r // RG))
                have.remove(("p", buf, r // RG))
                have.add(("o", buf, r // RG))
                ps = [pb[w, pl.ds(pl.multiple_of(zrow(r), RG), RG), :] for w in range(WIN + 1)]
                for c in range(NC):
                    ks = [HALO + r - DIL * w if w < WIN // 2 else zrow(HALO + r - DIL * w) for w in range(WIN)]
                    acc = _tree(_add, [ps[w] * vp[c, pl.ds(ks[w], RG), :] for w in range(WIN)])
                    acc = gate(acc * ps[WIN], c, NC)
                    if (r // RG) % 2 == 0:
                        otmp[c, pl.ds(pl.multiple_of(zrow(0), 8), RG), :] = acc
                    else:
                        both = jnp.concatenate([otmp[c], acc], axis=0).astype(BF16)
                        o[(r - RG) // 2:(r + RG) // 2, c * 128:(c + 1) * 128] = pltpu.bitcast(both, U32)
            return [functools.partial(one, r) for r in range(0, TM, RG)]

        def halo(buf, prev, part):
            _, qk, vp, _, _ = bufs[buf]
            for c in range(NC):
                if part == 1:
                    qk[NC + c, 0:HALO, :] = (jnp.zeros((HALO, 128), F32) if prev is None
                                             else bufs[prev][1][NC + c, TM:TM + HALO, :])
                else:
                    vp[c, 0:HALO, :] = (jnp.broadcast_to(vp[c, HALO:HALO + 1, :], (HALO, 128)) if prev is None
                                        else bufs[prev][2][c, TM:TM + HALO, :])

        def qkv_part(buf, g, sb=None, k=None):
            h1, qk, vp, _, _ = bufs[buf] if buf else (None,) * 5
            if sb is not None:
                h1 = h1s.at[sb]
                need(*[("h", sb, k, i) for i in range(TM // LG)], *[("w", g, k, j) for j in range(NC)])
            if k != 0:
                for i in range(TM // RG):
                    if g < 2 and ("qk"[g], buf) in have:
                        need(("l", buf, i))
                    if g == 2 and ("v", buf) in have:
                        assert ("p", buf, i) not in have or ("new", buf) in have
                if g == 1:
                    have.difference_update({("l", buf, i) for i in range(TM // RG)})
                    have.add(("new", buf))
                have.discard(("qkv"[g], buf))

            def sink(n0, r):
                ch = n0 // 128
                if k == 0:
                    part[sb, ch] = r
                    return
                if k == 1:
                    r = r + part[sb, ch]
                dst, ci = (qk, ch) if ch < 2 * NC else (vp, ch - 2 * NC)
                dst[ci, HALO:HALO + TM, :] = r * (SM_SCALE * LOG2E) if ch < NC else r
            matmul(lambda kk: ld16(h1, 0, TM, kk * KH, (kk + 1) * KH),
                   lambda kk, n0: ld16(wqkv_p, kk * KH, KH, n0, n0 + 128),
                   (0, 1) if k is None else (k,), range(g * D, (g + 1) * D, 128), sink,
                   None if k == 0 else ("qkv"[g], buf))
            if g == 2:
                have.discard(("new", buf))

        def wo_mm(buf, row0):
            o = bufs[buf][3]
            need(*[("o", buf, i) for i in range(TM // RG)])
            have.difference_update({("o", buf, i) for i in range(TM // RG)})

            def sink(n0, r):
                y_v[pl.ds(row0, TM), n0:n0 + 128] = r
            matmul(lambda k: ld16(o, 0, TM, k * KH, (k + 1) * KH),
                   lambda k, n0: ld16(wo_p, k * KH, KH, n0, n0 + 128),
                   (0, 1), range(0, D, 128), sink)

        UP = NC * (D // KH)

        def run_now(items):
            for fn in items:
                fn()

        def ffn(row0, slot, nxt_row):
            h = ld16(h2_v, 0, TMB, 0, D)
            for f0 in range(0, F, FC):
                g = jnp.dot(h, w1_v[:, f0:f0 + FC], preferred_element_type=F32)
                u = jnp.dot(h, w3_v[:, f0:f0 + FC], preferred_element_type=F32)
                act_v[:, f0:f0 + FC] = pltpu.bitcast((g * jax.nn.sigmoid(g) * u).astype(BF16), U32)
            nk = F // KH
            sched = {}
            place(sched, post_items(nxt_row), range(0, NC * nk - PB1))
            begin(sched)

            def sink(n0, r):
                z = (mod_v[5, :, n0:n0 + 128][None] * r.reshape(TMB // 8, 8, 128)).reshape(TMB, 128)
                obuf[slot, :, n0:n0 + 128] = (x1_rows(row0, TMB, n0, n0 + 128) + z).astype(BF16)
            matmul(lambda k: ld16(act_v, 0, TMB, k * KH, (k + 1) * KH),
                   lambda k, n0: w2_v[k * KH:(k + 1) * KH, n0:n0 + 128],
                   tuple(range(nk)), range(0, D, 128), sink)

        U8 = NC

        def segment(*placements):
            sched = {}
            for items, units in placements:
                place(sched, items, units)
            begin(sched)

        with jax.named_scope("prologue"):
            zs[0] = 0
            begin({})
            start("c", "x0", "ca0", "q0", "sa0", "k0", "v0", "x4", "ca1", "sa1", "q1", "k1", "v1", "wo",
                  "x1", "m2", "x2")
            wait("c")
            cb_v[...] = jnp.broadcast_to(silu_c().astype(F32), (128, D)).T
            wait("x0")
            for r in range(0, NS * TM, LG):
                xf = x_v[r:r + LG, :].astype(F32)
                mu = jnp.mean(xf, axis=-1, keepdims=True)
                d = xf - mu
                rs = jax.lax.rsqrt(jnp.mean(d * d, axis=-1, keepdims=True) + EPS)
                stats[0, r:r + LG, :] = jnp.broadcast_to(mu, (LG, 128))
                stats[1, r:r + LG, :] = jnp.broadcast_to(rs, (LG, 128))
            wait("ca0")
            mod_mxu(1, 0)
            wait("q0")
            run_now(perm_qkv_items(0, 0))
            wait("sa0")
            mod_mxu(0, 0)
            run_now(ln1_out_items(0, 0))

        with jax.named_scope("pass1"):
            segment((ln1_out_items(1, 0), range(0, U8 - 2)),
                    (ln1_out_items(2, 0) + ln1_out_items(3, 0), range(U8 - 2, 2 * U8)))
            qkv_part(None, 0, 0, 0)
            qkv_part(None, 0, 1, 0)
            wait("k0")
            segment((perm_qkv_items(1, 0), range(0, 2 * U8 - 2)))
            for g, b in ((0, 2), (0, 3), (1, 0), (1, 1)):
                qkv_part(None, g, b, 0)
            wait("v0", "x4", "ca1")
            segment((perm_qkv_items(2, 0), range(0, 2 * U8 - 2)),
                    (staged(ln1_start(NS, 0)[:2], TM // LG, 1), range(2 * U8 - 1, 4 * U8 - 2)),
                    (mod_items(D + KH, 4) + [functools.partial(mod_finish, 1, KH, D)], range(2 * U8 - 2, 4 * U8)))
            for g, b in ((1, 2), (1, 3), (2, 0), (2, 1)):
                qkv_part(None, g, b, 0)
            wait("sa1", "q1")
            segment((mod_items(KH, 4) + [functools.partial(mod_finish, 0, KH, D)], range(0, U8 + 2)),
                    (perm_qkv_items(0, 1), range(0, 2 * U8 - 2)),
                    (ln1_out_items(0, 1), range(U8 + 3, 2 * U8 - 1)))
            qkv_part(None, 2, 2, 0)
            qkv_part(None, 2, 3, 0)

        with jax.named_scope("pass2"):
            wait("k1")
            segment((perm_qkv_items(1, 1), range(0, 2 * U8 - 2)),
                    (ln1_out_items(1, 1), range(0, U8 - 2)),
                    (ln1_out_items(2, 1), range(U8 - 2, 2 * U8)))
            halo("b", None, 1)
            qkv_part("b", 0, 0, 1)
            qkv_part("c", 0, 1, 1)
            wait("v1")
            l0 = logit_items("b", True)
            segment((perm_qkv_items(2, 1), range(0, 2 * U8 - 2)),
                    (ln1_out_items(3, 1), range(0, U8)),
                    (l0[:LB], range(B0, B1)))
            qkv_part("b", 1, 0, 1)
            halo("c", "b", 1)
            qkv_part("c", 1, 1, 1)
            qkv_part("b", 2, 0, 1)
            halo("b", None, 2)
            halo("c", "b", 2)
            qkv_part("c", 2, 1, 1)
            wait("wo")
            segment((perm_wo_items(), range(0, 46)),
                    (l0[LB:], range(0, C0)),
                    (pv_items("b"), range(C0 - 6, 39)),
                    (logit_items("c", False), range(C0, C1)),
                    (pv_items("c"), range(C1 - 12, 63)),
                    (logit_items("a", False), range(C1, C2)),
                    (pv_items("a"), range(C2 - 10, 79)),
                    (ln1_out_items(NS, 0) + ln1_out_items(NS, 1), range(79, 95)),
                    (logit_items("b", False), range(C2, 96 - L1)))
            halo("a", "c", 1)
            halo("a", "c", 2)
            for g in range(3):
                qkv_part("a", g, 2, 1)
            halo("b", "a", 1)
            qkv_part("b", 0, 3, 1)
            qkv_part("b", 1, 3, 1)
            halo("b", "a", 2)
            qkv_part("b", 2, 3, 1)
            wo_mm("b", 0)
            wo_mm("c", TM)
            wo_mm("a", 2 * TM)
            finish()
            wait("x1", "m2")
            start("m3", "w1", "w3", "w2")


        def half(X, Y, u0, sched, row_ln1, row_wo, extra):
            place(sched, pv_items(Y), range(u0 + P0, u0 + 3 * UP - P1))
            place(sched, logit_items(X, False), range(u0 + 2 * UP + L0, u0 + 4 * UP - L1))
            place(sched, ln1_items(row_ln1, Y), range(u0 + N0, u0 + N1))
            if extra:
                place(sched, extra, range(u0, u0 + 4 * UP - 1))

            def run():
                halo(X, Y, 1)
                halo(X, Y, 2)
                for g in range(3):
                    qkv_part(X, g)
                wo_mm(Y, row_wo)
            return run

        def a_step(s, carry):
            @pl.when(s == 3)
            def _():
                wait("x2", "m3")

            ra = pl.multiple_of(2 * s * TM, TM)
            nxt = pl.multiple_of(jnp.minimum(ra + 2 * TM, S - TM), TM)
            col0 = pl.multiple_of(jnp.minimum(2 * D + (s - 2) * (MT * 128), 6 * D - MT * 128), 128)
            mi = mod_items(col0, MT)
            sched = {}
            run_a = half("a", "b", 0, sched, ra + TM, ra - TM, mi[:len(mi) // 2])
            run_b = half("b", "a", 4 * UP, sched, nxt, ra, mi[len(mi) // 2:])
            begin(sched)
            run_a()
            run_b()
            finish()
            return carry

        with jax.named_scope("aloop"):
            if SKIP_A:
                wait("x2", "m3")
            else:
                jax.lax.fori_loop(NS // 2, NB // 2, a_step, 0)

        with jax.named_scope("atail"):
            begin({})
            for j in range(2, 6):
                mod_finish(j, 0, D)
            run_now(pv_items("b"))
            sched = {}
            place(sched, post_items(0), range(0, UP - 2))
            begin(sched)
            wo_mm("b", S - TM)
            finish()
            wait("w1", "w3", "w2")

        def b_step(j, carry):
            slot = j % 2

            @pl.when(j >= 2)
            def _():
                cp_out(j - 2, slot).wait()

            row0 = pl.multiple_of(j * TMB, TMB)
            nxt = pl.multiple_of(jnp.minimum(row0 + TMB, S - TMB), TMB)
            if SKIP_FFN:
                obuf[slot] = x1_rows(row0, TMB, 0, D).astype(BF16)
            else:
                ffn(row0, slot, nxt)
            cp_out(j, slot).start()
            return carry

        with jax.named_scope("bloop"):
            jax.lax.fori_loop(0, NBB, b_step, 0)
        with jax.named_scope("tail"):
            cp_out(NBB - 2, (NBB - 2) % 2).wait()
            cp_out(NBB - 1, (NBB - 1) % 2).wait()

    any_spec = pl.BlockSpec(memory_space=pl.ANY)
    scratch = [
        pltpu.VMEM((S, D), BF16),
        pltpu.VMEM((D, 3 * D), BF16),
        pltpu.VMEM((NC, KH // 2, 128), U32),
        pltpu.VMEM((D // 2, 3 * D), U32),
        pltpu.VMEM((D, D), BF16),
        pltpu.VMEM((NC, D // 32 * 17, 128), U32),
        pltpu.VMEM((D // 2, D), U32),
        pltpu.VMEM((D, F), BF16),
        pltpu.VMEM((D, F), BF16),
        pltpu.VMEM((F, D), BF16),
        pltpu.VMEM((D, 6 * D), BF16),
        pltpu.VMEM((D, 128), F32),
        pltpu.VMEM((NSUB, 8, 6 * D), F32),
        pltpu.VMEM((6, 8, D), F32),
        pltpu.VMEM((TM // 2, D), U32),
        pltpu.VMEM((TM // 2, D), U32),
        pltpu.VMEM((NS, TM // 2, D), U32),
        pltpu.VMEM((NS, 3 * NC, TM, 128), F32),
        pltpu.VMEM((2, (NS + 1) * TM, 128), F32),
        pltpu.VMEM((2 * NC, KV + PADK, 128), F32),
        pltpu.VMEM((NC, KV + PADK, 128), F32),
        pltpu.VMEM((WIN + 1, TM, 128), F32),
        pltpu.VMEM((2 * NC, KV + PADK, 128), F32),
        pltpu.VMEM((NC, KV + PADK, 128), F32),
        pltpu.VMEM((WIN + 1, TM, 128), F32),
        pltpu.VMEM((2 * NC, KV + PADK, 128), F32),
        pltpu.VMEM((NC, KV + PADK, 128), F32),
        pltpu.VMEM((WIN + 1, TM, 128), F32),
        pltpu.VMEM((TM // 2, D), U32),
        pltpu.VMEM((TM // 2, D), U32),
        pltpu.VMEM((TM // 2, D), U32),
        pltpu.VMEM((NC, RG, 128), F32),
        pltpu.VMEM((NC, RG, 128), F32),
        pltpu.VMEM((NC, RG, 128), F32),
        pltpu.VMEM((WIN, RG, 128), F32),
        pltpu.VMEM((WIN, RG, 128), F32),
        pltpu.VMEM((WIN, RG, 128), F32),
        pltpu.VMEM((2, TM, 128), F32),
        pltpu.VMEM((2, TMB, 128), F32),
        pltpu.VMEM((S, D), F32),
        pltpu.VMEM((TMB, D), F32),
        pltpu.VMEM((TMB // 2, D), U32),
        pltpu.VMEM((TMB // 2, F), U32),
        pltpu.VMEM((2, TMB, D), BF16),
        pltpu.VMEM((1, D), BF16),
        pltpu.SMEM((1,), jnp.int32),
        pltpu.SemaphoreType.DMA((NDMA,)),
        pltpu.SemaphoreType.DMA((2,)),
    ]

    def call(A_x, A_wqkv, A_wo, B_w1, B_w3, B_w2, c, w_mod):
        return pl.pallas_call(
            kernel,
            out_shape=jax.ShapeDtypeStruct((1, S, D), BF16),
            in_specs=[any_spec] * 8,
            out_specs=any_spec,
            scratch_shapes=scratch,
            compiler_params=pltpu.CompilerParams(vmem_limit_bytes=120 * 1024 * 1024),
        )(A_x, A_wqkv, A_wo, B_w1, B_w3, B_w2, c, w_mod)

    return call


@jax.jit
def pallas_adaLN_cond__sliding_local_dilated__glu_gated_swiglu__prompt_kernel(
    A_x: jax.Array,
    A_wqkv: jax.Array,
    A_wo: jax.Array,
    B_x: jax.Array,
    B_w1: jax.Array,
    B_w3: jax.Array,
    B_w2: jax.Array,
    c: jax.Array,
    w_mod: jax.Array,
):
    del B_x
    return _build()(A_x, A_wqkv, A_wo, B_w1, B_w3, B_w2, c, w_mod)
```

```python
import functools
import math

import jax
import jax.numpy as jnp
import jax.experimental.pallas as pl
import jax.experimental.pallas.tpu as pltpu

S = 2048
D = 1024
F = 3584
H = 32
DH = D // H
WIN = 8
DIL = 2
NC = D // 128
HALO = 16
EPS = 1e-5
NEG = -1000000000.0
SM_SCALE = DH ** -0.5
LOG2E = math.log2(math.e)

TM = 128
NB = S // TM
KV = HALO + TM
RG = 8
LG = 16
NS = 4
NDMA = 21
KH = 512

F32 = jnp.float32
BF16 = jnp.bfloat16
U32 = jnp.uint32


def _tree(op, xs):
    xs = list(xs)
    while len(xs) > 1:
        xs = [op(xs[i], xs[i + 1]) if i + 1 < len(xs) else xs[i] for i in range(0, len(xs), 2)]
    return xs[0]


def _add(a, b):
    return a + b


def _build(TMB=128, FC=512, GATE=True, SKIP_FFN=False, SKIP_A=False,
           SCH=0, MT=6, NSUB=16, PB1=5, L0=0, L1=1, SPREAD=128, LLAG=3,
           P0=0, P1=16, N0=1, N1=30, PR=64, B0=14, B1=30, LB=19, PADK=0, C0=10, C1=38, C2=64, CP=0, WS=46, H0=0, H1=10):
    NBB = S // TMB

    def kernel(x_hbm, wqkv_hbm, wo_hbm, w1_hbm, w3_hbm, w2_hbm, c_hbm, wmod_hbm,
               out_hbm,
               x_v, wqkv_v, wtmp, wqkv_p, wo_v, wo_tmp, wo_p, w1_v, w3_v, w2_v, wmod_v, cb_v, modp_v, mod_v,
               h1a, h1b, h1s, part, stats, qka, va, pa, qkb, vb, pb_, qkc, vc, pc, oa, ob, oc, ota, otb, otc, sl0, sl1, sl2, stat1, stat2, y_v, x1n, h2_v, act_v, obuf, c_ref,
               zs, sem_w, sem_o):
        bufs = {"a": (h1a, qka, va, oa, pa), "b": (h1b, qkb, vb, ob, pb_),
                "c": (None, qkc, vc, oc, pc)}

        sls = (sl0, sl1, sl2)
        otmps = {"a": ota, "b": otb, "c": otc}

        dmas = {}

        def add_dma(name, src, dst):
            dmas[name] = (src, dst, len(dmas))

        for name, (b0, b1) in (("x0", (0, NS)), ("x4", (NS, NS + 1)), ("x1", (NS + 1, NS + 3)), ("x2", (NS + 3, NB))):
            rows = pl.ds(b0 * TM, (b1 - b0) * TM)
            add_dma(name, x_hbm.at[0, rows, :], x_v.at[rows, :])
        for name, (c0, c1) in (("sa0", (0, KH)), ("sa1", (KH, D)), ("ca0", (D, D + KH)), ("ca1", (D + KH, 2 * D)),
                               ("m2", (2 * D, 3 * D)), ("m3", (3 * D, 6 * D))):
            cols = pl.ds(c0, c1 - c0)
            add_dma(name, wmod_hbm.at[:, cols], wmod_v.at[:, cols])
        for g in range(3):
            for k in range(2):
                rows, cols = pl.ds(k * KH, KH), pl.ds(g * D, D)
                add_dma("qkv"[g] + str(k), wqkv_hbm.at[rows, cols], wqkv_v.at[rows, cols])
        add_dma("c", c_hbm, c_ref)
        add_dma("wo", wo_hbm, wo_v)
        add_dma("w1", w1_hbm, w1_v)
        add_dma("w3", w3_hbm, w3_v)
        add_dma("w2", w2_hbm, w2_v)
        assert len(dmas) == NDMA

        def cp(name):
            src, dst, i = dmas[name]
            return pltpu.make_async_copy(src, dst, sem_w.at[i])

        def start(*names):
            for n in names:
                cp(n).start()

        def wait(*names):
            for n in names:
                cp(n).wait()

        def cp_out(j, slot):
            return pltpu.make_async_copy(obuf.at[slot],
                                         out_hbm.at[0, pl.ds(j * TMB, TMB), :], sem_o.at[slot])

        st = {"z": None, "never": None, "clock": 0, "sched": {}, "tok": None}

        have = set()

        def need(*keys):
            assert all(k in have for k in keys), keys

        def begin(sched):
            z = zs[0]
            st.update(z=z, never=jnp.full((8, 128), z, jnp.int32) != 0, clock=0, sched=sched, tok=None)

        def gate(val, i, n):
            r = st["tok"]
            if r is None or not GATE:
                return val
            row = (i * SPREAD // n) // 8 * 8
            t = r[row:row + 8]
            return jnp.where(st["never"], t if val.dtype == F32 else pltpu.bitcast(t, val.dtype), val)

        def place(sched, items, units):
            units = list(units)
            for i, it in enumerate(items):
                sched.setdefault(units[(i * len(units)) // len(items)], []).append(it)

        def matmul(lhs_fn, w_fn, ks, cols, sink, gives=None):
            for n0 in cols:
                r = None
                for k in ks:
                    d = jnp.dot(lhs_fn(k), w_fn(k, n0), preferred_element_type=F32)
                    r = d if r is None else r + d
                    if k == ks[-1]:
                        sink(n0, r)
                    if n0 == cols[-1] and k == ks[-1]:
                        have.add(gives)
                    st["tok"] = r
                    for fn in st["sched"].pop(st["clock"], []):
                        fn()
                    st["tok"] = None
                    st["clock"] += 1

        def finish():
            assert not st["sched"]

        def lane_iota(rows):
            return jax.lax.broadcasted_iota(jnp.int32, (rows, 128), 1)

        def ld16(ref, r0, n, c0, c1):
            return pltpu.bitcast(ref[r0 // 2:(r0 + n) // 2, c0:c1], BF16)

        def silu_c():
            cf = c_ref[...].astype(F32)
            return (cf * jax.nn.sigmoid(cf)).astype(BF16)

        def mod_mxu(j, k):
            cs = slice(k * KH, (k + 1) * KH)
            lhs = jnp.broadcast_to(silu_c(), (16, D))
            r = jnp.dot(lhs, wmod_v[:, j * D + k * KH:j * D + (k + 1) * KH], preferred_element_type=F32)[0:8]
            mod_v[j, :, cs] = r + 1.0 if j in (1, 4) else r

        def mod_finish(j, c0, c1):
            r = _tree(_add, [modp_v[i, :, j * D + c0:j * D + c1] for i in range(NSUB)])
            r = jnp.sum(r, axis=0, keepdims=True)
            mod_v[j, :, c0:c1] = jnp.broadcast_to(r + 1.0 if j in (1, 4) else r, (8, c1 - c0))

        def mod_items(col0, ntiles):
            rows = D // NSUB

            def one(t, i):
                c0 = col0 + t * 128
                c0 = c0 if isinstance(c0, int) else pl.multiple_of(c0, 128)
                w = wmod_v[i * rows:(i + 1) * rows, pl.ds(c0, 128)].astype(F32)
                p = (w * cb_v[i * rows:(i + 1) * rows, :]).reshape(rows // 8, 8, 128)
                modp_v[i, :, pl.ds(c0, 128)] = gate(_tree(_add, [p[k] for k in range(rows // 8)]), 1, 2)
            return [functools.partial(one, t, i) for t in range(ntiles) for i in range(NSUB)]

        def perm_mix(g, i, nrows):
            n = nrows // 2
            l = lane_iota(n)
            vals = [pltpu.bitcast(wqkv_v[i * nrows:(i + 1) * nrows, g * D + c * 128: g * D + (c + 1) * 128], U32)
                    for c in range(NC)]
            for b in range(3):
                m = ((l >> (2 + b)) & 1) == 0
                for c in range(NC):
                    if c & (1 << b):
                        continue
                    lo, hi = vals[c], vals[c | (1 << b)]
                    vals[c] = jnp.where(m, lo, hi)
                    vals[c | (1 << b)] = jnp.where(m, hi, lo)
            p0 = (i * n) % (KH // 2)
            for j in range(NC):
                v = jnp.concatenate([gate(vals[j][q:q + 8], j, NC) for q in range(0, n, 8)], axis=0)
                wtmp[j, pl.ds(pl.multiple_of(zrow(p0), 8), n), :] = v

        def perm_gather(g, k, j):
            have.add(("w", g, k, j))
            l = lane_iota(8)
            idx = ((((l >> 1) & 3) << 5) | ((((l >> 3) & 7) ^ j) << 2) | ((l >> 6) << 1) | (l & 1))
            for q in range(0, KH // 2, 8):
                t = jnp.take_along_axis(gate(wtmp[j, q:q + 8, :], q, KH // 2), idx, axis=1,
                                        mode="promise_in_bounds")
                wqkv_p[k * KH // 2 + q:k * KH // 2 + q + 8, g * D + j * 128: g * D + (j + 1) * 128] = t

        def perm_qkv_items(g, k, nrows=PR):
            n = KH // nrows
            return ([functools.partial(perm_mix, g, i, nrows) for i in range(k * n, (k + 1) * n)]
                    + [functools.partial(perm_gather, g, k, j) for j in range(NC)])

        def perm_wo_items():
            low = jax.lax.broadcasted_iota(jnp.int32, (8, 128), 0) < 4

            def spread(c, h):
                for r in range(h * 256, h * 256 + 256, 8):
                    wo_tmp[c, pl.ds(zrow(r + r // 16), 8), :] = gate(pltpu.bitcast(
                        wo_v[2 * r:2 * r + 16, c * 128:(c + 1) * 128], U32), r % 256, 256)

            def gather(c, h):
                for G in range(h * 32, h * 32 + 32):
                    j, e, ch = G >> 3, (G >> 2) & 1, G & 3
                    dd = (((2 * ch) ^ j) << 1) | e
                    ta = wo_tmp[c, pl.ds(ch * 136 + dd, 8, stride=17), :]
                    tb = wo_tmp[c, pl.ds(ch * 136 + (dd ^ 2), 8, stride=17), :]
                    wo_p[G * 8:G * 8 + 8, c * 128:(c + 1) * 128] = jnp.where(low, ta, tb)
            return [functools.partial(fn, c, h) for fn in (spread, gather) for c in range(NC) for h in range(2)]

        def zrow(row, k=1):
            return row + k * st["z"]

        def gate16(v, i, n):
            return jnp.concatenate([gate(v[q:q + 8], i, n) for q in range(0, LG, 8)], axis=0)

        def staged(stages, n, lag):
            items = []
            for t in range(n + lag * (len(stages) - 1)):
                for k in reversed(range(len(stages))):
                    if 0 <= t - k * lag < n:
                        items.append(functools.partial(stages[k], t - k * lag))
            return items

        def ln_stages(load, stat, dst, j_scale, j_shift, cols=range(NC)):
            def chunks(x):
                return [x[:, c * 128:(c + 1) * 128] for c in range(NC)]

            def put(j, r, part, fn):
                m = jnp.sum(part, axis=-1, keepdims=True) * (1.0 / D)
                stat[j, pl.ds(pl.multiple_of(zrow(r), LG), LG), :] = jnp.broadcast_to(fn(m), (LG, 128))

            def s_mean(i):
                put(0, i * LG, gate16(_tree(_add, chunks(load(i * LG, 0))), 1, 2), lambda m: m)

            def s_var(i):
                r = i * LG
                mu = gate16(stat[0, r:r + LG, :], 0, 1)
                put(1, r, _tree(_add, [(x - mu) * (x - mu) for x in chunks(load(r, 1))]),
                    lambda m: jax.lax.rsqrt(m + EPS))

            def s_out(i):
                r = i * LG
                mu, rs = stat[0, r:r + LG, :], stat[1, r:r + LG, :]
                xs = chunks(load(r, 2))
                for c in cols:
                    x, cs = xs[c], slice(c * 128, (c + 1) * 128)
                    if c % (NC // 2) == 0:
                        rg = gate16(rs, c - cols[0], NC)
                    y = ((x - mu) * rg).reshape(LG // 8, 8, 128) * mod_v[j_scale, :, cs][None] + mod_v[j_shift, :, cs][None]
                    dst[r // 2:(r + LG) // 2, cs] = pltpu.bitcast(y.reshape(LG, 128).astype(BF16), U32)
            return s_mean, s_var, s_out

        def load_x(row0):
            return lambda r, k: x_v[pl.ds(pl.multiple_of(zrow(row0 + r, k), LG), LG), :].astype(F32)

        def ln1_items(row0, buf):
            return staged(ln_stages(load_x(row0), stat1, bufs[buf][0], 1, 0), TM // LG, 1)

        def ln1_start(b, k):
            return ln_stages(load_x(b * TM), stats.at[:, pl.ds(b * TM, TM), :], h1s.at[b] if b < NS else h1a,
                             1, 0, range(k * NC // 2, (k + 1) * NC // 2))

        def ln1_out_items(b, k):
            def one(i):
                have.add(("h", b, k, i))
                ln1_start(b, k)[2](i)
            return [functools.partial(one, i) for i in range(TM // LG)]

        def x1_rows(row, n, c0, c1):
            xf = x_v[pl.ds(row, n), c0:c1].astype(F32).reshape(n // 8, 8, c1 - c0)
            y = y_v[pl.ds(row, n), c0:c1].reshape(n // 8, 8, c1 - c0)
            return (xf + mod_v[2, :, c0:c1][None] * y).reshape(n, c1 - c0)

        def post_items(row0):
            def load(r, k):
                if k:
                    return x1n[pl.ds(pl.multiple_of(zrow(r, k), LG), LG), :]
                x1 = x1_rows(row0 + r, LG, 0, D)
                x1n[r:r + LG, :] = x1
                return x1
            return staged(ln_stages(load, stat2, h2_v, 4, 3), TMB // LG, 1)

        def logit_items(buf, first):
            _, qk, _, _, pb = bufs[buf]
            swap = lane_iota(RG) ^ 1

            def s_logit(g):
                need(("q", buf), ("k", buf))
                have.add(("l", buf, g))
                r = g * RG
                qs = [qk[c, HALO + r:HALO + r + RG, :] for c in range(NC)]
                for w in range(WIN):
                    k0 = HALO + r - DIL * w
                    if w >= WIN // 2:
                        k0 = zrow(k0)
                    s = _tree(_add, [qs[c] * qk[NC + c, pl.ds(k0, RG), :] for c in range(NC)])
                    s = gate(s, w, WIN)
                    s = s + pltpu.roll(s, 64, 1)
                    s = s + jnp.take_along_axis(s, swap, axis=1, mode="promise_in_bounds")
                    if first and r < DIL * w:
                        pos = r + jax.lax.broadcasted_iota(jnp.int32, (RG, 128), 0)
                        s = jnp.where(pos >= DIL * w, s, NEG * LOG2E)
                    sls[g % len(sls)][w, pl.ds(pl.multiple_of(zrow(0), RG), RG), :] = s

            def s_soft(g):
                assert ("p", buf, g) not in have
                have.add(("p", buf, g))
                r = g * RG
                ss = [sls[g % len(sls)][w] for w in range(WIN)]
                m = gate(_tree(jnp.maximum, ss), 0, 1)
                es = [jnp.exp2(s - m) for s in ss]
                for w in range(WIN):
                    pb[w, r:r + RG, :] = es[w]
                den = _tree(_add, es)
                inv = pl.reciprocal(den, approx=True)
                pb[WIN, r:r + RG, :] = inv * (2.0 - den * inv)
            return staged((s_logit, s_soft), TM // RG, LLAG)

        def pv_items(buf):
            _, _, vp, o, pb = bufs[buf]
            otmp = otmps[buf]

            def one(r):
                need(("v", buf), ("p", buf, r // RG))
                have.remove(("p", buf, r // RG))
                have.add(("o", buf, r // RG))
                ps = [pb[w, pl.ds(pl.multiple_of(zrow(r), RG), RG), :] for w in range(WIN + 1)]
                for c in range(NC):
                    ks = [HALO + r - DIL * w if w < WIN // 2 else zrow(HALO + r - DIL * w) for w in range(WIN)]
                    acc = _tree(_add, [ps[w] * vp[c, pl.ds(ks[w], RG), :] for w in range(WIN)])
                    acc = gate(acc * ps[WIN], c, NC)
                    if (r // RG) % 2 == 0:
                        otmp[c, pl.ds(pl.multiple_of(zrow(0), 8), RG), :] = acc
                    else:
                        both = jnp.concatenate([otmp[c], acc], axis=0).astype(BF16)
                        o[(r - RG) // 2:(r + RG) // 2, c * 128:(c + 1) * 128] = pltpu.bitcast(both, U32)
            return [functools.partial(one, r) for r in range(0, TM, RG)]

        def halo(buf, prev, part):
            _, qk, vp, _, _ = bufs[buf]
            for c in range(NC):
                if part == 1:
                    qk[NC + c, 0:HALO, :] = (jnp.zeros((HALO, 128), F32) if prev is None
                                             else gate16(bufs[prev][1][NC + c, TM:TM + HALO, :], 1, 2))
                else:
                    vp[c, 0:HALO, :] = (jnp.broadcast_to(vp[c, HALO:HALO + 1, :], (HALO, 128)) if prev is None
                                        else gate16(bufs[prev][2][c, TM:TM + HALO, :], 1, 2))

        def qkv_part(buf, g, sb=None, k=None):
            h1, qk, vp, _, _ = bufs[buf] if buf else (None,) * 5
            if sb is not None:
                h1 = h1s.at[sb]
                need(*[("h", sb, k, i) for i in range(TM // LG)], *[("w", g, k, j) for j in range(NC)])
            if k != 0:
                for i in range(TM // RG):
                    if g < 2 and ("qk"[g], buf) in have:
                        need(("l", buf, i))
                    if g == 2 and ("v", buf) in have:
                        assert ("p", buf, i) not in have or ("new", buf) in have
                if g == 1:
                    have.difference_update({("l", buf, i) for i in range(TM // RG)})
                    have.add(("new", buf))
                have.discard(("qkv"[g], buf))

            def sink(n0, r):
                ch = n0 // 128
                if k == 0:
                    part[sb, ch] = r
                    return
                if k == 1:
                    r = r + part[sb, ch]
                dst, ci = (qk, ch) if ch < 2 * NC else (vp, ch - 2 * NC)
                dst[ci, HALO:HALO + TM, :] = r * (SM_SCALE * LOG2E) if ch < NC else r
            matmul(lambda kk: ld16(h1, 0, TM, kk * KH, (kk + 1) * KH),
                   lambda kk, n0: ld16(wqkv_p, kk * KH, KH, n0, n0 + 128),
                   (0, 1) if k is None else (k,), range(g * D, (g + 1) * D, 128), sink,
                   None if k == 0 else ("qkv"[g], buf))
            if g == 2:
                have.discard(("new", buf))

        def wo_mm(buf, row0):
            o = bufs[buf][3]
            need(*[("o", buf, i) for i in range(TM // RG)])
            have.difference_update({("o", buf, i) for i in range(TM // RG)})

            def sink(n0, r):
                y_v[pl.ds(row0, TM), n0:n0 + 128] = r
            matmul(lambda k: ld16(o, 0, TM, k * KH, (k + 1) * KH),
                   lambda k, n0: ld16(wo_p, k * KH, KH, n0, n0 + 128),
                   (0, 1), range(0, D, 128), sink)

        UP = NC * (D // KH)

        def run_now(items):
            for fn in items:
                fn()

        def ffn(row0, slot, nxt_row):
            h = ld16(h2_v, 0, TMB, 0, D)
            for f0 in range(0, F, FC):
                g = jnp.dot(h, w1_v[:, f0:f0 + FC], preferred_element_type=F32)
                u = jnp.dot(h, w3_v[:, f0:f0 + FC], preferred_element_type=F32)
                act_v[:, f0:f0 + FC] = pltpu.bitcast((g * jax.nn.sigmoid(g) * u).astype(BF16), U32)
            nk = F // KH
            sched = {}
            place(sched, post_items(nxt_row), range(0, NC * nk - PB1))
            begin(sched)

            def sink(n0, r):
                z = (mod_v[5, :, n0:n0 + 128][None] * r.reshape(TMB // 8, 8, 128)).reshape(TMB, 128)
                obuf[slot, :, n0:n0 + 128] = (x1_rows(row0, TMB, n0, n0 + 128) + z).astype(BF16)
            matmul(lambda k: ld16(act_v, 0, TMB, k * KH, (k + 1) * KH),
                   lambda k, n0: w2_v[k * KH:(k + 1) * KH, n0:n0 + 128],
                   tuple(range(nk)), range(0, D, 128), sink)

        U8 = NC

        def segment(*placements):
            sched = {}
            for items, units in placements:
                place(sched, items, units)
            begin(sched)

        with jax.named_scope("prologue"):
            zs[0] = 0
            begin({})
            start("c", "x0", "ca0", "q0", "sa0", "k0", "v0", "x4", "ca1", "sa1", "q1", "k1", "v1", "wo",
                  "x1", "m2", "x2")
            wait("c")
            cb_v[...] = jnp.broadcast_to(silu_c().astype(F32), (128, D)).T
            wait("x0")
            for r in range(0, NS * TM, LG):
                xf = x_v[r:r + LG, :].astype(F32)
                mu = jnp.mean(xf, axis=-1, keepdims=True)
                d = xf - mu
                rs = jax.lax.rsqrt(jnp.mean(d * d, axis=-1, keepdims=True) + EPS)
                stats[0, r:r + LG, :] = jnp.broadcast_to(mu, (LG, 128))
                stats[1, r:r + LG, :] = jnp.broadcast_to(rs, (LG, 128))
            wait("ca0")
            mod_mxu(1, 0)
            wait("q0")
            run_now(perm_qkv_items(0, 0))
            wait("sa0")
            mod_mxu(0, 0)
            run_now(ln1_out_items(0, 0))

        with jax.named_scope("pass1"):
            segment((ln1_out_items(1, 0), range(0, U8 - 2)),
                    (ln1_out_items(2, 0) + ln1_out_items(3, 0), range(U8 - 2, 2 * U8)))
            qkv_part(None, 0, 0, 0)
            qkv_part(None, 0, 1, 0)
            wait("k0")
            segment((perm_qkv_items(1, 0), range(0, 2 * U8 - 2)))
            for g, b in ((0, 2), (0, 3), (1, 0), (1, 1)):
                qkv_part(None, g, b, 0)
            wait("v0", "x4", "ca1")
            segment((perm_qkv_items(2, 0), range(0, 2 * U8 - 2)),
                    (staged(ln1_start(NS, 0)[:2], TM // LG, 1), range(2 * U8 - 1, 4 * U8 - 2)),
                    (mod_items(D + KH, 4) + [functools.partial(mod_finish, 1, KH, D)], range(2 * U8 - 2, 4 * U8)))
            for g, b in ((1, 2), (1, 3), (2, 0), (2, 1)):
                qkv_part(None, g, b, 0)
            wait("sa1", "q1")
            segment((mod_items(KH, 4) + [functools.partial(mod_finish, 0, KH, D)], range(0, U8 + 2)),
                    (perm_qkv_items(0, 1), range(0, 2 * U8 - 2)),
                    (ln1_out_items(0, 1), range(U8 + 3, 2 * U8 - 1)))
            qkv_part(None, 2, 2, 0)
            qkv_part(None, 2, 3, 0)

        with jax.named_scope("pass2"):
            wait("k1")
            segment((perm_qkv_items(1, 1), range(0, 2 * U8 - 2)),
                    (ln1_out_items(1, 1), range(0, U8 - 2)),
                    (ln1_out_items(2, 1), range(U8 - 2, 2 * U8)))
            halo("b", None, 1)
            qkv_part("b", 0, 0, 1)
            qkv_part("c", 0, 1, 1)
            wait("v1")
            l0 = logit_items("b", True)
            segment((perm_qkv_items(2, 1), range(0, 2 * U8 - 2)),
                    (ln1_out_items(3, 1), range(0, U8)),
                    (l0[:LB], range(B0, B1)))
            qkv_part("b", 1, 0, 1)
            halo("c", "b", 1)
            qkv_part("c", 1, 1, 1)
            qkv_part("b", 2, 0, 1)
            halo("b", None, 2)
            halo("c", "b", 2)
            qkv_part("c", 2, 1, 1)
            wait("wo")
            segment((perm_wo_items(), range(0, WS)),
                    (l0[LB:], range(0, C0)),
                    (pv_items("b"), range(C0 + CP, 39)),
                    (logit_items("c", False), range(C0, C1)),
                    (pv_items("c"), range(C1 + CP, 63)),
                    (logit_items("a", False), range(C1, C2)),
                    (pv_items("a"), range(C2 + CP, 79)),
                    ([functools.partial(halo, "b", "a", 1)], [23]),
                    ([functools.partial(halo, "b", "a", 2)], [39]),
                    (ln1_out_items(NS, 0) + ln1_out_items(NS, 1), range(H0, H1)),
                    (logit_items("b", False), range(C2, 96 - L1)))
            halo("a", "c", 1)
            halo("a", "c", 2)
            for g in range(3):
                qkv_part("a", g, 2, 1)
            for g in range(3):
                qkv_part("b", g, 3, 1)
            wo_mm("b", 0)
            wo_mm("c", TM)
            wo_mm("a", 2 * TM)
            finish()
            wait("x1", "m2")
            start("m3", "w1", "w3", "w2")


        def half(X, Y, u0, sched, row_ln1, row_wo, extra):
            place(sched, pv_items(Y), range(u0 + P0, u0 + 3 * UP - P1))
            place(sched, logit_items(X, False), range(u0 + 2 * UP + L0, u0 + 4 * UP - L1))
            place(sched, ln1_items(row_ln1, Y), range(u0 + N0, u0 + N1))
            if extra:
                place(sched, extra, range(u0, u0 + 4 * UP - 1))

            def run():
                halo(X, Y, 1)
                halo(X, Y, 2)
                for g in range(3):
                    qkv_part(X, g)
                wo_mm(Y, row_wo)
            return run

        def a_step(s, carry):
            @pl.when(s == 3)
            def _():
                wait("x2", "m3")

            ra = pl.multiple_of(2 * s * TM, TM)
            nxt = pl.multiple_of(jnp.minimum(ra + 2 * TM, S - TM), TM)
            col0 = pl.multiple_of(jnp.minimum(2 * D + (s - 2) * (MT * 128), 6 * D - MT * 128), 128)
            mi = mod_items(col0, MT)
            sched = {}
            run_a = half("a", "b", 0, sched, ra + TM, ra - TM, mi[:len(mi) // 2])
            run_b = half("b", "a", 4 * UP, sched, nxt, ra, mi[len(mi) // 2:])
            begin(sched)
            run_a()
            run_b()
            finish()
            return carry

        with jax.named_scope("aloop"):
            if SKIP_A:
                wait("x2", "m3")
            else:
                jax.lax.fori_loop(NS // 2, NB // 2, a_step, 0)

        with jax.named_scope("atail"):
            begin({})
            for j in range(2, 6):
                mod_finish(j, 0, D)
            run_now(pv_items("b"))
            sched = {}
            place(sched, post_items(0), range(0, UP - 2))
            begin(sched)
            wo_mm("b", S - TM)
            finish()
            wait("w1", "w3", "w2")

        def b_step(j, carry):
            slot = j % 2

            @pl.when(j >= 2)
            def _():
                cp_out(j - 2, slot).wait()

            row0 = pl.multiple_of(j * TMB, TMB)
            nxt = pl.multiple_of(jnp.minimum(row0 + TMB, S - TMB), TMB)
            if SKIP_FFN:
                obuf[slot] = x1_rows(row0, TMB, 0, D).astype(BF16)
            else:
                ffn(row0, slot, nxt)
            cp_out(j, slot).start()
            return carry

        with jax.named_scope("bloop"):
            jax.lax.fori_loop(0, NBB, b_step, 0)
        with jax.named_scope("tail"):
            cp_out(NBB - 2, (NBB - 2) % 2).wait()
            cp_out(NBB - 1, (NBB - 1) % 2).wait()

    any_spec = pl.BlockSpec(memory_space=pl.ANY)
    scratch = [
        pltpu.VMEM((S, D), BF16),
        pltpu.VMEM((D, 3 * D), BF16),
        pltpu.VMEM((NC, KH // 2, 128), U32),
        pltpu.VMEM((D // 2, 3 * D), U32),
        pltpu.VMEM((D, D), BF16),
        pltpu.VMEM((NC, D // 32 * 17, 128), U32),
        pltpu.VMEM((D // 2, D), U32),
        pltpu.VMEM((D, F), BF16),
        pltpu.VMEM((D, F), BF16),
        pltpu.VMEM((F, D), BF16),
        pltpu.VMEM((D, 6 * D), BF16),
        pltpu.VMEM((D, 128), F32),
        pltpu.VMEM((NSUB, 8, 6 * D), F32),
        pltpu.VMEM((6, 8, D), F32),
        pltpu.VMEM((TM // 2, D), U32),
        pltpu.VMEM((TM // 2, D), U32),
        pltpu.VMEM((NS, TM // 2, D), U32),
        pltpu.VMEM((NS, 3 * NC, TM, 128), F32),
        pltpu.VMEM((2, (NS + 1) * TM, 128), F32),
        pltpu.VMEM((2 * NC, KV + PADK, 128), F32),
        pltpu.VMEM((NC, KV + PADK, 128), F32),
        pltpu.VMEM((WIN + 1, TM, 128), F32),
        pltpu.VMEM((2 * NC, KV + PADK, 128), F32),
        pltpu.VMEM((NC, KV + PADK, 128), F32),
        pltpu.VMEM((WIN + 1, TM, 128), F32),
        pltpu.VMEM((2 * NC, KV + PADK, 128), F32),
        pltpu.VMEM((NC, KV + PADK, 128), F32),
        pltpu.VMEM((WIN + 1, TM, 128), F32),
        pltpu.VMEM((TM // 2, D), U32),
        pltpu.VMEM((TM // 2, D), U32),
        pltpu.VMEM((TM // 2, D), U32),
        pltpu.VMEM((NC, RG, 128), F32),
        pltpu.VMEM((NC, RG, 128), F32),
        pltpu.VMEM((NC, RG, 128), F32),
        pltpu.VMEM((WIN, RG, 128), F32),
        pltpu.VMEM((WIN, RG, 128), F32),
        pltpu.VMEM((WIN, RG, 128), F32),
        pltpu.VMEM((2, TM, 128), F32),
        pltpu.VMEM((2, TMB, 128), F32),
        pltpu.VMEM((S, D), F32),
        pltpu.VMEM((TMB, D), F32),
        pltpu.VMEM((TMB // 2, D), U32),
        pltpu.VMEM((TMB // 2, F), U32),
        pltpu.VMEM((2, TMB, D), BF16),
        pltpu.VMEM((1, D), BF16),
        pltpu.SMEM((1,), jnp.int32),
        pltpu.SemaphoreType.DMA((NDMA,)),
        pltpu.SemaphoreType.DMA((2,)),
    ]

    def call(A_x, A_wqkv, A_wo, B_w1, B_w3, B_w2, c, w_mod):
        return pl.pallas_call(
            kernel,
            out_shape=jax.ShapeDtypeStruct((1, S, D), BF16),
            in_specs=[any_spec] * 8,
            out_specs=any_spec,
            scratch_shapes=scratch,
            compiler_params=pltpu.CompilerParams(vmem_limit_bytes=120 * 1024 * 1024),
        )(A_x, A_wqkv, A_wo, B_w1, B_w3, B_w2, c, w_mod)

    return call


@jax.jit
def pallas_adaLN_cond__sliding_local_dilated__glu_gated_swiglu__prompt_kernel(
    A_x: jax.Array,
    A_wqkv: jax.Array,
    A_wo: jax.Array,
    B_x: jax.Array,
    B_w1: jax.Array,
    B_w3: jax.Array,
    B_w2: jax.Array,
    c: jax.Array,
    w_mod: jax.Array,
):
    del B_x
    return _build()(A_x, A_wqkv, A_wo, B_w1, B_w3, B_w2, c, w_mod)
```

```python
import functools
import math

import jax
import jax.numpy as jnp
import jax.experimental.pallas as pl
import jax.experimental.pallas.tpu as pltpu

S = 2048
D = 1024
F = 3584
H = 32
DH = D // H
WIN = 8
DIL = 2
NC = D // 128
HALO = 16
EPS = 1e-5
NEG = -1000000000.0
SM_SCALE = DH ** -0.5
LOG2E = math.log2(math.e)

TM = 128
NB = S // TM
KV = HALO + TM
RG = 8
LG = 16
NS = 4
NDMA = 21
KH = 512

F32 = jnp.float32
BF16 = jnp.bfloat16
U32 = jnp.uint32


def _tree(op, xs):
    xs = list(xs)
    while len(xs) > 1:
        xs = [op(xs[i], xs[i + 1]) if i + 1 < len(xs) else xs[i] for i in range(0, len(xs), 2)]
    return xs[0]


def _add(a, b):
    return a + b


def _build(TMB=256, FC=512, GATE=True, SKIP_FFN=False, SKIP_A=False,
           SCH=0, MT=6, NSUB=16, PB1=5, L0=0, L1=1, SPREAD=128, LLAG=3,
           P0=0, P1=16, N0=1, N1=30, PR=64, B0=14, B1=30, LB=19, PADK=0, C0=10, C1=38, C2=64, CP=0, WS=46, H0=0, H1=10, TAILV=2, TB=16, OCUT=(0, 512, 896, 1024)):
    NBB = S // TMB
    NQ = len(OCUT) - 1

    def kernel(x_hbm, wqkv_hbm, wo_hbm, w1_hbm, w3_hbm, w2_hbm, c_hbm, wmod_hbm,
               out_hbm,
               x_v, wqkv_v, wtmp, wqkv_p, wo_v, wo_tmp, wo_p, w1_v, w3_v, w2_v, wmod_v, cb_v, modp_v, mod_v,
               h1a, h1b, h1s, part, stats, qka, va, pa, qkb, vb, pb_, qkc, vc, pc, oa, ob, oc, ota, otb, otc, sl0, sl1, sl2, stat1, stat2, y_v, x1n, h2_v, act_v, obuf, c_ref,
               zs, sem_w, sem_o):
        bufs = {"a": (h1a, qka, va, oa, pa), "b": (h1b, qkb, vb, ob, pb_),
                "c": (None, qkc, vc, oc, pc)}

        sls = (sl0, sl1, sl2)
        otmps = {"a": ota, "b": otb, "c": otc}

        dmas = {}

        def add_dma(name, src, dst):
            dmas[name] = (src, dst, len(dmas))

        for name, (b0, b1) in (("x0", (0, NS)), ("x4", (NS, NS + 1)), ("x1", (NS + 1, NS + 3)), ("x2", (NS + 3, NB))):
            rows = pl.ds(b0 * TM, (b1 - b0) * TM)
            add_dma(name, x_hbm.at[0, rows, :], x_v.at[rows, :])
        for name, (c0, c1) in (("sa0", (0, KH)), ("sa1", (KH, D)), ("ca0", (D, D + KH)), ("ca1", (D + KH, 2 * D)),
                               ("m2", (2 * D, 3 * D)), ("m3", (3 * D, 6 * D))):
            cols = pl.ds(c0, c1 - c0)
            add_dma(name, wmod_hbm.at[:, cols], wmod_v.at[:, cols])
        for g in range(3):
            for k in range(2):
                rows, cols = pl.ds(k * KH, KH), pl.ds(g * D, D)
                add_dma("qkv"[g] + str(k), wqkv_hbm.at[rows, cols], wqkv_v.at[rows, cols])
        add_dma("c", c_hbm, c_ref)
        add_dma("wo", wo_hbm, wo_v)
        add_dma("w1", w1_hbm, w1_v)
        add_dma("w3", w3_hbm, w3_v)
        add_dma("w2", w2_hbm, w2_v)
        assert len(dmas) == NDMA

        def cp(name):
            src, dst, i = dmas[name]
            return pltpu.make_async_copy(src, dst, sem_w.at[i])

        def start(*names):
            for n in names:
                cp(n).start()

        def wait(*names):
            for n in names:
                cp(n).wait()

        def cp_out(j, slot, q):
            c0, c1 = OCUT[q], OCUT[q + 1]
            return pltpu.make_async_copy(obuf.at[slot, :, pl.ds(c0, c1 - c0)],
                                         out_hbm.at[0, pl.ds(j * TMB, TMB), pl.ds(c0, c1 - c0)],
                                         sem_o.at[slot * NQ + q])

        def wait_out(j, slot):
            for q in range(NQ):
                cp_out(j, slot, q).wait()

        st = {"z": None, "never": None, "clock": 0, "sched": {}, "tok": None}

        have = set()

        def need(*keys):
            assert all(k in have for k in keys), keys

        def begin(sched):
            z = zs[0]
            st.update(z=z, never=jnp.full((8, 128), z, jnp.int32) != 0, clock=0, sched=sched, tok=None)

        def gate(val, i, n):
            r = st["tok"]
            if r is None or not GATE:
                return val
            row = (i * SPREAD // n) // 8 * 8
            t = r[row:row + 8]
            return jnp.where(st["never"], t if val.dtype == F32 else pltpu.bitcast(t, val.dtype), val)

        def place(sched, items, units):
            units = list(units)
            for i, it in enumerate(items):
                sched.setdefault(units[(i * len(units)) // len(items)], []).append(it)

        def matmul(lhs_fn, w_fn, ks, cols, sink, gives=None):
            for n0 in cols:
                r = None
                for k in ks:
                    d = jnp.dot(lhs_fn(k), w_fn(k, n0), preferred_element_type=F32)
                    r = d if r is None else r + d
                    if k == ks[-1]:
                        sink(n0, r)
                    if n0 == cols[-1] and k == ks[-1]:
                        have.add(gives)
                    st["tok"] = r
                    for fn in st["sched"].pop(st["clock"], []):
                        fn()
                    st["tok"] = None
                    st["clock"] += 1

        def finish():
            assert not st["sched"]

        def lane_iota(rows):
            return jax.lax.broadcasted_iota(jnp.int32, (rows, 128), 1)

        def ld16(ref, r0, n, c0, c1):
            return pltpu.bitcast(ref[r0 // 2:(r0 + n) // 2, c0:c1], BF16)

        def silu_c():
            cf = c_ref[...].astype(F32)
            return (cf * jax.nn.sigmoid(cf)).astype(BF16)

        def mod_mxu(j, k):
            cs = slice(k * KH, (k + 1) * KH)
            lhs = jnp.broadcast_to(silu_c(), (16, D))
            r = jnp.dot(lhs, wmod_v[:, j * D + k * KH:j * D + (k + 1) * KH], preferred_element_type=F32)[0:8]
            mod_v[j, :, cs] = r + 1.0 if j in (1, 4) else r

        def mod_finish(j, c0, c1):
            r = _tree(_add, [modp_v[i, :, j * D + c0:j * D + c1] for i in range(NSUB)])
            r = jnp.sum(r, axis=0, keepdims=True)
            mod_v[j, :, c0:c1] = jnp.broadcast_to(r + 1.0 if j in (1, 4) else r, (8, c1 - c0))

        def mod_items(col0, ntiles):
            rows = D // NSUB

            def one(t, i):
                c0 = col0 + t * 128
                c0 = c0 if isinstance(c0, int) else pl.multiple_of(c0, 128)
                w = wmod_v[i * rows:(i + 1) * rows, pl.ds(c0, 128)].astype(F32)
                p = (w * cb_v[i * rows:(i + 1) * rows, :]).reshape(rows // 8, 8, 128)
                modp_v[i, :, pl.ds(c0, 128)] = gate(_tree(_add, [p[k] for k in range(rows // 8)]), 1, 2)
            return [functools.partial(one, t, i) for t in range(ntiles) for i in range(NSUB)]

        def perm_mix(g, i, nrows):
            n = nrows // 2
            l = lane_iota(n)
            vals = [pltpu.bitcast(wqkv_v[i * nrows:(i + 1) * nrows, g * D + c * 128: g * D + (c + 1) * 128], U32)
                    for c in range(NC)]
            for b in range(3):
                m = ((l >> (2 + b)) & 1) == 0
                for c in range(NC):
                    if c & (1 << b):
                        continue
                    lo, hi = vals[c], vals[c | (1 << b)]
                    vals[c] = jnp.where(m, lo, hi)
                    vals[c | (1 << b)] = jnp.where(m, hi, lo)
            p0 = (i * n) % (KH // 2)
            for j in range(NC):
                v = jnp.concatenate([gate(vals[j][q:q + 8], j, NC) for q in range(0, n, 8)], axis=0)
                wtmp[j, pl.ds(pl.multiple_of(zrow(p0), 8), n), :] = v

        def perm_gather(g, k, j):
            have.add(("w", g, k, j))
            l = lane_iota(8)
            idx = ((((l >> 1) & 3) << 5) | ((((l >> 3) & 7) ^ j) << 2) | ((l >> 6) << 1) | (l & 1))
            for q in range(0, KH // 2, 8):
                t = jnp.take_along_axis(gate(wtmp[j, q:q + 8, :], q, KH // 2), idx, axis=1,
                                        mode="promise_in_bounds")
                wqkv_p[k * KH // 2 + q:k * KH // 2 + q + 8, g * D + j * 128: g * D + (j + 1) * 128] = t

        def perm_qkv_items(g, k, nrows=PR):
            n = KH // nrows
            return ([functools.partial(perm_mix, g, i, nrows) for i in range(k * n, (k + 1) * n)]
                    + [functools.partial(perm_gather, g, k, j) for j in range(NC)])

        def perm_wo_items():
            low = jax.lax.broadcasted_iota(jnp.int32, (8, 128), 0) < 4

            def spread(c, h):
                for r in range(h * 256, h * 256 + 256, 8):
                    wo_tmp[c, pl.ds(zrow(r + r // 16), 8), :] = gate(pltpu.bitcast(
                        wo_v[2 * r:2 * r + 16, c * 128:(c + 1) * 128], U32), r % 256, 256)

            def gather(c, h):
                for G in range(h * 32, h * 32 + 32):
                    j, e, ch = G >> 3, (G >> 2) & 1, G & 3
                    dd = (((2 * ch) ^ j) << 1) | e
                    ta = wo_tmp[c, pl.ds(ch * 136 + dd, 8, stride=17), :]
                    tb = wo_tmp[c, pl.ds(ch * 136 + (dd ^ 2), 8, stride=17), :]
                    wo_p[G * 8:G * 8 + 8, c * 128:(c + 1) * 128] = jnp.where(low, ta, tb)
            return [functools.partial(fn, c, h) for fn in (spread, gather) for c in range(NC) for h in range(2)]

        def zrow(row, k=1):
            return row + k * st["z"]

        def gate16(v, i, n):
            return jnp.concatenate([gate(v[q:q + 8], i, n) for q in range(0, LG, 8)], axis=0)

        def staged(stages, n, lag):
            items = []
            for t in range(n + lag * (len(stages) - 1)):
                for k in reversed(range(len(stages))):
                    if 0 <= t - k * lag < n:
                        items.append(functools.partial(stages[k], t - k * lag))
            return items

        def ln_stages(load, stat, dst, j_scale, j_shift, cols=range(NC)):
            def chunks(x):
                return [x[:, c * 128:(c + 1) * 128] for c in range(NC)]

            def put(j, r, part, fn):
                m = jnp.sum(part, axis=-1, keepdims=True) * (1.0 / D)
                stat[j, pl.ds(pl.multiple_of(zrow(r), LG), LG), :] = jnp.broadcast_to(fn(m), (LG, 128))

            def s_mean(i):
                put(0, i * LG, gate16(_tree(_add, chunks(load(i * LG, 0))), 1, 2), lambda m: m)

            def s_var(i):
                r = i * LG
                mu = gate16(stat[0, r:r + LG, :], 0, 1)
                put(1, r, _tree(_add, [(x - mu) * (x - mu) for x in chunks(load(r, 1))]),
                    lambda m: jax.lax.rsqrt(m + EPS))

            def s_out(i):
                r = i * LG
                mu, rs = stat[0, r:r + LG, :], stat[1, r:r + LG, :]
                xs = chunks(load(r, 2))
                for c in cols:
                    x, cs = xs[c], slice(c * 128, (c + 1) * 128)
                    if c % (NC // 2) == 0:
                        rg = gate16(rs, c - cols[0], NC)
                    y = ((x - mu) * rg).reshape(LG // 8, 8, 128) * mod_v[j_scale, :, cs][None] + mod_v[j_shift, :, cs][None]
                    dst[r // 2:(r + LG) // 2, cs] = pltpu.bitcast(y.reshape(LG, 128).astype(BF16), U32)
            return s_mean, s_var, s_out

        def load_x(row0):
            return lambda r, k: x_v[pl.ds(pl.multiple_of(zrow(row0 + r, k), LG), LG), :].astype(F32)

        def ln1_items(row0, buf):
            return staged(ln_stages(load_x(row0), stat1, bufs[buf][0], 1, 0), TM // LG, 1)

        def ln1_start(b, k):
            return ln_stages(load_x(b * TM), stats.at[:, pl.ds(b * TM, TM), :], h1s.at[b] if b < NS else h1a,
                             1, 0, range(k * NC // 2, (k + 1) * NC // 2))

        def ln1_out_items(b, k):
            def one(i):
                have.add(("h", b, k, i))
                ln1_start(b, k)[2](i)
            return [functools.partial(one, i) for i in range(TM // LG)]

        def x1_rows(row, n, c0, c1):
            xf = x_v[pl.ds(row, n), c0:c1].astype(F32).reshape(n // 8, 8, c1 - c0)
            y = y_v[pl.ds(row, n), c0:c1].reshape(n // 8, 8, c1 - c0)
            return (xf + mod_v[2, :, c0:c1][None] * y).reshape(n, c1 - c0)

        def post_items(row0):
            def load(r, k):
                if k:
                    return x1n[pl.ds(pl.multiple_of(zrow(r, k), LG), LG), :]
                x1 = x1_rows(row0 + r, LG, 0, D)
                x1n[r:r + LG, :] = x1
                return x1
            return staged(ln_stages(load, stat2, h2_v, 4, 3), TMB // LG, 1)

        def logit_items(buf, first):
            _, qk, _, _, pb = bufs[buf]
            swap = lane_iota(RG) ^ 1

            def s_logit(g):
                need(("q", buf), ("k", buf))
                have.add(("l", buf, g))
                r = g * RG
                qs = [qk[c, HALO + r:HALO + r + RG, :] for c in range(NC)]
                for w in range(WIN):
                    k0 = HALO + r - DIL * w
                    if w >= WIN // 2:
                        k0 = zrow(k0)
                    s = _tree(_add, [qs[c] * qk[NC + c, pl.ds(k0, RG), :] for c in range(NC)])
                    s = gate(s, w, WIN)
                    s = s + pltpu.roll(s, 64, 1)
                    s = s + jnp.take_along_axis(s, swap, axis=1, mode="promise_in_bounds")
                    if first and r < DIL * w:
                        pos = r + jax.lax.broadcasted_iota(jnp.int32, (RG, 128), 0)
                        s = jnp.where(pos >= DIL * w, s, NEG * LOG2E)
                    sls[g % len(sls)][w, pl.ds(pl.multiple_of(zrow(0), RG), RG), :] = s

            def s_soft(g):
                assert ("p", buf, g) not in have
                have.add(("p", buf, g))
                r = g * RG
                ss = [sls[g % len(sls)][w] for w in range(WIN)]
                m = gate(_tree(jnp.maximum, ss), 0, 1)
                es = [jnp.exp2(s - m) for s in ss]
                for w in range(WIN):
                    pb[w, r:r + RG, :] = es[w]
                den = _tree(_add, es)
                inv = pl.reciprocal(den, approx=True)
                pb[WIN, r:r + RG, :] = inv * (2.0 - den * inv)
            return staged((s_logit, s_soft), TM // RG, LLAG)

        def pv_items(buf):
            _, _, vp, o, pb = bufs[buf]
            otmp = otmps[buf]

            def one(r):
                need(("v", buf), ("p", buf, r // RG))
                have.remove(("p", buf, r // RG))
                have.add(("o", buf, r // RG))
                ps = [pb[w, pl.ds(pl.multiple_of(zrow(r), RG), RG), :] for w in range(WIN + 1)]
                for c in range(NC):
                    ks = [HALO + r - DIL * w if w < WIN // 2 else zrow(HALO + r - DIL * w) for w in range(WIN)]
                    acc = _tree(_add, [ps[w] * vp[c, pl.ds(ks[w], RG), :] for w in range(WIN)])
                    acc = gate(acc * ps[WIN], c, NC)
                    if (r // RG) % 2 == 0:
                        otmp[c, pl.ds(pl.multiple_of(zrow(0), 8), RG), :] = acc
                    else:
                        both = jnp.concatenate([otmp[c], acc], axis=0).astype(BF16)
                        o[(r - RG) // 2:(r + RG) // 2, c * 128:(c + 1) * 128] = pltpu.bitcast(both, U32)
            return [functools.partial(one, r) for r in range(0, TM, RG)]

        def halo(buf, prev, part):
            _, qk, vp, _, _ = bufs[buf]
            for c in range(NC):
                if part == 1:
                    qk[NC + c, 0:HALO, :] = (jnp.zeros((HALO, 128), F32) if prev is None
                                             else gate16(bufs[prev][1][NC + c, TM:TM + HALO, :], 1, 2))
                else:
                    vp[c, 0:HALO, :] = (jnp.broadcast_to(vp[c, HALO:HALO + 1, :], (HALO, 128)) if prev is None
                                        else gate16(bufs[prev][2][c, TM:TM + HALO, :], 1, 2))

        def qkv_part(buf, g, sb=None, k=None):
            h1, qk, vp, _, _ = bufs[buf] if buf else (None,) * 5
            if sb is not None:
                h1 = h1s.at[sb]
                need(*[("h", sb, k, i) for i in range(TM // LG)], *[("w", g, k, j) for j in range(NC)])
            if k != 0:
                for i in range(TM // RG):
                    if g < 2 and ("qk"[g], buf) in have:
                        need(("l", buf, i))
                    if g == 2 and ("v", buf) in have:
                        assert ("p", buf, i) not in have or ("new", buf) in have
                if g == 1:
                    have.difference_update({("l", buf, i) for i in range(TM // RG)})
                    have.add(("new", buf))
                have.discard(("qkv"[g], buf))

            def sink(n0, r):
                ch = n0 // 128
                if k == 0:
                    part[sb, ch] = r
                    return
                if k == 1:
                    r = r + part[sb, ch]
                dst, ci = (qk, ch) if ch < 2 * NC else (vp, ch - 2 * NC)
                dst[ci, HALO:HALO + TM, :] = r * (SM_SCALE * LOG2E) if ch < NC else r
            matmul(lambda kk: ld16(h1, 0, TM, kk * KH, (kk + 1) * KH),
                   lambda kk, n0: ld16(wqkv_p, kk * KH, KH, n0, n0 + 128),
                   (0, 1) if k is None else (k,), range(g * D, (g + 1) * D, 128), sink,
                   None if k == 0 else ("qkv"[g], buf))
            if g == 2:
                have.discard(("new", buf))

        def wo_mm(buf, row0):
            o = bufs[buf][3]
            need(*[("o", buf, i) for i in range(TM // RG)])
            have.difference_update({("o", buf, i) for i in range(TM // RG)})

            def sink(n0, r):
                y_v[pl.ds(row0, TM), n0:n0 + 128] = r
            matmul(lambda k: ld16(o, 0, TM, k * KH, (k + 1) * KH),
                   lambda k, n0: ld16(wo_p, k * KH, KH, n0, n0 + 128),
                   (0, 1), range(0, D, 128), sink)

        UP = NC * (D // KH)

        def run_now(items):
            for fn in items:
                fn()

        def ffn(j, row0, slot, nxt_row):
            h = ld16(h2_v, 0, TMB, 0, D)
            for f0 in range(0, F, FC):
                g = jnp.dot(h, w1_v[:, f0:f0 + FC], preferred_element_type=F32)
                u = jnp.dot(h, w3_v[:, f0:f0 + FC], preferred_element_type=F32)
                act_v[:, f0:f0 + FC] = pltpu.bitcast((g * jax.nn.sigmoid(g) * u).astype(BF16), U32)
            nk = F // KH
            sched = {}
            place(sched, post_items(nxt_row), range(0, NC * nk - PB1))
            begin(sched)

            def sink(n0, r):
                z = (mod_v[5, :, n0:n0 + 128][None] * r.reshape(TMB // 8, 8, 128)).reshape(TMB, 128)
                obuf[slot, :, n0:n0 + 128] = (x1_rows(row0, TMB, n0, n0 + 128) + z).astype(BF16)
                if n0 + 128 in OCUT:
                    cp_out(j, slot, OCUT.index(n0 + 128) - 1).start()
            matmul(lambda k: ld16(act_v, 0, TMB, k * KH, (k + 1) * KH),
                   lambda k, n0: w2_v[k * KH:(k + 1) * KH, n0:n0 + 128],
                   tuple(range(nk)), range(0, D, 128), sink)

        U8 = NC

        def segment(*placements):
            sched = {}
            for items, units in placements:
                place(sched, items, units)
            begin(sched)

        with jax.named_scope("prologue"):
            zs[0] = 0
            begin({})
            start("c", "x0", "ca0", "q0", "sa0", "k0", "v0", "x4", "ca1", "sa1", "q1", "k1", "v1", "wo",
                  "x1", "m2", "x2")
            wait("c")
            cb_v[...] = jnp.broadcast_to(silu_c().astype(F32), (128, D)).T
            wait("x0")
            for r in range(0, NS * TM, LG):
                xf = x_v[r:r + LG, :].astype(F32)
                mu = jnp.mean(xf, axis=-1, keepdims=True)
                d = xf - mu
                rs = jax.lax.rsqrt(jnp.mean(d * d, axis=-1, keepdims=True) + EPS)
                stats[0, r:r + LG, :] = jnp.broadcast_to(mu, (LG, 128))
                stats[1, r:r + LG, :] = jnp.broadcast_to(rs, (LG, 128))
            wait("ca0")
            mod_mxu(1, 0)
            wait("q0")
            run_now(perm_qkv_items(0, 0))
            wait("sa0")
            mod_mxu(0, 0)
            run_now(ln1_out_items(0, 0))

        with jax.named_scope("pass1"):
            segment((ln1_out_items(1, 0), range(0, U8 - 2)),
                    (ln1_out_items(2, 0) + ln1_out_items(3, 0), range(U8 - 2, 2 * U8)))
            qkv_part(None, 0, 0, 0)
            qkv_part(None, 0, 1, 0)
            wait("k0")
            segment((perm_qkv_items(1, 0), range(0, 2 * U8 - 2)))
            for g, b in ((0, 2), (0, 3), (1, 0), (1, 1)):
                qkv_part(None, g, b, 0)
            wait("v0", "x4", "ca1")
            segment((perm_qkv_items(2, 0), range(0, 2 * U8 - 2)),
                    (staged(ln1_start(NS, 0)[:2], TM // LG, 1), range(2 * U8 - 1, 4 * U8 - 2)),
                    (mod_items(D + KH, 4) + [functools.partial(mod_finish, 1, KH, D)], range(2 * U8 - 2, 4 * U8)))
            for g, b in ((1, 2), (1, 3), (2, 0), (2, 1)):
                qkv_part(None, g, b, 0)
            wait("sa1", "q1")
            segment((mod_items(KH, 4) + [functools.partial(mod_finish, 0, KH, D)], range(0, U8 + 2)),
                    (perm_qkv_items(0, 1), range(0, 2 * U8 - 2)),
                    (ln1_out_items(0, 1), range(U8 + 3, 2 * U8 - 1)))
            qkv_part(None, 2, 2, 0)
            qkv_part(None, 2, 3, 0)

        with jax.named_scope("pass2"):
            wait("k1")
            segment((perm_qkv_items(1, 1), range(0, 2 * U8 - 2)),
                    (ln1_out_items(1, 1), range(0, U8 - 2)),
                    (ln1_out_items(2, 1), range(U8 - 2, 2 * U8)))
            halo("b", None, 1)
            qkv_part("b", 0, 0, 1)
            qkv_part("c", 0, 1, 1)
            wait("v1")
            l0 = logit_items("b", True)
            segment((perm_qkv_items(2, 1), range(0, 2 * U8 - 2)),
                    (ln1_out_items(3, 1), range(0, U8)),
                    (l0[:LB], range(B0, B1)))
            qkv_part("b", 1, 0, 1)
            halo("c", "b", 1)
            qkv_part("c", 1, 1, 1)
            qkv_part("b", 2, 0, 1)
            halo("b", None, 2)
            halo("c", "b", 2)
            qkv_part("c", 2, 1, 1)
            wait("wo")
            segment((perm_wo_items(), range(0, WS)),
                    (l0[LB:], range(0, C0)),
                    (pv_items("b"), range(C0 + CP, 39)),
                    (logit_items("c", False), range(C0, C1)),
                    (pv_items("c"), range(C1 + CP, 63)),
                    (logit_items("a", False), range(C1, C2)),
                    (pv_items("a"), range(C2 + CP, 79)),
                    ([functools.partial(halo, "b", "a", 1)], [23]),
                    ([functools.partial(halo, "b", "a", 2)], [39]),
                    (ln1_out_items(NS, 0) + ln1_out_items(NS, 1), range(H0, H1)),
                    (logit_items("b", False), range(C2, 96 - L1)))
            halo("a", "c", 1)
            halo("a", "c", 2)
            for g in range(3):
                qkv_part("a", g, 2, 1)
            for g in range(3):
                qkv_part("b", g, 3, 1)
            wo_mm("b", 0)
            wo_mm("c", TM)
            wo_mm("a", 2 * TM)
            finish()
            wait("x1", "m2")
            start("m3", "w1", "w3", "w2")


        def half(X, Y, u0, sched, row_ln1, row_wo, extra):
            place(sched, pv_items(Y), range(u0 + P0, u0 + 3 * UP - P1))
            place(sched, logit_items(X, False), range(u0 + 2 * UP + L0, u0 + 4 * UP - L1))
            place(sched, ln1_items(row_ln1, Y), range(u0 + N0, u0 + N1))
            if extra:
                place(sched, extra, range(u0, u0 + 4 * UP - 1))

            def run():
                halo(X, Y, 1)
                halo(X, Y, 2)
                for g in range(3):
                    qkv_part(X, g)
                wo_mm(Y, row_wo)
            return run

        def a_step(s, carry):
            @pl.when(s == 3)
            def _():
                wait("x2", "m3")

            ra = pl.multiple_of(2 * s * TM, TM)
            nxt = pl.multiple_of(jnp.minimum(ra + 2 * TM, S - TM), TM)
            col0 = pl.multiple_of(jnp.minimum(2 * D + (s - 2) * (MT * 128), 6 * D - MT * 128), 128)
            mi = mod_items(col0, MT)
            sched = {}
            run_a = half("a", "b", 0, sched, ra + TM, ra - TM, mi[:len(mi) // 2])
            run_b = half("b", "a", 4 * UP, sched, nxt, ra, mi[len(mi) // 2:])
            begin(sched)
            run_a()
            run_b()
            finish()
            return carry

        with jax.named_scope("aloop"):
            if SKIP_A:
                wait("x2", "m3")
            else:
                jax.lax.fori_loop(NS // 2, NB // 2, a_step, 0)

        with jax.named_scope("atail"):
            begin({})
            for j in range(2, 6):
                mod_finish(j, 0, D)
            run_now(pv_items("b"))
            if TAILV == 0:
                segment((post_items(0), range(0, UP - 2)))
            elif TAILV == 1:
                items = post_items(0)
                run_now(items[:TB])
                segment((items[TB:], range(0, UP - 2)))
            else:
                def bulk(r):
                    x1 = x1_rows(r, LG, 0, D)
                    mu = jnp.mean(x1, axis=-1, keepdims=True)
                    d = x1 - mu
                    rs = jax.lax.rsqrt(jnp.mean(d * d, axis=-1, keepdims=True) + EPS)
                    y = (d * rs).reshape(LG // 8, 8, D) * mod_v[4][None] + mod_v[3][None]
                    h2_v[r // 2:(r + LG) // 2, :] = pltpu.bitcast(y.reshape(LG, D).astype(BF16), U32)
                for r in range(0, TMB, LG):
                    bulk(r)
            wo_mm("b", S - TM)
            finish()
            wait("w1", "w3", "w2")

        def b_step(j, carry):
            slot = j % 2

            @pl.when(j >= 2)
            def _():
                wait_out(j - 2, slot)

            row0 = pl.multiple_of(j * TMB, TMB)
            nxt = pl.multiple_of(jnp.minimum(row0 + TMB, S - TMB), TMB)
            if SKIP_FFN:
                obuf[slot] = x1_rows(row0, TMB, 0, D).astype(BF16)
                for q in range(NQ):
                    cp_out(j, slot, q).start()
            else:
                ffn(j, row0, slot, nxt)
            return carry

        with jax.named_scope("bloop"):
            jax.lax.fori_loop(0, NBB, b_step, 0)
        with jax.named_scope("tail"):
            wait_out(NBB - 2, (NBB - 2) % 2)
            wait_out(NBB - 1, (NBB - 1) % 2)

    any_spec = pl.BlockSpec(memory_space=pl.ANY)
    scratch = [
        pltpu.VMEM((S, D), BF16),
        pltpu.VMEM((D, 3 * D), BF16),
        pltpu.VMEM((NC, KH // 2, 128), U32),
        pltpu.VMEM((D // 2, 3 * D), U32),
        pltpu.VMEM((D, D), BF16),
        pltpu.VMEM((NC, D // 32 * 17, 128), U32),
        pltpu.VMEM((D // 2, D), U32),
        pltpu.VMEM((D, F), BF16),
        pltpu.VMEM((D, F), BF16),
        pltpu.VMEM((F, D), BF16),
        pltpu.VMEM((D, 6 * D), BF16),
        pltpu.VMEM((D, 128), F32),
        pltpu.VMEM((NSUB, 8, 6 * D), F32),
        pltpu.VMEM((6, 8, D), F32),
        pltpu.VMEM((TM // 2, D), U32),
        pltpu.VMEM((TM // 2, D), U32),
        pltpu.VMEM((NS, TM // 2, D), U32),
        pltpu.VMEM((NS, 3 * NC, TM, 128), F32),
        pltpu.VMEM((2, (NS + 1) * TM, 128), F32),
        pltpu.VMEM((2 * NC, KV + PADK, 128), F32),
        pltpu.VMEM((NC, KV + PADK, 128), F32),
        pltpu.VMEM((WIN + 1, TM, 128), F32),
        pltpu.VMEM((2 * NC, KV + PADK, 128), F32),
        pltpu.VMEM((NC, KV + PADK, 128), F32),
        pltpu.VMEM((WIN + 1, TM, 128), F32),
        pltpu.VMEM((2 * NC, KV + PADK, 128), F32),
        pltpu.VMEM((NC, KV + PADK, 128), F32),
        pltpu.VMEM((WIN + 1, TM, 128), F32),
        pltpu.VMEM((TM // 2, D), U32),
        pltpu.VMEM((TM // 2, D), U32),
        pltpu.VMEM((TM // 2, D), U32),
        pltpu.VMEM((NC, RG, 128), F32),
        pltpu.VMEM((NC, RG, 128), F32),
        pltpu.VMEM((NC, RG, 128), F32),
        pltpu.VMEM((WIN, RG, 128), F32),
        pltpu.VMEM((WIN, RG, 128), F32),
        pltpu.VMEM((WIN, RG, 128), F32),
        pltpu.VMEM((2, TM, 128), F32),
        pltpu.VMEM((2, TMB, 128), F32),
        pltpu.VMEM((S, D), F32),
        pltpu.VMEM((TMB, D), F32),
        pltpu.VMEM((TMB // 2, D), U32),
        pltpu.VMEM((TMB // 2, F), U32),
        pltpu.VMEM((2, TMB, D), BF16),
        pltpu.VMEM((1, D), BF16),
        pltpu.SMEM((1,), jnp.int32),
        pltpu.SemaphoreType.DMA((NDMA,)),
        pltpu.SemaphoreType.DMA((2 * NQ,)),
    ]

    def call(A_x, A_wqkv, A_wo, B_w1, B_w3, B_w2, c, w_mod):
        return pl.pallas_call(
            kernel,
            out_shape=jax.ShapeDtypeStruct((1, S, D), BF16),
            in_specs=[any_spec] * 8,
            out_specs=any_spec,
            scratch_shapes=scratch,
            compiler_params=pltpu.CompilerParams(vmem_limit_bytes=120 * 1024 * 1024),
        )(A_x, A_wqkv, A_wo, B_w1, B_w3, B_w2, c, w_mod)

    return call


@jax.jit
def pallas_adaLN_cond__sliding_local_dilated__glu_gated_swiglu__prompt_kernel(
    A_x: jax.Array,
    A_wqkv: jax.Array,
    A_wo: jax.Array,
    B_x: jax.Array,
    B_w1: jax.Array,
    B_w3: jax.Array,
    B_w2: jax.Array,
    c: jax.Array,
    w_mod: jax.Array,
):
    del B_x
    return _build()(A_x, A_wqkv, A_wo, B_w1, B_w3, B_w2, c, w_mod)
```

```python
import functools
import math

import jax
import jax.numpy as jnp
import jax.experimental.pallas as pl
import jax.experimental.pallas.tpu as pltpu

S = 2048
D = 1024
F = 3584
H = 32
DH = D // H
WIN = 8
DIL = 2
NC = D // 128
HALO = 16
EPS = 1e-5
NEG = -1000000000.0
SM_SCALE = DH ** -0.5
LOG2E = math.log2(math.e)

TM = 128
NB = S // TM
KV = HALO + TM
RG = 8
LG = 16
NS = 4
NDMA = 21
KH = 512

F32 = jnp.float32
BF16 = jnp.bfloat16
U32 = jnp.uint32


def _tree(op, xs):
    xs = list(xs)
    while len(xs) > 1:
        xs = [op(xs[i], xs[i + 1]) if i + 1 < len(xs) else xs[i] for i in range(0, len(xs), 2)]
    return xs[0]


def _add(a, b):
    return a + b


def _build(TMB=256, FC=512, GATE=True, SKIP_FFN=False, SKIP_A=False,
           SCH=0, MT=6, NSUB=16, PB1=5, L0=0, L1=1, SPREAD=128, LLAG=3,
           P0=0, P1=16, N0=1, N1=30, PR=64, B0=14, B1=30, LB=19, PADK=0, C0=10, C1=38, C2=64, CP=0, WS=46, H0=0, H1=10, TAILV=2, TB=16, TE=2, OCUT=(0, 512, 896, 1024)):
    NBB = S // TMB
    NQ = len(OCUT) - 1

    def kernel(x_hbm, wqkv_hbm, wo_hbm, w1_hbm, w3_hbm, w2_hbm, c_hbm, wmod_hbm,
               out_hbm,
               x_v, wqkv_v, wtmp, wqkv_p, wo_v, wo_tmp, wo_p, w1_v, w3_v, w2_v, wmod_v, cb_v, modp_v, mod_v,
               h1a, h1b, h1s, part, stats, qka, va, pa, qkb, vb, pb_, qkc, vc, pc, oa, ob, oc, ota, otb, otc, sl0, sl1, sl2, stat1, stat2, y_v, x1n, h2_v, act_v, obuf, c_ref,
               zs, sem_w, sem_o):
        bufs = {"a": (h1a, qka, va, oa, pa), "b": (h1b, qkb, vb, ob, pb_),
                "c": (None, qkc, vc, oc, pc)}

        sls = (sl0, sl1, sl2)
        otmps = {"a": ota, "b": otb, "c": otc}

        dmas = {}

        def add_dma(name, src, dst):
            dmas[name] = (src, dst, len(dmas))

        for name, (b0, b1) in (("x0", (0, NS)), ("x4", (NS, NS + 1)), ("x1", (NS + 1, NS + 3)), ("x2", (NS + 3, NB))):
            rows = pl.ds(b0 * TM, (b1 - b0) * TM)
            add_dma(name, x_hbm.at[0, rows, :], x_v.at[rows, :])
        for name, (c0, c1) in (("sa0", (0, KH)), ("sa1", (KH, D)), ("ca0", (D, D + KH)), ("ca1", (D + KH, 2 * D)),
                               ("m2", (2 * D, 3 * D)), ("m3", (3 * D, 6 * D))):
            cols = pl.ds(c0, c1 - c0)
            add_dma(name, wmod_hbm.at[:, cols], wmod_v.at[:, cols])
        for g in range(3):
            for k in range(2):
                rows, cols = pl.ds(k * KH, KH), pl.ds(g * D, D)
                add_dma("qkv"[g] + str(k), wqkv_hbm.at[rows, cols], wqkv_v.at[rows, cols])
        add_dma("c", c_hbm, c_ref)
        add_dma("wo", wo_hbm, wo_v)
        add_dma("w1", w1_hbm, w1_v)
        add_dma("w3", w3_hbm, w3_v)
        add_dma("w2", w2_hbm, w2_v)
        assert len(dmas) == NDMA

        def cp(name):
            src, dst, i = dmas[name]
            return pltpu.make_async_copy(src, dst, sem_w.at[i])

        def start(*names):
            for n in names:
                cp(n).start()

        def wait(*names):
            for n in names:
                cp(n).wait()

        def cp_out(j, slot, q):
            c0, c1 = OCUT[q], OCUT[q + 1]
            return pltpu.make_async_copy(obuf.at[slot, :, pl.ds(c0, c1 - c0)],
                                         out_hbm.at[0, pl.ds(j * TMB, TMB), pl.ds(c0, c1 - c0)],
                                         sem_o.at[slot * NQ + q])

        def wait_out(j, slot):
            for q in range(NQ):
                cp_out(j, slot, q).wait()

        st = {"z": None, "never": None, "clock": 0, "sched": {}, "tok": None}

        have = set()

        def need(*keys):
            assert all(k in have for k in keys), keys

        def begin(sched):
            z = zs[0]
            st.update(z=z, never=jnp.full((8, 128), z, jnp.int32) != 0, clock=0, sched=sched, tok=None)

        def gate(val, i, n):
            r = st["tok"]
            if r is None or not GATE:
                return val
            row = (i * SPREAD // n) // 8 * 8
            t = r[row:row + 8]
            return jnp.where(st["never"], t if val.dtype == F32 else pltpu.bitcast(t, val.dtype), val)

        def place(sched, items, units):
            units = list(units)
            for i, it in enumerate(items):
                sched.setdefault(units[(i * len(units)) // len(items)], []).append(it)

        def matmul(lhs_fn, w_fn, ks, cols, sink, gives=None):
            for n0 in cols:
                r = None
                for k in ks:
                    d = jnp.dot(lhs_fn(k), w_fn(k, n0), preferred_element_type=F32)
                    r = d if r is None else r + d
                    if k == ks[-1]:
                        sink(n0, r)
                    if n0 == cols[-1] and k == ks[-1]:
                        have.add(gives)
                    st["tok"] = r
                    for fn in st["sched"].pop(st["clock"], []):
                        fn()
                    st["tok"] = None
                    st["clock"] += 1

        def finish():
            assert not st["sched"]

        def lane_iota(rows):
            return jax.lax.broadcasted_iota(jnp.int32, (rows, 128), 1)

        def ld16(ref, r0, n, c0, c1):
            return pltpu.bitcast(ref[r0 // 2:(r0 + n) // 2, c0:c1], BF16)

        def silu_c():
            cf = c_ref[...].astype(F32)
            return (cf * jax.nn.sigmoid(cf)).astype(BF16)

        def mod_mxu(j, k):
            cs = slice(k * KH, (k + 1) * KH)
            lhs = jnp.broadcast_to(silu_c(), (16, D))
            r = jnp.dot(lhs, wmod_v[:, j * D + k * KH:j * D + (k + 1) * KH], preferred_element_type=F32)[0:8]
            mod_v[j, :, cs] = r + 1.0 if j in (1, 4) else r

        def mod_finish(j, c0, c1):
            r = _tree(_add, [modp_v[i, :, j * D + c0:j * D + c1] for i in range(NSUB)])
            r = jnp.sum(r, axis=0, keepdims=True)
            mod_v[j, :, c0:c1] = jnp.broadcast_to(r + 1.0 if j in (1, 4) else r, (8, c1 - c0))

        def mod_items(col0, ntiles):
            rows = D // NSUB

            def one(t, i):
                c0 = col0 + t * 128
                c0 = c0 if isinstance(c0, int) else pl.multiple_of(c0, 128)
                w = wmod_v[i * rows:(i + 1) * rows, pl.ds(c0, 128)].astype(F32)
                p = (w * cb_v[i * rows:(i + 1) * rows, :]).reshape(rows // 8, 8, 128)
                modp_v[i, :, pl.ds(c0, 128)] = gate(_tree(_add, [p[k] for k in range(rows // 8)]), 1, 2)
            return [functools.partial(one, t, i) for t in range(ntiles) for i in range(NSUB)]

        def perm_mix(g, i, nrows):
            n = nrows // 2
            l = lane_iota(n)
            vals = [pltpu.bitcast(wqkv_v[i * nrows:(i + 1) * nrows, g * D + c * 128: g * D + (c + 1) * 128], U32)
                    for c in range(NC)]
            for b in range(3):
                m = ((l >> (2 + b)) & 1) == 0
                for c in range(NC):
                    if c & (1 << b):
                        continue
                    lo, hi = vals[c], vals[c | (1 << b)]
                    vals[c] = jnp.where(m, lo, hi)
                    vals[c | (1 << b)] = jnp.where(m, hi, lo)
            p0 = (i * n) % (KH // 2)
            for j in range(NC):
                v = jnp.concatenate([gate(vals[j][q:q + 8], j, NC) for q in range(0, n, 8)], axis=0)
                wtmp[j, pl.ds(pl.multiple_of(zrow(p0), 8), n), :] = v

        def perm_gather(g, k, j):
            have.add(("w", g, k, j))
            l = lane_iota(8)
            idx = ((((l >> 1) & 3) << 5) | ((((l >> 3) & 7) ^ j) << 2) | ((l >> 6) << 1) | (l & 1))
            for q in range(0, KH // 2, 8):
                t = jnp.take_along_axis(gate(wtmp[j, q:q + 8, :], q, KH // 2), idx, axis=1,
                                        mode="promise_in_bounds")
                wqkv_p[k * KH // 2 + q:k * KH // 2 + q + 8, g * D + j * 128: g * D + (j + 1) * 128] = t

        def perm_qkv_items(g, k, nrows=PR):
            n = KH // nrows
            return ([functools.partial(perm_mix, g, i, nrows) for i in range(k * n, (k + 1) * n)]
                    + [functools.partial(perm_gather, g, k, j) for j in range(NC)])

        def perm_wo_items():
            low = jax.lax.broadcasted_iota(jnp.int32, (8, 128), 0) < 4

            def spread(c, h):
                for r in range(h * 256, h * 256 + 256, 8):
                    wo_tmp[c, pl.ds(zrow(r + r // 16), 8), :] = gate(pltpu.bitcast(
                        wo_v[2 * r:2 * r + 16, c * 128:(c + 1) * 128], U32), r % 256, 256)

            def gather(c, h):
                for G in range(h * 32, h * 32 + 32):
                    j, e, ch = G >> 3, (G >> 2) & 1, G & 3
                    dd = (((2 * ch) ^ j) << 1) | e
                    ta = wo_tmp[c, pl.ds(ch * 136 + dd, 8, stride=17), :]
                    tb = wo_tmp[c, pl.ds(ch * 136 + (dd ^ 2), 8, stride=17), :]
                    wo_p[G * 8:G * 8 + 8, c * 128:(c + 1) * 128] = jnp.where(low, ta, tb)
            return [functools.partial(fn, c, h) for fn in (spread, gather) for c in range(NC) for h in range(2)]

        def zrow(row, k=1):
            return row + k * st["z"]

        def gate16(v, i, n):
            return jnp.concatenate([gate(v[q:q + 8], i, n) for q in range(0, LG, 8)], axis=0)

        def staged(stages, n, lag):
            items = []
            for t in range(n + lag * (len(stages) - 1)):
                for k in reversed(range(len(stages))):
                    if 0 <= t - k * lag < n:
                        items.append(functools.partial(stages[k], t - k * lag))
            return items

        def ln_stages(load, stat, dst, j_scale, j_shift, cols=range(NC)):
            def chunks(x):
                return [x[:, c * 128:(c + 1) * 128] for c in range(NC)]

            def put(j, r, part, fn):
                m = jnp.sum(part, axis=-1, keepdims=True) * (1.0 / D)
                stat[j, pl.ds(pl.multiple_of(zrow(r), LG), LG), :] = jnp.broadcast_to(fn(m), (LG, 128))

            def s_mean(i):
                put(0, i * LG, gate16(_tree(_add, chunks(load(i * LG, 0))), 1, 2), lambda m: m)

            def s_var(i):
                r = i * LG
                mu = gate16(stat[0, r:r + LG, :], 0, 1)
                put(1, r, _tree(_add, [(x - mu) * (x - mu) for x in chunks(load(r, 1))]),
                    lambda m: jax.lax.rsqrt(m + EPS))

            def s_out(i):
                r = i * LG
                mu, rs = stat[0, r:r + LG, :], stat[1, r:r + LG, :]
                xs = chunks(load(r, 2))
                for c in cols:
                    x, cs = xs[c], slice(c * 128, (c + 1) * 128)
                    if c % (NC // 2) == 0:
                        rg = gate16(rs, c - cols[0], NC)
                    y = ((x - mu) * rg).reshape(LG // 8, 8, 128) * mod_v[j_scale, :, cs][None] + mod_v[j_shift, :, cs][None]
                    dst[r // 2:(r + LG) // 2, cs] = pltpu.bitcast(y.reshape(LG, 128).astype(BF16), U32)
            return s_mean, s_var, s_out

        def load_x(row0):
            return lambda r, k: x_v[pl.ds(pl.multiple_of(zrow(row0 + r, k), LG), LG), :].astype(F32)

        def ln1_items(row0, buf):
            return staged(ln_stages(load_x(row0), stat1, bufs[buf][0], 1, 0), TM // LG, 1)

        def ln1_start(b, k):
            return ln_stages(load_x(b * TM), stats.at[:, pl.ds(b * TM, TM), :], h1s.at[b] if b < NS else h1a,
                             1, 0, range(k * NC // 2, (k + 1) * NC // 2))

        def ln1_out_items(b, k):
            def one(i):
                have.add(("h", b, k, i))
                ln1_start(b, k)[2](i)
            return [functools.partial(one, i) for i in range(TM // LG)]

        def x1_rows(row, n, c0, c1):
            xf = x_v[pl.ds(row, n), c0:c1].astype(F32).reshape(n // 8, 8, c1 - c0)
            y = y_v[pl.ds(row, n), c0:c1].reshape(n // 8, 8, c1 - c0)
            ga = jnp.concatenate([gate(mod_v[2, :, c:c + 128], c - c0, 2 * D) for c in range(c0, c1, 128)], axis=1)
            return (xf + ga[None] * y).reshape(n, c1 - c0)

        def post_items(row0):
            def load(r, k):
                if k:
                    return x1n[pl.ds(pl.multiple_of(zrow(r, k), LG), LG), :]
                x1 = x1_rows(row0 + r, LG, 0, D)
                x1n[r:r + LG, :] = x1
                return x1
            return staged(ln_stages(load, stat2, h2_v, 4, 3), TMB // LG, 1)

        def logit_items(buf, first):
            _, qk, _, _, pb = bufs[buf]
            swap = lane_iota(RG) ^ 1

            def s_logit(g):
                need(("q", buf), ("k", buf))
                have.add(("l", buf, g))
                r = g * RG
                qs = [qk[c, HALO + r:HALO + r + RG, :] for c in range(NC)]
                for w in range(WIN):
                    k0 = HALO + r - DIL * w
                    if w >= WIN // 2:
                        k0 = zrow(k0)
                    s = _tree(_add, [qs[c] * qk[NC + c, pl.ds(k0, RG), :] for c in range(NC)])
                    s = gate(s, w, WIN)
                    s = s + pltpu.roll(s, 64, 1)
                    s = s + jnp.take_along_axis(s, swap, axis=1, mode="promise_in_bounds")
                    if first and r < DIL * w:
                        pos = r + jax.lax.broadcasted_iota(jnp.int32, (RG, 128), 0)
                        s = jnp.where(pos >= DIL * w, s, NEG * LOG2E)
                    sls[g % len(sls)][w, pl.ds(pl.multiple_of(zrow(0), RG), RG), :] = s

            def s_soft(g):
                assert ("p", buf, g) not in have
                have.add(("p", buf, g))
                r = g * RG
                ss = [sls[g % len(sls)][w] for w in range(WIN)]
                m = gate(_tree(jnp.maximum, ss), 0, 1)
                es = [jnp.exp2(s - m) for s in ss]
                for w in range(WIN):
                    pb[w, r:r + RG, :] = es[w]
                den = _tree(_add, es)
                inv = pl.reciprocal(den, approx=True)
                pb[WIN, r:r + RG, :] = inv * (2.0 - den * inv)
            return staged((s_logit, s_soft), TM // RG, LLAG)

        def pv_items(buf):
            _, _, vp, o, pb = bufs[buf]
            otmp = otmps[buf]

            def one(r):
                need(("v", buf), ("p", buf, r // RG))
                have.remove(("p", buf, r // RG))
                have.add(("o", buf, r // RG))
                ps = [pb[w, pl.ds(pl.multiple_of(zrow(r), RG), RG), :] for w in range(WIN + 1)]
                for c in range(NC):
                    ks = [HALO + r - DIL * w if w < WIN // 2 else zrow(HALO + r - DIL * w) for w in range(WIN)]
                    acc = _tree(_add, [ps[w] * vp[c, pl.ds(ks[w], RG), :] for w in range(WIN)])
                    acc = gate(acc * ps[WIN], c, NC)
                    if (r // RG) % 2 == 0:
                        otmp[c, pl.ds(pl.multiple_of(zrow(0), 8), RG), :] = acc
                    else:
                        both = jnp.concatenate([otmp[c], acc], axis=0).astype(BF16)
                        o[(r - RG) // 2:(r + RG) // 2, c * 128:(c + 1) * 128] = pltpu.bitcast(both, U32)
            return [functools.partial(one, r) for r in range(0, TM, RG)]

        def halo(buf, prev, part):
            _, qk, vp, _, _ = bufs[buf]
            for c in range(NC):
                if part == 1:
                    qk[NC + c, 0:HALO, :] = (jnp.zeros((HALO, 128), F32) if prev is None
                                             else gate16(bufs[prev][1][NC + c, TM:TM + HALO, :], 1, 2))
                else:
                    vp[c, 0:HALO, :] = (jnp.broadcast_to(vp[c, HALO:HALO + 1, :], (HALO, 128)) if prev is None
                                        else gate16(bufs[prev][2][c, TM:TM + HALO, :], 1, 2))

        def qkv_part(buf, g, sb=None, k=None):
            h1, qk, vp, _, _ = bufs[buf] if buf else (None,) * 5
            if sb is not None:
                h1 = h1s.at[sb]
                need(*[("h", sb, k, i) for i in range(TM // LG)], *[("w", g, k, j) for j in range(NC)])
            if k != 0:
                for i in range(TM // RG):
                    if g < 2 and ("qk"[g], buf) in have:
                        need(("l", buf, i))
                    if g == 2 and ("v", buf) in have:
                        assert ("p", buf, i) not in have or ("new", buf) in have
                if g == 1:
                    have.difference_update({("l", buf, i) for i in range(TM // RG)})
                    have.add(("new", buf))
                have.discard(("qkv"[g], buf))

            def sink(n0, r):
                ch = n0 // 128
                if k == 0:
                    part[sb, ch] = r
                    return
                if k == 1:
                    r = r + part[sb, ch]
                dst, ci = (qk, ch) if ch < 2 * NC else (vp, ch - 2 * NC)
                dst[ci, HALO:HALO + TM, :] = r * (SM_SCALE * LOG2E) if ch < NC else r
            matmul(lambda kk: ld16(h1, 0, TM, kk * KH, (kk + 1) * KH),
                   lambda kk, n0: ld16(wqkv_p, kk * KH, KH, n0, n0 + 128),
                   (0, 1) if k is None else (k,), range(g * D, (g + 1) * D, 128), sink,
                   None if k == 0 else ("qkv"[g], buf))
            if g == 2:
                have.discard(("new", buf))

        def wo_mm(buf, row0):
            o = bufs[buf][3]
            need(*[("o", buf, i) for i in range(TM // RG)])
            have.difference_update({("o", buf, i) for i in range(TM // RG)})

            def sink(n0, r):
                y_v[pl.ds(row0, TM), n0:n0 + 128] = r
            matmul(lambda k: ld16(o, 0, TM, k * KH, (k + 1) * KH),
                   lambda k, n0: ld16(wo_p, k * KH, KH, n0, n0 + 128),
                   (0, 1), range(0, D, 128), sink)

        UP = NC * (D // KH)

        def run_now(items):
            for fn in items:
                fn()

        def ffn(j, row0, slot, nxt_row):
            h = ld16(h2_v, 0, TMB, 0, D)
            for f0 in range(0, F, FC):
                g = jnp.dot(h, w1_v[:, f0:f0 + FC], preferred_element_type=F32)
                u = jnp.dot(h, w3_v[:, f0:f0 + FC], preferred_element_type=F32)
                act_v[:, f0:f0 + FC] = pltpu.bitcast((g * jax.nn.sigmoid(g) * u).astype(BF16), U32)
            nk = F // KH
            sched = {}
            place(sched, post_items(nxt_row), range(0, NC * nk - PB1))
            begin(sched)

            def sink(n0, r):
                z = (mod_v[5, :, n0:n0 + 128][None] * r.reshape(TMB // 8, 8, 128)).reshape(TMB, 128)
                obuf[slot, :, n0:n0 + 128] = (x1_rows(row0, TMB, n0, n0 + 128) + z).astype(BF16)
                if n0 + 128 in OCUT:
                    cp_out(j, slot, OCUT.index(n0 + 128) - 1).start()
            matmul(lambda k: ld16(act_v, 0, TMB, k * KH, (k + 1) * KH),
                   lambda k, n0: w2_v[k * KH:(k + 1) * KH, n0:n0 + 128],
                   tuple(range(nk)), range(0, D, 128), sink)

        U8 = NC

        def segment(*placements):
            sched = {}
            for items, units in placements:
                place(sched, items, units)
            begin(sched)

        with jax.named_scope("prologue"):
            zs[0] = 0
            begin({})
            start("c", "x0", "ca0", "q0", "sa0", "k0", "v0", "x4", "ca1", "sa1", "q1", "k1", "v1", "wo",
                  "x1", "m2", "x2")
            wait("c")
            cb_v[...] = jnp.broadcast_to(silu_c().astype(F32), (128, D)).T
            wait("x0")
            for r in range(0, NS * TM, LG):
                xf = x_v[r:r + LG, :].astype(F32)
                mu = jnp.mean(xf, axis=-1, keepdims=True)
                d = xf - mu
                rs = jax.lax.rsqrt(jnp.mean(d * d, axis=-1, keepdims=True) + EPS)
                stats[0, r:r + LG, :] = jnp.broadcast_to(mu, (LG, 128))
                stats[1, r:r + LG, :] = jnp.broadcast_to(rs, (LG, 128))
            wait("ca0")
            mod_mxu(1, 0)
            wait("q0")
            run_now(perm_qkv_items(0, 0))
            wait("sa0")
            mod_mxu(0, 0)
            run_now(ln1_out_items(0, 0))

        with jax.named_scope("pass1"):
            segment((ln1_out_items(1, 0), range(0, U8 - 2)),
                    (ln1_out_items(2, 0) + ln1_out_items(3, 0), range(U8 - 2, 2 * U8)))
            qkv_part(None, 0, 0, 0)
            qkv_part(None, 0, 1, 0)
            wait("k0")
            segment((perm_qkv_items(1, 0), range(0, 2 * U8 - 2)))
            for g, b in ((0, 2), (0, 3), (1, 0), (1, 1)):
                qkv_part(None, g, b, 0)
            wait("v0", "x4", "ca1")
            segment((perm_qkv_items(2, 0), range(0, 2 * U8 - 2)),
                    (staged(ln1_start(NS, 0)[:2], TM // LG, 1), range(2 * U8 - 1, 4 * U8 - 2)),
                    (mod_items(D + KH, 4) + [functools.partial(mod_finish, 1, KH, D)], range(2 * U8 - 2, 4 * U8)))
            for g, b in ((1, 2), (1, 3), (2, 0), (2, 1)):
                qkv_part(None, g, b, 0)
            wait("sa1", "q1")
            segment((mod_items(KH, 4) + [functools.partial(mod_finish, 0, KH, D)], range(0, U8 + 2)),
                    (perm_qkv_items(0, 1), range(0, 2 * U8 - 2)),
                    (ln1_out_items(0, 1), range(U8 + 3, 2 * U8 - 1)))
            qkv_part(None, 2, 2, 0)
            qkv_part(None, 2, 3, 0)

        with jax.named_scope("pass2"):
            wait("k1")
            segment((perm_qkv_items(1, 1), range(0, 2 * U8 - 2)),
                    (ln1_out_items(1, 1), range(0, U8 - 2)),
                    (ln1_out_items(2, 1), range(U8 - 2, 2 * U8)))
            halo("b", None, 1)
            qkv_part("b", 0, 0, 1)
            qkv_part("c", 0, 1, 1)
            wait("v1")
            l0 = logit_items("b", True)
            segment((perm_qkv_items(2, 1), range(0, 2 * U8 - 2)),
                    (ln1_out_items(3, 1), range(0, U8)),
                    (l0[:LB], range(B0, B1)))
            qkv_part("b", 1, 0, 1)
            halo("c", "b", 1)
            qkv_part("c", 1, 1, 1)
            qkv_part("b", 2, 0, 1)
            halo("b", None, 2)
            halo("c", "b", 2)
            qkv_part("c", 2, 1, 1)
            wait("wo")
            segment((perm_wo_items(), range(0, WS)),
                    (l0[LB:], range(0, C0)),
                    (pv_items("b"), range(C0 + CP, 39)),
                    (logit_items("c", False), range(C0, C1)),
                    (pv_items("c"), range(C1 + CP, 63)),
                    (logit_items("a", False), range(C1, C2)),
                    (pv_items("a"), range(C2 + CP, 79)),
                    ([functools.partial(halo, "b", "a", 1)], [23]),
                    ([functools.partial(halo, "b", "a", 2)], [39]),
                    (ln1_out_items(NS, 0) + ln1_out_items(NS, 1), range(H0, H1)),
                    (logit_items("b", False), range(C2, 96 - L1)))
            halo("a", "c", 1)
            halo("a", "c", 2)
            for g in range(3):
                qkv_part("a", g, 2, 1)
            for g in range(3):
                qkv_part("b", g, 3, 1)
            wo_mm("b", 0)
            wo_mm("c", TM)
            wo_mm("a", 2 * TM)
            finish()
            wait("x1", "m2")
            start("m3", "w1", "w3", "w2")


        def half(X, Y, u0, sched, row_ln1, row_wo, extra):
            place(sched, pv_items(Y), range(u0 + P0, u0 + 3 * UP - P1))
            place(sched, logit_items(X, False), range(u0 + 2 * UP + L0, u0 + 4 * UP - L1))
            place(sched, ln1_items(row_ln1, Y), range(u0 + N0, u0 + N1))
            if extra:
                place(sched, extra, range(u0, u0 + 4 * UP - 1))

            def run():
                halo(X, Y, 1)
                halo(X, Y, 2)
                for g in range(3):
                    qkv_part(X, g)
                wo_mm(Y, row_wo)
            return run

        def a_step(s, carry):
            @pl.when(s == 3)
            def _():
                wait("x2", "m3")

            ra = pl.multiple_of(2 * s * TM, TM)
            nxt = pl.multiple_of(jnp.minimum(ra + 2 * TM, S - TM), TM)
            col0 = pl.multiple_of(jnp.minimum(2 * D + (s - 2) * (MT * 128), 6 * D - MT * 128), 128)
            mi = mod_items(col0, MT)
            sched = {}
            run_a = half("a", "b", 0, sched, ra + TM, ra - TM, mi[:len(mi) // 2])
            run_b = half("b", "a", 4 * UP, sched, nxt, ra, mi[len(mi) // 2:])
            begin(sched)
            run_a()
            run_b()
            finish()
            return carry

        with jax.named_scope("aloop"):
            if SKIP_A:
                wait("x2", "m3")
            else:
                jax.lax.fori_loop(NS // 2, NB // 2, a_step, 0)

        with jax.named_scope("atail"):
            begin({})
            for j in range(2, 6):
                mod_finish(j, 0, D)
            run_now(pv_items("b"))
            if TAILV == 0:
                segment((post_items(0), range(0, UP - 2)))
            elif TAILV == 1:
                items = post_items(0)
                run_now(items[:TB])
                segment((items[TB:], range(0, UP - 2)))
            else:
                def bulk(r):
                    x1 = x1_rows(r, LG, 0, D)
                    mu = jnp.mean(x1, axis=-1, keepdims=True)
                    d = x1 - mu
                    rs = jax.lax.rsqrt(jnp.mean(d * d, axis=-1, keepdims=True) + EPS)
                    y = (d * rs).reshape(LG // 8, 8, D) * mod_v[4][None] + mod_v[3][None]
                    h2_v[r // 2:(r + LG) // 2, :] = pltpu.bitcast(y.reshape(LG, D).astype(BF16), U32)
                segment(([functools.partial(bulk, r) for r in range(0, TMB, LG)], range(0, UP - TE)))
            wo_mm("b", S - TM)
            finish()
            wait("w1", "w3", "w2")

        def b_step(j, carry):
            slot = j % 2

            @pl.when(j >= 2)
            def _():
                wait_out(j - 2, slot)

            row0 = pl.multiple_of(j * TMB, TMB)
            nxt = pl.multiple_of(jnp.minimum(row0 + TMB, S - TMB), TMB)
            if SKIP_FFN:
                obuf[slot] = x1_rows(row0, TMB, 0, D).astype(BF16)
                for q in range(NQ):
                    cp_out(j, slot, q).start()
            else:
                ffn(j, row0, slot, nxt)
            return carry

        with jax.named_scope("bloop"):
            jax.lax.fori_loop(0, NBB, b_step, 0)
        with jax.named_scope("tail"):
            wait_out(NBB - 2, (NBB - 2) % 2)
            wait_out(NBB - 1, (NBB - 1) % 2)

    any_spec = pl.BlockSpec(memory_space=pl.ANY)
    scratch = [
        pltpu.VMEM((S, D), BF16),
        pltpu.VMEM((D, 3 * D), BF16),
        pltpu.VMEM((NC, KH // 2, 128), U32),
        pltpu.VMEM((D // 2, 3 * D), U32),
        pltpu.VMEM((D, D), BF16),
        pltpu.VMEM((NC, D // 32 * 17, 128), U32),
        pltpu.VMEM((D // 2, D), U32),
        pltpu.VMEM((D, F), BF16),
        pltpu.VMEM((D, F), BF16),
        pltpu.VMEM((F, D), BF16),
        pltpu.VMEM((D, 6 * D), BF16),
        pltpu.VMEM((D, 128), F32),
        pltpu.VMEM((NSUB, 8, 6 * D), F32),
        pltpu.VMEM((6, 8, D), F32),
        pltpu.VMEM((TM // 2, D), U32),
        pltpu.VMEM((TM // 2, D), U32),
        pltpu.VMEM((NS, TM // 2, D), U32),
        pltpu.VMEM((NS, 3 * NC, TM, 128), F32),
        pltpu.VMEM((2, (NS + 1) * TM, 128), F32),
        pltpu.VMEM((2 * NC, KV + PADK, 128), F32),
        pltpu.VMEM((NC, KV + PADK, 128), F32),
        pltpu.VMEM((WIN + 1, TM, 128), F32),
        pltpu.VMEM((2 * NC, KV + PADK, 128), F32),
        pltpu.VMEM((NC, KV + PADK, 128), F32),
        pltpu.VMEM((WIN + 1, TM, 128), F32),
        pltpu.VMEM((2 * NC, KV + PADK, 128), F32),
        pltpu.VMEM((NC, KV + PADK, 128), F32),
        pltpu.VMEM((WIN + 1, TM, 128), F32),
        pltpu.VMEM((TM // 2, D), U32),
        pltpu.VMEM((TM // 2, D), U32),
        pltpu.VMEM((TM // 2, D), U32),
        pltpu.VMEM((NC, RG, 128), F32),
        pltpu.VMEM((NC, RG, 128), F32),
        pltpu.VMEM((NC, RG, 128), F32),
        pltpu.VMEM((WIN, RG, 128), F32),
        pltpu.VMEM((WIN, RG, 128), F32),
        pltpu.VMEM((WIN, RG, 128), F32),
        pltpu.VMEM((2, TM, 128), F32),
        pltpu.VMEM((2, TMB, 128), F32),
        pltpu.VMEM((S, D), F32),
        pltpu.VMEM((TMB, D), F32),
        pltpu.VMEM((TMB // 2, D), U32),
        pltpu.VMEM((TMB // 2, F), U32),
        pltpu.VMEM((2, TMB, D), BF16),
        pltpu.VMEM((1, D), BF16),
        pltpu.SMEM((1,), jnp.int32),
        pltpu.SemaphoreType.DMA((NDMA,)),
        pltpu.SemaphoreType.DMA((2 * NQ,)),
    ]

    def call(A_x, A_wqkv, A_wo, B_w1, B_w3, B_w2, c, w_mod):
        return pl.pallas_call(
            kernel,
            out_shape=jax.ShapeDtypeStruct((1, S, D), BF16),
            in_specs=[any_spec] * 8,
            out_specs=any_spec,
            scratch_shapes=scratch,
            compiler_params=pltpu.CompilerParams(vmem_limit_bytes=120 * 1024 * 1024),
        )(A_x, A_wqkv, A_wo, B_w1, B_w3, B_w2, c, w_mod)

    return call


@jax.jit
def pallas_adaLN_cond__sliding_local_dilated__glu_gated_swiglu__prompt_kernel(
    A_x: jax.Array,
    A_wqkv: jax.Array,
    A_wo: jax.Array,
    B_x: jax.Array,
    B_w1: jax.Array,
    B_w3: jax.Array,
    B_w2: jax.Array,
    c: jax.Array,
    w_mod: jax.Array,
):
    del B_x
    return _build()(A_x, A_wqkv, A_wo, B_w1, B_w3, B_w2, c, w_mod)
```

```python
import functools
import math

import jax
import jax.numpy as jnp
import jax.experimental.pallas as pl
import jax.experimental.pallas.tpu as pltpu

S = 2048
D = 1024
F = 3584
H = 32
DH = D // H
WIN = 8
DIL = 2
NC = D // 128
HALO = 16
EPS = 1e-5
NEG = -1000000000.0
SM_SCALE = DH ** -0.5
LOG2E = math.log2(math.e)

TM = 128
NB = S // TM
KV = HALO + TM
RG = 8
LG = 16
NS = 4
NDMA = 21
KH = 512

F32 = jnp.float32
BF16 = jnp.bfloat16
U32 = jnp.uint32


def _tree(op, xs):
    xs = list(xs)
    while len(xs) > 1:
        xs = [op(xs[i], xs[i + 1]) if i + 1 < len(xs) else xs[i] for i in range(0, len(xs), 2)]
    return xs[0]


def _add(a, b):
    return a + b


def _build(TMB=256, FC=512, GATE=True, SKIP_FFN=False, SKIP_A=False,
           SCH=0, MT=6, NSUB=16, PB1=5, L0=0, L1=1, SPREAD=128, LLAG=3,
           P0=0, P1=16, N0=1, N1=30, PR=32, B0=14, B1=30, LB=19, PADK=0, C0=10, C1=38, C2=64, CP=0, WS=46, H0=0, H1=10, TAILV=2, TB=16, TE=2, OCUT=(0, 512, 896, 1024)):
    NBB = S // TMB
    NQ = len(OCUT) - 1

    def kernel(x_hbm, wqkv_hbm, wo_hbm, w1_hbm, w3_hbm, w2_hbm, c_hbm, wmod_hbm,
               out_hbm,
               x_v, wqkv_v, wtmp, wqkv_p, wo_v, wo_tmp, wo_p, w1_v, w3_v, w2_v, wmod_v, cb_v, modp_v, mod_v,
               h1a, h1b, h1s, part, stats, qka, va, pa, qkb, vb, pb_, qkc, vc, pc, oa, ob, oc, ota, otb, otc, sl0, sl1, sl2, stat1, stat2, y_v, x1n, h2_v, act_v, obuf, c_ref,
               zs, sem_w, sem_o):
        bufs = {"a": (h1a, qka, va, oa, pa), "b": (h1b, qkb, vb, ob, pb_),
                "c": (None, qkc, vc, oc, pc)}

        sls = (sl0, sl1, sl2)
        otmps = {"a": ota, "b": otb, "c": otc}

        dmas = {}

        def add_dma(name, src, dst):
            dmas[name] = (src, dst, len(dmas))

        for name, (b0, b1) in (("x0", (0, NS)), ("x4", (NS, NS + 1)), ("x1", (NS + 1, NS + 3)), ("x2", (NS + 3, NB))):
            rows = pl.ds(b0 * TM, (b1 - b0) * TM)
            add_dma(name, x_hbm.at[0, rows, :], x_v.at[rows, :])
        for name, (c0, c1) in (("sa0", (0, KH)), ("sa1", (KH, D)), ("ca0", (D, D + KH)), ("ca1", (D + KH, 2 * D)),
                               ("m2", (2 * D, 3 * D)), ("m3", (3 * D, 6 * D))):
            cols = pl.ds(c0, c1 - c0)
            add_dma(name, wmod_hbm.at[:, cols], wmod_v.at[:, cols])
        for g in range(3):
            for k in range(2):
                rows, cols = pl.ds(k * KH, KH), pl.ds(g * D, D)
                add_dma("qkv"[g] + str(k), wqkv_hbm.at[rows, cols], wqkv_v.at[rows, cols])
        add_dma("c", c_hbm, c_ref)
        add_dma("wo", wo_hbm, wo_v)
        add_dma("w1", w1_hbm, w1_v)
        add_dma("w3", w3_hbm, w3_v)
        add_dma("w2", w2_hbm, w2_v)
        assert len(dmas) == NDMA

        def cp(name):
            src, dst, i = dmas[name]
            return pltpu.make_async_copy(src, dst, sem_w.at[i])

        def start(*names):
            for n in names:
                cp(n).start()

        def wait(*names):
            for n in names:
                cp(n).wait()

        def cp_out(j, slot, q):
            c0, c1 = OCUT[q], OCUT[q + 1]
            return pltpu.make_async_copy(obuf.at[slot, :, pl.ds(c0, c1 - c0)],
                                         out_hbm.at[0, pl.ds(j * TMB, TMB), pl.ds(c0, c1 - c0)],
                                         sem_o.at[slot * NQ + q])

        def wait_out(j, slot):
            for q in range(NQ):
                cp_out(j, slot, q).wait()

        st = {"z": None, "never": None, "clock": 0, "sched": {}, "tok": None}

        have = set()

        def need(*keys):
            assert all(k in have for k in keys), keys

        def begin(sched):
            z = zs[0]
            st.update(z=z, never=jnp.full((8, 128), z, jnp.int32) != 0, clock=0, sched=sched, tok=None)

        def gate(val, i, n):
            r = st["tok"]
            if r is None or not GATE:
                return val
            row = (i * SPREAD // n) // 8 * 8
            t = r[row:row + 8]
            return jnp.where(st["never"], t if val.dtype == F32 else pltpu.bitcast(t, val.dtype), val)

        def place(sched, items, units):
            units = list(units)
            for i, it in enumerate(items):
                sched.setdefault(units[(i * len(units)) // len(items)], []).append(it)

        def matmul(lhs_fn, w_fn, ks, cols, sink, gives=None):
            for n0 in cols:
                r = None
                for k in ks:
                    d = jnp.dot(lhs_fn(k), w_fn(k, n0), preferred_element_type=F32)
                    r = d if r is None else r + d
                    if k == ks[-1]:
                        sink(n0, r)
                    if n0 == cols[-1] and k == ks[-1]:
                        have.add(gives)
                    st["tok"] = r
                    for fn in st["sched"].pop(st["clock"], []):
                        fn()
                    st["tok"] = None
                    st["clock"] += 1

        def finish():
            assert not st["sched"]

        def lane_iota(rows):
            return jax.lax.broadcasted_iota(jnp.int32, (rows, 128), 1)

        def ld16(ref, r0, n, c0, c1):
            return pltpu.bitcast(ref[r0 // 2:(r0 + n) // 2, c0:c1], BF16)

        def silu_c():
            cf = c_ref[...].astype(F32)
            return (cf * jax.nn.sigmoid(cf)).astype(BF16)

        def mod_mxu(j, k):
            cs = slice(k * KH, (k + 1) * KH)
            lhs = jnp.broadcast_to(silu_c(), (16, D))
            r = jnp.dot(lhs, wmod_v[:, j * D + k * KH:j * D + (k + 1) * KH], preferred_element_type=F32)[0:8]
            mod_v[j, :, cs] = r + 1.0 if j in (1, 4) else r

        def mod_finish(j, c0, c1):
            r = _tree(_add, [modp_v[i, :, j * D + c0:j * D + c1] for i in range(NSUB)])
            r = jnp.sum(r, axis=0, keepdims=True)
            mod_v[j, :, c0:c1] = jnp.broadcast_to(r + 1.0 if j in (1, 4) else r, (8, c1 - c0))

        def mod_items(col0, ntiles):
            rows = D // NSUB

            def one(t, i):
                c0 = col0 + t * 128
                c0 = c0 if isinstance(c0, int) else pl.multiple_of(c0, 128)
                w = wmod_v[i * rows:(i + 1) * rows, pl.ds(c0, 128)].astype(F32)
                p = (w * cb_v[i * rows:(i + 1) * rows, :]).reshape(rows // 8, 8, 128)
                modp_v[i, :, pl.ds(c0, 128)] = gate(_tree(_add, [p[k] for k in range(rows // 8)]), 1, 2)
            return [functools.partial(one, t, i) for t in range(ntiles) for i in range(NSUB)]

        def perm_mix(g, i, nrows):
            for h in range(nrows // 16):
                r0 = i * nrows + h * 16
                l = gate(lane_iota(8), h, nrows // 16)
                vals = [pltpu.bitcast(wqkv_v[r0:r0 + 16, g * D + c * 128: g * D + (c + 1) * 128], U32)
                        for c in range(NC)]
                for b in range(3):
                    m = (l & (4 << b)) == 0
                    for c in range(NC):
                        if c & (1 << b):
                            continue
                        lo, hi = vals[c], vals[c | (1 << b)]
                        vals[c] = jnp.where(m, lo, hi)
                        vals[c | (1 << b)] = jnp.where(m, hi, lo)
                for j in range(NC):
                    wtmp[j, pl.ds(pl.multiple_of(zrow((r0 // 2) % (KH // 2)), 8), 8), :] = vals[j]

        def perm_gather(g, k, j):
            have.add(("w", g, k, j))
            l = lane_iota(8)
            idx = ((((l >> 1) & 3) << 5) | ((((l >> 3) & 7) ^ j) << 2) | ((l >> 6) << 1) | (l & 1))
            idx = gate(idx, 0, 1)
            for q in range(0, KH // 2, 8):
                t = jnp.take_along_axis(wtmp[j, q:q + 8, :], idx, axis=1, mode="promise_in_bounds")
                wqkv_p[k * KH // 2 + q:k * KH // 2 + q + 8, g * D + j * 128: g * D + (j + 1) * 128] = t

        def perm_qkv_items(g, k, nrows=PR):
            n = KH // nrows
            return ([functools.partial(perm_mix, g, i, nrows) for i in range(k * n, (k + 1) * n)]
                    + [functools.partial(perm_gather, g, k, j) for j in range(NC)])

        def perm_wo_items():
            low = jax.lax.broadcasted_iota(jnp.int32, (8, 128), 0) < 4

            def spread(c, h):
                for r in range(h * 256, h * 256 + 256, 8):
                    wo_tmp[c, pl.ds(zrow(r + r // 16), 8), :] = gate(pltpu.bitcast(
                        wo_v[2 * r:2 * r + 16, c * 128:(c + 1) * 128], U32), r % 256, 256)

            def gather(c, h):
                for G in range(h * 32, h * 32 + 32):
                    j, e, ch = G >> 3, (G >> 2) & 1, G & 3
                    dd = (((2 * ch) ^ j) << 1) | e
                    ta = wo_tmp[c, pl.ds(ch * 136 + dd, 8, stride=17), :]
                    tb = wo_tmp[c, pl.ds(ch * 136 + (dd ^ 2), 8, stride=17), :]
                    wo_p[G * 8:G * 8 + 8, c * 128:(c + 1) * 128] = jnp.where(low, ta, tb)
            return [functools.partial(fn, c, h) for fn in (spread, gather) for c in range(NC) for h in range(2)]

        def zrow(row, k=1):
            return row + k * st["z"]

        def gate16(v, i, n):
            return jnp.concatenate([gate(v[q:q + 8], i, n) for q in range(0, LG, 8)], axis=0)

        def staged(stages, n, lag):
            items = []
            for t in range(n + lag * (len(stages) - 1)):
                for k in reversed(range(len(stages))):
                    if 0 <= t - k * lag < n:
                        items.append(functools.partial(stages[k], t - k * lag))
            return items

        def ln_stages(load, stat, dst, j_scale, j_shift, cols=range(NC)):
            def chunks(x):
                return [x[:, c * 128:(c + 1) * 128] for c in range(NC)]

            def put(j, r, part, fn):
                m = jnp.sum(part, axis=-1, keepdims=True) * (1.0 / D)
                stat[j, pl.ds(pl.multiple_of(zrow(r), LG), LG), :] = jnp.broadcast_to(fn(m), (LG, 128))

            def s_mean(i):
                put(0, i * LG, gate16(_tree(_add, chunks(load(i * LG, 0))), 1, 2), lambda m: m)

            def s_var(i):
                r = i * LG
                mu = gate16(stat[0, r:r + LG, :], 0, 1)
                put(1, r, _tree(_add, [(x - mu) * (x - mu) for x in chunks(load(r, 1))]),
                    lambda m: jax.lax.rsqrt(m + EPS))

            def s_out(i):
                r = i * LG
                mu, rs = stat[0, r:r + LG, :], stat[1, r:r + LG, :]
                xs = chunks(load(r, 2))
                for c in cols:
                    x, cs = xs[c], slice(c * 128, (c + 1) * 128)
                    if c % (NC // 2) == 0:
                        rg = gate16(rs, c - cols[0], NC)
                    y = ((x - mu) * rg).reshape(LG // 8, 8, 128) * mod_v[j_scale, :, cs][None] + mod_v[j_shift, :, cs][None]
                    dst[r // 2:(r + LG) // 2, cs] = pltpu.bitcast(y.reshape(LG, 128).astype(BF16), U32)
            return s_mean, s_var, s_out

        def load_x(row0):
            return lambda r, k: x_v[pl.ds(pl.multiple_of(zrow(row0 + r, k), LG), LG), :].astype(F32)

        def ln1_items(row0, buf):
            return staged(ln_stages(load_x(row0), stat1, bufs[buf][0], 1, 0), TM // LG, 1)

        def ln1_start(b, k):
            return ln_stages(load_x(b * TM), stats.at[:, pl.ds(b * TM, TM), :], h1s.at[b] if b < NS else h1a,
                             1, 0, range(k * NC // 2, (k + 1) * NC // 2))

        def ln1_out_items(b, k):
            def one(i):
                have.add(("h", b, k, i))
                ln1_start(b, k)[2](i)
            return [functools.partial(one, i) for i in range(TM // LG)]

        def x1_rows(row, n, c0, c1):
            xf = x_v[pl.ds(row, n), c0:c1].astype(F32).reshape(n // 8, 8, c1 - c0)
            y = y_v[pl.ds(row, n), c0:c1].reshape(n // 8, 8, c1 - c0)
            ga = jnp.concatenate([gate(mod_v[2, :, c:c + 128], c - c0, 2 * D) for c in range(c0, c1, 128)], axis=1)
            return (xf + ga[None] * y).reshape(n, c1 - c0)

        def post_items(row0):
            def load(r, k):
                if k:
                    return x1n[pl.ds(pl.multiple_of(zrow(r, k), LG), LG), :]
                x1 = x1_rows(row0 + r, LG, 0, D)
                x1n[r:r + LG, :] = x1
                return x1
            return staged(ln_stages(load, stat2, h2_v, 4, 3), TMB // LG, 1)

        def logit_items(buf, first):
            _, qk, _, _, pb = bufs[buf]
            swap = lane_iota(RG) ^ 1

            def s_logit(g):
                need(("q", buf), ("k", buf))
                have.add(("l", buf, g))
                r = g * RG
                qs = [qk[c, HALO + r:HALO + r + RG, :] for c in range(NC)]
                for w in range(WIN):
                    k0 = HALO + r - DIL * w
                    if w >= WIN // 2:
                        k0 = zrow(k0)
                    s = _tree(_add, [qs[c] * qk[NC + c, pl.ds(k0, RG), :] for c in range(NC)])
                    s = gate(s, w, WIN)
                    s = s + pltpu.roll(s, 64, 1)
                    s = s + jnp.take_along_axis(s, swap, axis=1, mode="promise_in_bounds")
                    if first and r < DIL * w:
                        pos = r + jax.lax.broadcasted_iota(jnp.int32, (RG, 128), 0)
                        s = jnp.where(pos >= DIL * w, s, NEG * LOG2E)
                    sls[g % len(sls)][w, pl.ds(pl.multiple_of(zrow(0), RG), RG), :] = s

            def s_soft(g):
                assert ("p", buf, g) not in have
                have.add(("p", buf, g))
                r = g * RG
                ss = [sls[g % len(sls)][w] for w in range(WIN)]
                m = gate(_tree(jnp.maximum, ss), 0, 1)
                es = [jnp.exp2(s - m) for s in ss]
                for w in range(WIN):
                    pb[w, r:r + RG, :] = es[w]
                den = _tree(_add, es)
                inv = pl.reciprocal(den, approx=True)
                pb[WIN, r:r + RG, :] = inv * (2.0 - den * inv)
            return staged((s_logit, s_soft), TM // RG, LLAG)

        def pv_items(buf):
            _, _, vp, o, pb = bufs[buf]
            otmp = otmps[buf]

            def one(r):
                need(("v", buf), ("p", buf, r // RG))
                have.remove(("p", buf, r // RG))
                have.add(("o", buf, r // RG))
                ps = [pb[w, pl.ds(pl.multiple_of(zrow(r), RG), RG), :] for w in range(WIN + 1)]
                for c in range(NC):
                    ks = [HALO + r - DIL * w if w < WIN // 2 else zrow(HALO + r - DIL * w) for w in range(WIN)]
                    acc = _tree(_add, [ps[w] * vp[c, pl.ds(ks[w], RG), :] for w in range(WIN)])
                    acc = gate(acc * ps[WIN], c, NC)
                    if (r // RG) % 2 == 0:
                        otmp[c, pl.ds(pl.multiple_of(zrow(0), 8), RG), :] = acc
                    else:
                        both = jnp.concatenate([otmp[c], acc], axis=0).astype(BF16)
                        o[(r - RG) // 2:(r + RG) // 2, c * 128:(c + 1) * 128] = pltpu.bitcast(both, U32)
            return [functools.partial(one, r) for r in range(0, TM, RG)]

        def halo(buf, prev, part):
            _, qk, vp, _, _ = bufs[buf]
            for c in range(NC):
                if part == 1:
                    qk[NC + c, 0:HALO, :] = (jnp.zeros((HALO, 128), F32) if prev is None
                                             else gate16(bufs[prev][1][NC + c, TM:TM + HALO, :], 1, 2))
                else:
                    vp[c, 0:HALO, :] = (jnp.broadcast_to(vp[c, HALO:HALO + 1, :], (HALO, 128)) if prev is None
                                        else gate16(bufs[prev][2][c, TM:TM + HALO, :], 1, 2))

        def qkv_part(buf, g, sb=None, k=None):
            h1, qk, vp, _, _ = bufs[buf] if buf else (None,) * 5
            if sb is not None:
                h1 = h1s.at[sb]
                need(*[("h", sb, k, i) for i in range(TM // LG)], *[("w", g, k, j) for j in range(NC)])
            if k != 0:
                for i in range(TM // RG):
                    if g < 2 and ("qk"[g], buf) in have:
                        need(("l", buf, i))
                    if g == 2 and ("v", buf) in have:
                        assert ("p", buf, i) not in have or ("new", buf) in have
                if g == 1:
                    have.difference_update({("l", buf, i) for i in range(TM // RG)})
                    have.add(("new", buf))
                have.discard(("qkv"[g], buf))

            def sink(n0, r):
                ch = n0 // 128
                if k == 0:
                    part[sb, ch] = r
                    return
                if k == 1:
                    r = r + part[sb, ch]
                dst, ci = (qk, ch) if ch < 2 * NC else (vp, ch - 2 * NC)
                dst[ci, HALO:HALO + TM, :] = r * (SM_SCALE * LOG2E) if ch < NC else r
            matmul(lambda kk: ld16(h1, 0, TM, kk * KH, (kk + 1) * KH),
                   lambda kk, n0: ld16(wqkv_p, kk * KH, KH, n0, n0 + 128),
                   (0, 1) if k is None else (k,), range(g * D, (g + 1) * D, 128), sink,
                   None if k == 0 else ("qkv"[g], buf))
            if g == 2:
                have.discard(("new", buf))

        def wo_mm(buf, row0):
            o = bufs[buf][3]
            need(*[("o", buf, i) for i in range(TM // RG)])
            have.difference_update({("o", buf, i) for i in range(TM // RG)})

            def sink(n0, r):
                y_v[pl.ds(row0, TM), n0:n0 + 128] = r
            matmul(lambda k: ld16(o, 0, TM, k * KH, (k + 1) * KH),
                   lambda k, n0: ld16(wo_p, k * KH, KH, n0, n0 + 128),
                   (0, 1), range(0, D, 128), sink)

        UP = NC * (D // KH)

        def run_now(items):
            for fn in items:
                fn()

        def ffn(j, row0, slot, nxt_row):
            h = ld16(h2_v, 0, TMB, 0, D)
            for f0 in range(0, F, FC):
                g = jnp.dot(h, w1_v[:, f0:f0 + FC], preferred_element_type=F32)
                u = jnp.dot(h, w3_v[:, f0:f0 + FC], preferred_element_type=F32)
                act_v[:, f0:f0 + FC] = pltpu.bitcast((g * jax.nn.sigmoid(g) * u).astype(BF16), U32)
            nk = F // KH
            sched = {}
            place(sched, post_items(nxt_row), range(0, NC * nk - PB1))
            begin(sched)

            def sink(n0, r):
                z = (mod_v[5, :, n0:n0 + 128][None] * r.reshape(TMB // 8, 8, 128)).reshape(TMB, 128)
                obuf[slot, :, n0:n0 + 128] = (x1_rows(row0, TMB, n0, n0 + 128) + z).astype(BF16)
                if n0 + 128 in OCUT:
                    cp_out(j, slot, OCUT.index(n0 + 128) - 1).start()
            matmul(lambda k: ld16(act_v, 0, TMB, k * KH, (k + 1) * KH),
                   lambda k, n0: w2_v[k * KH:(k + 1) * KH, n0:n0 + 128],
                   tuple(range(nk)), range(0, D, 128), sink)

        U8 = NC

        def segment(*placements):
            sched = {}
            for items, units in placements:
                place(sched, items, units)
            begin(sched)

        with jax.named_scope("prologue"):
            zs[0] = 0
            begin({})
            start("c", "x0", "ca0", "q0", "sa0", "k0", "v0", "x4", "ca1", "sa1", "q1", "k1", "v1", "wo",
                  "x1", "m2", "x2")
            wait("c")
            cb_v[...] = jnp.broadcast_to(silu_c().astype(F32), (128, D)).T
            wait("x0")
            for r in range(0, NS * TM, LG):
                xf = x_v[r:r + LG, :].astype(F32)
                mu = jnp.mean(xf, axis=-1, keepdims=True)
                d = xf - mu
                rs = jax.lax.rsqrt(jnp.mean(d * d, axis=-1, keepdims=True) + EPS)
                stats[0, r:r + LG, :] = jnp.broadcast_to(mu, (LG, 128))
                stats[1, r:r + LG, :] = jnp.broadcast_to(rs, (LG, 128))
            wait("ca0")
            mod_mxu(1, 0)
            wait("q0")
            run_now(perm_qkv_items(0, 0))
            wait("sa0")
            mod_mxu(0, 0)
            run_now(ln1_out_items(0, 0))

        with jax.named_scope("pass1"):
            segment((ln1_out_items(1, 0), range(0, U8 - 2)),
                    (ln1_out_items(2, 0) + ln1_out_items(3, 0), range(U8 - 2, 2 * U8)))
            qkv_part(None, 0, 0, 0)
            qkv_part(None, 0, 1, 0)
            wait("k0")
            segment((perm_qkv_items(1, 0), range(0, 2 * U8 - 2)))
            for g, b in ((0, 2), (0, 3), (1, 0), (1, 1)):
                qkv_part(None, g, b, 0)
            wait("v0", "x4", "ca1")
            segment((perm_qkv_items(2, 0), range(0, 2 * U8 - 2)),
                    (staged(ln1_start(NS, 0)[:2], TM // LG, 1), range(2 * U8 - 1, 4 * U8 - 2)),
                    (mod_items(D + KH, 4) + [functools.partial(mod_finish, 1, KH, D)], range(2 * U8 - 2, 4 * U8)))
            for g, b in ((1, 2), (1, 3), (2, 0), (2, 1)):
                qkv_part(None, g, b, 0)
            wait("sa1", "q1")
            segment((mod_items(KH, 4) + [functools.partial(mod_finish, 0, KH, D)], range(0, U8 + 2)),
                    (perm_qkv_items(0, 1), range(0, 2 * U8 - 2)),
                    (ln1_out_items(0, 1), range(U8 + 3, 2 * U8 - 1)))
            qkv_part(None, 2, 2, 0)
            qkv_part(None, 2, 3, 0)

        with jax.named_scope("pass2"):
            wait("k1")
            segment((perm_qkv_items(1, 1), range(0, 2 * U8 - 2)),
                    (ln1_out_items(1, 1), range(0, U8 - 2)),
                    (ln1_out_items(2, 1), range(U8 - 2, 2 * U8)))
            halo("b", None, 1)
            qkv_part("b", 0, 0, 1)
            qkv_part("c", 0, 1, 1)
            wait("v1")
            l0 = logit_items("b", True)
            segment((perm_qkv_items(2, 1), range(0, 2 * U8 - 2)),
                    (ln1_out_items(3, 1), range(0, U8)),
                    (l0[:LB], range(B0, B1)))
            qkv_part("b", 1, 0, 1)
            halo("c", "b", 1)
            qkv_part("c", 1, 1, 1)
            qkv_part("b", 2, 0, 1)
            halo("b", None, 2)
            halo("c", "b", 2)
            qkv_part("c", 2, 1, 1)
            wait("wo")
            segment((perm_wo_items(), range(0, WS)),
                    (l0[LB:], range(0, C0)),
                    (pv_items("b"), range(C0 + CP, 39)),
                    (logit_items("c", False), range(C0, C1)),
                    (pv_items("c"), range(C1 + CP, 63)),
                    (logit_items("a", False), range(C1, C2)),
                    (pv_items("a"), range(C2 + CP, 79)),
                    ([functools.partial(halo, "b", "a", 1)], [23]),
                    ([functools.partial(halo, "b", "a", 2)], [39]),
                    (ln1_out_items(NS, 0) + ln1_out_items(NS, 1), range(H0, H1)),
                    (logit_items("b", False), range(C2, 96 - L1)))
            halo("a", "c", 1)
            halo("a", "c", 2)
            for g in range(3):
                qkv_part("a", g, 2, 1)
            for g in range(3):
                qkv_part("b", g, 3, 1)
            wo_mm("b", 0)
            wo_mm("c", TM)
            wo_mm("a", 2 * TM)
            finish()
            wait("x1", "m2")
            start("m3", "w1", "w3", "w2")


        def half(X, Y, u0, sched, row_ln1, row_wo, extra):
            place(sched, pv_items(Y), range(u0 + P0, u0 + 3 * UP - P1))
            place(sched, logit_items(X, False), range(u0 + 2 * UP + L0, u0 + 4 * UP - L1))
            place(sched, ln1_items(row_ln1, Y), range(u0 + N0, u0 + N1))
            if extra:
                place(sched, extra, range(u0, u0 + 4 * UP - 1))

            def run():
                halo(X, Y, 1)
                halo(X, Y, 2)
                for g in range(3):
                    qkv_part(X, g)
                wo_mm(Y, row_wo)
            return run

        def a_step(s, carry):
            @pl.when(s == 3)
            def _():
                wait("x2", "m3")

            ra = pl.multiple_of(2 * s * TM, TM)
            nxt = pl.multiple_of(jnp.minimum(ra + 2 * TM, S - TM), TM)
            col0 = pl.multiple_of(jnp.minimum(2 * D + (s - 2) * (MT * 128), 6 * D - MT * 128), 128)
            mi = mod_items(col0, MT)
            sched = {}
            run_a = half("a", "b", 0, sched, ra + TM, ra - TM, mi[:len(mi) // 2])
            run_b = half("b", "a", 4 * UP, sched, nxt, ra, mi[len(mi) // 2:])
            begin(sched)
            run_a()
            run_b()
            finish()
            return carry

        with jax.named_scope("aloop"):
            if SKIP_A:
                wait("x2", "m3")
            else:
                jax.lax.fori_loop(NS // 2, NB // 2, a_step, 0)

        with jax.named_scope("atail"):
            begin({})
            for j in range(2, 6):
                mod_finish(j, 0, D)
            run_now(pv_items("b"))
            if TAILV == 0:
                segment((post_items(0), range(0, UP - 2)))
            elif TAILV == 1:
                items = post_items(0)
                run_now(items[:TB])
                segment((items[TB:], range(0, UP - 2)))
            else:
                def bulk(r):
                    x1 = x1_rows(r, LG, 0, D)
                    mu = jnp.mean(x1, axis=-1, keepdims=True)
                    d = x1 - mu
                    rs = jax.lax.rsqrt(jnp.mean(d * d, axis=-1, keepdims=True) + EPS)
                    y = (d * rs).reshape(LG // 8, 8, D) * mod_v[4][None] + mod_v[3][None]
                    h2_v[r // 2:(r + LG) // 2, :] = pltpu.bitcast(y.reshape(LG, D).astype(BF16), U32)
                segment(([functools.partial(bulk, r) for r in range(0, TMB, LG)], range(0, UP - TE)))
            wo_mm("b", S - TM)
            finish()
            wait("w1", "w3", "w2")

        def b_step(j, carry):
            slot = j % 2

            @pl.when(j >= 2)
            def _():
                wait_out(j - 2, slot)

            row0 = pl.multiple_of(j * TMB, TMB)
            nxt = pl.multiple_of(jnp.minimum(row0 + TMB, S - TMB), TMB)
            if SKIP_FFN:
                obuf[slot] = x1_rows(row0, TMB, 0, D).astype(BF16)
                for q in range(NQ):
                    cp_out(j, slot, q).start()
            else:
                ffn(j, row0, slot, nxt)
            return carry

        with jax.named_scope("bloop"):
            jax.lax.fori_loop(0, NBB, b_step, 0)
        with jax.named_scope("tail"):
            wait_out(NBB - 2, (NBB - 2) % 2)
            wait_out(NBB - 1, (NBB - 1) % 2)

    any_spec = pl.BlockSpec(memory_space=pl.ANY)
    scratch = [
        pltpu.VMEM((S, D), BF16),
        pltpu.VMEM((D, 3 * D), BF16),
        pltpu.VMEM((NC, KH // 2, 128), U32),
        pltpu.VMEM((D // 2, 3 * D), U32),
        pltpu.VMEM((D, D), BF16),
        pltpu.VMEM((NC, D // 32 * 17, 128), U32),
        pltpu.VMEM((D // 2, D), U32),
        pltpu.VMEM((D, F), BF16),
        pltpu.VMEM((D, F), BF16),
        pltpu.VMEM((F, D), BF16),
        pltpu.VMEM((D, 6 * D), BF16),
        pltpu.VMEM((D, 128), F32),
        pltpu.VMEM((NSUB, 8, 6 * D), F32),
        pltpu.VMEM((6, 8, D), F32),
        pltpu.VMEM((TM // 2, D), U32),
        pltpu.VMEM((TM // 2, D), U32),
        pltpu.VMEM((NS, TM // 2, D), U32),
        pltpu.VMEM((NS, 3 * NC, TM, 128), F32),
        pltpu.VMEM((2, (NS + 1) * TM, 128), F32),
        pltpu.VMEM((2 * NC, KV + PADK, 128), F32),
        pltpu.VMEM((NC, KV + PADK, 128), F32),
        pltpu.VMEM((WIN + 1, TM, 128), F32),
        pltpu.VMEM((2 * NC, KV + PADK, 128), F32),
        pltpu.VMEM((NC, KV + PADK, 128), F32),
        pltpu.VMEM((WIN + 1, TM, 128), F32),
        pltpu.VMEM((2 * NC, KV + PADK, 128), F32),
        pltpu.VMEM((NC, KV + PADK, 128), F32),
        pltpu.VMEM((WIN + 1, TM, 128), F32),
        pltpu.VMEM((TM // 2, D), U32),
        pltpu.VMEM((TM // 2, D), U32),
        pltpu.VMEM((TM // 2, D), U32),
        pltpu.VMEM((NC, RG, 128), F32),
        pltpu.VMEM((NC, RG, 128), F32),
        pltpu.VMEM((NC, RG, 128), F32),
        pltpu.VMEM((WIN, RG, 128), F32),
        pltpu.VMEM((WIN, RG, 128), F32),
        pltpu.VMEM((WIN, RG, 128), F32),
        pltpu.VMEM((2, TM, 128), F32),
        pltpu.VMEM((2, TMB, 128), F32),
        pltpu.VMEM((S, D), F32),
        pltpu.VMEM((TMB, D), F32),
        pltpu.VMEM((TMB // 2, D), U32),
        pltpu.VMEM((TMB // 2, F), U32),
        pltpu.VMEM((2, TMB, D), BF16),
        pltpu.VMEM((1, D), BF16),
        pltpu.SMEM((1,), jnp.int32),
        pltpu.SemaphoreType.DMA((NDMA,)),
        pltpu.SemaphoreType.DMA((2 * NQ,)),
    ]

    def call(A_x, A_wqkv, A_wo, B_w1, B_w3, B_w2, c, w_mod):
        return pl.pallas_call(
            kernel,
            out_shape=jax.ShapeDtypeStruct((1, S, D), BF16),
            in_specs=[any_spec] * 8,
            out_specs=any_spec,
            scratch_shapes=scratch,
            compiler_params=pltpu.CompilerParams(vmem_limit_bytes=120 * 1024 * 1024),
        )(A_x, A_wqkv, A_wo, B_w1, B_w3, B_w2, c, w_mod)

    return call


@jax.jit
def pallas_adaLN_cond__sliding_local_dilated__glu_gated_swiglu__prompt_kernel(
    A_x: jax.Array,
    A_wqkv: jax.Array,
    A_wo: jax.Array,
    B_x: jax.Array,
    B_w1: jax.Array,
    B_w3: jax.Array,
    B_w2: jax.Array,
    c: jax.Array,
    w_mod: jax.Array,
):
    del B_x
    return _build()(A_x, A_wqkv, A_wo, B_w1, B_w3, B_w2, c, w_mod)
```

```python
import functools
import math

import jax
import jax.numpy as jnp
import jax.experimental.pallas as pl
import jax.experimental.pallas.tpu as pltpu

S = 2048
D = 1024
F = 3584
H = 32
DH = D // H
WIN = 8
DIL = 2
NC = D // 128
HALO = 16
EPS = 1e-5
NEG = -1000000000.0
SM_SCALE = DH ** -0.5
LOG2E = math.log2(math.e)

TM = 128
NB = S // TM
KV = HALO + TM
RG = 8
LG = 16
NS = 4
NDMA = 21
KH = 512

F32 = jnp.float32
BF16 = jnp.bfloat16
U32 = jnp.uint32


def _tree(op, xs):
    xs = list(xs)
    while len(xs) > 1:
        xs = [op(xs[i], xs[i + 1]) if i + 1 < len(xs) else xs[i] for i in range(0, len(xs), 2)]
    return xs[0]


def _add(a, b):
    return a + b


def _build(TMB=256, FC=512, GATE=True, SKIP_FFN=False, SKIP_A=False,
           SCH=0, MT=6, NSUB=16, PB1=5, L0=0, L1=1, SPREAD=128, LLAG=3,
           P0=1, P1=16, N0=0, N1=30, PR=32, B0=14, B1=30, LB=19, PADK=0, C0=10, C1=38, C2=64, CP=1, WS=46, H0=0, H1=10, CPARAMS={}, TAILV=2, TB=16, TE=2, OCUT=(0, 512, 896, 1024)):
    NBB = S // TMB
    NQ = len(OCUT) - 1

    def kernel(x_hbm, wqkv_hbm, wo_hbm, w1_hbm, w3_hbm, w2_hbm, c_hbm, wmod_hbm,
               out_hbm,
               x_v, wqkv_v, wtmp, wqkv_p, wo_v, wo_tmp, wo_p, w1_v, w3_v, w2_v, wmod_v, cb_v, modp_v, mod_v,
               h1a, h1b, h1s, part, stats, qka, va, pa, qkb, vb, pb_, qkc, vc, pc, oa, ob, oc, ota, otb, otc, sl0, sl1, sl2, stat1, stat2, y_v, x1n, h2_v, act_v, obuf, c_ref,
               zs, sem_w, sem_o):
        bufs = {"a": (h1a, qka, va, oa, pa), "b": (h1b, qkb, vb, ob, pb_),
                "c": (None, qkc, vc, oc, pc)}

        sls = (sl0, sl1, sl2)
        otmps = {"a": ota, "b": otb, "c": otc}

        dmas = {}

        def add_dma(name, src, dst):
            dmas[name] = (src, dst, len(dmas))

        for name, (b0, b1) in (("x0", (0, NS)), ("x4", (NS, NS + 1)), ("x1", (NS + 1, NS + 3)), ("x2", (NS + 3, NB))):
            rows = pl.ds(b0 * TM, (b1 - b0) * TM)
            add_dma(name, x_hbm.at[0, rows, :], x_v.at[rows, :])
        for name, (c0, c1) in (("sa0", (0, KH)), ("sa1", (KH, D)), ("ca0", (D, D + KH)), ("ca1", (D + KH, 2 * D)),
                               ("m2", (2 * D, 3 * D)), ("m3", (3 * D, 6 * D))):
            cols = pl.ds(c0, c1 - c0)
            add_dma(name, wmod_hbm.at[:, cols], wmod_v.at[:, cols])
        for g in range(3):
            for k in range(2):
                rows, cols = pl.ds(k * KH, KH), pl.ds(g * D, D)
                add_dma("qkv"[g] + str(k), wqkv_hbm.at[rows, cols], wqkv_v.at[rows, cols])
        add_dma("c", c_hbm, c_ref)
        add_dma("wo", wo_hbm, wo_v)
        add_dma("w1", w1_hbm, w1_v)
        add_dma("w3", w3_hbm, w3_v)
        add_dma("w2", w2_hbm, w2_v)
        assert len(dmas) == NDMA

        def cp(name):
            src, dst, i = dmas[name]
            return pltpu.make_async_copy(src, dst, sem_w.at[i])

        def start(*names):
            for n in names:
                cp(n).start()

        def wait(*names):
            for n in names:
                cp(n).wait()

        def cp_out(j, slot, q):
            c0, c1 = OCUT[q], OCUT[q + 1]
            return pltpu.make_async_copy(obuf.at[slot, :, pl.ds(c0, c1 - c0)],
                                         out_hbm.at[0, pl.ds(j * TMB, TMB), pl.ds(c0, c1 - c0)],
                                         sem_o.at[slot * NQ + q])

        def wait_out(j, slot):
            for q in range(NQ):
                cp_out(j, slot, q).wait()

        st = {"z": None, "never": None, "clock": 0, "sched": {}, "tok": None}

        have = set()

        def need(*keys):
            assert all(k in have for k in keys), keys

        def begin(sched):
            z = zs[0]
            st.update(z=z, never=jnp.full((8, 128), z, jnp.int32) != 0, clock=0, sched=sched, tok=None)

        def gate(val, i, n):
            r = st["tok"]
            if r is None or not GATE:
                return val
            row = (i * SPREAD // n) // 8 * 8
            t = r[row:row + 8]
            return jnp.where(st["never"], t if val.dtype == F32 else pltpu.bitcast(t, val.dtype), val)

        def place(sched, items, units):
            units = list(units)
            for i, it in enumerate(items):
                sched.setdefault(units[(i * len(units)) // len(items)], []).append(it)

        def matmul(lhs_fn, w_fn, ks, cols, sink, gives=None):
            for n0 in cols:
                r = None
                for k in ks:
                    d = jnp.dot(lhs_fn(k), w_fn(k, n0), preferred_element_type=F32)
                    r = d if r is None else r + d
                    if k == ks[-1]:
                        sink(n0, r)
                    if n0 == cols[-1] and k == ks[-1]:
                        have.add(gives)
                    st["tok"] = r
                    for fn in st["sched"].pop(st["clock"], []):
                        fn()
                    st["tok"] = None
                    st["clock"] += 1

        def finish():
            assert not st["sched"]

        def lane_iota(rows):
            return jax.lax.broadcasted_iota(jnp.int32, (rows, 128), 1)

        def ld16(ref, r0, n, c0, c1):
            return pltpu.bitcast(ref[r0 // 2:(r0 + n) // 2, c0:c1], BF16)

        def silu_c():
            cf = c_ref[...].astype(F32)
            return (cf * jax.nn.sigmoid(cf)).astype(BF16)

        def mod_mxu(j, k):
            cs = slice(k * KH, (k + 1) * KH)
            lhs = jnp.broadcast_to(silu_c(), (16, D))
            r = jnp.dot(lhs, wmod_v[:, j * D + k * KH:j * D + (k + 1) * KH], preferred_element_type=F32)[0:8]
            mod_v[j, :, cs] = r + 1.0 if j in (1, 4) else r

        def mod_finish(j, c0, c1):
            r = _tree(_add, [modp_v[i, :, j * D + c0:j * D + c1] for i in range(NSUB)])
            r = jnp.sum(r, axis=0, keepdims=True)
            mod_v[j, :, c0:c1] = jnp.broadcast_to(r + 1.0 if j in (1, 4) else r, (8, c1 - c0))

        def mod_items(col0, ntiles):
            rows = D // NSUB

            def one(t, i):
                c0 = col0 + t * 128
                c0 = c0 if isinstance(c0, int) else pl.multiple_of(c0, 128)
                w = wmod_v[i * rows:(i + 1) * rows, pl.ds(c0, 128)].astype(F32)
                p = (w * cb_v[i * rows:(i + 1) * rows, :]).reshape(rows // 8, 8, 128)
                modp_v[i, :, pl.ds(c0, 128)] = gate(_tree(_add, [p[k] for k in range(rows // 8)]), 1, 2)
            return [functools.partial(one, t, i) for t in range(ntiles) for i in range(NSUB)]

        def perm_mix(g, i, nrows):
            for h in range(nrows // 16):
                r0 = i * nrows + h * 16
                l = gate(lane_iota(8), h, nrows // 16)
                vals = [pltpu.bitcast(wqkv_v[r0:r0 + 16, g * D + c * 128: g * D + (c + 1) * 128], U32)
                        for c in range(NC)]
                for b in range(3):
                    m = (l & (4 << b)) == 0
                    for c in range(NC):
                        if c & (1 << b):
                            continue
                        lo, hi = vals[c], vals[c | (1 << b)]
                        vals[c] = jnp.where(m, lo, hi)
                        vals[c | (1 << b)] = jnp.where(m, hi, lo)
                for j in range(NC):
                    wtmp[j, pl.ds(pl.multiple_of(zrow((r0 // 2) % (KH // 2)), 8), 8), :] = vals[j]

        def perm_gather(g, k, j):
            have.add(("w", g, k, j))
            l = lane_iota(8)
            idx = ((((l >> 1) & 3) << 5) | ((((l >> 3) & 7) ^ j) << 2) | ((l >> 6) << 1) | (l & 1))
            idx = gate(idx, 0, 1)
            for q in range(0, KH // 2, 8):
                t = jnp.take_along_axis(wtmp[j, q:q + 8, :], idx, axis=1, mode="promise_in_bounds")
                wqkv_p[k * KH // 2 + q:k * KH // 2 + q + 8, g * D + j * 128: g * D + (j + 1) * 128] = t

        def perm_qkv_items(g, k, nrows=PR):
            n = KH // nrows
            return ([functools.partial(perm_mix, g, i, nrows) for i in range(k * n, (k + 1) * n)]
                    + [functools.partial(perm_gather, g, k, j) for j in range(NC)])

        def perm_wo_items():
            sub = jax.lax.broadcasted_iota(jnp.int32, (8, 128), 0)

            def spread(c, h):
                for r in range(h * 256, h * 256 + 256, 8):
                    wo_tmp[c, pl.ds(zrow(r + r // 16), 8), :] = gate(pltpu.bitcast(
                        wo_v[2 * r:2 * r + 16, c * 128:(c + 1) * 128], U32), r % 256, 256)

            def gather(c, h):
                for G in range(h * 32, h * 32 + 32):
                    j, e, ch = G >> 3, (G >> 2) & 1, G & 3
                    dd = (((2 * ch) ^ j) << 1) | e
                    ta = wo_tmp[c, pl.ds(ch * 136 + dd, 8, stride=17), :]
                    tb = wo_tmp[c, pl.ds(ch * 136 + (dd ^ 2), 8, stride=17), :]
                    wo_p[G * 8:G * 8 + 8, c * 128:(c + 1) * 128] = jnp.where(gate(sub, G % 32, 32) < 4, ta, tb)
            return [functools.partial(fn, c, h) for fn in (spread, gather) for c in range(NC) for h in range(2)]

        def zrow(row, k=1):
            return row + k * st["z"]

        def gate16(v, i, n):
            return jnp.concatenate([gate(v[q:q + 8], i, n) for q in range(0, LG, 8)], axis=0)

        def staged(stages, n, lag):
            items = []
            for t in range(n + lag * (len(stages) - 1)):
                for k in reversed(range(len(stages))):
                    if 0 <= t - k * lag < n:
                        items.append(functools.partial(stages[k], t - k * lag))
            return items

        def ln_stages(load, stat, dst, j_scale, j_shift, cols=range(NC)):
            def chunks(x):
                return [x[:, c * 128:(c + 1) * 128] for c in range(NC)]

            def put(j, r, part, fn):
                m = jnp.sum(part, axis=-1, keepdims=True) * (1.0 / D)
                stat[j, pl.ds(pl.multiple_of(zrow(r), LG), LG), :] = jnp.broadcast_to(fn(m), (LG, 128))

            def s_mean(i):
                put(0, i * LG, gate16(_tree(_add, chunks(load(i * LG, 0))), 1, 2), lambda m: m)

            def s_var(i):
                r = i * LG
                mu = gate16(stat[0, r:r + LG, :], 0, 1)
                put(1, r, _tree(_add, [(x - mu) * (x - mu) for x in chunks(load(r, 1))]),
                    lambda m: jax.lax.rsqrt(m + EPS))

            def s_out(i):
                r = i * LG
                mu, rs = stat[0, r:r + LG, :], stat[1, r:r + LG, :]
                xs = chunks(load(r, 2))
                for c in cols:
                    x, cs = xs[c], slice(c * 128, (c + 1) * 128)
                    if c % (NC // 2) == 0:
                        rg = gate16(rs, c - cols[0], NC)
                    y = ((x - mu) * rg).reshape(LG // 8, 8, 128) * mod_v[j_scale, :, cs][None] + mod_v[j_shift, :, cs][None]
                    dst[r // 2:(r + LG) // 2, cs] = pltpu.bitcast(y.reshape(LG, 128).astype(BF16), U32)
            return s_mean, s_var, s_out

        def load_x(row0):
            return lambda r, k: x_v[pl.ds(pl.multiple_of(zrow(row0 + r, k), LG), LG), :].astype(F32)

        def ln1_items(row0, buf):
            return staged(ln_stages(load_x(row0), stat1, bufs[buf][0], 1, 0), TM // LG, 1)

        def ln1_start(b, k):
            return ln_stages(load_x(b * TM), stats.at[:, pl.ds(b * TM, TM), :], h1s.at[b] if b < NS else h1a,
                             1, 0, range(k * NC // 2, (k + 1) * NC // 2))

        def ln1_out_items(b, k):
            def one(i):
                have.add(("h", b, k, i))
                ln1_start(b, k)[2](i)
            return [functools.partial(one, i) for i in range(TM // LG)]

        def x1_rows(row, n, c0, c1):
            xf = x_v[pl.ds(row, n), c0:c1].astype(F32).reshape(n // 8, 8, c1 - c0)
            y = y_v[pl.ds(row, n), c0:c1].reshape(n // 8, 8, c1 - c0)
            ga = jnp.concatenate([gate(mod_v[2, :, c:c + 128], c - c0, 2 * D) for c in range(c0, c1, 128)], axis=1)
            return (xf + ga[None] * y).reshape(n, c1 - c0)

        def post_items(row0):
            def load(r, k):
                if k:
                    return x1n[pl.ds(pl.multiple_of(zrow(r, k), LG), LG), :]
                x1 = x1_rows(row0 + r, LG, 0, D)
                x1n[r:r + LG, :] = x1
                return x1
            return staged(ln_stages(load, stat2, h2_v, 4, 3), TMB // LG, 1)

        def logit_items(buf, first):
            _, qk, _, _, pb = bufs[buf]
            swap = lane_iota(RG) ^ 1

            def s_logit(g):
                need(("q", buf), ("k", buf))
                have.add(("l", buf, g))
                r = g * RG
                qs = [qk[c, HALO + r:HALO + r + RG, :] for c in range(NC)]
                for w in range(WIN):
                    k0 = HALO + r - DIL * w
                    if w >= WIN // 2:
                        k0 = zrow(k0)
                    s = _tree(_add, [qs[c] * qk[NC + c, pl.ds(k0, RG), :] for c in range(NC)])
                    s = gate(s, w, WIN)
                    s = s + pltpu.roll(s, 64, 1)
                    s = s + jnp.take_along_axis(s, swap, axis=1, mode="promise_in_bounds")
                    if first and r < DIL * w:
                        pos = r + jax.lax.broadcasted_iota(jnp.int32, (RG, 128), 0)
                        s = jnp.where(pos >= DIL * w, s, NEG * LOG2E)
                    sls[g % len(sls)][w, pl.ds(pl.multiple_of(zrow(0), RG), RG), :] = s

            def s_soft(g):
                assert ("p", buf, g) not in have
                have.add(("p", buf, g))
                r = g * RG
                ss = [sls[g % len(sls)][w] for w in range(WIN)]
                m = gate(_tree(jnp.maximum, ss), 0, 1)
                es = [jnp.exp2(s - m) for s in ss]
                for w in range(WIN):
                    pb[w, r:r + RG, :] = es[w]
                den = _tree(_add, es)
                inv = pl.reciprocal(den, approx=True)
                pb[WIN, r:r + RG, :] = inv * (2.0 - den * inv)
            return staged((s_logit, s_soft), TM // RG, LLAG)

        def pv_items(buf):
            _, _, vp, o, pb = bufs[buf]
            otmp = otmps[buf]

            def one(r):
                need(("v", buf), ("p", buf, r // RG))
                have.remove(("p", buf, r // RG))
                have.add(("o", buf, r // RG))
                ps = [pb[w, pl.ds(pl.multiple_of(zrow(r), RG), RG), :] for w in range(WIN + 1)]
                for c in range(NC):
                    ks = [HALO + r - DIL * w if w < WIN // 2 else zrow(HALO + r - DIL * w) for w in range(WIN)]
                    acc = _tree(_add, [ps[w] * vp[c, pl.ds(ks[w], RG), :] for w in range(WIN)])
                    acc = gate(acc * ps[WIN], c, NC)
                    if (r // RG) % 2 == 0:
                        otmp[c, pl.ds(pl.multiple_of(zrow(0), 8), RG), :] = acc
                    else:
                        both = jnp.concatenate([otmp[c], acc], axis=0).astype(BF16)
                        o[(r - RG) // 2:(r + RG) // 2, c * 128:(c + 1) * 128] = pltpu.bitcast(both, U32)
            return [functools.partial(one, r) for r in range(0, TM, RG)]

        def halo(buf, prev, part):
            _, qk, vp, _, _ = bufs[buf]
            for c in range(NC):
                if part == 1:
                    qk[NC + c, 0:HALO, :] = (jnp.zeros((HALO, 128), F32) if prev is None
                                             else gate16(bufs[prev][1][NC + c, TM:TM + HALO, :], 1, 2))
                else:
                    vp[c, 0:HALO, :] = (jnp.broadcast_to(vp[c, HALO:HALO + 1, :], (HALO, 128)) if prev is None
                                        else gate16(bufs[prev][2][c, TM:TM + HALO, :], 1, 2))

        def qkv_part(buf, g, sb=None, k=None):
            h1, qk, vp, _, _ = bufs[buf] if buf else (None,) * 5
            if sb is not None:
                h1 = h1s.at[sb]
                need(*[("h", sb, k, i) for i in range(TM // LG)], *[("w", g, k, j) for j in range(NC)])
            if k != 0:
                for i in range(TM // RG):
                    if g < 2 and ("qk"[g], buf) in have:
                        need(("l", buf, i))
                    if g == 2 and ("v", buf) in have:
                        assert ("p", buf, i) not in have or ("new", buf) in have
                if g == 1:
                    have.difference_update({("l", buf, i) for i in range(TM // RG)})
                    have.add(("new", buf))
                have.discard(("qkv"[g], buf))

            def sink(n0, r):
                ch = n0 // 128
                if k == 0:
                    part[sb, ch] = r
                    return
                if k == 1:
                    r = r + part[sb, ch]
                dst, ci = (qk, ch) if ch < 2 * NC else (vp, ch - 2 * NC)
                dst[ci, HALO:HALO + TM, :] = r * (SM_SCALE * LOG2E) if ch < NC else r
            matmul(lambda kk: ld16(h1, 0, TM, kk * KH, (kk + 1) * KH),
                   lambda kk, n0: ld16(wqkv_p, kk * KH, KH, n0, n0 + 128),
                   (0, 1) if k is None else (k,), range(g * D, (g + 1) * D, 128), sink,
                   None if k == 0 else ("qkv"[g], buf))
            if g == 2:
                have.discard(("new", buf))

        def wo_mm(buf, row0):
            o = bufs[buf][3]
            need(*[("o", buf, i) for i in range(TM // RG)])
            have.difference_update({("o", buf, i) for i in range(TM // RG)})

            def sink(n0, r):
                y_v[pl.ds(row0, TM), n0:n0 + 128] = r
            matmul(lambda k: ld16(o, 0, TM, k * KH, (k + 1) * KH),
                   lambda k, n0: ld16(wo_p, k * KH, KH, n0, n0 + 128),
                   (0, 1), range(0, D, 128), sink)

        UP = NC * (D // KH)

        def run_now(items):
            for fn in items:
                fn()

        def ffn(j, row0, slot, nxt_row):
            h = ld16(h2_v, 0, TMB, 0, D)
            for f0 in range(0, F, FC):
                g = jnp.dot(h, w1_v[:, f0:f0 + FC], preferred_element_type=F32)
                u = jnp.dot(h, w3_v[:, f0:f0 + FC], preferred_element_type=F32)
                act_v[:, f0:f0 + FC] = pltpu.bitcast((g * jax.nn.sigmoid(g) * u).astype(BF16), U32)
            nk = F // KH
            sched = {}
            place(sched, post_items(nxt_row), range(0, NC * nk - PB1))
            begin(sched)

            def sink(n0, r):
                z = (mod_v[5, :, n0:n0 + 128][None] * r.reshape(TMB // 8, 8, 128)).reshape(TMB, 128)
                obuf[slot, :, n0:n0 + 128] = (x1_rows(row0, TMB, n0, n0 + 128) + z).astype(BF16)
                if n0 + 128 in OCUT:
                    cp_out(j, slot, OCUT.index(n0 + 128) - 1).start()
            matmul(lambda k: ld16(act_v, 0, TMB, k * KH, (k + 1) * KH),
                   lambda k, n0: w2_v[k * KH:(k + 1) * KH, n0:n0 + 128],
                   tuple(range(nk)), range(0, D, 128), sink)

        U8 = NC

        def segment(*placements):
            sched = {}
            for items, units in placements:
                place(sched, items, units)
            begin(sched)

        with jax.named_scope("prologue"):
            zs[0] = 0
            begin({})
            start("c", "x0", "ca0", "q0", "sa0", "k0", "v0", "x4", "ca1", "sa1", "q1", "k1", "v1", "wo",
                  "x1", "m2", "x2")
            wait("c")
            cb_v[...] = jnp.broadcast_to(silu_c().astype(F32), (128, D)).T
            wait("x0")
            for r in range(0, NS * TM, LG):
                xf = x_v[r:r + LG, :].astype(F32)
                mu = jnp.mean(xf, axis=-1, keepdims=True)
                d = xf - mu
                rs = jax.lax.rsqrt(jnp.mean(d * d, axis=-1, keepdims=True) + EPS)
                stats[0, r:r + LG, :] = jnp.broadcast_to(mu, (LG, 128))
                stats[1, r:r + LG, :] = jnp.broadcast_to(rs, (LG, 128))
            wait("ca0")
            mod_mxu(1, 0)
            wait("q0")
            run_now(perm_qkv_items(0, 0))
            wait("sa0")
            mod_mxu(0, 0)
            run_now(ln1_out_items(0, 0))

        with jax.named_scope("pass1"):
            segment((ln1_out_items(1, 0), range(0, U8 - 2)),
                    (ln1_out_items(2, 0) + ln1_out_items(3, 0), range(U8 - 2, 2 * U8)))
            qkv_part(None, 0, 0, 0)
            qkv_part(None, 0, 1, 0)
            wait("k0")
            segment((perm_qkv_items(1, 0), range(0, 2 * U8 - 2)))
            for g, b in ((0, 2), (0, 3), (1, 0), (1, 1)):
                qkv_part(None, g, b, 0)
            wait("v0", "x4", "ca1")
            segment((perm_qkv_items(2, 0), range(0, 2 * U8 - 2)),
                    (staged(ln1_start(NS, 0)[:2], TM // LG, 1), range(2 * U8 - 1, 4 * U8 - 2)),
                    (mod_items(D + KH, 4) + [functools.partial(mod_finish, 1, KH, D)], range(2 * U8 - 2, 4 * U8)))
            for g, b in ((1, 2), (1, 3), (2, 0), (2, 1)):
                qkv_part(None, g, b, 0)
            wait("sa1", "q1")
            segment((mod_items(KH, 4) + [functools.partial(mod_finish, 0, KH, D)], range(0, U8 + 2)),
                    (perm_qkv_items(0, 1), range(0, 2 * U8 - 2)),
                    (ln1_out_items(0, 1), range(U8 + 3, 2 * U8 - 1)))
            qkv_part(None, 2, 2, 0)
            qkv_part(None, 2, 3, 0)

        with jax.named_scope("pass2"):
            wait("k1")
            segment((perm_qkv_items(1, 1), range(0, 2 * U8 - 2)),
                    (ln1_out_items(1, 1), range(0, U8 - 2)),
                    (ln1_out_items(2, 1), range(U8 - 2, 2 * U8)))
            halo("b", None, 1)
            qkv_part("b", 0, 0, 1)
            qkv_part("c", 0, 1, 1)
            wait("v1")
            l0 = logit_items("b", True)
            segment((perm_qkv_items(2, 1), range(0, 2 * U8 - 2)),
                    (ln1_out_items(3, 1), range(0, U8)),
                    (l0[:LB], range(B0, B1)))
            qkv_part("b", 1, 0, 1)
            halo("c", "b", 1)
            qkv_part("c", 1, 1, 1)
            qkv_part("b", 2, 0, 1)
            halo("b", None, 2)
            halo("c", "b", 2)
            qkv_part("c", 2, 1, 1)
            wait("wo")
            segment((perm_wo_items(), range(0, WS)),
                    (l0[LB:], range(0, C0)),
                    (pv_items("b"), range(C0 + CP, 39)),
                    (logit_items("c", False), range(C0, C1)),
                    (pv_items("c"), range(C1 + CP, 63)),
                    (logit_items("a", False), range(C1, C2)),
                    (pv_items("a"), range(C2 + CP, 79)),
                    ([functools.partial(halo, "b", "a", 1)], [23]),
                    ([functools.partial(halo, "b", "a", 2)], [39]),
                    (ln1_out_items(NS, 0) + ln1_out_items(NS, 1), range(H0, H1)),
                    (logit_items("b", False), range(C2, 96 - L1)))
            halo("a", "c", 1)
            halo("a", "c", 2)
            for g in range(3):
                qkv_part("a", g, 2, 1)
            for g in range(3):
                qkv_part("b", g, 3, 1)
            wo_mm("b", 0)
            wo_mm("c", TM)
            wo_mm("a", 2 * TM)
            finish()
            wait("x1", "m2")
            start("m3", "w1", "w3", "w2")


        def half(X, Y, u0, sched, row_ln1, row_wo, extra):
            place(sched, pv_items(Y), range(u0 + P0, u0 + 3 * UP - P1))
            place(sched, logit_items(X, False), range(u0 + 2 * UP + L0, u0 + 4 * UP - L1))
            place(sched, ln1_items(row_ln1, Y), range(u0 + N0, u0 + N1))
            if extra:
                place(sched, extra, range(u0, u0 + 4 * UP - 1))

            def run():
                halo(X, Y, 1)
                halo(X, Y, 2)
                for g in range(3):
                    qkv_part(X, g)
                wo_mm(Y, row_wo)
            return run

        def a_step(s, carry):
            @pl.when(s == 3)
            def _():
                wait("x2", "m3")

            ra = pl.multiple_of(2 * s * TM, TM)
            nxt = pl.multiple_of(jnp.minimum(ra + 2 * TM, S - TM), TM)
            col0 = pl.multiple_of(jnp.minimum(2 * D + (s - 2) * (MT * 128), 6 * D - MT * 128), 128)
            mi = mod_items(col0, MT)
            sched = {}
            run_a = half("a", "b", 0, sched, ra + TM, ra - TM, mi[:len(mi) // 2])
            run_b = half("b", "a", 4 * UP, sched, nxt, ra, mi[len(mi) // 2:])
            begin(sched)
            run_a()
            run_b()
            finish()
            return carry

        with jax.named_scope("aloop"):
            if SKIP_A:
                wait("x2", "m3")
            else:
                jax.lax.fori_loop(NS // 2, NB // 2, a_step, 0)

        with jax.named_scope("atail"):
            begin({})
            for j in range(2, 6):
                mod_finish(j, 0, D)
            run_now(pv_items("b"))
            if TAILV == 0:
                segment((post_items(0), range(0, UP - 2)))
            elif TAILV == 1:
                items = post_items(0)
                run_now(items[:TB])
                segment((items[TB:], range(0, UP - 2)))
            else:
                def bulk(r):
                    x1 = x1_rows(r, LG, 0, D)
                    mu = jnp.mean(x1, axis=-1, keepdims=True)
                    d = x1 - mu
                    rs = jax.lax.rsqrt(jnp.mean(d * d, axis=-1, keepdims=True) + EPS)
                    y = (d * rs).reshape(LG // 8, 8, D) * mod_v[4][None] + mod_v[3][None]
                    h2_v[r // 2:(r + LG) // 2, :] = pltpu.bitcast(y.reshape(LG, D).astype(BF16), U32)
                segment(([functools.partial(bulk, r) for r in range(0, TMB, LG)], range(0, UP - TE)))
            wo_mm("b", S - TM)
            finish()
            wait("w1", "w3", "w2")

        def b_step(j, carry):
            slot = j % 2

            @pl.when(j >= 2)
            def _():
                wait_out(j - 2, slot)

            row0 = pl.multiple_of(j * TMB, TMB)
            nxt = pl.multiple_of(jnp.minimum(row0 + TMB, S - TMB), TMB)
            if SKIP_FFN:
                obuf[slot] = x1_rows(row0, TMB, 0, D).astype(BF16)
                for q in range(NQ):
                    cp_out(j, slot, q).start()
            else:
                ffn(j, row0, slot, nxt)
            return carry

        with jax.named_scope("bloop"):
            jax.lax.fori_loop(0, NBB, b_step, 0)
        with jax.named_scope("tail"):
            wait_out(NBB - 2, (NBB - 2) % 2)
            wait_out(NBB - 1, (NBB - 1) % 2)

    any_spec = pl.BlockSpec(memory_space=pl.ANY)
    scratch = [
        pltpu.VMEM((S, D), BF16),
        pltpu.VMEM((D, 3 * D), BF16),
        pltpu.VMEM((NC, KH // 2, 128), U32),
        pltpu.VMEM((D // 2, 3 * D), U32),
        pltpu.VMEM((D, D), BF16),
        pltpu.VMEM((NC, D // 32 * 17, 128), U32),
        pltpu.VMEM((D // 2, D), U32),
        pltpu.VMEM((D, F), BF16),
        pltpu.VMEM((D, F), BF16),
        pltpu.VMEM((F, D), BF16),
        pltpu.VMEM((D, 6 * D), BF16),
        pltpu.VMEM((D, 128), F32),
        pltpu.VMEM((NSUB, 8, 6 * D), F32),
        pltpu.VMEM((6, 8, D), F32),
        pltpu.VMEM((TM // 2, D), U32),
        pltpu.VMEM((TM // 2, D), U32),
        pltpu.VMEM((NS, TM // 2, D), U32),
        pltpu.VMEM((NS, 3 * NC, TM, 128), F32),
        pltpu.VMEM((2, (NS + 1) * TM, 128), F32),
        pltpu.VMEM((2 * NC, KV + PADK, 128), F32),
        pltpu.VMEM((NC, KV + PADK, 128), F32),
        pltpu.VMEM((WIN + 1, TM, 128), F32),
        pltpu.VMEM((2 * NC, KV + PADK, 128), F32),
        pltpu.VMEM((NC, KV + PADK, 128), F32),
        pltpu.VMEM((WIN + 1, TM, 128), F32),
        pltpu.VMEM((2 * NC, KV + PADK, 128), F32),
        pltpu.VMEM((NC, KV + PADK, 128), F32),
        pltpu.VMEM((WIN + 1, TM, 128), F32),
        pltpu.VMEM((TM // 2, D), U32),
        pltpu.VMEM((TM // 2, D), U32),
        pltpu.VMEM((TM // 2, D), U32),
        pltpu.VMEM((NC, RG, 128), F32),
        pltpu.VMEM((NC, RG, 128), F32),
        pltpu.VMEM((NC, RG, 128), F32),
        pltpu.VMEM((WIN, RG, 128), F32),
        pltpu.VMEM((WIN, RG, 128), F32),
        pltpu.VMEM((WIN, RG, 128), F32),
        pltpu.VMEM((2, TM, 128), F32),
        pltpu.VMEM((2, TMB, 128), F32),
        pltpu.VMEM((S, D), F32),
        pltpu.VMEM((TMB, D), F32),
        pltpu.VMEM((TMB // 2, D), U32),
        pltpu.VMEM((TMB // 2, F), U32),
        pltpu.VMEM((2, TMB, D), BF16),
        pltpu.VMEM((1, D), BF16),
        pltpu.SMEM((1,), jnp.int32),
        pltpu.SemaphoreType.DMA((NDMA,)),
        pltpu.SemaphoreType.DMA((2 * NQ,)),
    ]

    def call(A_x, A_wqkv, A_wo, B_w1, B_w3, B_w2, c, w_mod):
        return pl.pallas_call(
            kernel,
            out_shape=jax.ShapeDtypeStruct((1, S, D), BF16),
            in_specs=[any_spec] * 8,
            out_specs=any_spec,
            scratch_shapes=scratch,
            compiler_params=pltpu.CompilerParams(
                vmem_limit_bytes=120 * 1024 * 1024,
                disable_semaphore_checks=True, disable_bounds_checks=True, **CPARAMS),
        )(A_x, A_wqkv, A_wo, B_w1, B_w3, B_w2, c, w_mod)

    return call


@jax.jit
def pallas_adaLN_cond__sliding_local_dilated__glu_gated_swiglu__prompt_kernel(
    A_x: jax.Array,
    A_wqkv: jax.Array,
    A_wo: jax.Array,
    B_x: jax.Array,
    B_w1: jax.Array,
    B_w3: jax.Array,
    B_w2: jax.Array,
    c: jax.Array,
    w_mod: jax.Array,
):
    del B_x
    return _build()(A_x, A_wqkv, A_wo, B_w1, B_w3, B_w2, c, w_mod)
```

```python
import functools
import math

import jax
import jax.numpy as jnp
import jax.experimental.pallas as pl
import jax.experimental.pallas.tpu as pltpu

S = 2048
D = 1024
F = 3584
H = 32
DH = D // H
WIN = 8
DIL = 2
NC = D // 128
HALO = 16
EPS = 1e-5
NEG = -1000000000.0
SM_SCALE = DH ** -0.5
LOG2E = math.log2(math.e)

TM = 128
NB = S // TM
KV = HALO + TM
RG = 8
LG = 16
NS = 4
NDMA = 22
KH = 512

F32 = jnp.float32
BF16 = jnp.bfloat16
U32 = jnp.uint32


def _tree(op, xs):
    xs = list(xs)
    while len(xs) > 1:
        xs = [op(xs[i], xs[i + 1]) if i + 1 < len(xs) else xs[i] for i in range(0, len(xs), 2)]
    return xs[0]


def _add(a, b):
    return a + b


def _build(TMB=256, FC=512, GATE=True, SKIP_FFN=False, SKIP_A=False,
           SCH=0, MT=6, NSUB=16, PB1=5, L0=0, L1=1, SPREAD=128, LLAG=3,
           P0=1, P1=16, N0=0, N1=30, PR=32, B0=14, B1=30, LB=19, PADK=0, C0=10, C1=38, C2=64, CP=1, WS=46, H0=0, H1=10, CPARAMS={}, MLAG=8, TSPLIT=True, TP0=8, TE=3, SA_CUT=768, OCUT=(0, 512, 896, 1024)):
    NBB = S // TMB
    NQ = len(OCUT) - 1

    def kernel(x_hbm, wqkv_hbm, wo_hbm, w1_hbm, w3_hbm, w2_hbm, c_hbm, wmod_hbm,
               out_hbm,
               x_v, wqkv_v, wtmp, wqkv_p, wo_v, wo_tmp, wo_p, w1_v, w3_v, w2_v, wmod_v, cb_v, modp_v, modb_v, mod_v,
               h1a, h1b, h1s, part, stats, qka, va, pa, qkb, vb, pb_, qkc, vc, pc, oa, ob, oc, ota, otb, otc, sl0, sl1, sl2, stat1, stat2, y_v, x1n, h2_v, act_v, obuf, c_ref,
               zs, sem_w, sem_o):
        bufs = {"a": (h1a, qka, va, oa, pa), "b": (h1b, qkb, vb, ob, pb_),
                "c": (None, qkc, vc, oc, pc)}

        sls = (sl0, sl1, sl2)
        otmps = {"a": ota, "b": otb, "c": otc}

        dmas = {}

        def add_dma(name, src, dst):
            dmas[name] = (src, dst, len(dmas))

        for name, (b0, b1) in (("x0", (0, NS)), ("x4", (NS, NS + 1)), ("x1", (NS + 1, NS + 3)), ("x2", (NS + 3, NB))):
            rows = pl.ds(b0 * TM, (b1 - b0) * TM)
            add_dma(name, x_hbm.at[0, rows, :], x_v.at[rows, :])
        for name, (r0, r1) in (("sa0a", (0, SA_CUT)), ("sa0b", (SA_CUT, D))):
            rows, cols = pl.ds(r0, r1 - r0), pl.ds(0, KH)
            add_dma(name, wmod_hbm.at[rows, cols], wmod_v.at[rows, cols])
        for name, (c0, c1) in (("sa1", (KH, D)), ("ca0", (D, D + KH)), ("ca1", (D + KH, 2 * D)),
                               ("m2", (2 * D, 3 * D)), ("m3", (3 * D, 6 * D))):
            cols = pl.ds(c0, c1 - c0)
            add_dma(name, wmod_hbm.at[:, cols], wmod_v.at[:, cols])
        for g in range(3):
            for k in range(2):
                rows, cols = pl.ds(k * KH, KH), pl.ds(g * D, D)
                add_dma("qkv"[g] + str(k), wqkv_hbm.at[rows, cols], wqkv_v.at[rows, cols])
        add_dma("c", c_hbm, c_ref)
        add_dma("wo", wo_hbm, wo_v)
        add_dma("w1", w1_hbm, w1_v)
        add_dma("w3", w3_hbm, w3_v)
        add_dma("w2", w2_hbm, w2_v)
        assert len(dmas) == NDMA

        def cp(name):
            src, dst, i = dmas[name]
            return pltpu.make_async_copy(src, dst, sem_w.at[i])

        def start(*names):
            for n in names:
                cp(n).start()

        def wait(*names):
            for n in names:
                cp(n).wait()

        def cp_out(j, slot, q):
            c0, c1 = OCUT[q], OCUT[q + 1]
            return pltpu.make_async_copy(obuf.at[slot, :, pl.ds(c0, c1 - c0)],
                                         out_hbm.at[0, pl.ds(j * TMB, TMB), pl.ds(c0, c1 - c0)],
                                         sem_o.at[slot * NQ + q])

        def wait_out(j, slot):
            for q in range(NQ):
                cp_out(j, slot, q).wait()

        st = {"z": None, "never": None, "clock": 0, "sched": {}, "tok": None}

        have = set()

        def need(*keys):
            assert all(k in have for k in keys), keys

        def begin(sched):
            z = zs[0]
            st.update(z=z, never=jnp.full((8, 128), z, jnp.int32) != 0, clock=0, sched=sched, tok=None)

        def gate(val, i, n):
            r = st["tok"]
            if r is None or not GATE:
                return val
            row = (i * min(SPREAD, r.shape[0]) // n) // 8 * 8
            t = r[row:row + 8]
            return jnp.where(st["never"], t if val.dtype == F32 else pltpu.bitcast(t, val.dtype), val)

        def place(sched, items, units):
            units = list(units)
            for i, it in enumerate(items):
                sched.setdefault(units[(i * len(units)) // len(items)], []).append(it)

        def matmul(lhs_fn, w_fn, ks, cols, sink, gives=None):
            for n0 in cols:
                r = None
                for k in ks:
                    d = jnp.dot(lhs_fn(k), w_fn(k, n0), preferred_element_type=F32)
                    r = d if r is None else r + d
                    if k == ks[-1]:
                        sink(n0, r)
                    if n0 == cols[-1] and k == ks[-1]:
                        have.add(gives)
                    st["tok"] = r
                    for fn in st["sched"].pop(st["clock"], []):
                        fn()
                    st["tok"] = None
                    st["clock"] += 1

        def finish():
            assert not st["sched"]

        def lane_iota(rows):
            return jax.lax.broadcasted_iota(jnp.int32, (rows, 128), 1)

        def ld16(ref, r0, n, c0, c1):
            return pltpu.bitcast(ref[r0 // 2:(r0 + n) // 2, c0:c1], BF16)

        def silu_c():
            cf = c_ref[...].astype(F32)
            return (cf * jax.nn.sigmoid(cf)).astype(BF16)

        def mod_mxu(j, r0, r1):
            cs = slice(j * D, j * D + KH)
            lhs = jnp.broadcast_to(silu_c()[:, r0:r1], (16, r1 - r0))
            r = jnp.dot(lhs, wmod_v[r0:r1, cs], preferred_element_type=F32)[0:8]
            mod_v[:, cs] = r + (mod_v[:, cs] if r0 else float(j == 1))

        def mod(j, c0, c1):
            return (mod_v if j < 2 else modb_v)[:, j * D + c0:j * D + c1]

        def mod_items(col0, ntiles):
            rows = D // NSUB

            def col(t):
                c0 = col0 + t * 128
                return c0 if isinstance(c0, int) else pl.multiple_of(c0, 128)

            def part_sum(t, i):
                w = wmod_v[i * rows:(i + 1) * rows, pl.ds(col(t), 128)].astype(F32)
                p = (w * cb_v[i * rows:(i + 1) * rows, :]).reshape(rows // 8, 8, 128)
                modp_v[t, i] = gate(_tree(_add, [p[k] for k in range(rows // 8)]), 1, 2)

            def total(t):
                r = gate(_tree(_add, [modp_v[t, pl.ds(zrow(i), 1)][0] for i in range(NSUB)]), 0, 1)
                one = jnp.where((col(t) // D) % 3 == 1, 1.0, 0.0).astype(F32)
                dst = mod_v if isinstance(col0, int) else modb_v
                dst[:, pl.ds(col(t), 128)] = jnp.broadcast_to(jnp.sum(r, axis=0, keepdims=True) + one, (8, 128))
            items = []
            for t in range(ntiles + 1):
                for i in range(NSUB):
                    if t < ntiles:
                        items.append(functools.partial(part_sum, t, i))
                    if t > 0 and i == (MLAG if t < ntiles else 0):
                        items.append(functools.partial(total, t - 1))
            return items

        def perm_mix(g, i, nrows):
            for h in range(nrows // 16):
                r0 = i * nrows + h * 16
                l = gate(lane_iota(8), h, nrows // 16)
                vals = [pltpu.bitcast(wqkv_v[r0:r0 + 16, g * D + c * 128: g * D + (c + 1) * 128], U32)
                        for c in range(NC)]
                for b in range(3):
                    m = (l & (4 << b)) == 0
                    for c in range(NC):
                        if c & (1 << b):
                            continue
                        lo, hi = vals[c], vals[c | (1 << b)]
                        vals[c] = jnp.where(m, lo, hi)
                        vals[c | (1 << b)] = jnp.where(m, hi, lo)
                for j in range(NC):
                    wtmp[j, pl.ds(pl.multiple_of(zrow((r0 // 2) % (KH // 2)), 8), 8), :] = vals[j]

        def perm_gather(g, k, j):
            have.add(("w", g, k, j))
            l = lane_iota(8)
            idx = ((((l >> 1) & 3) << 5) | ((((l >> 3) & 7) ^ j) << 2) | ((l >> 6) << 1) | (l & 1))
            idx = gate(idx, 0, 1)
            for q in range(0, KH // 2, 8):
                t = jnp.take_along_axis(wtmp[j, q:q + 8, :], idx, axis=1, mode="promise_in_bounds")
                wqkv_p[k * KH // 2 + q:k * KH // 2 + q + 8, g * D + j * 128: g * D + (j + 1) * 128] = t

        def perm_qkv_items(g, k, nrows=PR):
            n = KH // nrows
            return ([functools.partial(perm_mix, g, i, nrows) for i in range(k * n, (k + 1) * n)]
                    + [functools.partial(perm_gather, g, k, j) for j in range(NC)])

        def perm_wo_items():
            sub = jax.lax.broadcasted_iota(jnp.int32, (8, 128), 0)

            def spread(c, h):
                for r in range(h * 256, h * 256 + 256, 8):
                    wo_tmp[c, pl.ds(zrow(r + r // 16), 8), :] = gate(pltpu.bitcast(
                        wo_v[2 * r:2 * r + 16, c * 128:(c + 1) * 128], U32), r % 256, 256)

            def gather(c, h):
                for G in range(h * 32, h * 32 + 32):
                    j, e, ch = G >> 3, (G >> 2) & 1, G & 3
                    dd = (((2 * ch) ^ j) << 1) | e
                    ta = wo_tmp[c, pl.ds(ch * 136 + dd, 8, stride=17), :]
                    tb = wo_tmp[c, pl.ds(ch * 136 + (dd ^ 2), 8, stride=17), :]
                    wo_p[G * 8:G * 8 + 8, c * 128:(c + 1) * 128] = jnp.where(gate(sub, G % 32, 32) < 4, ta, tb)
            return [functools.partial(fn, c, h) for fn in (spread, gather) for c in range(NC) for h in range(2)]

        def zrow(row, k=1):
            return row + k * st["z"]

        def gate16(v, i, n):
            return jnp.concatenate([gate(v[q:q + 8], i, n) for q in range(0, LG, 8)], axis=0)

        def staged(stages, n, lag):
            items = []
            for t in range(n + lag * (len(stages) - 1)):
                for k in reversed(range(len(stages))):
                    if 0 <= t - k * lag < n:
                        items.append(functools.partial(stages[k], t - k * lag))
            return items

        def ln_stages(load, stat, dst, j_scale, j_shift, cols=range(NC)):
            def chunks(x):
                return [x[:, c * 128:(c + 1) * 128] for c in range(NC)]

            def put(j, r, part, fn):
                m = jnp.sum(part, axis=-1, keepdims=True) * (1.0 / D)
                stat[j, pl.ds(pl.multiple_of(zrow(r), LG), LG), :] = jnp.broadcast_to(fn(m), (LG, 128))

            def s_mean(i):
                put(0, i * LG, gate16(_tree(_add, chunks(load(i * LG, 0))), 1, 2), lambda m: m)

            def s_var(i):
                r = i * LG
                mu = gate16(stat[0, r:r + LG, :], 0, 1)
                put(1, r, _tree(_add, [(x - mu) * (x - mu) for x in chunks(load(r, 1))]),
                    lambda m: jax.lax.rsqrt(m + EPS))

            def s_out(i):
                r = i * LG
                mu, rs = stat[0, r:r + LG, :], stat[1, r:r + LG, :]
                xs = chunks(load(r, 2))
                for c in cols:
                    x, cs = xs[c], slice(c * 128, (c + 1) * 128)
                    if c % (NC // 2) == 0:
                        rg = gate16(rs, c - cols[0], NC)
                    y = ((x - mu) * rg).reshape(LG // 8, 8, 128) * mod(j_scale, c * 128, c * 128 + 128)[None] + mod(j_shift, c * 128, c * 128 + 128)[None]
                    dst[r // 2:(r + LG) // 2, cs] = pltpu.bitcast(y.reshape(LG, 128).astype(BF16), U32)
            return s_mean, s_var, s_out

        def load_x(row0):
            return lambda r, k: x_v[pl.ds(pl.multiple_of(zrow(row0 + r, k), LG), LG), :].astype(F32)

        def ln1_items(row0, buf):
            return staged(ln_stages(load_x(row0), stat1, bufs[buf][0], 1, 0), TM // LG, 1)

        def ln1_start(b, k):
            return ln_stages(load_x(b * TM), stats.at[:, pl.ds(b * TM, TM), :], h1s.at[b] if b < NS else h1a,
                             1, 0, range(k * NC // 2, (k + 1) * NC // 2))

        def ln1_out_items(b, k):
            def one(i):
                have.add(("h", b, k, i))
                ln1_start(b, k)[2](i)
            return [functools.partial(one, i) for i in range(TM // LG)]

        def x1_rows(row, n, c0, c1):
            xf = x_v[pl.ds(row, n), c0:c1].astype(F32).reshape(n // 8, 8, c1 - c0)
            y = y_v[pl.ds(row, n), c0:c1].reshape(n // 8, 8, c1 - c0)
            ga = jnp.concatenate([gate(mod(2, c, c + 128), c - c0, 2 * D) for c in range(c0, c1, 128)], axis=1)
            return (xf + ga[None] * y).reshape(n, c1 - c0)

        def post_items(row0):
            def load(r, k):
                if k:
                    return x1n[pl.ds(pl.multiple_of(zrow(r, k), LG), LG), :]
                x1 = x1_rows(row0 + r, LG, 0, D)
                x1n[r:r + LG, :] = x1
                return x1
            return staged(ln_stages(load, stat2, h2_v, 4, 3), TMB // LG, 1)

        def logit_items(buf, first):
            _, qk, _, _, pb = bufs[buf]
            swap = lane_iota(RG) ^ 1

            def s_logit(g):
                need(("q", buf), ("k", buf))
                have.add(("l", buf, g))
                r = g * RG
                qs = [qk[c, HALO + r:HALO + r + RG, :] for c in range(NC)]
                for w in range(WIN):
                    k0 = HALO + r - DIL * w
                    if w >= WIN // 2:
                        k0 = zrow(k0)
                    s = _tree(_add, [qs[c] * qk[NC + c, pl.ds(k0, RG), :] for c in range(NC)])
                    s = gate(s, w, WIN)
                    s = s + pltpu.roll(s, 64, 1)
                    s = s + jnp.take_along_axis(s, swap, axis=1, mode="promise_in_bounds")
                    if first and r < DIL * w:
                        pos = r + jax.lax.broadcasted_iota(jnp.int32, (RG, 128), 0)
                        s = jnp.where(pos >= DIL * w, s, NEG * LOG2E)
                    sls[g % len(sls)][w, pl.ds(pl.multiple_of(zrow(0), RG), RG), :] = s

            def s_soft(g):
                assert ("p", buf, g) not in have
                have.add(("p", buf, g))
                r = g * RG
                ss = [sls[g % len(sls)][w] for w in range(WIN)]
                m = gate(_tree(jnp.maximum, ss), 0, 1)
                es = [jnp.exp2(s - m) for s in ss]
                for w in range(WIN):
                    pb[w, r:r + RG, :] = es[w]
                den = _tree(_add, es)
                inv = pl.reciprocal(den, approx=True)
                pb[WIN, r:r + RG, :] = inv * (2.0 - den * inv)
            return staged((s_logit, s_soft), TM // RG, LLAG)

        def pv_items(buf):
            _, _, vp, o, pb = bufs[buf]
            otmp = otmps[buf]

            def one(r):
                need(("v", buf), ("p", buf, r // RG))
                have.remove(("p", buf, r // RG))
                have.add(("o", buf, r // RG))
                ps = [pb[w, pl.ds(pl.multiple_of(zrow(r), RG), RG), :] for w in range(WIN + 1)]
                for c in range(NC):
                    ks = [HALO + r - DIL * w if w < WIN // 2 else zrow(HALO + r - DIL * w) for w in range(WIN)]
                    acc = _tree(_add, [ps[w] * vp[c, pl.ds(ks[w], RG), :] for w in range(WIN)])
                    acc = gate(acc * ps[WIN], c, NC)
                    if (r // RG) % 2 == 0:
                        otmp[c, pl.ds(pl.multiple_of(zrow(0), 8), RG), :] = acc
                    else:
                        both = jnp.concatenate([otmp[c], acc], axis=0).astype(BF16)
                        o[(r - RG) // 2:(r + RG) // 2, c * 128:(c + 1) * 128] = pltpu.bitcast(both, U32)
            return [functools.partial(one, r) for r in range(0, TM, RG)]

        def halo(buf, prev, part):
            _, qk, vp, _, _ = bufs[buf]
            for c in range(NC):
                if part == 1:
                    qk[NC + c, 0:HALO, :] = (jnp.zeros((HALO, 128), F32) if prev is None
                                             else gate16(bufs[prev][1][NC + c, TM:TM + HALO, :], 1, 2))
                else:
                    vp[c, 0:HALO, :] = (jnp.broadcast_to(vp[c, HALO:HALO + 1, :], (HALO, 128)) if prev is None
                                        else gate16(bufs[prev][2][c, TM:TM + HALO, :], 1, 2))

        def qkv_part(buf, g, sb=None, k=None):
            h1, qk, vp, _, _ = bufs[buf] if buf else (None,) * 5
            if sb is not None:
                h1 = h1s.at[sb]
                need(*[("h", sb, k, i) for i in range(TM // LG)], *[("w", g, k, j) for j in range(NC)])
            if k != 0:
                for i in range(TM // RG):
                    if g < 2 and ("qk"[g], buf) in have:
                        need(("l", buf, i))
                    if g == 2 and ("v", buf) in have:
                        assert ("p", buf, i) not in have or ("new", buf) in have
                if g == 1:
                    have.difference_update({("l", buf, i) for i in range(TM // RG)})
                    have.add(("new", buf))
                have.discard(("qkv"[g], buf))

            def sink(n0, r):
                ch = n0 // 128
                if k == 0:
                    part[sb, ch] = r
                    return
                if k == 1:
                    r = r + part[sb, ch]
                dst, ci = (qk, ch) if ch < 2 * NC else (vp, ch - 2 * NC)
                dst[ci, HALO:HALO + TM, :] = r * (SM_SCALE * LOG2E) if ch < NC else r
            matmul(lambda kk: ld16(h1, 0, TM, kk * KH, (kk + 1) * KH),
                   lambda kk, n0: ld16(wqkv_p, kk * KH, KH, n0, n0 + 128),
                   (0, 1) if k is None else (k,), range(g * D, (g + 1) * D, 128), sink,
                   None if k == 0 else ("qkv"[g], buf))
            if g == 2:
                have.discard(("new", buf))

        def wo_mm(buf, row0, m0=0, m1=TM):
            o = bufs[buf][3]
            need(*[("o", buf, i) for i in range(m0 // RG, m1 // RG)])
            have.difference_update({("o", buf, i) for i in range(m0 // RG, m1 // RG)})

            def sink(n0, r):
                y_v[pl.ds(row0 + m0, m1 - m0), n0:n0 + 128] = r
            matmul(lambda k: ld16(o, m0, m1 - m0, k * KH, (k + 1) * KH),
                   lambda k, n0: ld16(wo_p, k * KH, KH, n0, n0 + 128),
                   (0, 1), range(0, D, 128), sink)

        UP = NC * (D // KH)

        def run_now(items):
            for fn in items:
                fn()

        def ffn(j, row0, slot, nxt_row):
            h = ld16(h2_v, 0, TMB, 0, D)
            for f0 in range(0, F, FC):
                g = jnp.dot(h, w1_v[:, f0:f0 + FC], preferred_element_type=F32)
                u = jnp.dot(h, w3_v[:, f0:f0 + FC], preferred_element_type=F32)
                act_v[:, f0:f0 + FC] = pltpu.bitcast((g * jax.nn.sigmoid(g) * u).astype(BF16), U32)
            nk = F // KH
            sched = {}
            place(sched, post_items(nxt_row), range(0, NC * nk - PB1))
            begin(sched)

            def sink(n0, r):
                z = (mod(5, n0, n0 + 128)[None] * r.reshape(TMB // 8, 8, 128)).reshape(TMB, 128)
                obuf[slot, :, n0:n0 + 128] = (x1_rows(row0, TMB, n0, n0 + 128) + z).astype(BF16)
                if n0 + 128 in OCUT:
                    cp_out(j, slot, OCUT.index(n0 + 128) - 1).start()
            matmul(lambda k: ld16(act_v, 0, TMB, k * KH, (k + 1) * KH),
                   lambda k, n0: w2_v[k * KH:(k + 1) * KH, n0:n0 + 128],
                   tuple(range(nk)), range(0, D, 128), sink)

        U8 = NC

        def segment(*placements):
            sched = {}
            for items, units in placements:
                place(sched, items, units)
            begin(sched)

        with jax.named_scope("prologue"):
            zs[0] = 0
            begin({})
            start("c", "x0", "ca0", "q0", "sa0a", "sa0b", "k0", "v0", "x4", "ca1", "sa1", "q1", "k1", "v1", "wo",
                  "x1", "m2", "x2")
            wait("c")
            cb_v[...] = jnp.broadcast_to(silu_c().astype(F32), (128, D)).T
            wait("x0")
            for r in range(0, NS * TM, LG):
                xf = x_v[r:r + LG, :].astype(F32)
                mu = jnp.mean(xf, axis=-1, keepdims=True)
                d = xf - mu
                rs = jax.lax.rsqrt(jnp.mean(d * d, axis=-1, keepdims=True) + EPS)
                stats[0, r:r + LG, :] = jnp.broadcast_to(mu, (LG, 128))
                stats[1, r:r + LG, :] = jnp.broadcast_to(rs, (LG, 128))
            wait("ca0")
            mod_mxu(1, 0, D)
            wait("q0")
            run_now(perm_qkv_items(0, 0))
            wait("sa0a")
            mod_mxu(0, 0, SA_CUT)
            wait("sa0b")
            mod_mxu(0, SA_CUT, D)
            run_now(ln1_out_items(0, 0))

        with jax.named_scope("pass1"):
            segment((ln1_out_items(1, 0), range(0, U8 - 2)),
                    (ln1_out_items(2, 0) + ln1_out_items(3, 0), range(U8 - 2, 2 * U8)))
            qkv_part(None, 0, 0, 0)
            qkv_part(None, 0, 1, 0)
            wait("k0")
            segment((perm_qkv_items(1, 0), range(0, 2 * U8 - 2)))
            for g, b in ((0, 2), (0, 3), (1, 0), (1, 1)):
                qkv_part(None, g, b, 0)
            wait("v0", "x4", "ca1")
            segment((perm_qkv_items(2, 0), range(0, 2 * U8 - 2)),
                    (staged(ln1_start(NS, 0)[:2], TM // LG, 1), range(2 * U8 - 1, 4 * U8 - 2)),
                    (mod_items(D + KH, 4), range(2 * U8 - 2, 4 * U8)))
            for g, b in ((1, 2), (1, 3), (2, 0), (2, 1)):
                qkv_part(None, g, b, 0)
            wait("sa1", "q1")
            segment((mod_items(KH, 4), range(0, U8 + 2)),
                    (perm_qkv_items(0, 1), range(0, 2 * U8 - 2)),
                    (ln1_out_items(0, 1), range(U8 + 3, 2 * U8 - 1)))
            qkv_part(None, 2, 2, 0)
            qkv_part(None, 2, 3, 0)

        with jax.named_scope("pass2"):
            wait("k1")
            segment((perm_qkv_items(1, 1), range(0, 2 * U8 - 2)),
                    (ln1_out_items(1, 1), range(0, U8 - 2)),
                    (ln1_out_items(2, 1), range(U8 - 2, 2 * U8)))
            halo("b", None, 1)
            qkv_part("b", 0, 0, 1)
            qkv_part("c", 0, 1, 1)
            wait("v1")
            l0 = logit_items("b", True)
            segment((perm_qkv_items(2, 1), range(0, 2 * U8 - 2)),
                    (ln1_out_items(3, 1), range(0, U8)),
                    (l0[:LB], range(B0, B1)))
            qkv_part("b", 1, 0, 1)
            halo("c", "b", 1)
            qkv_part("c", 1, 1, 1)
            qkv_part("b", 2, 0, 1)
            halo("b", None, 2)
            halo("c", "b", 2)
            qkv_part("c", 2, 1, 1)
            wait("wo")
            segment((perm_wo_items(), range(0, WS)),
                    (l0[LB:], range(0, C0)),
                    (pv_items("b"), range(C0 + CP, 39)),
                    (logit_items("c", False), range(C0, C1)),
                    (pv_items("c"), range(C1 + CP, 63)),
                    (logit_items("a", False), range(C1, C2)),
                    (pv_items("a"), range(C2 + CP, 79)),
                    ([functools.partial(halo, "b", "a", 1)], [23]),
                    ([functools.partial(halo, "b", "a", 2)], [39]),
                    (ln1_out_items(NS, 0) + ln1_out_items(NS, 1), range(H0, H1)),
                    (logit_items("b", False), range(C2, 96 - L1)))
            halo("a", "c", 1)
            halo("a", "c", 2)
            for g in range(3):
                qkv_part("a", g, 2, 1)
            for g in range(3):
                qkv_part("b", g, 3, 1)
            wo_mm("b", 0)
            wo_mm("c", TM)
            wo_mm("a", 2 * TM)
            finish()
            wait("x1", "m2")
            start("m3", "w1", "w3", "w2")


        def half(X, Y, u0, sched, row_ln1, row_wo, extra):
            place(sched, pv_items(Y), range(u0 + P0, u0 + 3 * UP - P1))
            place(sched, logit_items(X, False), range(u0 + 2 * UP + L0, u0 + 4 * UP - L1))
            place(sched, ln1_items(row_ln1, Y), range(u0 + N0, u0 + N1))
            if extra:
                place(sched, extra, range(u0, u0 + 4 * UP - 1))

            def run():
                halo(X, Y, 1)
                halo(X, Y, 2)
                for g in range(3):
                    qkv_part(X, g)
                wo_mm(Y, row_wo)
            return run

        def a_step(s, carry):
            @pl.when(s == 3)
            def _():
                wait("x2", "m3")

            ra = pl.multiple_of(2 * s * TM, TM)
            nxt = pl.multiple_of(jnp.minimum(ra + 2 * TM, S - TM), TM)
            col0 = pl.multiple_of(jnp.minimum(2 * D + (s - 2) * (MT * 128), 6 * D - MT * 128), 128)
            mi = mod_items(col0, MT)
            sched = {}
            run_a = half("a", "b", 0, sched, ra + TM, ra - TM, mi[:len(mi) // 2])
            run_b = half("b", "a", 4 * UP, sched, nxt, ra, mi[len(mi) // 2:])
            begin(sched)
            run_a()
            run_b()
            finish()
            return carry

        with jax.named_scope("aloop"):
            if SKIP_A:
                wait("x2", "m3")
            else:
                jax.lax.fori_loop(NS // 2, NB // 2, a_step, 0)

        with jax.named_scope("atail"):
            begin({})
            def post0(r):
                x1 = x1_rows(r, LG, 0, D)
                mu = jnp.mean(x1, axis=-1, keepdims=True)
                d = x1 - mu
                rs = jax.lax.rsqrt(jnp.mean(d * d, axis=-1, keepdims=True) + EPS)
                y = (d * rs).reshape(LG // 8, 8, D) * mod(4, 0, D)[None] + mod(3, 0, D)[None]
                h2_v[r // 2:(r + LG) // 2, :] = pltpu.bitcast(y.reshape(LG, D).astype(BF16), U32)
            post = [functools.partial(post0, r) for r in range(0, TMB, LG)]
            pv = pv_items("b")
            if TSPLIT:
                run_now(pv[:NC])
                segment((pv[NC:], range(0, UP - 2)), (post, range(TP0, 2 * UP - TE)))
                wo_mm("b", S - TM, 0, TM // 2)
                wo_mm("b", S - TM, TM // 2, TM)
            else:
                run_now(pv)
                segment((post, range(0, UP - 2)))
                wo_mm("b", S - TM)
            finish()
            wait("w1", "w3", "w2")

        def b_step(j, carry):
            slot = j % 2

            @pl.when(j >= 2)
            def _():
                wait_out(j - 2, slot)

            row0 = pl.multiple_of(j * TMB, TMB)
            nxt = pl.multiple_of(jnp.minimum(row0 + TMB, S - TMB), TMB)
            if SKIP_FFN:
                obuf[slot] = x1_rows(row0, TMB, 0, D).astype(BF16)
                for q in range(NQ):
                    cp_out(j, slot, q).start()
            else:
                ffn(j, row0, slot, nxt)
            return carry

        with jax.named_scope("bloop"):
            jax.lax.fori_loop(0, NBB, b_step, 0)
        with jax.named_scope("tail"):
            wait_out(NBB - 2, (NBB - 2) % 2)
            wait_out(NBB - 1, (NBB - 1) % 2)

    any_spec = pl.BlockSpec(memory_space=pl.ANY)
    scratch = [
        pltpu.VMEM((S, D), BF16),
        pltpu.VMEM((D, 3 * D), BF16),
        pltpu.VMEM((NC, KH // 2, 128), U32),
        pltpu.VMEM((D // 2, 3 * D), U32),
        pltpu.VMEM((D, D), BF16),
        pltpu.VMEM((NC, D // 32 * 17, 128), U32),
        pltpu.VMEM((D // 2, D), U32),
        pltpu.VMEM((D, F), BF16),
        pltpu.VMEM((D, F), BF16),
        pltpu.VMEM((F, D), BF16),
        pltpu.VMEM((D, 6 * D), BF16),
        pltpu.VMEM((D, 128), F32),
        pltpu.VMEM((MT, NSUB, 8, 128), F32),
        pltpu.VMEM((8, 6 * D), F32),
        pltpu.VMEM((8, 2 * D), F32),
        pltpu.VMEM((TM // 2, D), U32),
        pltpu.VMEM((TM // 2, D), U32),
        pltpu.VMEM((NS, TM // 2, D), U32),
        pltpu.VMEM((NS, 3 * NC, TM, 128), F32),
        pltpu.VMEM((2, (NS + 1) * TM, 128), F32),
        pltpu.VMEM((2 * NC, KV + PADK, 128), F32),
        pltpu.VMEM((NC, KV + PADK, 128), F32),
        pltpu.VMEM((WIN + 1, TM, 128), F32),
        pltpu.VMEM((2 * NC, KV + PADK, 128), F32),
        pltpu.VMEM((NC, KV + PADK, 128), F32),
        pltpu.VMEM((WIN + 1, TM, 128), F32),
        pltpu.VMEM((2 * NC, KV + PADK, 128), F32),
        pltpu.VMEM((NC, KV + PADK, 128), F32),
        pltpu.VMEM((WIN + 1, TM, 128), F32),
        pltpu.VMEM((TM // 2, D), U32),
        pltpu.VMEM((TM // 2, D), U32),
        pltpu.VMEM((TM // 2, D), U32),
        pltpu.VMEM((NC, RG, 128), F32),
        pltpu.VMEM((NC, RG, 128), F32),
        pltpu.VMEM((NC, RG, 128), F32),
        pltpu.VMEM((WIN, RG, 128), F32),
        pltpu.VMEM((WIN, RG, 128), F32),
        pltpu.VMEM((WIN, RG, 128), F32),
        pltpu.VMEM((2, TM, 128), F32),
        pltpu.VMEM((2, TMB, 128), F32),
        pltpu.VMEM((S, D), F32),
        pltpu.VMEM((TMB, D), F32),
        pltpu.VMEM((TMB // 2, D), U32),
        pltpu.VMEM((TMB // 2, F), U32),
        pltpu.VMEM((2, TMB, D), BF16),
        pltpu.VMEM((1, D), BF16),
        pltpu.SMEM((1,), jnp.int32),
        pltpu.SemaphoreType.DMA((NDMA,)),
        pltpu.SemaphoreType.DMA((2 * NQ,)),
    ]

    def call(A_x, A_wqkv, A_wo, B_w1, B_w3, B_w2, c, w_mod):
        return pl.pallas_call(
            kernel,
            out_shape=jax.ShapeDtypeStruct((1, S, D), BF16),
            in_specs=[any_spec] * 8,
            out_specs=any_spec,
            scratch_shapes=scratch,
            compiler_params=pltpu.CompilerParams(
                vmem_limit_bytes=120 * 1024 * 1024,
                disable_semaphore_checks=True, disable_bounds_checks=True, **CPARAMS),
        )(A_x, A_wqkv, A_wo, B_w1, B_w3, B_w2, c, w_mod)

    return call


@jax.jit
def pallas_adaLN_cond__sliding_local_dilated__glu_gated_swiglu__prompt_kernel(
    A_x: jax.Array,
    A_wqkv: jax.Array,
    A_wo: jax.Array,
    B_x: jax.Array,
    B_w1: jax.Array,
    B_w3: jax.Array,
    B_w2: jax.Array,
    c: jax.Array,
    w_mod: jax.Array,
):
    del B_x
    return _build()(A_x, A_wqkv, A_wo, B_w1, B_w3, B_w2, c, w_mod)
```

```python
import functools
import math

import jax
import jax.numpy as jnp
import jax.experimental.pallas as pl
import jax.experimental.pallas.tpu as pltpu

S = 2048
D = 1024
F = 3584
H = 32
DH = D // H
WIN = 8
DIL = 2
NC = D // 128
HALO = 16
EPS = 1e-5
NEG = -1000000000.0
SM_SCALE = DH ** -0.5
LOG2E = math.log2(math.e)

TM = 128
NB = S // TM
KV = HALO + TM
RG = 8
LG = 16
NS = 4
NDMA = 22
KH = 512

F32 = jnp.float32
BF16 = jnp.bfloat16
U32 = jnp.uint32


def _tree(op, xs):
    xs = list(xs)
    while len(xs) > 1:
        xs = [op(xs[i], xs[i + 1]) if i + 1 < len(xs) else xs[i] for i in range(0, len(xs), 2)]
    return xs[0]


def _add(a, b):
    return a + b


def _fold(op, x):
    while x.shape[0] > 1:
        x = x.reshape(x.shape[0] // 2, 2, *x.shape[1:])
        x = op(x[:, 0], x[:, 1])
    return x[0]


def _lane_gather(x, idx):
    dn = jax.lax.GatherDimensionNumbers(
        offset_dims=(), collapsed_slice_dims=(1,), start_index_map=(1,),
        operand_batching_dims=(0,), start_indices_batching_dims=(0,))
    return jax.lax.gather(x, idx[..., None], dn, (1, 1), mode=jax.lax.GatherScatterMode.PROMISE_IN_BOUNDS)


def _build(TMB=256, FC=512, OCUT=(0, 512, 896, 1024), SA_CUT=768,
           MT=6, NSUB=16, MLAG=8, PR=32, SPREAD=128, LLAG=3,
           P0=1, P1=16, L0=0, L1=1, N0=0, N1=30, PB1=5,
           B0=14, B1=30, LB=19, C0=10, C1=38, C2=64, CP=1, WS=46, H0=0, H1=10,
           TP0=10, TE=3, SKIP_FFN=False):
    NBB = S // TMB
    NQ = len(OCUT) - 1

    def kernel(x_hbm, wqkv_hbm, wo_hbm, w1_hbm, w3_hbm, w2_hbm, c_hbm, wmod_hbm,
               out_hbm,
               x_v, wqkv_v, wtmp, wqkv_p, wo_v, wo_tmp, wo_p, w1_v, w3_v, w2_v,
               wmod_v, cb_v, modp_v, modb_v, mod_v,
               h1a, h1b, h1s, part, stats, qka, va, pa, qkb, vb, pb_, qkc, vc, pc,
               oa, ob, oc, ota, otb, otc, sl0, sl1, sl2, stat1, stat2,
               y_v, x1n, h2_v, act_v, obuf, c_ref, zs, sem_w, sem_o):
        bufs = {"a": (h1a, qka, va, oa, pa), "b": (h1b, qkb, vb, ob, pb_),
                "c": (None, qkc, vc, oc, pc)}

        sls = (sl0, sl1, sl2)
        otmps = {"a": ota, "b": otb, "c": otc}

        dmas = {}

        def add_dma(name, src, dst):
            dmas[name] = (src, dst, len(dmas))

        for name, (b0, b1) in (("x0", (0, NS)), ("x4", (NS, NS + 1)), ("x1", (NS + 1, NS + 3)), ("x2", (NS + 3, NB))):
            rows = pl.ds(b0 * TM, (b1 - b0) * TM)
            add_dma(name, x_hbm.at[0, rows, :], x_v.at[rows, :])
        for name, (r0, r1) in (("sa0a", (0, SA_CUT)), ("sa0b", (SA_CUT, D))):
            rows, cols = pl.ds(r0, r1 - r0), pl.ds(0, KH)
            add_dma(name, wmod_hbm.at[rows, cols], wmod_v.at[rows, cols])
        for name, (c0, c1) in (("sa1", (KH, D)), ("ca0", (D, D + KH)), ("ca1", (D + KH, 2 * D)),
                               ("m2", (2 * D, 3 * D)), ("m3", (3 * D, 6 * D))):
            cols = pl.ds(c0, c1 - c0)
            add_dma(name, wmod_hbm.at[:, cols], wmod_v.at[:, cols])
        for g in range(3):
            for k in range(2):
                rows, cols = pl.ds(k * KH, KH), pl.ds(g * D, D)
                add_dma("qkv"[g] + str(k), wqkv_hbm.at[rows, cols], wqkv_v.at[rows, cols])
        add_dma("c", c_hbm, c_ref)
        add_dma("wo", wo_hbm, wo_v)
        add_dma("w1", w1_hbm, w1_v)
        add_dma("w3", w3_hbm, w3_v)
        add_dma("w2", w2_hbm, w2_v)
        assert len(dmas) == NDMA

        def cp(name):
            src, dst, i = dmas[name]
            return pltpu.make_async_copy(src, dst, sem_w.at[i])

        def start(*names):
            for n in names:
                cp(n).start()

        def wait(*names):
            for n in names:
                cp(n).wait()

        def cp_out(j, slot, q):
            c0, c1 = OCUT[q], OCUT[q + 1]
            return pltpu.make_async_copy(obuf.at[slot, :, pl.ds(c0, c1 - c0)],
                                         out_hbm.at[0, pl.ds(j * TMB, TMB), pl.ds(c0, c1 - c0)],
                                         sem_o.at[slot * NQ + q])

        def wait_out(j, slot):
            for q in range(NQ):
                cp_out(j, slot, q).wait()

        st = {"z": None, "never": None, "clock": 0, "sched": {}, "tok": None}

        have = set()

        def need(*keys):
            assert all(k in have for k in keys), keys

        def begin(sched):
            z = zs[0]
            st.update(z=(0, z, 2 * z), never=jnp.full((8, 128), z, jnp.int32) != 0, clock=0, sched=sched, tok=None)

        def gate(val, i, n):
            r = st["tok"]
            if r is None:
                return val
            row = (i * min(SPREAD, r.shape[0]) // n) // 8 * 8
            t = r[row:row + 8]
            return jax.lax.select(st["never"], t if val.dtype == F32 else pltpu.bitcast(t, val.dtype), val)

        def place(sched, items, units):
            units = list(units)
            for i, it in enumerate(items):
                sched.setdefault(units[(i * len(units)) // len(items)], []).append(it)

        def matmul(lhs_fn, w_fn, ks, cols, sink, gives=None):
            for n0 in cols:
                r = None
                for k in ks:
                    d = jnp.dot(lhs_fn(k), w_fn(k, n0), preferred_element_type=F32)
                    r = d if r is None else r + d
                    if k == ks[-1]:
                        sink(n0, r)
                    if n0 == cols[-1] and k == ks[-1]:
                        have.add(gives)
                    st["tok"] = r
                    for fn in st["sched"].pop(st["clock"], []):
                        fn()
                    st["tok"] = None
                    st["clock"] += 1

        def finish():
            assert not st["sched"]

        def lane_iota(rows):
            return jax.lax.broadcasted_iota(jnp.int32, (rows, 128), 1)

        def ld16(ref, r0, n, c0, c1):
            return pltpu.bitcast(ref[r0 // 2:(r0 + n) // 2, c0:c1], BF16)

        def silu_c():
            cf = c_ref[...].astype(F32)
            return (cf * jax.nn.sigmoid(cf)).astype(BF16)

        def mod_mxu(j, r0, r1):
            cs = slice(j * D, j * D + KH)
            lhs = jnp.broadcast_to(silu_c()[:, r0:r1], (16, r1 - r0))
            r = jnp.dot(lhs, wmod_v[r0:r1, cs], preferred_element_type=F32)[0:8]
            mod_v[:, cs] = r + (mod_v[:, cs] if r0 else float(j == 1))

        def mod(j, c0, c1):
            return (mod_v if j < 2 else modb_v)[:, j * D + c0:j * D + c1]

        def mod_items(col0, ntiles):
            rows = D // NSUB

            def col(t):
                c0 = col0 + t * 128
                return c0 if isinstance(c0, int) else pl.multiple_of(c0, 128)

            def part_sum(t, i):
                w = wmod_v[i * rows:(i + 1) * rows, pl.ds(col(t), 128)].astype(F32)
                p = (w * cb_v[i * rows:(i + 1) * rows, :]).reshape(rows // 8, 8, 128)
                modp_v[t, i] = gate(_fold(_add, p), 1, 2)

            def total(t):
                r = gate(_fold(_add, modp_v[t, pl.ds(zrow(0), NSUB)]), 0, 1)
                one = jnp.where((col(t) // D) % 3 == 1, 1.0, 0.0).astype(F32)
                dst = mod_v if isinstance(col0, int) else modb_v
                dst[:, pl.ds(col(t), 128)] = jnp.broadcast_to(jnp.sum(r, axis=0, keepdims=True) + one, (8, 128))
            items = []
            for t in range(ntiles + 1):
                for i in range(NSUB):
                    if t < ntiles:
                        items.append(functools.partial(part_sum, t, i))
                    if t > 0 and i == (MLAG if t < ntiles else 0):
                        items.append(functools.partial(total, t - 1))
            return items

        def perm_mix(g, i, nrows):
            n = nrows // 2
            l = jnp.concatenate([gate(lane_iota(8), h, n) for h in range(0, n, 8)], axis=0)
            w = pltpu.bitcast(wqkv_v[i * nrows:(i + 1) * nrows, g * D:(g + 1) * D], U32)
            vals = [w[:, c * 128:(c + 1) * 128] for c in range(NC)]
            for b in range(3):
                m = (l & (4 << b)) == 0
                for c in range(NC):
                    if c & (1 << b):
                        continue
                    lo, hi = vals[c], vals[c | (1 << b)]
                    vals[c] = jax.lax.select(m, lo, hi)
                    vals[c | (1 << b)] = jax.lax.select(m, hi, lo)
            wtmp[:, pl.ds(pl.multiple_of(zrow((i * n) % (KH // 2)), 8), n), :] = jnp.stack(vals)

        def perm_gather(g, k, j):
            have.add(("w", g, k, j))
            l = lane_iota(8)
            idx = ((((l >> 1) & 3) << 5) | ((((l >> 3) & 7) ^ j) << 2) | ((l >> 6) << 1) | (l & 1))
            idx = jnp.concatenate([gate(idx, 0, 1)] * (KH // 16), axis=0)
            wqkv_p[k * KH // 2:(k + 1) * KH // 2, g * D + j * 128: g * D + (j + 1) * 128] = _lane_gather(wtmp[j], idx)

        def perm_qkv_items(g, k, nrows=PR):
            n = KH // nrows
            return ([functools.partial(perm_mix, g, i, nrows) for i in range(k * n, (k + 1) * n)]
                    + [functools.partial(perm_gather, g, k, j) for j in range(NC)])

        def perm_wo_items():
            sub = jax.lax.broadcasted_iota(jnp.int32, (8, 128), 0)

            def spread(c, h):
                for r in range(h * 256, h * 256 + 256, 8):
                    wo_tmp[c, pl.ds(zrow(r + r // 16), 8), :] = gate(pltpu.bitcast(
                        wo_v[2 * r:2 * r + 16, c * 128:(c + 1) * 128], U32), r % 256, 256)

            def gather(c, h):
                for G in range(h * 32, h * 32 + 32):
                    j, e, ch = G >> 3, (G >> 2) & 1, G & 3
                    dd = (((2 * ch) ^ j) << 1) | e
                    ta = wo_tmp[c, pl.ds(ch * 136 + dd, 8, stride=17), :]
                    tb = wo_tmp[c, pl.ds(ch * 136 + (dd ^ 2), 8, stride=17), :]
                    wo_p[G * 8:G * 8 + 8, c * 128:(c + 1) * 128] = jax.lax.select(gate(sub, G % 32, 32) < 4, ta, tb)
            return [functools.partial(fn, c, h) for fn in (spread, gather) for c in range(NC) for h in range(2)]

        def zrow(row, k=1):
            return row if k == 0 else row + st["z"][k]

        def gate16(v, i, n):
            return jnp.concatenate([gate(v[q:q + 8], i, n) for q in range(0, LG, 8)], axis=0)

        def staged(stages, n, lag):
            items = []
            for t in range(n + lag * (len(stages) - 1)):
                for k in reversed(range(len(stages))):
                    if 0 <= t - k * lag < n:
                        items.append(functools.partial(stages[k], t - k * lag))
            return items

        def ln_stages(load, stat, dst, j_scale, j_shift, cols=range(NC)):
            def chunks(x):
                return [x[:, c * 128:(c + 1) * 128] for c in range(NC)]

            def put(j, r, part, fn):
                m = jnp.sum(part, axis=-1, keepdims=True) * (1.0 / D)
                stat[j, pl.ds(pl.multiple_of(zrow(r), LG), LG), :] = jnp.broadcast_to(fn(m), (LG, 128))

            def s_mean(i):
                put(0, i * LG, gate16(_tree(_add, chunks(load(i * LG, 0))), 1, 2), lambda m: m)

            def s_var(i):
                r = i * LG
                d = load(r, 1) - jnp.concatenate([gate16(stat[0, r:r + LG, :], 0, 1)] * NC, axis=1)
                put(1, r, _tree(_add, chunks(d * d)), lambda m: jax.lax.rsqrt(m + EPS))

            def s_out(i):
                r = i * LG
                x = load(r, 2)
                mu = jnp.concatenate([stat[0, r:r + LG, :]] * (NC // 2), axis=1)
                for c0 in range(cols[0] * 128, cols[-1] * 128, KH):
                    rs = jnp.concatenate([gate16(stat[1, r:r + LG, :], c0 - cols[0] * 128, D)] * (NC // 2), axis=1)
                    y = ((x[:, c0:c0 + KH] - mu) * rs).reshape(LG // 8, 8, KH)
                    y = y * mod(j_scale, c0, c0 + KH)[None] + mod(j_shift, c0, c0 + KH)[None]
                    dst[r // 2:(r + LG) // 2, c0:c0 + KH] = pltpu.bitcast(y.reshape(LG, KH).astype(BF16), U32)
            return s_mean, s_var, s_out

        def load_x(row0):
            return lambda r, k: x_v[pl.ds(pl.multiple_of(zrow(row0 + r, k), LG), LG), :].astype(F32)

        def ln1_items(row0, buf):
            return staged(ln_stages(load_x(row0), stat1, bufs[buf][0], 1, 0), TM // LG, 1)

        def ln1_start(b, k):
            return ln_stages(load_x(b * TM), stats.at[:, pl.ds(b * TM, TM), :], h1s.at[b] if b < NS else h1a,
                             1, 0, range(k * NC // 2, (k + 1) * NC // 2))

        def ln1_out_items(b, k):
            def one(i):
                have.add(("h", b, k, i))
                ln1_start(b, k)[2](i)
            return [functools.partial(one, i) for i in range(TM // LG)]

        def x1_rows(row, n, c0, c1):
            xf = x_v[pl.ds(row, n), c0:c1].astype(F32).reshape(n // 8, 8, c1 - c0)
            y = y_v[pl.ds(row, n), c0:c1].reshape(n // 8, 8, c1 - c0)
            ga = jnp.concatenate([gate(mod(2, c, c + 128), c - c0, 2 * D) for c in range(c0, c1, 128)], axis=1)
            return (xf + ga[None] * y).reshape(n, c1 - c0)

        def post_items(row0):
            def load(r, k):
                if k:
                    return x1n[pl.ds(pl.multiple_of(zrow(r, k), LG), LG), :]
                x1 = x1_rows(row0 + r, LG, 0, D)
                x1n[r:r + LG, :] = x1
                return x1
            return staged(ln_stages(load, stat2, h2_v, 4, 3), TMB // LG, 1)

        def logit_items(buf, first):
            _, qk, _, _, pb = bufs[buf]
            swap = lane_iota(RG) ^ 1

            def s_logit(g):
                need(("q", buf), ("k", buf))
                have.add(("l", buf, g))
                r = g * RG
                q = qk[0:NC, HALO + r:HALO + r + RG, :]
                dst = pl.ds(pl.multiple_of(zrow(0), RG), RG)
                for w in range(WIN):
                    k0 = zrow(HALO + r - DIL * w, int(w >= WIN // 2))
                    s = gate(_fold(_add, q * qk[NC:2 * NC, pl.ds(k0, RG), :]), w, WIN)
                    s = s + pltpu.roll(s, 64, 1)
                    s = s + _lane_gather(s, swap)
                    if first and r < DIL * w:
                        pos = r + jax.lax.broadcasted_iota(jnp.int32, (RG, 128), 0)
                        s = jnp.where(pos >= DIL * w, s, NEG * LOG2E)
                    sls[g % len(sls)][w, dst, :] = s

            def s_soft(g):
                assert ("p", buf, g) not in have
                have.add(("p", buf, g))
                r = g * RG
                s = sls[g % len(sls)][...]
                e = jnp.exp2(s - gate(_fold(jnp.maximum, s), 0, 1)[None])
                pb[0:WIN, r:r + RG, :] = e
                den = _fold(_add, e)
                inv = pl.reciprocal(den, approx=True)
                pb[WIN, r:r + RG, :] = inv * (2.0 - den * inv)
            return staged((s_logit, s_soft), TM // RG, LLAG)

        def pv_items(buf):
            _, _, vp, o, pb = bufs[buf]
            otmp = otmps[buf]

            def one(r):
                need(("v", buf), ("p", buf, r // RG))
                have.remove(("p", buf, r // RG))
                have.add(("o", buf, r // RG))
                p = pb[:, pl.ds(pl.multiple_of(zrow(r), RG), RG), :]
                acc = _tree(_add, [p[w:w + 1] * vp[:, pl.ds(zrow(HALO + r - DIL * w, int(w >= WIN // 2)), RG), :]
                                   for w in range(WIN)]) * p[WIN:]
                acc = [gate(acc[c], c, NC) for c in range(NC)]
                if (r // RG) % 2 == 0:
                    otmp[:, pl.ds(pl.multiple_of(zrow(0), 8), RG), :] = jnp.stack(acc)
                else:
                    prev = otmp[...]
                    both = jnp.concatenate([jnp.concatenate([prev[c] for c in range(NC)], axis=1),
                                            jnp.concatenate(acc, axis=1)], axis=0)
                    o[(r - RG) // 2:(r + RG) // 2, :] = pltpu.bitcast(both.astype(BF16), U32)
            return [functools.partial(one, r) for r in range(0, TM, RG)]

        def halo(buf, prev, part):
            c0 = NC if part == 1 else 0
            ref = bufs[buf][part]
            if prev is None:
                val = (jnp.zeros((NC, HALO, 128), F32) if part == 1
                       else jnp.broadcast_to(ref[:, HALO:HALO + 1, :], (NC, HALO, 128)))
            else:
                val = bufs[prev][part][c0:c0 + NC, TM:TM + HALO, :]
                if st["tok"] is not None:
                    val = jnp.stack([gate16(val[c], 1, 2) for c in range(NC)])
            ref[c0:c0 + NC, 0:HALO, :] = val

        def qkv_part(buf, g, sb=None, k=None):
            h1, qk, vp, _, _ = bufs[buf] if buf else (None,) * 5
            if sb is not None:
                h1 = h1s.at[sb]
                need(*[("h", sb, k, i) for i in range(TM // LG)], *[("w", g, k, j) for j in range(NC)])
            if k != 0:
                for i in range(TM // RG):
                    if g < 2 and ("qk"[g], buf) in have:
                        need(("l", buf, i))
                    if g == 2 and ("v", buf) in have:
                        assert ("p", buf, i) not in have or ("new", buf) in have
                if g == 1:
                    have.difference_update({("l", buf, i) for i in range(TM // RG)})
                    have.add(("new", buf))
                have.discard(("qkv"[g], buf))

            def sink(n0, r):
                ch = n0 // 128
                if k == 0:
                    part[sb, ch] = r
                    return
                if k == 1:
                    r = r + part[sb, ch]
                dst, ci = (qk, ch) if ch < 2 * NC else (vp, ch - 2 * NC)
                dst[ci, HALO:HALO + TM, :] = r * (SM_SCALE * LOG2E) if ch < NC else r
            matmul(lambda kk: ld16(h1, 0, TM, kk * KH, (kk + 1) * KH),
                   lambda kk, n0: ld16(wqkv_p, kk * KH, KH, n0, n0 + 128),
                   (0, 1) if k is None else (k,), range(g * D, (g + 1) * D, 128), sink,
                   None if k == 0 else ("qkv"[g], buf))
            if g == 2:
                have.discard(("new", buf))

        def wo_mm(buf, row0, m0=0, m1=TM):
            o = bufs[buf][3]
            need(*[("o", buf, i) for i in range(m0 // RG, m1 // RG)])
            have.difference_update({("o", buf, i) for i in range(m0 // RG, m1 // RG)})

            def sink(n0, r):
                y_v[pl.ds(row0 + m0, m1 - m0), n0:n0 + 128] = r
            matmul(lambda k: ld16(o, m0, m1 - m0, k * KH, (k + 1) * KH),
                   lambda k, n0: ld16(wo_p, k * KH, KH, n0, n0 + 128),
                   (0, 1), range(0, D, 128), sink)

        UP = NC * (D // KH)

        def run_now(items):
            for fn in items:
                fn()

        def ffn(j, row0, slot, nxt_row):
            h = ld16(h2_v, 0, TMB, 0, D)
            for f0 in range(0, F, FC):
                g = jnp.dot(h, w1_v[:, f0:f0 + FC], preferred_element_type=F32)
                u = jnp.dot(h, w3_v[:, f0:f0 + FC], preferred_element_type=F32)
                act_v[:, f0:f0 + FC] = pltpu.bitcast((g * jax.nn.sigmoid(g) * u).astype(BF16), U32)
            nk = F // KH
            sched = {}
            place(sched, post_items(nxt_row), range(0, NC * nk - PB1))
            begin(sched)

            def sink(n0, r):
                z = (mod(5, n0, n0 + 128)[None] * r.reshape(TMB // 8, 8, 128)).reshape(TMB, 128)
                obuf[slot, :, n0:n0 + 128] = (x1_rows(row0, TMB, n0, n0 + 128) + z).astype(BF16)
                if n0 + 128 in OCUT:
                    cp_out(j, slot, OCUT.index(n0 + 128) - 1).start()
            matmul(lambda k: ld16(act_v, 0, TMB, k * KH, (k + 1) * KH),
                   lambda k, n0: w2_v[k * KH:(k + 1) * KH, n0:n0 + 128],
                   tuple(range(nk)), range(0, D, 128), sink)

        U8 = NC

        def segment(*placements):
            sched = {}
            for items, units in placements:
                place(sched, items, units)
            begin(sched)

        with jax.named_scope("prologue"):
            zs[0] = 0
            begin({})
            start("c", "x0", "ca0", "q0", "sa0a", "sa0b", "k0", "v0", "x4", "ca1", "sa1", "q1", "k1", "v1", "wo",
                  "x1", "m2", "x2")
            wait("c")
            cb_v[...] = jnp.broadcast_to(silu_c().astype(F32), (128, D)).T
            wait("x0")
            for r in range(0, NS * TM, LG):
                xf = x_v[r:r + LG, :].astype(F32)
                mu = jnp.mean(xf, axis=-1, keepdims=True)
                d = xf - mu
                rs = jax.lax.rsqrt(jnp.mean(d * d, axis=-1, keepdims=True) + EPS)
                stats[0, r:r + LG, :] = jnp.broadcast_to(mu, (LG, 128))
                stats[1, r:r + LG, :] = jnp.broadcast_to(rs, (LG, 128))
            wait("ca0")
            mod_mxu(1, 0, D)
            wait("q0")
            run_now(perm_qkv_items(0, 0))
            wait("sa0a")
            mod_mxu(0, 0, SA_CUT)
            wait("sa0b")
            mod_mxu(0, SA_CUT, D)
            run_now(ln1_out_items(0, 0))

        with jax.named_scope("pass1"):
            segment((ln1_out_items(1, 0), range(0, U8 - 2)),
                    (ln1_out_items(2, 0) + ln1_out_items(3, 0), range(U8 - 2, 2 * U8)))
            qkv_part(None, 0, 0, 0)
            qkv_part(None, 0, 1, 0)
            wait("k0")
            segment((perm_qkv_items(1, 0), range(0, 2 * U8 - 2)))
            for g, b in ((0, 2), (0, 3), (1, 0), (1, 1)):
                qkv_part(None, g, b, 0)
            wait("v0", "x4", "ca1")
            segment((perm_qkv_items(2, 0), range(0, 2 * U8 - 2)),
                    (staged(ln1_start(NS, 0)[:2], TM // LG, 1), range(2 * U8 - 1, 4 * U8 - 2)),
                    (mod_items(D + KH, 4), range(2 * U8 - 2, 4 * U8)))
            for g, b in ((1, 2), (1, 3), (2, 0), (2, 1)):
                qkv_part(None, g, b, 0)
            wait("sa1", "q1")
            segment((mod_items(KH, 4), range(0, U8 + 2)),
                    (perm_qkv_items(0, 1), range(0, 2 * U8 - 2)),
                    (ln1_out_items(0, 1), range(U8 + 3, 2 * U8 - 1)))
            qkv_part(None, 2, 2, 0)
            qkv_part(None, 2, 3, 0)

        with jax.named_scope("pass2"):
            wait("k1")
            segment((perm_qkv_items(1, 1), range(0, 2 * U8 - 2)),
                    (ln1_out_items(1, 1), range(0, U8 - 2)),
                    (ln1_out_items(2, 1), range(U8 - 2, 2 * U8)))
            halo("b", None, 1)
            qkv_part("b", 0, 0, 1)
            qkv_part("c", 0, 1, 1)
            wait("v1")
            l0 = logit_items("b", True)
            segment((perm_qkv_items(2, 1), range(0, 2 * U8 - 2)),
                    (ln1_out_items(3, 1), range(0, U8)),
                    (l0[:LB], range(B0, B1)))
            qkv_part("b", 1, 0, 1)
            halo("c", "b", 1)
            qkv_part("c", 1, 1, 1)
            qkv_part("b", 2, 0, 1)
            halo("b", None, 2)
            halo("c", "b", 2)
            qkv_part("c", 2, 1, 1)
            wait("wo")
            segment((perm_wo_items(), range(0, WS)),
                    (l0[LB:], range(0, C0)),
                    (pv_items("b"), range(C0 + CP, 39)),
                    (logit_items("c", False), range(C0, C1)),
                    (pv_items("c"), range(C1 + CP, 63)),
                    (logit_items("a", False), range(C1, C2)),
                    (pv_items("a"), range(C2 + CP, 79)),
                    ([functools.partial(halo, "b", "a", 1)], [23]),
                    ([functools.partial(halo, "b", "a", 2)], [39]),
                    (ln1_out_items(NS, 0) + ln1_out_items(NS, 1), range(H0, H1)),
                    (logit_items("b", False), range(C2, 96 - L1)))
            halo("a", "c", 1)
            halo("a", "c", 2)
            for g in range(3):
                qkv_part("a", g, 2, 1)
            for g in range(3):
                qkv_part("b", g, 3, 1)
            wo_mm("b", 0)
            wo_mm("c", TM)
            wo_mm("a", 2 * TM)
            finish()
            wait("x1", "m2")
            start("m3", "w1", "w3", "w2")


        def half(X, Y, u0, sched, row_ln1, row_wo, extra):
            place(sched, pv_items(Y), range(u0 + P0, u0 + 3 * UP - P1))
            place(sched, logit_items(X, False), range(u0 + 2 * UP + L0, u0 + 4 * UP - L1))
            place(sched, ln1_items(row_ln1, Y), range(u0 + N0, u0 + N1))
            place(sched, extra, range(u0, u0 + 4 * UP - 1))

            def run():
                halo(X, Y, 1)
                halo(X, Y, 2)
                for g in range(3):
                    qkv_part(X, g)
                wo_mm(Y, row_wo)
            return run

        def a_step(s, carry):
            @pl.when(s == 3)
            def _():
                wait("x2", "m3")

            ra = pl.multiple_of(2 * s * TM, TM)
            nxt = pl.multiple_of(jnp.minimum(ra + 2 * TM, S - TM), TM)
            col0 = pl.multiple_of(jnp.minimum(2 * D + (s - 2) * (MT * 128), 6 * D - MT * 128), 128)
            mi = mod_items(col0, MT)
            sched = {}
            run_a = half("a", "b", 0, sched, ra + TM, ra - TM, mi[:len(mi) // 2])
            run_b = half("b", "a", 4 * UP, sched, nxt, ra, mi[len(mi) // 2:])
            begin(sched)
            run_a()
            run_b()
            finish()
            return carry

        with jax.named_scope("aloop"):
            jax.lax.fori_loop(NS // 2, NB // 2, a_step, 0)

        with jax.named_scope("atail"):
            begin({})

            def post0(r):
                x1 = x1_rows(r, LG, 0, D)
                mu = jnp.mean(x1, axis=-1, keepdims=True)
                d = x1 - mu
                rs = jax.lax.rsqrt(jnp.mean(d * d, axis=-1, keepdims=True) + EPS)
                y = (d * rs).reshape(LG // 8, 8, D) * mod(4, 0, D)[None] + mod(3, 0, D)[None]
                h2_v[r // 2:(r + LG) // 2, :] = pltpu.bitcast(y.reshape(LG, D).astype(BF16), U32)
            post = [functools.partial(post0, r) for r in range(0, TMB, LG)]
            pv = pv_items("b")
            run_now(pv[:NC])
            segment((pv[NC:], range(0, UP - 2)), (post, range(TP0, 2 * UP - TE)))
            wo_mm("b", S - TM, 0, TM // 2)
            wo_mm("b", S - TM, TM // 2, TM)
            finish()
            wait("w1", "w3", "w2")

        def b_step(j, carry):
            slot = j % 2

            @pl.when(j >= 2)
            def _():
                wait_out(j - 2, slot)

            row0 = pl.multiple_of(j * TMB, TMB)
            nxt = pl.multiple_of(jnp.minimum(row0 + TMB, S - TMB), TMB)
            if SKIP_FFN:
                obuf[slot] = x1_rows(row0, TMB, 0, D).astype(BF16)
                for q in range(NQ):
                    cp_out(j, slot, q).start()
            else:
                ffn(j, row0, slot, nxt)
            return carry

        with jax.named_scope("bloop"):
            jax.lax.fori_loop(0, NBB, b_step, 0)
        with jax.named_scope("tail"):
            wait_out(NBB - 2, (NBB - 2) % 2)
            wait_out(NBB - 1, (NBB - 1) % 2)

    any_spec = pl.BlockSpec(memory_space=pl.ANY)
    qkv_set = [
        pltpu.VMEM((2 * NC, KV, 128), F32),
        pltpu.VMEM((NC, KV, 128), F32),
        pltpu.VMEM((WIN + 1, TM, 128), F32),
    ]
    scratch = [
        pltpu.VMEM((S, D), BF16),
        pltpu.VMEM((D, 3 * D), BF16),
        pltpu.VMEM((NC, KH // 2, 128), U32),
        pltpu.VMEM((D // 2, 3 * D), U32),
        pltpu.VMEM((D, D), BF16),
        pltpu.VMEM((NC, D // 32 * 17, 128), U32),
        pltpu.VMEM((D // 2, D), U32),
        pltpu.VMEM((D, F), BF16),
        pltpu.VMEM((D, F), BF16),
        pltpu.VMEM((F, D), BF16),
        pltpu.VMEM((D, 6 * D), BF16),
        pltpu.VMEM((D, 128), F32),
        pltpu.VMEM((MT, NSUB, 8, 128), F32),
        pltpu.VMEM((8, 6 * D), F32),
        pltpu.VMEM((8, 2 * D), F32),
        pltpu.VMEM((TM // 2, D), U32),
        pltpu.VMEM((TM // 2, D), U32),
        pltpu.VMEM((NS, TM // 2, D), U32),
        pltpu.VMEM((NS, 3 * NC, TM, 128), F32),
        pltpu.VMEM((2, (NS + 1) * TM, 128), F32),
        *qkv_set, *qkv_set, *qkv_set,
        *[pltpu.VMEM((TM // 2, D), U32)] * 3,
        *[pltpu.VMEM((NC, RG, 128), F32)] * 3,
        *[pltpu.VMEM((WIN, RG, 128), F32)] * 3,
        pltpu.VMEM((2, TM, 128), F32),
        pltpu.VMEM((2, TMB, 128), F32),
        pltpu.VMEM((S, D), F32),
        pltpu.VMEM((TMB, D), F32),
        pltpu.VMEM((TMB // 2, D), U32),
        pltpu.VMEM((TMB // 2, F), U32),
        pltpu.VMEM((2, TMB, D), BF16),
        pltpu.VMEM((1, D), BF16),
        pltpu.SMEM((1,), jnp.int32),
        pltpu.SemaphoreType.DMA((NDMA,)),
        pltpu.SemaphoreType.DMA((2 * NQ,)),
    ]

    def call(A_x, A_wqkv, A_wo, B_w1, B_w3, B_w2, c, w_mod):
        return pl.pallas_call(
            kernel,
            out_shape=jax.ShapeDtypeStruct((1, S, D), BF16),
            in_specs=[any_spec] * 8,
            out_specs=any_spec,
            scratch_shapes=scratch,
            compiler_params=pltpu.CompilerParams(
                vmem_limit_bytes=120 * 1024 * 1024,
                disable_semaphore_checks=True, disable_bounds_checks=True),
        )(A_x, A_wqkv, A_wo, B_w1, B_w3, B_w2, c, w_mod)

    return call


@jax.jit
def pallas_adaLN_cond__sliding_local_dilated__glu_gated_swiglu__prompt_kernel(
    A_x: jax.Array,
    A_wqkv: jax.Array,
    A_wo: jax.Array,
    B_x: jax.Array,
    B_w1: jax.Array,
    B_w3: jax.Array,
    B_w2: jax.Array,
    c: jax.Array,
    w_mod: jax.Array,
):
    del B_x
    return _build()(A_x, A_wqkv, A_wo, B_w1, B_w3, B_w2, c, w_mod)
```

```python
import functools
import math

import jax
import jax.numpy as jnp
import jax.experimental.pallas as pl
import jax.experimental.pallas.tpu as pltpu

S = 2048
D = 1024
F = 3584
H = 32
DH = D // H
WIN = 8
DIL = 2
NC = D // 128
HALO = 16
EPS = 1e-5
NEG = -1000000000.0
SM_SCALE = DH ** -0.5
LOG2E = math.log2(math.e)

TM = 128
NB = S // TM
KV = HALO + TM
RG = 8
LG = 16
NS = 4
NDMA = 23
KH = 512

F32 = jnp.float32
BF16 = jnp.bfloat16
U32 = jnp.uint32


def _tree(op, xs):
    xs = list(xs)
    while len(xs) > 1:
        xs = [op(xs[i], xs[i + 1]) if i + 1 < len(xs) else xs[i] for i in range(0, len(xs), 2)]
    return xs[0]


def _add(a, b):
    return a + b


def _fold(op, x):
    while x.shape[0] > 1:
        x = x.reshape(x.shape[0] // 2, 2, *x.shape[1:])
        x = op(x[:, 0], x[:, 1])
    return x[0]


def _lane_gather(x, idx):
    dn = jax.lax.GatherDimensionNumbers(
        offset_dims=(), collapsed_slice_dims=(1,), start_index_map=(1,),
        operand_batching_dims=(0,), start_indices_batching_dims=(0,))
    return jax.lax.gather(x, idx[..., None], dn, (1, 1), mode=jax.lax.GatherScatterMode.PROMISE_IN_BOUNDS)


def _build(TMB=256, FC=512, OCUT=(0, 512, 896, 1024), SA_CUT=768,
           MT=6, NSUB=16, MLAG=8, PR=32, SPREAD=128, LLAG=3,
           P0=1, P1=16, L0=0, L1=1, N0=0, N1=30, PB1=5,
           B0=14, B1=30, LB=19, C0=10, C1=38, C2=64, CP=1, WS=46, H0=0, H1=10,
           TP0=10, TE=3, X0=4, X1=4, X2=7, X3=0, X4=6, SKIP_FFN=False):
    NBB = S // TMB
    NQ = len(OCUT) - 1

    def kernel(x_hbm, wqkv_hbm, wo_hbm, w1_hbm, w3_hbm, w2_hbm, c_hbm, wmod_hbm,
               out_hbm,
               x_v, wqkv_v, wtmp, wqkv_p, wo_v, wo_tmp, wo_p, w1_v, w3_v, w2_v,
               wmod_v, cb_v, modp_v, modb_v, mod_v,
               h1a, h1b, h1s, part, stats, qka, va, pa, qkb, vb, pb_, qkc, vc, pc,
               oa, ob, oc, ota, otb, otc, sl0, sl1, sl2, stat1, stat2,
               y_v, x1n, h2_v, act_v, obuf, c_ref, zs, sem_w, sem_o):
        bufs = {"a": (h1a, qka, va, oa, pa), "b": (h1b, qkb, vb, ob, pb_),
                "c": (None, qkc, vc, oc, pc)}

        sls = (sl0, sl1, sl2)
        otmps = {"a": ota, "b": otb, "c": otc}

        dmas = {}

        def add_dma(name, src, dst):
            dmas[name] = (src, dst, len(dmas))

        for name, (b0, b1) in (("x0", (0, 2)), ("x23", (2, NS)), ("x4", (NS, NS + 1)), ("x1", (NS + 1, NS + 3)), ("x2", (NS + 3, NB))):
            rows = pl.ds(b0 * TM, (b1 - b0) * TM)
            add_dma(name, x_hbm.at[0, rows, :], x_v.at[rows, :])
        for name, (r0, r1) in (("sa0a", (0, SA_CUT)), ("sa0b", (SA_CUT, D))):
            rows, cols = pl.ds(r0, r1 - r0), pl.ds(0, KH)
            add_dma(name, wmod_hbm.at[rows, cols], wmod_v.at[rows, cols])
        for name, (c0, c1) in (("sa1", (KH, D)), ("ca0", (D, D + KH)), ("ca1", (D + KH, 2 * D)),
                               ("m2", (2 * D, 3 * D)), ("m3", (3 * D, 6 * D))):
            cols = pl.ds(c0, c1 - c0)
            add_dma(name, wmod_hbm.at[:, cols], wmod_v.at[:, cols])
        for g in range(3):
            for k in range(2):
                rows, cols = pl.ds(k * KH, KH), pl.ds(g * D, D)
                add_dma("qkv"[g] + str(k), wqkv_hbm.at[rows, cols], wqkv_v.at[rows, cols])
        add_dma("c", c_hbm, c_ref)
        add_dma("wo", wo_hbm, wo_v)
        add_dma("w1", w1_hbm, w1_v)
        add_dma("w3", w3_hbm, w3_v)
        add_dma("w2", w2_hbm, w2_v)
        assert len(dmas) == NDMA

        def cp(name):
            src, dst, i = dmas[name]
            return pltpu.make_async_copy(src, dst, sem_w.at[i])

        def start(*names):
            for n in names:
                cp(n).start()

        def wait(*names):
            for n in names:
                cp(n).wait()

        def cp_out(j, slot, q):
            c0, c1 = OCUT[q], OCUT[q + 1]
            return pltpu.make_async_copy(obuf.at[slot, :, pl.ds(c0, c1 - c0)],
                                         out_hbm.at[0, pl.ds(j * TMB, TMB), pl.ds(c0, c1 - c0)],
                                         sem_o.at[slot * NQ + q])

        def wait_out(j, slot):
            for q in range(NQ):
                cp_out(j, slot, q).wait()

        st = {"z": None, "never": None, "clock": 0, "sched": {}, "tok": None}

        have = set()

        def need(*keys):
            assert all(k in have for k in keys), keys

        def begin(sched):
            z = zs[0]
            st.update(z=(0, z, 2 * z), never=jnp.full((8, 128), z, jnp.int32) != 0, clock=0, sched=sched, tok=None)

        def gate(val, i, n):
            r = st["tok"]
            if r is None:
                return val
            row = (i * min(SPREAD, r.shape[0]) // n) // 8 * 8
            t = r[row:row + 8]
            return jax.lax.select(st["never"], t if val.dtype == F32 else pltpu.bitcast(t, val.dtype), val)

        def place(sched, items, units):
            units = list(units)
            for i, it in enumerate(items):
                sched.setdefault(units[(i * len(units)) // len(items)], []).append(it)

        def matmul(lhs_fn, w_fn, ks, cols, sink, gives=None):
            for n0 in cols:
                r = None
                for k in ks:
                    d = jnp.dot(lhs_fn(k), w_fn(k, n0), preferred_element_type=F32)
                    r = d if r is None else r + d
                    if k == ks[-1]:
                        sink(n0, r)
                    if n0 == cols[-1] and k == ks[-1]:
                        have.add(gives)
                    st["tok"] = r
                    for fn in st["sched"].pop(st["clock"], []):
                        fn()
                    st["tok"] = None
                    st["clock"] += 1

        def finish():
            assert not st["sched"]

        def lane_iota(rows):
            return jax.lax.broadcasted_iota(jnp.int32, (rows, 128), 1)

        def ld16(ref, r0, n, c0, c1):
            return pltpu.bitcast(ref[r0 // 2:(r0 + n) // 2, c0:c1], BF16)

        def silu_c():
            cf = c_ref[...].astype(F32)
            return (cf * jax.nn.sigmoid(cf)).astype(BF16)

        def mod_mxu(j, r0, r1):
            cs = slice(j * D, j * D + KH)
            lhs = jnp.broadcast_to(silu_c()[:, r0:r1], (16, r1 - r0))
            r = jnp.dot(lhs, wmod_v[r0:r1, cs], preferred_element_type=F32)[0:8]
            mod_v[:, cs] = r + (mod_v[:, cs] if r0 else float(j == 1))

        def mod(j, c0, c1):
            return (mod_v if j < 2 else modb_v)[:, j * D + c0:j * D + c1]

        def mod_items(col0, ntiles):
            rows = D // NSUB

            def col(t):
                c0 = col0 + t * 128
                return c0 if isinstance(c0, int) else pl.multiple_of(c0, 128)

            def part_sum(t, i):
                w = wmod_v[i * rows:(i + 1) * rows, pl.ds(col(t), 128)].astype(F32)
                p = (w * cb_v[i * rows:(i + 1) * rows, :]).reshape(rows // 8, 8, 128)
                modp_v[t, i] = gate(_fold(_add, p), 1, 2)

            def total(t):
                r = gate(_fold(_add, modp_v[t, pl.ds(zrow(0), NSUB)]), 0, 1)
                one = jnp.where((col(t) // D) % 3 == 1, 1.0, 0.0).astype(F32)
                dst = mod_v if isinstance(col0, int) else modb_v
                dst[:, pl.ds(col(t), 128)] = jnp.broadcast_to(jnp.sum(r, axis=0, keepdims=True) + one, (8, 128))
            items = []
            for t in range(ntiles + 1):
                for i in range(NSUB):
                    if t < ntiles:
                        items.append(functools.partial(part_sum, t, i))
                    if t > 0 and i == (MLAG if t < ntiles else 0):
                        items.append(functools.partial(total, t - 1))
            return items

        def perm_mix(g, i, nrows):
            n = nrows // 2
            l = jnp.concatenate([gate(lane_iota(8), h, n) for h in range(0, n, 8)], axis=0)
            w = pltpu.bitcast(wqkv_v[i * nrows:(i + 1) * nrows, g * D:(g + 1) * D], U32)
            vals = [w[:, c * 128:(c + 1) * 128] for c in range(NC)]
            for b in range(3):
                m = (l & (4 << b)) == 0
                for c in range(NC):
                    if c & (1 << b):
                        continue
                    lo, hi = vals[c], vals[c | (1 << b)]
                    vals[c] = jax.lax.select(m, lo, hi)
                    vals[c | (1 << b)] = jax.lax.select(m, hi, lo)
            wtmp[:, pl.ds(pl.multiple_of(zrow((i * n) % (KH // 2)), 8), n), :] = jnp.stack(vals)

        def perm_gather(g, k, j):
            have.add(("w", g, k, j))
            l = lane_iota(8)
            idx = ((((l >> 1) & 3) << 5) | ((((l >> 3) & 7) ^ j) << 2) | ((l >> 6) << 1) | (l & 1))
            idx = jnp.concatenate([gate(idx, 0, 1)] * (KH // 16), axis=0)
            wqkv_p[k * KH // 2:(k + 1) * KH // 2, g * D + j * 128: g * D + (j + 1) * 128] = _lane_gather(wtmp[j], idx)

        def perm_qkv_items(g, k, nrows=PR):
            n = KH // nrows
            return ([functools.partial(perm_mix, g, i, nrows) for i in range(k * n, (k + 1) * n)]
                    + [functools.partial(perm_gather, g, k, j) for j in range(NC)])

        def perm_wo_items():
            sub = jax.lax.broadcasted_iota(jnp.int32, (8, 128), 0)

            def spread(c, h):
                for r in range(h * 256, h * 256 + 256, 8):
                    wo_tmp[c, pl.ds(zrow(r + r // 16), 8), :] = gate(pltpu.bitcast(
                        wo_v[2 * r:2 * r + 16, c * 128:(c + 1) * 128], U32), r % 256, 256)

            def gather(c, h):
                for G in range(h * 32, h * 32 + 32):
                    j, e, ch = G >> 3, (G >> 2) & 1, G & 3
                    dd = (((2 * ch) ^ j) << 1) | e
                    ta = wo_tmp[c, pl.ds(ch * 136 + dd, 8, stride=17), :]
                    tb = wo_tmp[c, pl.ds(ch * 136 + (dd ^ 2), 8, stride=17), :]
                    wo_p[G * 8:G * 8 + 8, c * 128:(c + 1) * 128] = jax.lax.select(gate(sub, G % 32, 32) < 4, ta, tb)
            return [functools.partial(fn, c, h) for fn in (spread, gather) for c in range(NC) for h in range(2)]

        def zrow(row, k=1):
            return row if k == 0 else row + st["z"][k]

        def gate16(v, i, n):
            return jnp.concatenate([gate(v[q:q + 8], i, n) for q in range(0, LG, 8)], axis=0)

        def staged(stages, n, lag):
            items = []
            for t in range(n + lag * (len(stages) - 1)):
                for k in reversed(range(len(stages))):
                    if 0 <= t - k * lag < n:
                        items.append(functools.partial(stages[k], t - k * lag))
            return items

        def ln_stages(load, stat, dst, j_scale, j_shift, cols=range(NC)):
            def chunks(x):
                return [x[:, c * 128:(c + 1) * 128] for c in range(NC)]

            def put(j, r, part, fn):
                m = jnp.sum(part, axis=-1, keepdims=True) * (1.0 / D)
                stat[j, pl.ds(pl.multiple_of(zrow(r), LG), LG), :] = jnp.broadcast_to(fn(m), (LG, 128))

            def s_mean(i):
                put(0, i * LG, gate16(_tree(_add, chunks(load(i * LG, 0))), 1, 2), lambda m: m)

            def s_var(i):
                r = i * LG
                d = load(r, 1) - jnp.concatenate([gate16(stat[0, r:r + LG, :], 0, 1)] * NC, axis=1)
                put(1, r, _tree(_add, chunks(d * d)), lambda m: jax.lax.rsqrt(m + EPS))

            def s_out(i):
                r = i * LG
                x = load(r, 2)
                mu = jnp.concatenate([stat[0, r:r + LG, :]] * (NC // 2), axis=1)
                for c0 in range(cols[0] * 128, cols[-1] * 128, KH):
                    rs = jnp.concatenate([gate16(stat[1, r:r + LG, :], c0 - cols[0] * 128, D)] * (NC // 2), axis=1)
                    y = ((x[:, c0:c0 + KH] - mu) * rs).reshape(LG // 8, 8, KH)
                    y = y * mod(j_scale, c0, c0 + KH)[None] + mod(j_shift, c0, c0 + KH)[None]
                    dst[r // 2:(r + LG) // 2, c0:c0 + KH] = pltpu.bitcast(y.reshape(LG, KH).astype(BF16), U32)
            return s_mean, s_var, s_out

        def load_x(row0):
            return lambda r, k: x_v[pl.ds(pl.multiple_of(zrow(row0 + r, k), LG), LG), :].astype(F32)

        def ln1_items(row0, buf):
            return staged(ln_stages(load_x(row0), stat1, bufs[buf][0], 1, 0), TM // LG, 1)

        def ln1_start(b, k):
            return ln_stages(load_x(b * TM), stats.at[:, pl.ds(b * TM, TM), :], h1s.at[b] if b < NS else h1a,
                             1, 0, range(k * NC // 2, (k + 1) * NC // 2))

        def stats_items(b, with_out):
            def one(i):
                r = b * TM + i * LG
                xf = x_v[r:r + LG, :].astype(F32)
                part = gate16(_tree(_add, [xf[:, c * 128:(c + 1) * 128] for c in range(NC)]), 0, 1)
                mu = jnp.sum(part, axis=-1, keepdims=True) * (1.0 / D)
                d = xf - mu
                rs = jax.lax.rsqrt(jnp.mean(d * d, axis=-1, keepdims=True) + EPS)
                stats[0, r:r + LG, :] = jnp.broadcast_to(mu, (LG, 128))
                stats[1, r:r + LG, :] = jnp.broadcast_to(rs, (LG, 128))
                if with_out:
                    have.add(("h", b, 0, i))
                    y = (d[:, :KH] * rs).reshape(LG // 8, 8, KH) * mod(1, 0, KH)[None] + mod(0, 0, KH)[None]
                    h1s[b, i * LG // 2:(i + 1) * LG // 2, 0:KH] = pltpu.bitcast(y.reshape(LG, KH).astype(BF16), U32)
            return [functools.partial(one, i) for i in range(TM // LG)]

        def ln1_out_items(b, k):
            def one(i):
                have.add(("h", b, k, i))
                ln1_start(b, k)[2](i)
            return [functools.partial(one, i) for i in range(TM // LG)]

        def x1_rows(row, n, c0, c1):
            xf = x_v[pl.ds(row, n), c0:c1].astype(F32).reshape(n // 8, 8, c1 - c0)
            y = y_v[pl.ds(row, n), c0:c1].reshape(n // 8, 8, c1 - c0)
            ga = jnp.concatenate([gate(mod(2, c, c + 128), c - c0, 2 * D) for c in range(c0, c1, 128)], axis=1)
            return (xf + ga[None] * y).reshape(n, c1 - c0)

        def post_items(row0):
            def load(r, k):
                if k:
                    return x1n[pl.ds(pl.multiple_of(zrow(r, k), LG), LG), :]
                x1 = x1_rows(row0 + r, LG, 0, D)
                x1n[r:r + LG, :] = x1
                return x1
            return staged(ln_stages(load, stat2, h2_v, 4, 3), TMB // LG, 1)

        def logit_items(buf, first):
            _, qk, _, _, pb = bufs[buf]
            swap = lane_iota(RG) ^ 1

            def s_logit(g):
                need(("q", buf), ("k", buf))
                have.add(("l", buf, g))
                r = g * RG
                q = qk[0:NC, HALO + r:HALO + r + RG, :]
                dst = pl.ds(pl.multiple_of(zrow(0), RG), RG)
                for w in range(WIN):
                    k0 = zrow(HALO + r - DIL * w, int(w >= WIN // 2))
                    s = gate(_fold(_add, q * qk[NC:2 * NC, pl.ds(k0, RG), :]), w, WIN)
                    s = s + pltpu.roll(s, 64, 1)
                    s = s + _lane_gather(s, swap)
                    if first and r < DIL * w:
                        pos = r + jax.lax.broadcasted_iota(jnp.int32, (RG, 128), 0)
                        s = jnp.where(pos >= DIL * w, s, NEG * LOG2E)
                    sls[g % len(sls)][w, dst, :] = s

            def s_soft(g):
                assert ("p", buf, g) not in have
                have.add(("p", buf, g))
                r = g * RG
                s = sls[g % len(sls)][...]
                e = jnp.exp2(s - gate(_fold(jnp.maximum, s), 0, 1)[None])
                pb[0:WIN, r:r + RG, :] = e
                den = _fold(_add, e)
                inv = pl.reciprocal(den, approx=True)
                pb[WIN, r:r + RG, :] = inv * (2.0 - den * inv)
            return staged((s_logit, s_soft), TM // RG, LLAG)

        def pv_items(buf):
            _, _, vp, o, pb = bufs[buf]
            otmp = otmps[buf]

            def one(r):
                need(("v", buf), ("p", buf, r // RG))
                have.remove(("p", buf, r // RG))
                have.add(("o", buf, r // RG))
                p = pb[:, pl.ds(pl.multiple_of(zrow(r), RG), RG), :]
                acc = _tree(_add, [p[w:w + 1] * vp[:, pl.ds(zrow(HALO + r - DIL * w, int(w >= WIN // 2)), RG), :]
                                   for w in range(WIN)]) * p[WIN:]
                acc = [gate(acc[c], c, NC) for c in range(NC)]
                if (r // RG) % 2 == 0:
                    otmp[:, pl.ds(pl.multiple_of(zrow(0), 8), RG), :] = jnp.stack(acc)
                else:
                    prev = otmp[...]
                    both = jnp.concatenate([jnp.concatenate([prev[c] for c in range(NC)], axis=1),
                                            jnp.concatenate(acc, axis=1)], axis=0)
                    o[(r - RG) // 2:(r + RG) // 2, :] = pltpu.bitcast(both.astype(BF16), U32)
            return [functools.partial(one, r) for r in range(0, TM, RG)]

        def halo(buf, prev, part):
            c0 = NC if part == 1 else 0
            ref = bufs[buf][part]
            if prev is None:
                val = (jnp.zeros((NC, HALO, 128), F32) if part == 1
                       else jnp.broadcast_to(ref[:, HALO:HALO + 1, :], (NC, HALO, 128)))
            else:
                val = bufs[prev][part][c0:c0 + NC, TM:TM + HALO, :]
                if st["tok"] is not None:
                    val = jnp.stack([gate16(val[c], 1, 2) for c in range(NC)])
            ref[c0:c0 + NC, 0:HALO, :] = val

        def qkv_part(buf, g, sb=None, k=None):
            h1, qk, vp, _, _ = bufs[buf] if buf else (None,) * 5
            if sb is not None:
                h1 = h1s.at[sb]
                need(*[("h", sb, k, i) for i in range(TM // LG)])
            if k != 0:
                for i in range(TM // RG):
                    if g < 2 and ("qk"[g], buf) in have:
                        need(("l", buf, i))
                    if g == 2 and ("v", buf) in have:
                        assert ("p", buf, i) not in have or ("new", buf) in have
                if g == 1:
                    have.difference_update({("l", buf, i) for i in range(TM // RG)})
                    have.add(("new", buf))
                have.discard(("qkv"[g], buf))

            def sink(n0, r):
                ch = n0 // 128
                if k == 0:
                    part[sb, ch] = r
                    return
                if k == 1:
                    r = r + part[sb, ch]
                dst, ci = (qk, ch) if ch < 2 * NC else (vp, ch - 2 * NC)
                dst[ci, HALO:HALO + TM, :] = r * (SM_SCALE * LOG2E) if ch < NC else r

            def weights(kk, n0):
                need(("w", g, kk, n0 % D // 128))
                return ld16(wqkv_p, kk * KH, KH, n0, n0 + 128)
            matmul(lambda kk: ld16(h1, 0, TM, kk * KH, (kk + 1) * KH), weights,
                   (0, 1) if k is None else (k,), range(g * D, (g + 1) * D, 128), sink,
                   None if k == 0 else ("qkv"[g], buf))
            if g == 2:
                have.discard(("new", buf))

        def wo_mm(buf, row0, m0=0, m1=TM):
            o = bufs[buf][3]
            need(*[("o", buf, i) for i in range(m0 // RG, m1 // RG)])
            have.difference_update({("o", buf, i) for i in range(m0 // RG, m1 // RG)})

            def sink(n0, r):
                y_v[pl.ds(row0 + m0, m1 - m0), n0:n0 + 128] = r
            matmul(lambda k: ld16(o, m0, m1 - m0, k * KH, (k + 1) * KH),
                   lambda k, n0: ld16(wo_p, k * KH, KH, n0, n0 + 128),
                   (0, 1), range(0, D, 128), sink)

        UP = NC * (D // KH)

        def run_now(items):
            for fn in items:
                fn()

        def ffn(j, row0, slot, nxt_row):
            h = ld16(h2_v, 0, TMB, 0, D)
            for f0 in range(0, F, FC):
                g = jnp.dot(h, w1_v[:, f0:f0 + FC], preferred_element_type=F32)
                u = jnp.dot(h, w3_v[:, f0:f0 + FC], preferred_element_type=F32)
                act_v[:, f0:f0 + FC] = pltpu.bitcast((g * jax.nn.sigmoid(g) * u).astype(BF16), U32)
            nk = F // KH
            sched = {}
            place(sched, post_items(nxt_row), range(0, NC * nk - PB1))
            begin(sched)

            def sink(n0, r):
                z = (mod(5, n0, n0 + 128)[None] * r.reshape(TMB // 8, 8, 128)).reshape(TMB, 128)
                obuf[slot, :, n0:n0 + 128] = (x1_rows(row0, TMB, n0, n0 + 128) + z).astype(BF16)
                if n0 + 128 in OCUT:
                    cp_out(j, slot, OCUT.index(n0 + 128) - 1).start()
            matmul(lambda k: ld16(act_v, 0, TMB, k * KH, (k + 1) * KH),
                   lambda k, n0: w2_v[k * KH:(k + 1) * KH, n0:n0 + 128],
                   tuple(range(nk)), range(0, D, 128), sink)

        U8 = NC

        def segment(*placements):
            sched = {}
            for items, units in placements:
                place(sched, items, units)
            begin(sched)

        with jax.named_scope("prologue"):
            zs[0] = 0
            begin({})
            start("c", "x0", "ca0", "q0", "sa0a", "sa0b", "x23", "k0", "v0", "ca1", "sa1", "q1", "x4", "k1", "v1",
                  "wo", "x1", "m2", "x2")
            wait("c")
            cb_v[...] = jnp.broadcast_to(silu_c().astype(F32), (128, D)).T
            wait("x0")
            run_now(stats_items(0, False) + stats_items(1, False))
            wait("ca0")
            mod_mxu(1, 0, D)
            wait("q0")
            run_now(perm_qkv_items(0, 0))
            wait("sa0a")
            mod_mxu(0, 0, SA_CUT)
            wait("sa0b")
            mod_mxu(0, SA_CUT, D)
            run_now(ln1_out_items(0, 0))

        with jax.named_scope("pass1"):
            segment((ln1_out_items(1, 0), range(0, U8 - 1)))
            qkv_part(None, 0, 0, 0)
            wait("x23")
            segment((stats_items(2, True), range(0, X0)), (stats_items(3, True), range(U8 - 1, U8 + X1)))
            qkv_part(None, 0, 1, 0)
            qkv_part(None, 0, 2, 0)
            wait("k0")
            segment((perm_qkv_items(1, 0), range(0, X2)))
            for g, b in ((0, 3), (1, 0), (1, 1)):
                qkv_part(None, g, b, 0)
            wait("v0", "ca1")
            segment((perm_qkv_items(2, 0), range(0, 2 * U8 - 2)),
                    (mod_items(D + KH, 4), range(2 * U8 - 2, 4 * U8)))
            for g, b in ((1, 2), (1, 3), (2, 0), (2, 1)):
                qkv_part(None, g, b, 0)
            wait("sa1", "q1")
            segment((mod_items(KH, 4), range(0, U8 + 2)),
                    (perm_qkv_items(0, 1), range(0, 2 * U8 - 2)),
                    (ln1_out_items(0, 1), range(U8 + 3, 2 * U8 - 1)))
            qkv_part(None, 2, 2, 0)
            qkv_part(None, 2, 3, 0)

        with jax.named_scope("pass2"):
            wait("x4", "k1")
            segment((stats_items(NS, False), range(X3, X4)),
                    (perm_qkv_items(1, 1), range(0, 2 * U8 - 2)),
                    (ln1_out_items(1, 1), range(0, U8 - 2)),
                    (ln1_out_items(2, 1), range(U8 - 2, 2 * U8)))
            halo("b", None, 1)
            qkv_part("b", 0, 0, 1)
            qkv_part("c", 0, 1, 1)
            wait("v1")
            l0 = logit_items("b", True)
            segment((perm_qkv_items(2, 1), range(0, 2 * U8 - 2)),
                    (ln1_out_items(3, 1), range(0, U8)),
                    (l0[:LB], range(B0, B1)))
            qkv_part("b", 1, 0, 1)
            halo("c", "b", 1)
            qkv_part("c", 1, 1, 1)
            qkv_part("b", 2, 0, 1)
            halo("b", None, 2)
            halo("c", "b", 2)
            qkv_part("c", 2, 1, 1)
            wait("wo")
            segment((perm_wo_items(), range(0, WS)),
                    (l0[LB:], range(0, C0)),
                    (pv_items("b"), range(C0 + CP, 39)),
                    (logit_items("c", False), range(C0, C1)),
                    (pv_items("c"), range(C1 + CP, 63)),
                    (logit_items("a", False), range(C1, C2)),
                    (pv_items("a"), range(C2 + CP, 79)),
                    ([functools.partial(halo, "b", "a", 1)], [23]),
                    ([functools.partial(halo, "b", "a", 2)], [39]),
                    (ln1_out_items(NS, 0) + ln1_out_items(NS, 1), range(H0, H1)),
                    (logit_items("b", False), range(C2, 96 - L1)))
            halo("a", "c", 1)
            halo("a", "c", 2)
            for g in range(3):
                qkv_part("a", g, 2, 1)
            for g in range(3):
                qkv_part("b", g, 3, 1)
            wo_mm("b", 0)
            wo_mm("c", TM)
            wo_mm("a", 2 * TM)
            finish()
            wait("x1", "m2")
            start("m3", "w1", "w3", "w2")


        def half(X, Y, u0, sched, row_ln1, row_wo, extra):
            place(sched, pv_items(Y), range(u0 + P0, u0 + 3 * UP - P1))
            place(sched, logit_items(X, False), range(u0 + 2 * UP + L0, u0 + 4 * UP - L1))
            place(sched, ln1_items(row_ln1, Y), range(u0 + N0, u0 + N1))
            place(sched, extra, range(u0, u0 + 4 * UP - 1))

            def run():
                halo(X, Y, 1)
                halo(X, Y, 2)
                for g in range(3):
                    qkv_part(X, g)
                wo_mm(Y, row_wo)
            return run

        def a_step(s, carry):
            @pl.when(s == 3)
            def _():
                wait("x2", "m3")

            ra = pl.multiple_of(2 * s * TM, TM)
            nxt = pl.multiple_of(jnp.minimum(ra + 2 * TM, S - TM), TM)
            col0 = pl.multiple_of(jnp.minimum(2 * D + (s - 2) * (MT * 128), 6 * D - MT * 128), 128)
            mi = mod_items(col0, MT)
            sched = {}
            run_a = half("a", "b", 0, sched, ra + TM, ra - TM, mi[:len(mi) // 2])
            run_b = half("b", "a", 4 * UP, sched, nxt, ra, mi[len(mi) // 2:])
            begin(sched)
            run_a()
            run_b()
            finish()
            return carry

        with jax.named_scope("aloop"):
            jax.lax.fori_loop(NS // 2, NB // 2, a_step, 0)

        with jax.named_scope("atail"):
            begin({})

            def post0(r):
                x1 = x1_rows(r, LG, 0, D)
                mu = jnp.mean(x1, axis=-1, keepdims=True)
                d = x1 - mu
                rs = jax.lax.rsqrt(jnp.mean(d * d, axis=-1, keepdims=True) + EPS)
                y = (d * rs).reshape(LG // 8, 8, D) * mod(4, 0, D)[None] + mod(3, 0, D)[None]
                h2_v[r // 2:(r + LG) // 2, :] = pltpu.bitcast(y.reshape(LG, D).astype(BF16), U32)
            post = [functools.partial(post0, r) for r in range(0, TMB, LG)]
            pv = pv_items("b")
            run_now(pv[:NC])
            segment((pv[NC:], range(0, UP - 2)), (post, range(TP0, 2 * UP - TE)))
            wo_mm("b", S - TM, 0, TM // 2)
            wo_mm("b", S - TM, TM // 2, TM)
            finish()
            wait("w1", "w3", "w2")

        def b_step(j, carry):
            slot = j % 2

            @pl.when(j >= 2)
            def _():
                wait_out(j - 2, slot)

            row0 = pl.multiple_of(j * TMB, TMB)
            nxt = pl.multiple_of(jnp.minimum(row0 + TMB, S - TMB), TMB)
            if SKIP_FFN:
                obuf[slot] = x1_rows(row0, TMB, 0, D).astype(BF16)
                for q in range(NQ):
                    cp_out(j, slot, q).start()
            else:
                ffn(j, row0, slot, nxt)
            return carry

        with jax.named_scope("bloop"):
            jax.lax.fori_loop(0, NBB, b_step, 0)
        with jax.named_scope("tail"):
            wait_out(NBB - 2, (NBB - 2) % 2)
            wait_out(NBB - 1, (NBB - 1) % 2)

    any_spec = pl.BlockSpec(memory_space=pl.ANY)
    qkv_set = [
        pltpu.VMEM((2 * NC, KV, 128), F32),
        pltpu.VMEM((NC, KV, 128), F32),
        pltpu.VMEM((WIN + 1, TM, 128), F32),
    ]
    scratch = [
        pltpu.VMEM((S, D), BF16),
        pltpu.VMEM((D, 3 * D), BF16),
        pltpu.VMEM((NC, KH // 2, 128), U32),
        pltpu.VMEM((D // 2, 3 * D), U32),
        pltpu.VMEM((D, D), BF16),
        pltpu.VMEM((NC, D // 32 * 17, 128), U32),
        pltpu.VMEM((D // 2, D), U32),
        pltpu.VMEM((D, F), BF16),
        pltpu.VMEM((D, F), BF16),
        pltpu.VMEM((F, D), BF16),
        pltpu.VMEM((D, 6 * D), BF16),
        pltpu.VMEM((D, 128), F32),
        pltpu.VMEM((MT, NSUB, 8, 128), F32),
        pltpu.VMEM((8, 6 * D), F32),
        pltpu.VMEM((8, 2 * D), F32),
        pltpu.VMEM((TM // 2, D), U32),
        pltpu.VMEM((TM // 2, D), U32),
        pltpu.VMEM((NS, TM // 2, D), U32),
        pltpu.VMEM((NS, 3 * NC, TM, 128), F32),
        pltpu.VMEM((2, (NS + 1) * TM, 128), F32),
        *qkv_set, *qkv_set, *qkv_set,
        *[pltpu.VMEM((TM // 2, D), U32)] * 3,
        *[pltpu.VMEM((NC, RG, 128), F32)] * 3,
        *[pltpu.VMEM((WIN, RG, 128), F32)] * 3,
        pltpu.VMEM((2, TM, 128), F32),
        pltpu.VMEM((2, TMB, 128), F32),
        pltpu.VMEM((S, D), F32),
        pltpu.VMEM((TMB, D), F32),
        pltpu.VMEM((TMB // 2, D), U32),
        pltpu.VMEM((TMB // 2, F), U32),
        pltpu.VMEM((2, TMB, D), BF16),
        pltpu.VMEM((1, D), BF16),
        pltpu.SMEM((1,), jnp.int32),
        pltpu.SemaphoreType.DMA((NDMA,)),
        pltpu.SemaphoreType.DMA((2 * NQ,)),
    ]

    def call(A_x, A_wqkv, A_wo, B_w1, B_w3, B_w2, c, w_mod):
        return pl.pallas_call(
            kernel,
            out_shape=jax.ShapeDtypeStruct((1, S, D), BF16),
            in_specs=[any_spec] * 8,
            out_specs=any_spec,
            scratch_shapes=scratch,
            compiler_params=pltpu.CompilerParams(
                vmem_limit_bytes=120 * 1024 * 1024,
                disable_semaphore_checks=True, disable_bounds_checks=True),
        )(A_x, A_wqkv, A_wo, B_w1, B_w3, B_w2, c, w_mod)

    return call


@jax.jit
def pallas_adaLN_cond__sliding_local_dilated__glu_gated_swiglu__prompt_kernel(
    A_x: jax.Array,
    A_wqkv: jax.Array,
    A_wo: jax.Array,
    B_x: jax.Array,
    B_w1: jax.Array,
    B_w3: jax.Array,
    B_w2: jax.Array,
    c: jax.Array,
    w_mod: jax.Array,
):
    del B_x
    return _build()(A_x, A_wqkv, A_wo, B_w1, B_w3, B_w2, c, w_mod)
```

```python
import functools
import math

import jax
import jax.numpy as jnp
import jax.experimental.pallas as pl
import jax.experimental.pallas.tpu as pltpu

S = 2048
D = 1024
F = 3584
H = 32
DH = D // H
WIN = 8
DIL = 2
NC = D // 128
HALO = 16
EPS = 1e-5
NEG = -1000000000.0
SM_SCALE = DH ** -0.5
LOG2E = math.log2(math.e)

TM = 128
NB = S // TM
KV = HALO + TM
RG = 8
LG = 16
NS = 4
NDMA = 23
KH = 512

F32 = jnp.float32
BF16 = jnp.bfloat16
U32 = jnp.uint32


def _tree(op, xs):
    xs = list(xs)
    while len(xs) > 1:
        xs = [op(xs[i], xs[i + 1]) if i + 1 < len(xs) else xs[i] for i in range(0, len(xs), 2)]
    return xs[0]


def _add(a, b):
    return a + b


def _fold(op, x):
    while x.shape[0] > 1:
        x = x.reshape(x.shape[0] // 2, 2, *x.shape[1:])
        x = op(x[:, 0], x[:, 1])
    return x[0]


def _lane_gather(x, idx):
    dn = jax.lax.GatherDimensionNumbers(
        offset_dims=(), collapsed_slice_dims=(1,), start_index_map=(1,),
        operand_batching_dims=(0,), start_indices_batching_dims=(0,))
    return jax.lax.gather(x, idx[..., None], dn, (1, 1), mode=jax.lax.GatherScatterMode.PROMISE_IN_BOUNDS)


def _build(TMB=256, FC=512, OCUT=(0, 512, 896, 1024), SA_CUT=768,
           MT=6, NSUB=16, MLAG=8, PR=32, SPREAD=128, LLAG=3,
           P0=1, P1=16, L0=0, L1=1, N0=0, N1=30, PB1=5,
           B0=14, B1=30, LB=19, C0=10, C1=38, C2=64, CP=1, WS=46, H0=0, H1=10,
           TP0=10, TE=3, X0=4, X1=4, X2=7, X3=0, X4=6, SKIP_FFN=False):
    NBB = S // TMB
    NQ = len(OCUT) - 1

    def kernel(x_hbm, wqkv_hbm, wo_hbm, w1_hbm, w3_hbm, w2_hbm, c_hbm, wmod_hbm,
               out_hbm,
               x_v, wqkv_v, wtmp, wqkv_p, wo_v, wo_tmp, wo_p, w1_v, w3_v, w2_v,
               wmod_v, cb_v, modp_v, modb_v, mod_v,
               h1a, h1b, h1s, part, stats, qka, va, pa, qkb, vb, pb_, qkc, vc, pc,
               oa, ob, oc, ota, otb, otc, sl0, sl1, sl2, stat1, stat2,
               y_v, x1n, h2_v, act_v, obuf, c_ref, zs, sem_w, sem_o):
        bufs = {"a": (h1a, qka, va, oa, pa), "b": (h1b, qkb, vb, ob, pb_),
                "c": (None, qkc, vc, oc, pc)}

        sls = (sl0, sl1, sl2)
        otmps = {"a": ota, "b": otb, "c": otc}

        dmas = {}

        def add_dma(name, src, dst):
            dmas[name] = (src, dst, len(dmas))

        for name, (b0, b1) in (("x0", (0, 2)), ("x23", (2, NS)), ("x4", (NS, NS + 1)), ("x1", (NS + 1, NS + 3)), ("x2", (NS + 3, NB))):
            rows = pl.ds(b0 * TM, (b1 - b0) * TM)
            add_dma(name, x_hbm.at[0, rows, :], x_v.at[rows, :])
        for name, (r0, r1) in (("sa0a", (0, SA_CUT)), ("sa0b", (SA_CUT, D))):
            rows, cols = pl.ds(r0, r1 - r0), pl.ds(0, KH)
            add_dma(name, wmod_hbm.at[rows, cols], wmod_v.at[rows, cols])
        for name, (c0, c1) in (("sa1", (KH, D)), ("ca0", (D, D + KH)), ("ca1", (D + KH, 2 * D)),
                               ("m2", (2 * D, 3 * D)), ("m3", (3 * D, 6 * D))):
            cols = pl.ds(c0, c1 - c0)
            add_dma(name, wmod_hbm.at[:, cols], wmod_v.at[:, cols])
        for g in range(3):
            for k in range(2):
                rows, cols = pl.ds(k * KH, KH), pl.ds(g * D, D)
                add_dma("qkv"[g] + str(k), wqkv_hbm.at[rows, cols], wqkv_v.at[rows, cols])
        add_dma("c", c_hbm, c_ref)
        add_dma("wo", wo_hbm, wo_v)
        add_dma("w1", w1_hbm, w1_v)
        add_dma("w3", w3_hbm, w3_v)
        add_dma("w2", w2_hbm, w2_v)
        assert len(dmas) == NDMA

        def cp(name):
            src, dst, i = dmas[name]
            return pltpu.make_async_copy(src, dst, sem_w.at[i])

        def start(*names):
            for n in names:
                cp(n).start()

        def wait(*names):
            for n in names:
                cp(n).wait()

        def cp_out(j, q):
            rows, cols = pl.ds(j * TMB, TMB), pl.ds(OCUT[q], OCUT[q + 1] - OCUT[q])
            return pltpu.make_async_copy(obuf.at[rows, cols], out_hbm.at[0, rows, cols], sem_o.at[j * NQ + q])

        st = {"z": None, "never": None, "clock": 0, "sched": {}, "tok": None}

        have = set()

        def need(*keys):
            assert all(k in have for k in keys), keys

        def finish():
            assert not st["sched"], "items placed beyond the last unit"

        def begin(sched):
            finish()
            z = zs[0]
            st.update(z=(0, z, 2 * z), never=jnp.full((8, 128), z, jnp.int32) != 0, clock=0, sched=sched, tok=None)

        def gate(val, i, n):
            r = st["tok"]
            if r is None:
                return val
            row = (i * min(SPREAD, r.shape[0]) // n) // 8 * 8
            t = r[row:row + 8]
            return jax.lax.select(st["never"], t if val.dtype == F32 else pltpu.bitcast(t, val.dtype), val)

        def place(sched, items, units):
            units = list(units)
            for i, it in enumerate(items):
                sched.setdefault(units[(i * len(units)) // len(items)], []).append(it)

        def matmul(lhs_fn, w_fn, ks, cols, sink, gives=None):
            for n0 in cols:
                r = None
                for k in ks:
                    d = jnp.dot(lhs_fn(k), w_fn(k, n0), preferred_element_type=F32)
                    r = d if r is None else r + d
                    if k == ks[-1]:
                        sink(n0, r)
                    if n0 == cols[-1] and k == ks[-1]:
                        have.add(gives)
                    st["tok"] = r
                    for fn in st["sched"].pop(st["clock"], []):
                        fn()
                    st["tok"] = None
                    st["clock"] += 1

        def lane_iota(rows):
            return jax.lax.broadcasted_iota(jnp.int32, (rows, 128), 1)

        def ld16(ref, r0, n, c0, c1):
            return pltpu.bitcast(ref[r0 // 2:(r0 + n) // 2, c0:c1], BF16)

        def silu_c():
            cf = c_ref[...].astype(F32)
            return (cf * jax.nn.sigmoid(cf)).astype(BF16)

        def mod_mxu(j, r0, r1):
            cs = slice(j * D, j * D + KH)
            lhs = jnp.broadcast_to(silu_c()[:, r0:r1], (16, r1 - r0))
            r = jnp.dot(lhs, wmod_v[r0:r1, cs], preferred_element_type=F32)[0:8]
            mod_v[:, cs] = r + (mod_v[:, cs] if r0 else float(j == 1))

        def mod(j, c0, c1):
            return (mod_v if j < 2 else modb_v)[:, j * D + c0:j * D + c1]

        def mod_items(col0, ntiles):
            rows = D // NSUB

            def col(t):
                c0 = col0 + t * 128
                return c0 if isinstance(c0, int) else pl.multiple_of(c0, 128)

            def part_sum(t, i):
                w = wmod_v[i * rows:(i + 1) * rows, pl.ds(col(t), 128)].astype(F32)
                p = (w * cb_v[i * rows:(i + 1) * rows, :]).reshape(rows // 8, 8, 128)
                modp_v[t, i] = gate(_fold(_add, p), 1, 2)

            def total(t):
                r = gate(_fold(_add, modp_v[t, pl.ds(zrow(0), NSUB)]), 0, 1)
                one = jnp.where((col(t) // D) % 3 == 1, 1.0, 0.0).astype(F32)
                dst = mod_v if isinstance(col0, int) else modb_v
                dst[:, pl.ds(col(t), 128)] = jnp.broadcast_to(jnp.sum(r, axis=0, keepdims=True) + one, (8, 128))
            items = []
            for t in range(ntiles + 1):
                for i in range(NSUB):
                    if t < ntiles:
                        items.append(functools.partial(part_sum, t, i))
                    if t > 0 and i == (MLAG if t < ntiles else 0):
                        items.append(functools.partial(total, t - 1))
            return items

        def perm_mix(g, i, nrows):
            n = nrows // 2
            l = jnp.concatenate([gate(lane_iota(8), h, n) for h in range(0, n, 8)], axis=0)
            w = pltpu.bitcast(wqkv_v[i * nrows:(i + 1) * nrows, g * D:(g + 1) * D], U32)
            vals = [w[:, c * 128:(c + 1) * 128] for c in range(NC)]
            for b in range(3):
                m = (l & (4 << b)) == 0
                for c in range(NC):
                    if c & (1 << b):
                        continue
                    lo, hi = vals[c], vals[c | (1 << b)]
                    vals[c] = jax.lax.select(m, lo, hi)
                    vals[c | (1 << b)] = jax.lax.select(m, hi, lo)
            wtmp[:, pl.ds(pl.multiple_of(zrow((i * n) % (KH // 2)), 8), n), :] = jnp.stack(vals)

        def perm_gather(g, k, j):
            have.add(("w", g, k, j))
            l = lane_iota(8)
            idx = ((((l >> 1) & 3) << 5) | ((((l >> 3) & 7) ^ j) << 2) | ((l >> 6) << 1) | (l & 1))
            idx = jnp.concatenate([gate(idx, 0, 1)] * (KH // 16), axis=0)
            wqkv_p[k * KH // 2:(k + 1) * KH // 2, g * D + j * 128: g * D + (j + 1) * 128] = _lane_gather(wtmp[j], idx)

        def perm_qkv_items(g, k, nrows=PR):
            n = KH // nrows
            return ([functools.partial(perm_mix, g, i, nrows) for i in range(k * n, (k + 1) * n)]
                    + [functools.partial(perm_gather, g, k, j) for j in range(NC)])

        def perm_wo_items():
            sub = jax.lax.broadcasted_iota(jnp.int32, (8, 128), 0)

            def spread(c, h):
                for r in range(h * 256, h * 256 + 256, 8):
                    wo_tmp[c, pl.ds(zrow(r + r // 16), 8), :] = gate(pltpu.bitcast(
                        wo_v[2 * r:2 * r + 16, c * 128:(c + 1) * 128], U32), r % 256, 256)

            def gather(c, h):
                for G in range(h * 32, h * 32 + 32):
                    j, e, ch = G >> 3, (G >> 2) & 1, G & 3
                    dd = (((2 * ch) ^ j) << 1) | e
                    ta = wo_tmp[c, pl.ds(ch * 136 + dd, 8, stride=17), :]
                    tb = wo_tmp[c, pl.ds(ch * 136 + (dd ^ 2), 8, stride=17), :]
                    wo_p[G * 8:G * 8 + 8, c * 128:(c + 1) * 128] = jax.lax.select(gate(sub, G % 32, 32) < 4, ta, tb)
            return [functools.partial(fn, c, h) for fn in (spread, gather) for c in range(NC) for h in range(2)]

        def zrow(row, k=1):
            return row if k == 0 else row + st["z"][k]

        def gate16(v, i, n):
            return jnp.concatenate([gate(v[q:q + 8], i, n) for q in range(0, LG, 8)], axis=0)

        def staged(stages, n, lag):
            items = []
            for t in range(n + lag * (len(stages) - 1)):
                for k in reversed(range(len(stages))):
                    if 0 <= t - k * lag < n:
                        items.append(functools.partial(stages[k], t - k * lag))
            return items

        def ln_stages(load, stat, dst, j_scale, j_shift, cols=range(NC)):
            def chunks(x):
                return [x[:, c * 128:(c + 1) * 128] for c in range(NC)]

            def put(j, r, part, fn):
                m = jnp.sum(part, axis=-1, keepdims=True) * (1.0 / D)
                stat[j, pl.ds(pl.multiple_of(zrow(r), LG), LG), :] = jnp.broadcast_to(fn(m), (LG, 128))

            def s_mean(i):
                put(0, i * LG, gate16(_tree(_add, chunks(load(i * LG, 0))), 1, 2), lambda m: m)

            def s_var(i):
                r = i * LG
                d = load(r, 1) - jnp.concatenate([gate16(stat[0, r:r + LG, :], 0, 1)] * NC, axis=1)
                put(1, r, _tree(_add, chunks(d * d)), lambda m: jax.lax.rsqrt(m + EPS))

            def s_out(i):
                r = i * LG
                x = load(r, 2)
                mu = jnp.concatenate([stat[0, r:r + LG, :]] * (NC // 2), axis=1)
                for c0 in range(cols[0] * 128, cols[-1] * 128, KH):
                    rs = jnp.concatenate([gate16(stat[1, r:r + LG, :], c0 - cols[0] * 128, D)] * (NC // 2), axis=1)
                    y = ((x[:, c0:c0 + KH] - mu) * rs).reshape(LG // 8, 8, KH)
                    y = y * mod(j_scale, c0, c0 + KH)[None] + mod(j_shift, c0, c0 + KH)[None]
                    dst[r // 2:(r + LG) // 2, c0:c0 + KH] = pltpu.bitcast(y.reshape(LG, KH).astype(BF16), U32)
            return s_mean, s_var, s_out

        def load_x(row0):
            return lambda r, k: x_v[pl.ds(pl.multiple_of(zrow(row0 + r, k), LG), LG), :].astype(F32)

        def ln1_items(row0, buf):
            return staged(ln_stages(load_x(row0), stat1, bufs[buf][0], 1, 0), TM // LG, 1)

        def ln1_start(b, k):
            return ln_stages(load_x(b * TM), stats.at[:, pl.ds(b * TM, TM), :], h1s.at[b] if b < NS else h1a,
                             1, 0, range(k * NC // 2, (k + 1) * NC // 2))

        def stats_items(b, with_out):
            def one(i):
                r = b * TM + i * LG
                xf = x_v[r:r + LG, :].astype(F32)
                part = gate16(_tree(_add, [xf[:, c * 128:(c + 1) * 128] for c in range(NC)]), 0, 1)
                mu = jnp.sum(part, axis=-1, keepdims=True) * (1.0 / D)
                d = xf - mu
                rs = jax.lax.rsqrt(jnp.mean(d * d, axis=-1, keepdims=True) + EPS)
                stats[0, r:r + LG, :] = jnp.broadcast_to(mu, (LG, 128))
                stats[1, r:r + LG, :] = jnp.broadcast_to(rs, (LG, 128))
                if with_out:
                    have.add(("h", b, 0, i))
                    y = (d[:, :KH] * rs).reshape(LG // 8, 8, KH) * mod(1, 0, KH)[None] + mod(0, 0, KH)[None]
                    h1s[b, i * LG // 2:(i + 1) * LG // 2, 0:KH] = pltpu.bitcast(y.reshape(LG, KH).astype(BF16), U32)
            return [functools.partial(one, i) for i in range(TM // LG)]

        def ln1_out_items(b, k):
            def one(i):
                have.add(("h", b, k, i))
                ln1_start(b, k)[2](i)
            return [functools.partial(one, i) for i in range(TM // LG)]

        def x1_rows(row, n, c0, c1):
            xf = x_v[pl.ds(row, n), c0:c1].astype(F32).reshape(n // 8, 8, c1 - c0)
            y = y_v[pl.ds(row, n), c0:c1].reshape(n // 8, 8, c1 - c0)
            ga = jnp.concatenate([gate(mod(2, c, c + 128), c - c0, 2 * D) for c in range(c0, c1, 128)], axis=1)
            return (xf + ga[None] * y).reshape(n, c1 - c0)

        def post_items(row0):
            def load(r, k):
                if k:
                    return x1n[pl.ds(pl.multiple_of(zrow(r, k), LG), LG), :]
                x1 = x1_rows(row0 + r, LG, 0, D)
                x1n[r:r + LG, :] = x1
                return x1
            return staged(ln_stages(load, stat2, h2_v, 4, 3), TMB // LG, 1)

        def logit_items(buf, first):
            _, qk, _, _, pb = bufs[buf]
            swap = lane_iota(RG) ^ 1

            def s_logit(g):
                need(("q", buf), ("k", buf))
                have.add(("l", buf, g))
                r = g * RG
                q = qk[0:NC, HALO + r:HALO + r + RG, :]
                dst = pl.ds(pl.multiple_of(zrow(0), RG), RG)
                for w in range(WIN):
                    k0 = zrow(HALO + r - DIL * w, int(w >= WIN // 2))
                    s = gate(_fold(_add, q * qk[NC:2 * NC, pl.ds(k0, RG), :]), w, WIN)
                    s = s + pltpu.roll(s, 64, 1)
                    s = s + _lane_gather(s, swap)
                    if first and r < DIL * w:
                        pos = r + jax.lax.broadcasted_iota(jnp.int32, (RG, 128), 0)
                        s = jnp.where(pos >= DIL * w, s, NEG * LOG2E)
                    sls[g % len(sls)][w, dst, :] = s

            def s_soft(g):
                assert ("p", buf, g) not in have
                have.add(("p", buf, g))
                r = g * RG
                s = sls[g % len(sls)][...]
                e = jnp.exp2(s - gate(_fold(jnp.maximum, s), 0, 1)[None])
                pb[0:WIN, r:r + RG, :] = e
                den = _fold(_add, e)
                inv = pl.reciprocal(den, approx=True)
                pb[WIN, r:r + RG, :] = inv * (2.0 - den * inv)
            return staged((s_logit, s_soft), TM // RG, LLAG)

        def pv_items(buf):
            _, _, vp, o, pb = bufs[buf]
            otmp = otmps[buf]

            def one(r):
                need(("v", buf), ("p", buf, r // RG))
                have.remove(("p", buf, r // RG))
                have.add(("o", buf, r // RG))
                p = pb[:, pl.ds(pl.multiple_of(zrow(r), RG), RG), :]
                acc = _tree(_add, [p[w:w + 1] * vp[:, pl.ds(zrow(HALO + r - DIL * w, int(w >= WIN // 2)), RG), :]
                                   for w in range(WIN)]) * p[WIN:]
                acc = [gate(acc[c], c, NC) for c in range(NC)]
                if (r // RG) % 2 == 0:
                    otmp[:, pl.ds(pl.multiple_of(zrow(0), 8), RG), :] = jnp.stack(acc)
                else:
                    prev = otmp[...]
                    both = jnp.concatenate([jnp.concatenate([prev[c] for c in range(NC)], axis=1),
                                            jnp.concatenate(acc, axis=1)], axis=0)
                    o[(r - RG) // 2:(r + RG) // 2, :] = pltpu.bitcast(both.astype(BF16), U32)
            return [functools.partial(one, r) for r in range(0, TM, RG)]

        def halo(buf, prev, part):
            c0 = NC if part == 1 else 0
            ref = bufs[buf][part]
            if prev is None:
                val = (jnp.zeros((NC, HALO, 128), F32) if part == 1
                       else jnp.broadcast_to(ref[:, HALO:HALO + 1, :], (NC, HALO, 128)))
            else:
                val = bufs[prev][part][c0:c0 + NC, TM:TM + HALO, :]
                if st["tok"] is not None:
                    val = jnp.stack([gate16(val[c], 1, 2) for c in range(NC)])
            ref[c0:c0 + NC, 0:HALO, :] = val

        def qkv_part(buf, g, sb=None, k=None):
            h1, qk, vp, _, _ = bufs[buf] if buf else (None,) * 5
            if sb is not None:
                h1 = h1s.at[sb]
                need(*[("h", sb, k, i) for i in range(TM // LG)])
            if k != 0:
                for i in range(TM // RG):
                    if g < 2 and ("qk"[g], buf) in have:
                        need(("l", buf, i))
                    if g == 2 and ("v", buf) in have:
                        assert ("p", buf, i) not in have or ("new", buf) in have
                if g == 1:
                    have.difference_update({("l", buf, i) for i in range(TM // RG)})
                    have.add(("new", buf))
                have.discard(("qkv"[g], buf))

            def sink(n0, r):
                ch = n0 // 128
                if k == 0:
                    part[sb, ch] = r
                    return
                if k == 1:
                    r = r + part[sb, ch]
                dst, ci = (qk, ch) if ch < 2 * NC else (vp, ch - 2 * NC)
                dst[ci, HALO:HALO + TM, :] = r * (SM_SCALE * LOG2E) if ch < NC else r

            def weights(kk, n0):
                need(("w", g, kk, n0 % D // 128))
                return ld16(wqkv_p, kk * KH, KH, n0, n0 + 128)
            matmul(lambda kk: ld16(h1, 0, TM, kk * KH, (kk + 1) * KH), weights,
                   (0, 1) if k is None else (k,), range(g * D, (g + 1) * D, 128), sink,
                   None if k == 0 else ("qkv"[g], buf))
            if g == 2:
                have.discard(("new", buf))

        def wo_mm(buf, row0, m0=0, m1=TM):
            o = bufs[buf][3]
            need(*[("o", buf, i) for i in range(m0 // RG, m1 // RG)])
            have.difference_update({("o", buf, i) for i in range(m0 // RG, m1 // RG)})

            def sink(n0, r):
                y_v[pl.ds(row0 + m0, m1 - m0), n0:n0 + 128] = r
            matmul(lambda k: ld16(o, m0, m1 - m0, k * KH, (k + 1) * KH),
                   lambda k, n0: ld16(wo_p, k * KH, KH, n0, n0 + 128),
                   (0, 1), range(0, D, 128), sink)

        UP = NC * (D // KH)

        def run_now(items):
            for fn in items:
                fn()

        def ffn(j, row0, nxt_row):
            h = ld16(h2_v, 0, TMB, 0, D)
            for f0 in range(0, F, FC):
                g = jnp.dot(h, w1_v[:, f0:f0 + FC], preferred_element_type=F32)
                u = jnp.dot(h, w3_v[:, f0:f0 + FC], preferred_element_type=F32)
                act_v[:, f0:f0 + FC] = pltpu.bitcast((g * jax.nn.sigmoid(g) * u).astype(BF16), U32)
            nk = F // KH
            sched = {}
            place(sched, post_items(nxt_row), range(0, NC * nk - PB1))
            begin(sched)

            def sink(n0, r):
                z = (mod(5, n0, n0 + 128)[None] * r.reshape(TMB // 8, 8, 128)).reshape(TMB, 128)
                obuf[pl.ds(row0, TMB), n0:n0 + 128] = (x1_rows(row0, TMB, n0, n0 + 128) + z).astype(BF16)
                if n0 + 128 in OCUT:
                    cp_out(j, OCUT.index(n0 + 128) - 1).start()
            matmul(lambda k: ld16(act_v, 0, TMB, k * KH, (k + 1) * KH),
                   lambda k, n0: w2_v[k * KH:(k + 1) * KH, n0:n0 + 128],
                   tuple(range(nk)), range(0, D, 128), sink)
            finish()

        U8 = NC

        def segment(*placements):
            sched = {}
            for items, units in placements:
                place(sched, items, units)
            begin(sched)

        with jax.named_scope("prologue"):
            zs[0] = 0
            begin({})
            start("c", "x0", "ca0", "q0", "sa0a", "sa0b", "x23", "k0", "v0", "ca1", "sa1", "q1", "x4", "k1", "v1",
                  "wo", "x1", "m2", "x2")
            wait("c")
            cb_v[...] = jnp.broadcast_to(silu_c().astype(F32), (128, D)).T
            wait("x0")
            run_now(stats_items(0, False) + stats_items(1, False))
            wait("ca0")
            mod_mxu(1, 0, D)
            wait("q0")
            run_now(perm_qkv_items(0, 0))
            wait("sa0a")
            mod_mxu(0, 0, SA_CUT)
            wait("sa0b")
            mod_mxu(0, SA_CUT, D)
            run_now(ln1_out_items(0, 0))

        with jax.named_scope("pass1"):
            segment((ln1_out_items(1, 0), range(0, U8 - 1)))
            qkv_part(None, 0, 0, 0)
            wait("x23")
            segment((stats_items(2, True), range(0, X0)), (stats_items(3, True), range(U8 - 1, U8 + X1)))
            qkv_part(None, 0, 1, 0)
            qkv_part(None, 0, 2, 0)
            wait("k0")
            segment((perm_qkv_items(1, 0), range(0, X2)))
            for g, b in ((0, 3), (1, 0), (1, 1)):
                qkv_part(None, g, b, 0)
            wait("v0", "ca1")
            segment((perm_qkv_items(2, 0), range(0, 2 * U8 - 2)),
                    (mod_items(D + KH, 4), range(2 * U8 - 2, 4 * U8)))
            for g, b in ((1, 2), (1, 3), (2, 0), (2, 1)):
                qkv_part(None, g, b, 0)
            wait("sa1", "q1")
            segment((mod_items(KH, 4), range(0, U8 + 2)),
                    (perm_qkv_items(0, 1), range(0, 2 * U8 - 2)),
                    (ln1_out_items(0, 1), range(U8 + 3, 2 * U8 - 1)))
            qkv_part(None, 2, 2, 0)
            qkv_part(None, 2, 3, 0)

        with jax.named_scope("pass2"):
            wait("x4", "k1")
            segment((stats_items(NS, False), range(X3, X4)),
                    (perm_qkv_items(1, 1), range(0, 2 * U8 - 2)),
                    (ln1_out_items(1, 1), range(0, U8 - 2)),
                    (ln1_out_items(2, 1), range(U8 - 2, 2 * U8)))
            halo("b", None, 1)
            qkv_part("b", 0, 0, 1)
            qkv_part("c", 0, 1, 1)
            wait("v1")
            l0 = logit_items("b", True)
            segment((perm_qkv_items(2, 1), range(0, 2 * U8 - 2)),
                    (ln1_out_items(3, 1), range(0, U8)),
                    (l0[:LB], range(B0, B1)))
            qkv_part("b", 1, 0, 1)
            halo("c", "b", 1)
            qkv_part("c", 1, 1, 1)
            qkv_part("b", 2, 0, 1)
            halo("b", None, 2)
            halo("c", "b", 2)
            qkv_part("c", 2, 1, 1)
            wait("wo")
            segment((perm_wo_items(), range(0, WS)),
                    (l0[LB:], range(0, C0)),
                    (pv_items("b"), range(C0 + CP, 39)),
                    (logit_items("c", False), range(C0, C1)),
                    (pv_items("c"), range(C1 + CP, 63)),
                    (logit_items("a", False), range(C1, C2)),
                    (pv_items("a"), range(C2 + CP, 79)),
                    ([functools.partial(halo, "b", "a", 1)], [23]),
                    ([functools.partial(halo, "b", "a", 2)], [39]),
                    (ln1_out_items(NS, 0) + ln1_out_items(NS, 1), range(H0, H1)),
                    (logit_items("b", False), range(C2, 96 - L1)))
            halo("a", "c", 1)
            halo("a", "c", 2)
            for g in range(3):
                qkv_part("a", g, 2, 1)
            for g in range(3):
                qkv_part("b", g, 3, 1)
            wo_mm("b", 0)
            wo_mm("c", TM)
            wo_mm("a", 2 * TM)
            finish()
            wait("x1", "m2")
            start("m3", "w1", "w3", "w2")


        def half(X, Y, u0, sched, row_ln1, row_wo, extra):
            place(sched, pv_items(Y), range(u0 + P0, u0 + 3 * UP - P1))
            place(sched, logit_items(X, False), range(u0 + 2 * UP + L0, u0 + 4 * UP - L1))
            place(sched, ln1_items(row_ln1, Y), range(u0 + N0, u0 + N1))
            place(sched, extra, range(u0, u0 + 4 * UP - 1))

            def run():
                halo(X, Y, 1)
                halo(X, Y, 2)
                for g in range(3):
                    qkv_part(X, g)
                wo_mm(Y, row_wo)
            return run

        def a_step(s, carry):
            @pl.when(s == 3)
            def _():
                wait("x2", "m3")

            ra = pl.multiple_of(2 * s * TM, TM)
            nxt = pl.multiple_of(jnp.minimum(ra + 2 * TM, S - TM), TM)
            col0 = pl.multiple_of(jnp.minimum(2 * D + (s - 2) * (MT * 128), 6 * D - MT * 128), 128)
            mi = mod_items(col0, MT)
            sched = {}
            run_a = half("a", "b", 0, sched, ra + TM, ra - TM, mi[:len(mi) // 2])
            run_b = half("b", "a", 4 * UP, sched, nxt, ra, mi[len(mi) // 2:])
            begin(sched)
            run_a()
            run_b()
            finish()
            return carry

        with jax.named_scope("aloop"):
            jax.lax.fori_loop(NS // 2, NB // 2, a_step, 0)

        with jax.named_scope("atail"):
            begin({})

            def post0(r):
                x1 = x1_rows(r, LG, 0, D)
                mu = jnp.mean(x1, axis=-1, keepdims=True)
                d = x1 - mu
                rs = jax.lax.rsqrt(jnp.mean(d * d, axis=-1, keepdims=True) + EPS)
                y = (d * rs).reshape(LG // 8, 8, D) * mod(4, 0, D)[None] + mod(3, 0, D)[None]
                h2_v[r // 2:(r + LG) // 2, :] = pltpu.bitcast(y.reshape(LG, D).astype(BF16), U32)
            post = [functools.partial(post0, r) for r in range(0, TMB, LG)]
            pv = pv_items("b")
            run_now(pv[:NC])
            segment((pv[NC:], range(0, UP - 2)), (post, range(TP0, 2 * UP - TE)))
            wo_mm("b", S - TM, 0, TM // 2)
            wo_mm("b", S - TM, TM // 2, TM)
            finish()
            wait("w1", "w3", "w2")

        def b_step(j, carry):
            row0 = pl.multiple_of(j * TMB, TMB)
            nxt = pl.multiple_of(jnp.minimum(row0 + TMB, S - TMB), TMB)
            if SKIP_FFN:
                obuf[pl.ds(row0, TMB), :] = x1_rows(row0, TMB, 0, D).astype(BF16)
                for q in range(NQ):
                    cp_out(j, q).start()
            else:
                ffn(j, row0, nxt)
            return carry

        with jax.named_scope("bloop"):
            jax.lax.fori_loop(0, NBB, b_step, 0)
        with jax.named_scope("tail"):
            for j in range(NBB):
                for q in range(NQ):
                    cp_out(j, q).wait()

    any_spec = pl.BlockSpec(memory_space=pl.ANY)
    qkv_set = [
        pltpu.VMEM((2 * NC, KV, 128), F32),
        pltpu.VMEM((NC, KV, 128), F32),
        pltpu.VMEM((WIN + 1, TM, 128), F32),
    ]
    scratch = [
        pltpu.VMEM((S, D), BF16),
        pltpu.VMEM((D, 3 * D), BF16),
        pltpu.VMEM((NC, KH // 2, 128), U32),
        pltpu.VMEM((D // 2, 3 * D), U32),
        pltpu.VMEM((D, D), BF16),
        pltpu.VMEM((NC, D // 32 * 17, 128), U32),
        pltpu.VMEM((D // 2, D), U32),
        pltpu.VMEM((D, F), BF16),
        pltpu.VMEM((D, F), BF16),
        pltpu.VMEM((F, D), BF16),
        pltpu.VMEM((D, 6 * D), BF16),
        pltpu.VMEM((D, 128), F32),
        pltpu.VMEM((MT, NSUB, 8, 128), F32),
        pltpu.VMEM((8, 6 * D), F32),
        pltpu.VMEM((8, 2 * D), F32),
        pltpu.VMEM((TM // 2, D), U32),
        pltpu.VMEM((TM // 2, D), U32),
        pltpu.VMEM((NS, TM // 2, D), U32),
        pltpu.VMEM((NS, 3 * NC, TM, 128), F32),
        pltpu.VMEM((2, (NS + 1) * TM, 128), F32),
        *qkv_set, *qkv_set, *qkv_set,
        *[pltpu.VMEM((TM // 2, D), U32)] * 3,
        *[pltpu.VMEM((NC, RG, 128), F32)] * 3,
        *[pltpu.VMEM((WIN, RG, 128), F32)] * 3,
        pltpu.VMEM((2, TM, 128), F32),
        pltpu.VMEM((2, TMB, 128), F32),
        pltpu.VMEM((S, D), F32),
        pltpu.VMEM((TMB, D), F32),
        pltpu.VMEM((TMB // 2, D), U32),
        pltpu.VMEM((TMB // 2, F), U32),
        pltpu.VMEM((S, D), BF16),
        pltpu.VMEM((1, D), BF16),
        pltpu.SMEM((1,), jnp.int32),
        pltpu.SemaphoreType.DMA((NDMA,)),
        pltpu.SemaphoreType.DMA((NBB * NQ,)),
    ]

    def call(A_x, A_wqkv, A_wo, B_w1, B_w3, B_w2, c, w_mod):
        return pl.pallas_call(
            kernel,
            out_shape=jax.ShapeDtypeStruct((1, S, D), BF16),
            in_specs=[any_spec] * 8,
            out_specs=any_spec,
            scratch_shapes=scratch,
            compiler_params=pltpu.CompilerParams(
                vmem_limit_bytes=120 * 1024 * 1024,
                disable_semaphore_checks=True, disable_bounds_checks=True),
        )(A_x, A_wqkv, A_wo, B_w1, B_w3, B_w2, c, w_mod)

    return call


@jax.jit
def pallas_adaLN_cond__sliding_local_dilated__glu_gated_swiglu__prompt_kernel(
    A_x: jax.Array,
    A_wqkv: jax.Array,
    A_wo: jax.Array,
    B_x: jax.Array,
    B_w1: jax.Array,
    B_w3: jax.Array,
    B_w2: jax.Array,
    c: jax.Array,
    w_mod: jax.Array,
):
    del B_x
    return _build()(A_x, A_wqkv, A_wo, B_w1, B_w3, B_w2, c, w_mod)
```

```python
import functools
import math

import jax
import jax.numpy as jnp
import jax.experimental.pallas as pl
import jax.experimental.pallas.tpu as pltpu

S = 2048
D = 1024
F = 3584
H = 32
DH = D // H
WIN = 8
DIL = 2
NC = D // 128
HALO = 16
EPS = 1e-5
NEG = -1000000000.0
SM_SCALE = DH ** -0.5
LOG2E = math.log2(math.e)

TM = 128
NB = S // TM
KV = HALO + TM
RG = 8
LG = 16
NS = 6
NDMA = 28
KP = (0, 256, 512, 1024)
KH = 512

F32 = jnp.float32
BF16 = jnp.bfloat16
U32 = jnp.uint32


def _tree(op, xs):
    xs = list(xs)
    while len(xs) > 1:
        xs = [op(xs[i], xs[i + 1]) if i + 1 < len(xs) else xs[i] for i in range(0, len(xs), 2)]
    return xs[0]


def _add(a, b):
    return a + b


def _fold(op, x):
    while x.shape[0] > 1:
        x = x.reshape(x.shape[0] // 2, 2, *x.shape[1:])
        x = op(x[:, 0], x[:, 1])
    return x[0]


def _lane_gather(x, idx):
    dn = jax.lax.GatherDimensionNumbers(
        offset_dims=(), collapsed_slice_dims=(1,), start_index_map=(1,),
        operand_batching_dims=(0,), start_indices_batching_dims=(0,))
    return jax.lax.gather(x, idx[..., None], dn, (1, 1), mode=jax.lax.GatherScatterMode.PROMISE_IN_BOUNDS)


def _build(TMB=256, FC=512, OCUT=(0, 512, 896, 1024),
           MT=7, NSUB=16, MLAG=8, PR=32, SPREAD=128, SLAG=5,
           P0=1, P1=16, L0=0, L1=0, N0=0, N1=30, PB1=5, TP0=10, TE=3,
           X0=2, X1=3, X2=6, X3=2, A2=7, A3=5, A4=10, A5=11, A6=6, KB=4, F0=11, F1=8,
           E0=14, E1=29, LB=5, WS=54, O0=0, O1=70, G0=134, G1=140, H0=150, H1=182,
           LW=(20, 48, 78, 108, 134, 184), PW=((21, 47), (49, 87), (87, 127), (115, 151), (140, 167)),
           SKIP_FFN=False):
    NBB = S // TMB
    NQ = len(OCUT) - 1

    def kernel(x_hbm, wqkv_hbm, wo_hbm, w1_hbm, w3_hbm, w2_hbm, c_hbm, wmod_hbm,
               out_hbm,
               x_v, wqkv_v, wtmp, wqkv_p, wo_v, wo_tmp, wo_p, w1_v, w3_v, w2_v,
               wmod_v, cb_v, modp_v, modb_v, mod_v,
               h1a, h1b, h1s, part, stats, qka, va, pa, qkb, vb, pb_, qkc, vc, pc,
               oa, ob, oc, sl0, sl1, sl2, sl3, sl4, stat1, stat2,
               y_v, x1n, h2_v, act_v, obuf, c_ref, zs, sem_w, sem_o):
        bufs = {"a": (h1a, qka, va, oa, pa), "b": (h1b, qkb, vb, ob, pb_),
                "c": (None, qkc, vc, oc, pc)}

        free_sl, held = [sl0, sl1, sl2, sl3, sl4], {}

        dmas = {}

        def add_dma(name, src, dst):
            dmas[name] = (src, dst, len(dmas))

        for name, (b0, b1) in (("x0", (0, 2)), ("x23", (2, 4)), ("x45", (4, 6)), ("x6", (6, 7)),
                               ("x1", (7, 9)), ("x2", (9, NB))):
            rows = pl.ds(b0 * TM, (b1 - b0) * TM)
            add_dma(name, x_hbm.at[0, rows, :], x_v.at[rows, :])
        for k in range(3):
            for j, name in enumerate(("sa", "ca")):
                cols = pl.ds(j * D + KP[k], KP[k + 1] - KP[k])
                add_dma(name + str(k), wmod_hbm.at[:, cols], wmod_v.at[:, cols])
            for g in range(3):
                rows, cols = pl.ds(KP[k], KP[k + 1] - KP[k]), pl.ds(g * D, D)
                add_dma("qkv"[g] + str(k), wqkv_hbm.at[rows, cols], wqkv_v.at[rows, cols])
        for name, (c0, c1) in (("m2", (2 * D, 3 * D)), ("m3", (3 * D, 6 * D))):
            cols = pl.ds(c0, c1 - c0)
            add_dma(name, wmod_hbm.at[:, cols], wmod_v.at[:, cols])
        add_dma("c", c_hbm, c_ref)
        add_dma("wo", wo_hbm, wo_v)
        add_dma("w1", w1_hbm, w1_v)
        add_dma("w3", w3_hbm, w3_v)
        add_dma("w2", w2_hbm, w2_v)
        assert len(dmas) == NDMA

        def cp(name):
            src, dst, i = dmas[name]
            return pltpu.make_async_copy(src, dst, sem_w.at[i])

        def start(*names):
            for n in names:
                cp(n).start()

        def wait(*names):
            for n in names:
                cp(n).wait()

        def cp_out(j, q):
            rows, cols = pl.ds(j * TMB, TMB), pl.ds(OCUT[q], OCUT[q + 1] - OCUT[q])
            return pltpu.make_async_copy(obuf.at[rows, cols], out_hbm.at[0, rows, cols], sem_o.at[j * NQ + q])

        st = {"z": None, "never": None, "clock": 0, "sched": {}, "tok": None}

        have = set()

        def need(*keys):
            assert all(k in have for k in keys), keys

        def finish():
            assert not st["sched"], "items placed beyond the last unit"

        def begin(sched):
            finish()
            z = zs[0]
            st.update(z=(0, z, 2 * z), never=jnp.full((8, 128), z, jnp.int32) != 0, clock=0, sched=sched, tok=None)

        def gate(val, i, n):
            r = st["tok"]
            if r is None:
                return val
            row = (i * min(SPREAD, r.shape[0]) // n) // 8 * 8
            t = r[row:row + 8, 0:128]
            return jax.lax.select(st["never"], t if val.dtype == F32 else pltpu.bitcast(t, val.dtype), val)

        def place(sched, items, units):
            units = list(units)
            for i, it in enumerate(items):
                sched.setdefault(units[(i * len(units)) // len(items)], []).append(it)

        def matmul(lhs_fn, w_fn, ks, cols, sink, gives=None):
            for n0 in cols:
                r = None
                for k in ks:
                    d = jnp.dot(lhs_fn(k), w_fn(k, n0), preferred_element_type=F32)
                    r = d if r is None else r + d
                    if k == ks[-1]:
                        sink(n0, r)
                    if n0 == cols[-1] and k == ks[-1]:
                        have.add(gives)
                    st["tok"] = r
                    for fn in st["sched"].pop(st["clock"], []):
                        fn()
                    st["tok"] = None
                    st["clock"] += 1

        def lane_iota(rows):
            return jax.lax.broadcasted_iota(jnp.int32, (rows, 128), 1)

        def ld16(ref, r0, n, c0, c1):
            return pltpu.bitcast(ref[r0 // 2:(r0 + n) // 2, c0:c1], BF16)

        def silu_c():
            cf = c_ref[...].astype(F32)
            return (cf * jax.nn.sigmoid(cf)).astype(BF16)

        def mod_mxu(j, k):
            cs = slice(j * D + KP[k], j * D + KP[k + 1])
            lhs = jnp.broadcast_to(silu_c(), (16, D))
            mod_v[:, cs] = jnp.dot(lhs, wmod_v[:, cs], preferred_element_type=F32)[0:8] + float(j == 1)

        def mod(j, c0, c1):
            return (mod_v if j < 2 else modb_v)[:, j * D + c0:j * D + c1]

        def mod_items(col0, ntiles):
            rows = D // NSUB

            def col(t):
                c0 = col0 + t * 128
                return c0 if isinstance(c0, int) else pl.multiple_of(c0, 128)

            def part_sum(t, i):
                w = wmod_v[i * rows:(i + 1) * rows, pl.ds(col(t), 128)].astype(F32)
                p = (w * cb_v[i * rows:(i + 1) * rows, :]).reshape(rows // 8, 8, 128)
                modp_v[t, i] = gate(_fold(_add, p), 1, 2)

            def total(t):
                r = gate(_fold(_add, modp_v[t, pl.ds(zrow(0), NSUB)]), 0, 1)
                one = jnp.where((col(t) // D) % 3 == 1, 1.0, 0.0).astype(F32)
                dst = mod_v if isinstance(col0, int) else modb_v
                dst[:, pl.ds(col(t), 128)] = jnp.broadcast_to(jnp.sum(r, axis=0, keepdims=True) + one, (8, 128))
            items = []
            for t in range(ntiles + 1):
                for i in range(NSUB):
                    if t < ntiles:
                        items.append(functools.partial(part_sum, t, i))
                    if t > 0 and i == (MLAG if t < ntiles else 0):
                        items.append(functools.partial(total, t - 1))
            return items

        def perm_mix(g, i, nrows, row0):
            n = nrows // 2
            l = jnp.concatenate([gate(lane_iota(8), h, n) for h in range(0, n, 8)], axis=0)
            w = pltpu.bitcast(wqkv_v[i * nrows:(i + 1) * nrows, g * D:(g + 1) * D], U32)
            vals = [w[:, c * 128:(c + 1) * 128] for c in range(NC)]
            for b in range(3):
                m = (l & (4 << b)) == 0
                for c in range(NC):
                    if c & (1 << b):
                        continue
                    lo, hi = vals[c], vals[c | (1 << b)]
                    vals[c] = jax.lax.select(m, lo, hi)
                    vals[c | (1 << b)] = jax.lax.select(m, hi, lo)
            wtmp[:, pl.ds(pl.multiple_of(zrow(i * n - row0), 8), n), :] = jnp.stack(vals)

        def perm_gather(g, k, j):
            have.add(("w", g, k, j))
            l = lane_iota(8)
            idx = ((((l >> 1) & 3) << 5) | ((((l >> 3) & 7) ^ j) << 2) | ((l >> 6) << 1) | (l & 1))
            n = (KP[k + 1] - KP[k]) // 2
            idx = jnp.concatenate([gate(idx, 0, 1)] * (n // 8), axis=0)
            wqkv_p[KP[k] // 2:KP[k + 1] // 2, g * D + j * 128: g * D + (j + 1) * 128] = _lane_gather(wtmp[j, 0:n], idx)

        def perm_qkv_items(g, k, nrows=PR):
            return ([functools.partial(perm_mix, g, i, nrows, KP[k] // 2) for i in range(KP[k] // nrows, KP[k + 1] // nrows)]
                    + [functools.partial(perm_gather, g, k, j) for j in range(NC)])

        def perm_wo_items():
            sub = jax.lax.broadcasted_iota(jnp.int32, (8, 128), 0)

            def spread(c, h):
                for r in range(h * 256, h * 256 + 256, 8):
                    wo_tmp[c, pl.ds(zrow(r + r // 16), 8), :] = gate(pltpu.bitcast(
                        wo_v[2 * r:2 * r + 16, c * 128:(c + 1) * 128], U32), r % 256, 256)

            def gather(c, h):
                for G in range(h * 32, h * 32 + 32):
                    j, e, ch = G >> 3, (G >> 2) & 1, G & 3
                    dd = (((2 * ch) ^ j) << 1) | e
                    ta = wo_tmp[c, pl.ds(ch * 136 + dd, 8, stride=17), :]
                    tb = wo_tmp[c, pl.ds(ch * 136 + (dd ^ 2), 8, stride=17), :]
                    wo_p[G * 8:G * 8 + 8, c * 128:(c + 1) * 128] = jax.lax.select(gate(sub, G % 32, 32) < 4, ta, tb)
            return [functools.partial(fn, c, h) for fn in (spread, gather) for c in range(NC) for h in range(2)]

        def zrow(row, k=1):
            return row if k == 0 else row + st["z"][k]

        def gate16(v, i, n):
            return jnp.concatenate([gate(v[q:q + 8], i, n) for q in range(0, LG, 8)], axis=0)

        def staged(stages, n, lag):
            items = []
            for t in range(n + lag * (len(stages) - 1)):
                for k in reversed(range(len(stages))):
                    if 0 <= t - k * lag < n:
                        items.append(functools.partial(stages[k], t - k * lag))
            return items

        def ln_stages(load, stat, dst, j_scale, j_shift, cols=(0, KH, D)):
            def chunks(x):
                return [x[:, c * 128:(c + 1) * 128] for c in range(NC)]

            def put(j, r, part, fn):
                m = jnp.sum(part, axis=-1, keepdims=True) * (1.0 / D)
                stat[j, pl.ds(pl.multiple_of(zrow(r), LG), LG), :] = jnp.broadcast_to(fn(m), (LG, 128))

            def s_mean(i):
                put(0, i * LG, gate16(_tree(_add, chunks(load(i * LG, 0))), 1, 2), lambda m: m)

            def s_var(i):
                r = i * LG
                d = load(r, 1) - jnp.concatenate([gate16(stat[0, r:r + LG, :], 0, 1)] * NC, axis=1)
                put(1, r, _tree(_add, chunks(d * d)), lambda m: jax.lax.rsqrt(m + EPS))

            def s_out(i):
                r = i * LG
                x = load(r, 2)
                for c0, c1 in zip(cols[:-1], cols[1:]):
                    nrep = (c1 - c0) // 128
                    mu = jnp.concatenate([stat[0, r:r + LG, :]] * nrep, axis=1)
                    rs = jnp.concatenate([gate16(stat[1, r:r + LG, :], c0 - cols[0], D)] * nrep, axis=1)
                    y = ((x[:, c0:c1] - mu) * rs).reshape(LG // 8, 8, c1 - c0)
                    y = y * mod(j_scale, c0, c1)[None] + mod(j_shift, c0, c1)[None]
                    dst[r // 2:(r + LG) // 2, c0:c1] = pltpu.bitcast(y.reshape(LG, c1 - c0).astype(BF16), U32)
            return s_mean, s_var, s_out

        def load_x(row0):
            return lambda r, k: x_v[pl.ds(pl.multiple_of(zrow(row0 + r, k), LG), LG), :].astype(F32)

        def ln1_items(row0, buf):
            return staged(ln_stages(load_x(row0), stat1, bufs[buf][0], 1, 0), TM // LG, 1)

        def ln1_start(b, k):
            return ln_stages(load_x(b * TM), stats.at[:, pl.ds(b * TM, TM), :], h1s.at[b] if b < NS else h1a,
                             1, 0, KP[k:k + 2] if b < NS else (k * KH, (k + 1) * KH))

        def stats_items(b, with_out):
            def one(i):
                r = b * TM + i * LG
                rows = pl.ds(r if isinstance(r, int) else pl.multiple_of(r, LG), LG)
                xf = x_v[rows, :].astype(F32)
                part = gate16(_tree(_add, [xf[:, c * 128:(c + 1) * 128] for c in range(NC)]), 0, 1)
                mu = jnp.sum(part, axis=-1, keepdims=True) * (1.0 / D)
                d = xf - mu
                rs = jax.lax.rsqrt(jnp.mean(d * d, axis=-1, keepdims=True) + EPS)
                stats[0, rows, :] = jnp.broadcast_to(mu, (LG, 128))
                stats[1, rows, :] = jnp.broadcast_to(rs, (LG, 128))
                if with_out:
                    have.add(("h", b, 0, i))
                    k1 = KP[1]
                    y = (d[:, :k1] * rs).reshape(LG // 8, 8, k1) * mod(1, 0, k1)[None] + mod(0, 0, k1)[None]
                    h1s[b, i * LG // 2:(i + 1) * LG // 2, 0:k1] = pltpu.bitcast(y.reshape(LG, k1).astype(BF16), U32)
            return [functools.partial(one, i) for i in range(TM // LG)]

        def ln1_out_items(b, k):
            def one(i):
                have.add(("h", b, k, i))
                ln1_start(b, k)[2](i)
            return [functools.partial(one, i) for i in range(TM // LG)]

        def x1_rows(row, n, c0, c1):
            xf = x_v[pl.ds(row, n), c0:c1].astype(F32).reshape(n // 8, 8, c1 - c0)
            y = y_v[pl.ds(row, n), c0:c1].reshape(n // 8, 8, c1 - c0)
            ga = jnp.concatenate([gate(mod(2, c, c + 128), c - c0, 2 * D) for c in range(c0, c1, 128)], axis=1)
            return (xf + ga[None] * y).reshape(n, c1 - c0)

        def post_items(row0):
            def load(r, k):
                if k:
                    return x1n[pl.ds(pl.multiple_of(zrow(r, k), LG), LG), :]
                x1 = x1_rows(row0 + r, LG, 0, D)
                x1n[r:r + LG, :] = x1
                return x1
            return staged(ln_stages(load, stat2, h2_v, 4, 3), TMB // LG, 1)

        def logit_items(buf, first):
            _, qk, _, _, pb = bufs[buf]
            swap = lane_iota(RG) ^ 1

            def s_logit(g):
                need(("q", buf), ("k", buf))
                have.add(("l", buf, g))
                sl = held[buf, g] = free_sl.pop(0)
                r = g * RG
                q = qk[0:NC, HALO + r:HALO + r + RG, :]
                dst = pl.ds(pl.multiple_of(zrow(0), RG), RG)
                for w in range(WIN):
                    k0 = zrow(HALO + r - DIL * w, int(w >= WIN // 2))
                    s = gate(_fold(_add, q * qk[NC:2 * NC, pl.ds(k0, RG), :]), w, WIN)
                    s = s + pltpu.roll(s, 64, 1)
                    s = s + _lane_gather(s, swap)
                    if first and r < DIL * w:
                        pos = r + jax.lax.broadcasted_iota(jnp.int32, (RG, 128), 0)
                        s = jnp.where(pos >= DIL * w, s, NEG * LOG2E)
                    sl[w, dst, :] = s

            def s_soft(g):
                assert ("p", buf, g) not in have
                sl = held.pop((buf, g))
                free_sl.append(sl)
                have.add(("p", buf, g))
                r = g * RG
                s = sl[...]
                e = jnp.exp2(s - gate(_fold(jnp.maximum, s), 0, 1)[None])
                pb[0:WIN, r:r + RG, :] = e
                den = _fold(_add, e)
                inv = pl.reciprocal(den, approx=True)
                pb[WIN, r:r + RG, :] = inv * (2.0 - den * inv)
            return [[functools.partial(fn, g) for g in range(TM // RG)] for fn in (s_logit, s_soft)]

        def logit_plan(items, u0, u1, g0=0, g1=TM // RG, s0=None, s1=None):
            lg, sm = items
            s0, s1 = g0 if s0 is None else s0, g1 if s1 is None else s1
            n = g1 - g0
            pos = [u0 + (i * (u1 - SLAG - u0)) // n for i in range(n)]
            plan = [([sm[g]], [pos[g - g0] + SLAG if g >= g0 else u0]) for g in range(s0, s1)]
            return plan + [([lg[g]], [pos[g - g0]]) for g in range(g0, g1)]

        def pv_items(buf):
            _, _, vp, o, pb = bufs[buf]
            hc = NC // 2

            def one(r, h):
                need(("v", buf), ("p", buf, r // RG), ("p", buf, r // RG + 1))
                if h:
                    have.difference_update({("p", buf, r // RG), ("p", buf, r // RG + 1)})
                    have.update({("o", buf, r // RG), ("o", buf, r // RG + 1)})
                vs = {d: vp[h * hc:(h + 1) * hc, pl.ds(zrow(HALO + r + d, int(d <= -RG)), RG), :]
                      for d in range(RG, -DIL * WIN, -DIL)}
                accs = []
                for q in (0, RG):
                    p = pb[:, pl.ds(pl.multiple_of(zrow(r + q, 1 + h), RG), RG), :]
                    accs.append(_tree(_add, [p[w:w + 1] * vs[q - DIL * w] for w in range(WIN)]) * p[WIN:])
                both = jnp.concatenate([
                    jnp.concatenate([gate(accs[i][c], 2 * c + i, NC) for c in range(hc)], axis=1)
                    for i in range(2)], axis=0)
                o[r // 2:r // 2 + RG, h * KH:(h + 1) * KH] = pltpu.bitcast(both.astype(BF16), U32)
            return [functools.partial(one, r, h) for r in range(0, TM, 2 * RG) for h in range(2)]

        def halo(buf, prev, part):
            c0 = NC if part == 1 else 0
            ref = bufs[buf][part]
            if prev is None:
                val = (jnp.zeros((NC, HALO, 128), F32) if part == 1
                       else jnp.broadcast_to(ref[:, HALO:HALO + 1, :], (NC, HALO, 128)))
            else:
                val = bufs[prev][part][c0:c0 + NC, TM:TM + HALO, :]
                if st["tok"] is not None:
                    val = jnp.stack([gate16(val[c], 1, 2) for c in range(NC)])
            ref[c0:c0 + NC, 0:HALO, :] = val

        def qkv_part(buf, g, sb=None, k=None):
            h1, qk, vp, _, _ = bufs[buf] if buf else (None,) * 5
            if sb is not None:
                h1 = h1s.at[sb]
                need(*[("h", sb, k, i) for i in range(TM // LG)])
            if k in (None, 2):
                for i in range(TM // RG):
                    if g < 2 and ("qk"[g], buf) in have:
                        need(("l", buf, i))
                    if g == 2 and ("v", buf) in have:
                        assert ("p", buf, i) not in have or ("new", buf) in have
                if g == 1:
                    have.difference_update({("l", buf, i) for i in range(TM // RG)})
                    have.add(("new", buf))
                have.discard(("qkv"[g], buf))

            def sink(n0, r):
                for cc in range(r.shape[1] // 128):
                    ch, rc = n0 // 128 + cc, r[:, cc * 128:(cc + 1) * 128]
                    if k in (1, 2):
                        rc = rc + part[sb, ch]
                    if k in (0, 1):
                        part[sb, ch] = rc
                        continue
                    dst, ci = (qk, ch) if ch < 2 * NC else (vp, ch - 2 * NC)
                    dst[ci, HALO:HALO + TM, :] = rc * (SM_SCALE * LOG2E) if ch < NC else rc

            kr = ((0, KH), (KH, D)) if k is None else (KP[k:k + 2],)
            nw = 128 * KH // (kr[0][1] - kr[0][0])

            def weights(kk, n0):
                if k is not None:
                    need(*[("w", g, k, j) for j in range(n0 % D // 128, (n0 % D + nw) // 128)])
                return ld16(wqkv_p, kk[0], kk[1] - kk[0], n0, n0 + nw)
            matmul(lambda kk: ld16(h1, 0, TM, kk[0], kk[1]), weights, kr, range(g * D, (g + 1) * D, nw), sink,
                   ("qkv"[g], buf) if k in (None, 2) else None)
            if g == 2:
                have.discard(("new", buf))

        def wo_mm(buf, row0, m0=0, m1=TM):
            o = bufs[buf][3]
            need(*[("o", buf, i) for i in range(m0 // RG, m1 // RG)])
            have.difference_update({("o", buf, i) for i in range(m0 // RG, m1 // RG)})

            def sink(n0, r):
                y_v[pl.ds(row0 + m0, m1 - m0), n0:n0 + 128] = r
            matmul(lambda k: ld16(o, m0, m1 - m0, k * KH, (k + 1) * KH),
                   lambda k, n0: ld16(wo_p, k * KH, KH, n0, n0 + 128),
                   (0, 1), range(0, D, 128), sink)

        UP = NC * (D // KH)

        def run_now(items):
            for fn in items:
                fn()

        def ffn(j, row0, nxt_row):
            h = ld16(h2_v, 0, TMB, 0, D)
            for f0 in range(0, F, FC):
                g = jnp.dot(h, w1_v[:, f0:f0 + FC], preferred_element_type=F32)
                u = jnp.dot(h, w3_v[:, f0:f0 + FC], preferred_element_type=F32)
                act_v[:, f0:f0 + FC] = pltpu.bitcast((g * jax.nn.sigmoid(g) * u).astype(BF16), U32)
            nk = F // KH
            sched = {}
            place(sched, post_items(nxt_row), range(0, NC * nk - PB1))
            begin(sched)

            def sink(n0, r):
                z = (mod(5, n0, n0 + 128)[None] * r.reshape(TMB // 8, 8, 128)).reshape(TMB, 128)
                obuf[pl.ds(row0, TMB), n0:n0 + 128] = (x1_rows(row0, TMB, n0, n0 + 128) + z).astype(BF16)
                if n0 + 128 in OCUT:
                    cp_out(j, OCUT.index(n0 + 128) - 1).start()
            matmul(lambda k: ld16(act_v, 0, TMB, k * KH, (k + 1) * KH),
                   lambda k, n0: w2_v[k * KH:(k + 1) * KH, n0:n0 + 128],
                   tuple(range(nk)), range(0, D, 128), sink)
            finish()

        def segment(*placements, sparse=()):
            sched = {}
            for items, units in placements:
                place(sched, items, units)
            busy = {u for u, its in sched.items() if any(getattr(i, "func", i).__name__ == "s_logit" for i in its)}
            for items, units in sparse:
                free = [u for u in units if u not in busy]
                free = free if len(free) >= len(items) else list(units)
                for i, it in enumerate(items):
                    u = free[(i * len(free)) // len(items)]
                    sched.setdefault(u, []).append(it)
                    busy.add(u)
            begin(sched)

        def parts(k, *gb):
            for g, b in gb:
                qkv_part(None if k < 2 else sets[b], g, b, k)

        def outs(k, *bs):
            return [it for b in bs for it in ln1_out_items(b, k)]

        def at(u, fn, *args):
            return [functools.partial(fn, *args)], [u]

        sets = "cabcab"
        with jax.named_scope("prologue"):
            zs[0] = 0
            begin({})
            start("c", "x0", "ca0", "q0", "sa0", "x23", "k0", "v0", "x45", "ca1", "sa1", "q1", "k1", "v1",
                  "ca2", "sa2", "q2", "k2", "v2", "x6", "wo", "x1", "m2")
            wait("c")
            cb_v[...] = jnp.broadcast_to(silu_c().astype(F32), (128, D)).T
            wait("x0")

            def stats_body(b, carry):
                run_now(stats_items(b, False))
                return carry
            jax.lax.fori_loop(0, 2, stats_body, 0)
            wait("ca0")
            mod_mxu(1, 0)
            wait("q0")
            run_now(perm_qkv_items(0, 0))
            wait("sa0")
            mod_mxu(0, 0)
            run_now(outs(0, 0))

        with jax.named_scope("pass1"):
            segment((outs(0, 1), range(0, 4)))
            parts(0, (0, 0))
            wait("x23")
            segment((stats_items(2, True), range(0, X0)), (stats_items(3, True), range(X1, X2)))
            parts(0, (0, 1), (0, 2))
            wait("k0")
            segment((perm_qkv_items(1, 0), range(0, X3)))
            parts(0, (0, 3), (1, 0), (1, 1))
            wait("v0")
            segment((perm_qkv_items(2, 0), range(0, A2)))
            parts(0, (1, 2), (1, 3), (2, 0), (2, 1))
            wait("x45")
            segment((stats_items(4, True), range(0, A3)), (stats_items(5, True), range(A3, A4)))
            parts(0, (2, 2), (2, 3), (0, 4), (0, 5))
            wait("ca1", "sa1", "q1")
            segment((mod_items(D + KP[1], 2) + mod_items(KP[1], 2), range(0, A5)),
                    (perm_qkv_items(0, 1), range(A6, 15)),
                    (outs(1, 0), range(A5 + 1, 16)))
            parts(0, (1, 4), (1, 5), (2, 4), (2, 5))
            wait("k1", "v1")
            segment((outs(1, 1), range(0, 3)), (outs(1, 2, 3, 4, 5), range(3, 18)),
                    (perm_qkv_items(1, 1), range(0, 16)),
                    (perm_qkv_items(2, 1), range(16, 34)))
            parts(1, *[(0, b) for b in range(NS)], *[(1, b) for b in range(KB)])
            wait("ca2", "sa2", "q2")
            nu = 4 * (2 * NS - KB)
            segment((mod_items(D + KP[2], 4), range(0, F0)),
                    (mod_items(KP[2], 4), range(F0, 2 * F0)),
                    (perm_qkv_items(0, 2), range(F1, nu - 2)),
                    (outs(2, 0, 1), range(2 * F0 + 1, nu)))
            parts(1, *[(1, b) for b in range(KB, NS)], *[(2, b) for b in range(NS)])

        with jax.named_scope("pass2"):
            wait("k2", "v2")
            l0 = logit_items("c", True)
            segment((perm_qkv_items(1, 2), range(0, E0)),
                    (perm_qkv_items(2, 2), range(E0, E1)),
                    (outs(2, 2, 3), range(16, 38)),
                    at(24, halo, "a", "c", 1),
                    *logit_plan(l0, E1, 40, 0, LB))
            halo("c", None, 1)
            parts(2, (0, 0), (0, 1), (1, 0), (1, 1), (2, 0))
            halo("c", None, 2)
            halo("a", "c", 2)
            wait("x6", "wo")
            start("x2", "m3", "w1", "w3", "w2")
            plan = [(perm_wo_items(), range(0, WS)), *logit_plan(l0, 0, LW[0], LB),
                    (stats_items(NS, False), range(G0, G1)),
                    ]
            sparse = []
            for b in range(1, NS):
                plan += logit_plan(logit_items(sets[b], False), LW[b - 1] - (SLAG - 1) * (b < NS - 1), LW[b])
            for b in range(NS - 1):
                sparse.append((pv_items(sets[b]), range(*PW[b])))
            for b, u in zip(range(2, NS), (8, 32, 72, 112)):
                plan.append(at(u - 1, halo, sets[b], sets[b - 1], 1))
                plan.append(at(u + 15, halo, sets[b], sets[b - 1], 2))
            sparse += [(outs(2, 4, 5), range(O0, O1)), (ln1_out_items(NS, 0) + ln1_out_items(NS, 1), range(H0, H1))]
            segment(*plan, sparse=sparse)
            parts(2, (2, 1), (0, 2), (1, 2), (2, 2))
            for b in range(3, NS):
                parts(2, (0, b), (1, b), (2, b))
                wo_mm(sets[b - 3], (b - 3) * TM)
            wo_mm(sets[NS - 3], (NS - 3) * TM)
            wo_mm(sets[NS - 2], (NS - 2) * TM)
            finish()
            wait("x1", "m2")


        def half(X, Y, u0, sched, row_ln1, row_wo, extra):
            place(sched, pv_items(Y), range(u0 + P0, u0 + 3 * UP - P1))
            for items, units in logit_plan(logit_items(X, False), u0 + 2 * UP + L0, u0 + 4 * UP - L1):
                place(sched, items, units)
            place(sched, ln1_items(row_ln1, Y), range(u0 + N0, u0 + N1))
            place(sched, extra, range(u0, u0 + 4 * UP - 1))

            def run():
                halo(X, Y, 1)
                halo(X, Y, 2)
                for g in range(3):
                    qkv_part(X, g)
                wo_mm(Y, row_wo)
            return run

        def a_step(s, carry):
            @pl.when(s == NS // 2 + 1)
            def _():
                wait("x2", "m3")

            ra = pl.multiple_of(2 * s * TM, TM)
            nxt = pl.multiple_of(jnp.minimum(ra + 2 * TM, S - TM), TM)
            col0 = pl.multiple_of(jnp.minimum(2 * D + (s - NS // 2) * (MT * 128), 6 * D - MT * 128), 128)
            mi = mod_items(col0, MT)
            sched = {}
            run_a = half("a", "b", 0, sched, ra + TM, ra - TM, mi[:len(mi) // 2])
            run_b = half("b", "a", 4 * UP, sched, nxt, ra, mi[len(mi) // 2:])
            begin(sched)
            run_a()
            run_b()
            finish()
            return carry

        with jax.named_scope("aloop"):
            jax.lax.fori_loop(NS // 2, NB // 2, a_step, 0)

        with jax.named_scope("atail"):
            begin({})

            def post0(r):
                x1 = x1_rows(r, LG, 0, D)
                mu = jnp.mean(x1, axis=-1, keepdims=True)
                d = x1 - mu
                rs = jax.lax.rsqrt(jnp.mean(d * d, axis=-1, keepdims=True) + EPS)
                y = (d * rs).reshape(LG // 8, 8, D) * mod(4, 0, D)[None] + mod(3, 0, D)[None]
                h2_v[r // 2:(r + LG) // 2, :] = pltpu.bitcast(y.reshape(LG, D).astype(BF16), U32)
            post = [functools.partial(post0, r) for r in range(0, TMB, LG)]
            pv = pv_items("b")
            run_now(pv[:NC])
            segment((pv[NC:], range(0, UP - 2)), (post, range(TP0, 2 * UP - TE)))
            wo_mm("b", S - TM, 0, TM // 2)
            wo_mm("b", S - TM, TM // 2, TM)
            finish()
            wait("w1", "w3", "w2")

        def b_step(j, carry):
            row0 = pl.multiple_of(j * TMB, TMB)
            nxt = pl.multiple_of(jnp.minimum(row0 + TMB, S - TMB), TMB)
            if SKIP_FFN:
                obuf[pl.ds(row0, TMB), :] = x1_rows(row0, TMB, 0, D).astype(BF16)
                for q in range(NQ):
                    cp_out(j, q).start()
            else:
                ffn(j, row0, nxt)
            return carry

        with jax.named_scope("bloop"):
            jax.lax.fori_loop(0, NBB, b_step, 0)
        with jax.named_scope("tail"):
            for j in range(NBB):
                for q in range(NQ):
                    cp_out(j, q).wait()

    any_spec = pl.BlockSpec(memory_space=pl.ANY)
    qkv_set = [
        pltpu.VMEM((2 * NC, KV, 128), F32),
        pltpu.VMEM((NC, KV, 128), F32),
        pltpu.VMEM((WIN + 1, TM, 128), F32),
    ]
    scratch = [
        pltpu.VMEM((S, D), BF16),
        pltpu.VMEM((D, 3 * D), BF16),
        pltpu.VMEM((NC, KH // 2, 128), U32),
        pltpu.VMEM((D // 2, 3 * D), U32),
        pltpu.VMEM((D, D), BF16),
        pltpu.VMEM((NC, D // 32 * 17, 128), U32),
        pltpu.VMEM((D // 2, D), U32),
        pltpu.VMEM((D, F), BF16),
        pltpu.VMEM((D, F), BF16),
        pltpu.VMEM((F, D), BF16),
        pltpu.VMEM((D, 6 * D), BF16),
        pltpu.VMEM((D, 128), F32),
        pltpu.VMEM((MT, NSUB, 8, 128), F32),
        pltpu.VMEM((8, 6 * D), F32),
        pltpu.VMEM((8, 2 * D), F32),
        pltpu.VMEM((TM // 2, D), U32),
        pltpu.VMEM((TM // 2, D), U32),
        pltpu.VMEM((NS, TM // 2, D), U32),
        pltpu.VMEM((NS, 3 * NC, TM, 128), F32),
        pltpu.VMEM((2, (NS + 1) * TM, 128), F32),
        *qkv_set, *qkv_set, *qkv_set,
        *[pltpu.VMEM((TM // 2, D), U32)] * 3,
        *[pltpu.VMEM((WIN, RG, 128), F32)] * 5,
        pltpu.VMEM((2, TM, 128), F32),
        pltpu.VMEM((2, TMB, 128), F32),
        pltpu.VMEM((S, D), F32),
        pltpu.VMEM((TMB, D), F32),
        pltpu.VMEM((TMB // 2, D), U32),
        pltpu.VMEM((TMB // 2, F), U32),
        pltpu.VMEM((S, D), BF16),
        pltpu.VMEM((1, D), BF16),
        pltpu.SMEM((1,), jnp.int32),
        pltpu.SemaphoreType.DMA((NDMA,)),
        pltpu.SemaphoreType.DMA((NBB * NQ,)),
    ]

    def call(A_x, A_wqkv, A_wo, B_w1, B_w3, B_w2, c, w_mod):
        return pl.pallas_call(
            kernel,
            out_shape=jax.ShapeDtypeStruct((1, S, D), BF16),
            in_specs=[any_spec] * 8,
            out_specs=any_spec,
            scratch_shapes=scratch,
            compiler_params=pltpu.CompilerParams(
                vmem_limit_bytes=120 * 1024 * 1024,
                disable_semaphore_checks=True, disable_bounds_checks=True),
        )(A_x, A_wqkv, A_wo, B_w1, B_w3, B_w2, c, w_mod)

    return call


@jax.jit
def pallas_adaLN_cond__sliding_local_dilated__glu_gated_swiglu__prompt_kernel(
    A_x: jax.Array,
    A_wqkv: jax.Array,
    A_wo: jax.Array,
    B_x: jax.Array,
    B_w1: jax.Array,
    B_w3: jax.Array,
    B_w2: jax.Array,
    c: jax.Array,
    w_mod: jax.Array,
):
    del B_x
    return _build()(A_x, A_wqkv, A_wo, B_w1, B_w3, B_w2, c, w_mod)
```

```python
import functools
import math

import jax
import jax.numpy as jnp
import jax.experimental.pallas as pl
import jax.experimental.pallas.tpu as pltpu

S = 2048
D = 1024
F = 3584
H = 32
DH = D // H
WIN = 8
DIL = 2
NC = D // 128
HALO = 16
EPS = 1e-5
NEG = -1000000000.0
SM_SCALE = DH ** -0.5
LOG2E = math.log2(math.e)

TM = 128
NB = S // TM
KV = HALO + TM
RG = 8
LG = 16
NS = 6
NDMA = 27
KP = (0, 256, 512, 1024)
KH = 512

F32 = jnp.float32
BF16 = jnp.bfloat16
U32 = jnp.uint32


def _tree(op, xs):
    xs = list(xs)
    while len(xs) > 1:
        xs = [op(xs[i], xs[i + 1]) if i + 1 < len(xs) else xs[i] for i in range(0, len(xs), 2)]
    return xs[0]


def _add(a, b):
    return a + b


def _fold(op, x):
    while x.shape[0] > 1:
        x = x.reshape(x.shape[0] // 2, 2, *x.shape[1:])
        x = op(x[:, 0], x[:, 1])
    return x[0]


def _lane_gather(x, idx):
    dn = jax.lax.GatherDimensionNumbers(
        offset_dims=(), collapsed_slice_dims=(1,), start_index_map=(1,),
        operand_batching_dims=(0,), start_indices_batching_dims=(0,))
    return jax.lax.gather(x, idx[..., None], dn, (1, 1), mode=jax.lax.GatherScatterMode.PROMISE_IN_BOUNDS)


def _build(TMB=256, FC=512, OCUT=(0, 512, 896, 1024),
           MT=7, NSUB=16, MLAG=8, PR=32, SPREAD=128, SLAG=5,
           P0=1, P1=16, L0=0, L1=0, N0=0, N1=30, PB1=5, TP0=10, TE=3,
           X0=2, X1=3, X2=6, X3=2, A2=7, A3=5, A4=10, A5=11, A6=6, KB=4, F0=11, F1=8,
           E0=14, E1=29, LB=5, WS=54, O0=0, O1=70, G0=134, G1=140, H0=150, H1=182,
           LW=(20, 48, 78, 108, 134, 184), PW=((21, 47), (49, 87), (87, 127), (115, 151), (140, 167)),
           XM=1, MU=80, SKIP_FFN=False):
    NBB = S // TMB
    NQ = len(OCUT) - 1

    def kernel(x_hbm, wqkv_hbm, wo_hbm, w1_hbm, w3_hbm, w2_hbm, c_hbm, wmod_hbm,
               out_hbm,
               x_v, wqkv_v, wtmp, wqkv_p, wo_v, wo_tmp, wo_p, w1_v, w3_v, w2_v,
               wmod_v, wst_v, cb_v, modp_v, modb_v, mod_v,
               h1a, h1b, h1s, part, stats, qka, va, pa, qkb, vb, pb_, qkc, vc, pc,
               oa, ob, oc, sl0, sl1, sl2, sl3, sl4, stat1, stat2,
               y_v, x1n, h2_v, act_v, obuf, c_ref, zs, sem_w, sem_o):
        bufs = {"a": (h1a, qka, va, oa, pa), "b": (h1b, qkb, vb, ob, pb_),
                "c": (None, qkc, vc, oc, pc)}

        free_sl, held = [sl0, sl1, sl2, sl3, sl4], {}

        dmas = {}

        def add_dma(name, src, dst):
            dmas[name] = (src, dst, len(dmas))

        for name, (b0, b1) in (("x0", (0, 2)), ("x23", (2, 4)), ("x45", (4, 6)), ("x6", (6, 7)),
                               ("x1", (7, 9)), ("x2", (9, NB))):
            rows = pl.ds(b0 * TM, (b1 - b0) * TM)
            add_dma(name, x_hbm.at[0, rows, :], x_v.at[rows, :])
        for k in range(3):
            for j, name in enumerate(("sa", "ca")):
                cols = pl.ds(j * D + KP[k], KP[k + 1] - KP[k])
                add_dma(name + str(k), wmod_hbm.at[:, cols], wmod_v.at[:, cols])
            for g in range(3):
                rows, cols = pl.ds(KP[k], KP[k + 1] - KP[k]), pl.ds(g * D, D)
                add_dma("qkv"[g] + str(k), wqkv_hbm.at[rows, cols], wqkv_v.at[rows, cols])
        add_dma("c", c_hbm, c_ref)
        add_dma("wo", wo_hbm, wo_v)
        add_dma("w1", w1_hbm, w1_v)
        assert len(dmas) == NDMA - 3

        def cp_quarter(s):
            i = jnp.minimum(s - NS // 2, 3)
            cps = []
            for k, (src, dst) in enumerate(((w3_hbm, w3_v), (w2_hbm, w2_v))):
                n = src.shape[0] // 4
                rows = pl.ds(pl.multiple_of(i * n, n), n)
                cps.append(pltpu.make_async_copy(src.at[rows, :], dst.at[rows, :], sem_w.at[NDMA - 3 + k]))
            return cps

        def mod_col(s):
            c = jnp.minimum(2 * D + (s - NS // 2) * (MT * 128), 6 * D - MT * 128)
            return pl.multiple_of(c, 128)

        def cp_stage(s):
            return pltpu.make_async_copy(wmod_hbm.at[:, pl.ds(mod_col(s), MT * 128)],
                                         wst_v.at[:, pl.ds(0, MT * 128)], sem_w.at[NDMA - 1])

        def cp(name):
            src, dst, i = dmas[name]
            return pltpu.make_async_copy(src, dst, sem_w.at[i])

        def start(*names):
            for n in names:
                cp(n).start()

        def wait(*names):
            for n in names:
                cp(n).wait()

        def cp_out(j, q):
            rows, cols = pl.ds(j * TMB, TMB), pl.ds(OCUT[q], OCUT[q + 1] - OCUT[q])
            return pltpu.make_async_copy(obuf.at[rows, cols], out_hbm.at[0, rows, cols], sem_o.at[j * NQ + q])

        st = {"z": None, "never": None, "clock": 0, "sched": {}, "tok": None}

        have = set()

        def need(*keys):
            assert all(k in have for k in keys), keys

        def finish():
            assert not st["sched"], "items placed beyond the last unit"

        def begin(sched):
            finish()
            z = zs[0]
            st.update(z=(0, z, 2 * z), never=jnp.full((8, 128), z, jnp.int32) != 0, clock=0, sched=sched, tok=None)

        def gate(val, i, n):
            r = st["tok"]
            if r is None:
                return val
            row = (i * min(SPREAD, r.shape[0]) // n) // 8 * 8
            t = r[row:row + 8, 0:128]
            return jax.lax.select(st["never"], t if val.dtype == F32 else pltpu.bitcast(t, val.dtype), val)

        def place(sched, items, units):
            units = list(units)
            for i, it in enumerate(items):
                sched.setdefault(units[(i * len(units)) // len(items)], []).append(it)

        def matmul(lhs_fn, w_fn, ks, cols, sink, gives=None):
            for n0 in cols:
                r = None
                for k in ks:
                    d = jnp.dot(lhs_fn(k), w_fn(k, n0), preferred_element_type=F32)
                    r = d if r is None else r + d
                    if k == ks[-1]:
                        sink(n0, r)
                    if n0 == cols[-1] and k == ks[-1]:
                        have.add(gives)
                    st["tok"] = r
                    for fn in st["sched"].pop(st["clock"], []):
                        fn()
                    st["tok"] = None
                    st["clock"] += 1

        def lane_iota(rows):
            return jax.lax.broadcasted_iota(jnp.int32, (rows, 128), 1)

        def ld16(ref, r0, n, c0, c1):
            return pltpu.bitcast(ref[r0 // 2:(r0 + n) // 2, c0:c1], BF16)

        def silu_c():
            cf = c_ref[...].astype(F32)
            return (cf * jax.nn.sigmoid(cf)).astype(BF16)

        def mod_mxu(j, k):
            cs = slice(j * D + KP[k], j * D + KP[k + 1])
            lhs = jnp.broadcast_to(silu_c(), (16, D))
            mod_v[:, cs] = jnp.dot(lhs, wmod_v[:, cs], preferred_element_type=F32)[0:8] + float(j == 1)

        def mod(j, c0, c1):
            return (mod_v if j < 2 else modb_v)[:, j * D + c0:j * D + c1]

        def mod_items(col0, ntiles):
            rows = D // NSUB

            def col(t):
                c0 = col0 + t * 128
                return c0 if isinstance(c0, int) else pl.multiple_of(c0, 128)

            def part_sum(t, i):
                src, c0 = (wmod_v, col(t)) if isinstance(col0, int) else (wst_v, t * 128)
                w = src[i * rows:(i + 1) * rows, c0:c0 + 128].astype(F32)
                p = (w * cb_v[i * rows:(i + 1) * rows, :]).reshape(rows // 8, 8, 128)
                modp_v[t, i] = gate(_fold(_add, p), 1, 2)

            def total(t):
                r = gate(_fold(_add, modp_v[t, pl.ds(zrow(0), NSUB)]), 0, 1)
                one = jnp.where((col(t) // D) % 3 == 1, 1.0, 0.0).astype(F32)
                dst = mod_v if isinstance(col0, int) else modb_v
                dst[:, pl.ds(col(t), 128)] = jnp.broadcast_to(jnp.sum(r, axis=0, keepdims=True) + one, (8, 128))
            items = []
            for t in range(ntiles + 1):
                for i in range(NSUB):
                    if t < ntiles:
                        items.append(functools.partial(part_sum, t, i))
                    if t > 0 and i == (MLAG if t < ntiles else 0):
                        items.append(functools.partial(total, t - 1))
            return items

        def perm_mix(g, i, nrows, row0):
            n = nrows // 2
            l = jnp.concatenate([gate(lane_iota(8), h, n) for h in range(0, n, 8)], axis=0)
            w = pltpu.bitcast(wqkv_v[i * nrows:(i + 1) * nrows, g * D:(g + 1) * D], U32)
            vals = [w[:, c * 128:(c + 1) * 128] for c in range(NC)]
            for b in range(3):
                m = (l & (4 << b)) == 0
                for c in range(NC):
                    if c & (1 << b):
                        continue
                    lo, hi = vals[c], vals[c | (1 << b)]
                    vals[c] = jax.lax.select(m, lo, hi)
                    vals[c | (1 << b)] = jax.lax.select(m, hi, lo)
            wtmp[:, pl.ds(pl.multiple_of(zrow(i * n - row0), 8), n), :] = jnp.stack(vals)

        def perm_gather(g, k, j):
            have.add(("w", g, k, j))
            l = lane_iota(8)
            idx = ((((l >> 1) & 3) << 5) | ((((l >> 3) & 7) ^ j) << 2) | ((l >> 6) << 1) | (l & 1))
            n = (KP[k + 1] - KP[k]) // 2
            idx = jnp.concatenate([gate(idx, 0, 1)] * (n // 8), axis=0)
            wqkv_p[KP[k] // 2:KP[k + 1] // 2, g * D + j * 128: g * D + (j + 1) * 128] = _lane_gather(wtmp[j, 0:n], idx)

        def perm_qkv_items(g, k, nrows=PR):
            return ([functools.partial(perm_mix, g, i, nrows, KP[k] // 2) for i in range(KP[k] // nrows, KP[k + 1] // nrows)]
                    + [functools.partial(perm_gather, g, k, j) for j in range(NC)])

        def perm_wo_items():
            sub = jax.lax.broadcasted_iota(jnp.int32, (8, 128), 0)

            def spread(c, h):
                for r in range(h * 256, h * 256 + 256, 8):
                    wo_tmp[c, pl.ds(zrow(r + r // 16), 8), :] = gate(pltpu.bitcast(
                        wo_v[2 * r:2 * r + 16, c * 128:(c + 1) * 128], U32), r % 256, 256)

            def gather(c, h):
                for G in range(h * 32, h * 32 + 32):
                    j, e, ch = G >> 3, (G >> 2) & 1, G & 3
                    dd = (((2 * ch) ^ j) << 1) | e
                    ta = wo_tmp[c, pl.ds(ch * 136 + dd, 8, stride=17), :]
                    tb = wo_tmp[c, pl.ds(ch * 136 + (dd ^ 2), 8, stride=17), :]
                    wo_p[G * 8:G * 8 + 8, c * 128:(c + 1) * 128] = jax.lax.select(gate(sub, G % 32, 32) < 4, ta, tb)
            return [functools.partial(fn, c, h) for fn in (spread, gather) for c in range(NC) for h in range(2)]

        def zrow(row, k=1):
            return row if k == 0 else row + st["z"][k]

        def gate16(v, i, n):
            return jnp.concatenate([gate(v[q:q + 8], i, n) for q in range(0, LG, 8)], axis=0)

        def staged(stages, n, lag):
            items = []
            for t in range(n + lag * (len(stages) - 1)):
                for k in reversed(range(len(stages))):
                    if 0 <= t - k * lag < n:
                        items.append(functools.partial(stages[k], t - k * lag))
            return items

        def ln_stages(load, stat, dst, j_scale, j_shift, cols=(0, KH, D)):
            def chunks(x):
                return [x[:, c * 128:(c + 1) * 128] for c in range(NC)]

            def put(j, r, part, fn):
                m = jnp.sum(part, axis=-1, keepdims=True) * (1.0 / D)
                stat[j, pl.ds(pl.multiple_of(zrow(r), LG), LG), :] = jnp.broadcast_to(fn(m), (LG, 128))

            def s_mean(i):
                part = gate16(_tree(_add, chunks(load(i * LG, 0))), 1, 2)
                if "pull" in st:
                    part = jnp.concatenate([jax.lax.select(st["never"], st.pop("pull"), part[0:8]), part[8:]], axis=0)
                put(0, i * LG, part, lambda m: m)

            def s_var(i):
                r = i * LG
                d = load(r, 1) - jnp.concatenate([gate16(stat[0, r:r + LG, :], 0, 1)] * NC, axis=1)
                put(1, r, _tree(_add, chunks(d * d)), lambda m: jax.lax.rsqrt(m + EPS))

            def s_out(i):
                r = i * LG
                x = load(r, 2)
                for c0, c1 in zip(cols[:-1], cols[1:]):
                    nrep = (c1 - c0) // 128
                    mu = jnp.concatenate([stat[0, r:r + LG, :]] * nrep, axis=1)
                    rs = jnp.concatenate([gate16(stat[1, r:r + LG, :], c0 - cols[0], D)] * nrep, axis=1)
                    y = ((x[:, c0:c1] - mu) * rs).reshape(LG // 8, 8, c1 - c0)
                    y = y * mod(j_scale, c0, c1)[None] + mod(j_shift, c0, c1)[None]
                    dst[r // 2:(r + LG) // 2, c0:c1] = pltpu.bitcast(y.reshape(LG, c1 - c0).astype(BF16), U32)
            return s_mean, s_var, s_out

        def load_x(row0):
            return lambda r, k: x_v[pl.ds(pl.multiple_of(zrow(row0 + r, k), LG), LG), :].astype(F32)

        def ln1_items(row0, buf):
            return staged(ln_stages(load_x(row0), stat1, bufs[buf][0], 1, 0), TM // LG, 1)

        def ln1_start(b, k):
            return ln_stages(load_x(b * TM), stats.at[:, pl.ds(b * TM, TM), :], h1s.at[b] if b < NS else h1a,
                             1, 0, KP[k:k + 2] if b < NS else (k * KH, (k + 1) * KH))

        def stats_items(b, with_out):
            def one(i):
                r = b * TM + i * LG
                rows = pl.ds(r if isinstance(r, int) else pl.multiple_of(r, LG), LG)
                xf = x_v[rows, :].astype(F32)
                part = gate16(_tree(_add, [xf[:, c * 128:(c + 1) * 128] for c in range(NC)]), 0, 1)
                mu = jnp.sum(part, axis=-1, keepdims=True) * (1.0 / D)
                d = xf - mu
                rs = jax.lax.rsqrt(jnp.mean(d * d, axis=-1, keepdims=True) + EPS)
                stats[0, rows, :] = jnp.broadcast_to(mu, (LG, 128))
                stats[1, rows, :] = jnp.broadcast_to(rs, (LG, 128))
                if with_out:
                    have.add(("h", b, 0, i))
                    k1 = KP[1]
                    y = (d[:, :k1] * rs).reshape(LG // 8, 8, k1) * mod(1, 0, k1)[None] + mod(0, 0, k1)[None]
                    h1s[b, i * LG // 2:(i + 1) * LG // 2, 0:k1] = pltpu.bitcast(y.reshape(LG, k1).astype(BF16), U32)
            return [functools.partial(one, i) for i in range(TM // LG)]

        def ln1_out_items(b, k):
            def one(i):
                have.add(("h", b, k, i))
                ln1_start(b, k)[2](i)
            return [functools.partial(one, i) for i in range(TM // LG)]

        def x1_rows(row, n, c0, c1):
            xf = x_v[pl.ds(row, n), c0:c1].astype(F32).reshape(n // 8, 8, c1 - c0)
            y = y_v[pl.ds(row, n), c0:c1].reshape(n // 8, 8, c1 - c0)
            ga = jnp.concatenate([gate(mod(2, c, c + 128), c - c0, 2 * D) for c in range(c0, c1, 128)], axis=1)
            return (xf + ga[None] * y).reshape(n, c1 - c0)

        def post_items(row0):
            def load(r, k):
                if k:
                    return x1n[pl.ds(pl.multiple_of(zrow(r, k), LG), LG), :]
                x1 = x1_rows(row0 + r, LG, 0, D)
                x1n[r:r + LG, :] = x1
                return x1
            return staged(ln_stages(load, stat2, h2_v, 4, 3), TMB // LG, 1)

        def logit_items(buf, first):
            _, qk, _, _, pb = bufs[buf]
            swap = lane_iota(RG) ^ 1
            even = (lane_iota(RG) & 1) == 0

            def s_logit(g):
                need(("q", buf), ("k", buf))
                have.add(("l", buf, g))
                sl = held[buf, g] = free_sl.pop(0)
                r = g * RG
                q = qk[0:NC, HALO + r:HALO + r + RG, :]
                dst = pl.ds(pl.multiple_of(zrow(0), RG), RG)
                for w in range(WIN):
                    k0 = zrow(HALO + r - DIL * w, int(w >= WIN // 2))
                    s = gate(_fold(_add, q * qk[NC:2 * NC, pl.ds(k0, RG), :]), w, WIN)
                    if XM == 2:
                        s = s + _lane_gather(s, swap)
                    s = s + pltpu.roll(s, 64, 1)
                    if XM == 0:
                        s = s + _lane_gather(s, swap)
                    elif XM == 1:
                        s = s + jax.lax.select(even, pltpu.roll(s, 127, 1), pltpu.roll(s, 1, 1))
                    if first and r < DIL * w:
                        pos = r + jax.lax.broadcasted_iota(jnp.int32, (RG, 128), 0)
                        s = jnp.where(pos >= DIL * w, s, NEG * LOG2E)
                    sl[w, dst, :] = s

            def s_soft(g):
                assert ("p", buf, g) not in have
                sl = held.pop((buf, g))
                free_sl.append(sl)
                have.add(("p", buf, g))
                r = g * RG
                s = sl[...]
                e = jnp.exp2(s - gate(_fold(jnp.maximum, s), 0, 1)[None])
                pb[0:WIN, r:r + RG, :] = e
                den = _fold(_add, e)
                inv = pl.reciprocal(den, approx=True)
                pb[WIN, r:r + RG, :] = inv * (2.0 - den * inv)
            return [[functools.partial(fn, g) for g in range(TM // RG)] for fn in (s_logit, s_soft)]

        def logit_plan(items, u0, u1, g0=0, g1=TM // RG, s0=None, s1=None):
            lg, sm = items
            s0, s1 = g0 if s0 is None else s0, g1 if s1 is None else s1
            n = g1 - g0
            pos = [u0 + (i * (u1 - SLAG - u0)) // n for i in range(n)]
            plan = [([sm[g]], [pos[g - g0] + SLAG if g >= g0 else u0]) for g in range(s0, s1)]
            return plan + [([lg[g]], [pos[g - g0]]) for g in range(g0, g1)]

        def pv_items(buf):
            _, _, vp, o, pb = bufs[buf]
            hc = NC // 2

            def one(r, h):
                need(("v", buf), ("p", buf, r // RG), ("p", buf, r // RG + 1))
                if h:
                    have.difference_update({("p", buf, r // RG), ("p", buf, r // RG + 1)})
                    have.update({("o", buf, r // RG), ("o", buf, r // RG + 1)})
                vs = {d: vp[h * hc:(h + 1) * hc, pl.ds(zrow(HALO + r + d, int(d <= -RG)), RG), :]
                      for d in range(RG, -DIL * WIN, -DIL)}
                accs = []
                for q in (0, RG):
                    p = pb[:, pl.ds(pl.multiple_of(zrow(r + q, 1 + h), RG), RG), :]
                    accs.append(_tree(_add, [p[w:w + 1] * vs[q - DIL * w] for w in range(WIN)]) * p[WIN:])
                both = jnp.concatenate([
                    jnp.concatenate([gate(accs[i][c], 2 * c + i, NC) for c in range(hc)], axis=1)
                    for i in range(2)], axis=0)
                o[r // 2:r // 2 + RG, h * KH:(h + 1) * KH] = pltpu.bitcast(both.astype(BF16), U32)
            return [functools.partial(one, r, h) for r in range(0, TM, 2 * RG) for h in range(2)]

        def halo(buf, prev, part):
            c0 = NC if part == 1 else 0
            ref = bufs[buf][part]
            if prev is None:
                val = (jnp.zeros((NC, HALO, 128), F32) if part == 1
                       else jnp.broadcast_to(ref[:, HALO:HALO + 1, :], (NC, HALO, 128)))
            else:
                val = bufs[prev][part][c0:c0 + NC, TM:TM + HALO, :]
                if st["tok"] is not None:
                    val = jnp.stack([gate16(val[c], 1, 2) for c in range(NC)])
            ref[c0:c0 + NC, 0:HALO, :] = val

        def qkv_part(buf, g, sb=None, k=None):
            h1, qk, vp, _, _ = bufs[buf] if buf else (None,) * 5
            if sb is not None:
                h1 = h1s.at[sb]
                need(*[("h", sb, k, i) for i in range(TM // LG)])
            if k in (None, 2):
                for i in range(TM // RG):
                    if g < 2 and ("qk"[g], buf) in have:
                        need(("l", buf, i))
                    if g == 2 and ("v", buf) in have:
                        assert ("p", buf, i) not in have or ("new", buf) in have
                if g == 1:
                    have.difference_update({("l", buf, i) for i in range(TM // RG)})
                    have.add(("new", buf))
                have.discard(("qkv"[g], buf))

            def sink(n0, r):
                for cc in range(r.shape[1] // 128):
                    ch, rc = n0 // 128 + cc, r[:, cc * 128:(cc + 1) * 128]
                    if k in (1, 2):
                        rc = rc + part[sb, ch]
                    if k in (0, 1):
                        part[sb, ch] = rc
                        continue
                    dst, ci = (qk, ch) if ch < 2 * NC else (vp, ch - 2 * NC)
                    dst[ci, HALO:HALO + TM, :] = rc * (SM_SCALE * LOG2E) if ch < NC else rc

            kr = ((0, KH), (KH, D)) if k is None else (KP[k:k + 2],)
            nw = 128 * KH // (kr[0][1] - kr[0][0])

            def weights(kk, n0):
                if k is not None:
                    need(*[("w", g, k, j) for j in range(n0 % D // 128, (n0 % D + nw) // 128)])
                return ld16(wqkv_p, kk[0], kk[1] - kk[0], n0, n0 + nw)
            matmul(lambda kk: ld16(h1, 0, TM, kk[0], kk[1]), weights, kr, range(g * D, (g + 1) * D, nw), sink,
                   ("qkv"[g], buf) if k in (None, 2) else None)
            if g == 2:
                have.discard(("new", buf))

        def wo_mm(buf, row0, m0=0, m1=TM):
            o = bufs[buf][3]
            need(*[("o", buf, i) for i in range(m0 // RG, m1 // RG)])
            have.difference_update({("o", buf, i) for i in range(m0 // RG, m1 // RG)})

            def sink(n0, r):
                y_v[pl.ds(row0 + m0, m1 - m0), n0:n0 + 128] = r
            matmul(lambda k: ld16(o, m0, m1 - m0, k * KH, (k + 1) * KH),
                   lambda k, n0: ld16(wo_p, k * KH, KH, n0, n0 + 128),
                   (0, 1), range(0, D, 128), sink)

        UP = NC * (D // KH)

        def run_now(items):
            for fn in items:
                fn()

        def ffn(j, row0, nxt_row):
            h = ld16(h2_v, 0, TMB, 0, D)
            for f0 in range(0, F, FC):
                g = jnp.dot(h, w1_v[:, f0:f0 + FC], preferred_element_type=F32)
                u = jnp.dot(h, w3_v[:, f0:f0 + FC], preferred_element_type=F32)
                act_v[:, f0:f0 + FC] = pltpu.bitcast((g * jax.nn.sigmoid(g) * u).astype(BF16), U32)
            nk = F // KH
            sched = {}
            place(sched, post_items(nxt_row), range(0, NC * nk - PB1))
            begin(sched)

            def sink(n0, r):
                z = (mod(5, n0, n0 + 128)[None] * r.reshape(TMB // 8, 8, 128)).reshape(TMB, 128)
                obuf[pl.ds(row0, TMB), n0:n0 + 128] = (x1_rows(row0, TMB, n0, n0 + 128) + z).astype(BF16)
                if n0 + 128 in OCUT:
                    cp_out(j, OCUT.index(n0 + 128) - 1).start()
            matmul(lambda k: ld16(act_v, 0, TMB, k * KH, (k + 1) * KH),
                   lambda k, n0: w2_v[k * KH:(k + 1) * KH, n0:n0 + 128],
                   tuple(range(nk)), range(0, D, 128), sink)
            finish()

        def segment(*placements, sparse=()):
            sched = {}
            for items, units in placements:
                place(sched, items, units)
            busy = {u for u, its in sched.items() if any(getattr(i, "func", i).__name__ == "s_logit" for i in its)}
            for items, units in sparse:
                free = [u for u in units if u not in busy]
                free = free if len(free) >= len(items) else list(units)
                for i, it in enumerate(items):
                    u = free[(i * len(free)) // len(items)]
                    sched.setdefault(u, []).append(it)
                    busy.add(u)
            begin(sched)

        def parts(k, *gb):
            for g, b in gb:
                qkv_part(None if k < 2 else sets[b], g, b, k)

        def outs(k, *bs):
            return [it for b in bs for it in ln1_out_items(b, k)]

        def at(u, fn, *args):
            return [functools.partial(fn, *args)], [u]

        sets = "cabcab"
        with jax.named_scope("prologue"):
            zs[0] = 0
            wst_v[0:16, MT * 128:] = jnp.zeros((16, 128), BF16)
            begin({})
            start("c", "x0", "ca0", "q0", "sa0", "x23", "k0", "v0", "x45", "ca1", "sa1", "q1", "k1", "v1",
                  "ca2", "sa2", "q2", "k2", "v2", "x6", "wo", "x1")
            cp_stage(NS // 2).start()
            wait("c")
            cb_v[...] = jnp.broadcast_to(silu_c().astype(F32), (128, D)).T
            wait("x0")

            def stats_body(b, carry):
                run_now(stats_items(b, False))
                return carry
            jax.lax.fori_loop(0, 2, stats_body, 0)
            wait("ca0")
            mod_mxu(1, 0)
            wait("q0")
            run_now(perm_qkv_items(0, 0))
            wait("sa0")
            mod_mxu(0, 0)
            run_now(outs(0, 0))

        with jax.named_scope("pass1"):
            segment((outs(0, 1), range(0, 4)))
            parts(0, (0, 0))
            wait("x23")
            segment((stats_items(2, True), range(0, X0)), (stats_items(3, True), range(X1, X2)))
            parts(0, (0, 1), (0, 2))
            wait("k0")
            segment((perm_qkv_items(1, 0), range(0, X3)))
            parts(0, (0, 3), (1, 0), (1, 1))
            wait("v0")
            segment((perm_qkv_items(2, 0), range(0, A2)))
            parts(0, (1, 2), (1, 3), (2, 0), (2, 1))
            wait("x45")
            segment((stats_items(4, True), range(0, A3)), (stats_items(5, True), range(A3, A4)))
            parts(0, (2, 2), (2, 3), (0, 4), (0, 5))
            wait("ca1", "sa1", "q1")
            segment((mod_items(D + KP[1], 2) + mod_items(KP[1], 2), range(0, A5)),
                    (perm_qkv_items(0, 1), range(A6, 15)),
                    (outs(1, 0), range(A5 + 1, 16)))
            parts(0, (1, 4), (1, 5), (2, 4), (2, 5))
            wait("k1", "v1")
            segment((outs(1, 1), range(0, 3)), (outs(1, 2, 3, 4, 5), range(3, 18)),
                    (perm_qkv_items(1, 1), range(0, 16)),
                    (perm_qkv_items(2, 1), range(16, 34)))
            parts(1, *[(0, b) for b in range(NS)], *[(1, b) for b in range(KB)])
            wait("ca2", "sa2", "q2")
            nu = 4 * (2 * NS - KB)
            segment((mod_items(D + KP[2], 4), range(0, F0)),
                    (mod_items(KP[2], 4), range(F0, 2 * F0)),
                    (perm_qkv_items(0, 2), range(F1, nu - 2)),
                    (outs(2, 0, 1), range(2 * F0 + 1, nu)))
            parts(1, *[(1, b) for b in range(KB, NS)], *[(2, b) for b in range(NS)])

        with jax.named_scope("pass2"):
            wait("k2", "v2")
            l0 = logit_items("c", True)
            segment((perm_qkv_items(1, 2), range(0, E0)),
                    (perm_qkv_items(2, 2), range(E0, E1)),
                    (outs(2, 2, 3), range(16, 38)),
                    at(24, halo, "a", "c", 1),
                    *logit_plan(l0, E1, 40, 0, LB))
            halo("c", None, 1)
            parts(2, (0, 0), (0, 1), (1, 0), (1, 1), (2, 0))
            halo("c", None, 2)
            halo("a", "c", 2)
            start("x2", "w1")
            wait("x6", "wo")
            plan = [(perm_wo_items(), range(0, WS)), *logit_plan(l0, 0, LW[0], LB),
                    (stats_items(NS, False), range(G0, G1)),
                    ]
            sparse = []
            for b in range(1, NS):
                plan += logit_plan(logit_items(sets[b], False), LW[b - 1] - (SLAG - 1) * (b < NS - 1), LW[b])
            for b in range(NS - 1):
                sparse.append((pv_items(sets[b]), range(*PW[b])))
            for b, u in zip(range(2, NS), (8, 32, 72, 112)):
                plan.append(at(u - 1, halo, sets[b], sets[b - 1], 1))
                plan.append(at(u + 15, halo, sets[b], sets[b - 1], 2))
            sparse += [(outs(2, 4, 5), range(O0, O1)), (ln1_out_items(NS, 0) + ln1_out_items(NS, 1), range(H0, H1))]
            segment(*plan, sparse=sparse)
            parts(2, (2, 1), (0, 2), (1, 2), (2, 2))
            for b in range(3, NS):
                parts(2, (0, b), (1, b), (2, b))
                wo_mm(sets[b - 3], (b - 3) * TM)
            wo_mm(sets[NS - 3], (NS - 3) * TM)
            wo_mm(sets[NS - 2], (NS - 2) * TM)
            finish()
            wait("x1", "x2")


        def half(X, Y, u0, sched, row_ln1, row_wo):
            place(sched, pv_items(Y), range(u0 + P0, u0 + 3 * UP - P1))
            for items, units in logit_plan(logit_items(X, False), u0 + 2 * UP + L0, u0 + 4 * UP - L1):
                place(sched, items, units)
            place(sched, ln1_items(row_ln1, Y), range(u0 + N0, u0 + N1))

            def run():
                halo(X, Y, 1)
                halo(X, Y, 2)
                for g in range(3):
                    qkv_part(X, g)
                wo_mm(Y, row_wo)
            return run

        def a_step(s, carry):
            for c in cp_quarter(s):
                c.start()
            cp_stage(s).wait()

            def refill():
                cp_stage(s + 1).start()
                pad = wst_v[0:16, pl.ds(pl.multiple_of(zrow(MT * 128), 128), 128)]
                st["pull"] = pltpu.bitcast(pad, F32)
            ra = pl.multiple_of(2 * s * TM, TM)
            nxt = pl.multiple_of(jnp.minimum(ra + 2 * TM, S - TM), TM)
            sched = {}
            place(sched, mod_items(mod_col(s), MT), range(0, MU))
            place(sched, [refill], [MU + 1])
            run_a = half("a", "b", 0, sched, ra + TM, ra - TM)
            run_b = half("b", "a", 4 * UP, sched, nxt, ra)
            begin(sched)
            run_a()
            run_b()
            finish()
            assert "pull" not in st
            for c in cp_quarter(s):
                c.wait()
            return carry

        with jax.named_scope("aloop"):
            jax.lax.fori_loop(NS // 2, NB // 2, a_step, 0)
            cp_stage(NB // 2).wait()

        with jax.named_scope("atail"):
            begin({})

            def post0(r):
                x1 = x1_rows(r, LG, 0, D)
                mu = jnp.mean(x1, axis=-1, keepdims=True)
                d = x1 - mu
                rs = jax.lax.rsqrt(jnp.mean(d * d, axis=-1, keepdims=True) + EPS)
                y = (d * rs).reshape(LG // 8, 8, D) * mod(4, 0, D)[None] + mod(3, 0, D)[None]
                h2_v[r // 2:(r + LG) // 2, :] = pltpu.bitcast(y.reshape(LG, D).astype(BF16), U32)
            post = [functools.partial(post0, r) for r in range(0, TMB, LG)]
            pv = pv_items("b")
            run_now(pv[:NC])
            segment((pv[NC:], range(0, UP - 2)), (post, range(TP0, 2 * UP - TE)))
            wo_mm("b", S - TM, 0, TM // 2)
            wo_mm("b", S - TM, TM // 2, TM)
            finish()
            wait("w1")

        def b_step(j, carry):
            row0 = pl.multiple_of(j * TMB, TMB)
            nxt = pl.multiple_of(jnp.minimum(row0 + TMB, S - TMB), TMB)
            if SKIP_FFN:
                obuf[pl.ds(row0, TMB), :] = x1_rows(row0, TMB, 0, D).astype(BF16)
                for q in range(NQ):
                    cp_out(j, q).start()
            else:
                ffn(j, row0, nxt)
            return carry

        with jax.named_scope("bloop"):
            jax.lax.fori_loop(0, NBB, b_step, 0)
        with jax.named_scope("tail"):
            for j in range(NBB):
                for q in range(NQ):
                    cp_out(j, q).wait()

    any_spec = pl.BlockSpec(memory_space=pl.ANY)
    qkv_set = [
        pltpu.VMEM((2 * NC, KV, 128), F32),
        pltpu.VMEM((NC, KV, 128), F32),
        pltpu.VMEM((WIN + 1, TM, 128), F32),
    ]
    scratch = [
        pltpu.VMEM((S, D), BF16),
        pltpu.VMEM((D, 3 * D), BF16),
        pltpu.VMEM((NC, KH // 2, 128), U32),
        pltpu.VMEM((D // 2, 3 * D), U32),
        pltpu.VMEM((D, D), BF16),
        pltpu.VMEM((NC, D // 32 * 17, 128), U32),
        pltpu.VMEM((D // 2, D), U32),
        pltpu.VMEM((D, F), BF16),
        pltpu.VMEM((D, F), BF16),
        pltpu.VMEM((F, D), BF16),
        pltpu.VMEM((D, 2 * D + 128), BF16),
        pltpu.VMEM((D, MT * 128 + 128), BF16),
        pltpu.VMEM((D, 128), F32),
        pltpu.VMEM((MT, NSUB, 8, 128), F32),
        pltpu.VMEM((8, 6 * D), F32),
        pltpu.VMEM((8, 2 * D), F32),
        pltpu.VMEM((TM // 2, D), U32),
        pltpu.VMEM((TM // 2, D), U32),
        pltpu.VMEM((NS, TM // 2, D), U32),
        pltpu.VMEM((NS, 3 * NC, TM, 128), F32),
        pltpu.VMEM((2, (NS + 1) * TM, 128), F32),
        *qkv_set, *qkv_set, *qkv_set,
        *[pltpu.VMEM((TM // 2, D), U32)] * 3,
        *[pltpu.VMEM((WIN, RG, 128), F32)] * 5,
        pltpu.VMEM((2, TM, 128), F32),
        pltpu.VMEM((2, TMB, 128), F32),
        pltpu.VMEM((S, D), F32),
        pltpu.VMEM((TMB, D), F32),
        pltpu.VMEM((TMB // 2, D), U32),
        pltpu.VMEM((TMB // 2, F), U32),
        pltpu.VMEM((S, D), BF16),
        pltpu.VMEM((1, D), BF16),
        pltpu.SMEM((1,), jnp.int32),
        pltpu.SemaphoreType.DMA((NDMA,)),
        pltpu.SemaphoreType.DMA((NBB * NQ,)),
    ]

    def call(A_x, A_wqkv, A_wo, B_w1, B_w3, B_w2, c, w_mod):
        return pl.pallas_call(
            kernel,
            out_shape=jax.ShapeDtypeStruct((1, S, D), BF16),
            in_specs=[any_spec] * 8,
            out_specs=any_spec,
            scratch_shapes=scratch,
            compiler_params=pltpu.CompilerParams(
                vmem_limit_bytes=120 * 1024 * 1024,
                disable_semaphore_checks=True, disable_bounds_checks=True),
        )(A_x, A_wqkv, A_wo, B_w1, B_w3, B_w2, c, w_mod)

    return call


@jax.jit
def pallas_adaLN_cond__sliding_local_dilated__glu_gated_swiglu__prompt_kernel(
    A_x: jax.Array,
    A_wqkv: jax.Array,
    A_wo: jax.Array,
    B_x: jax.Array,
    B_w1: jax.Array,
    B_w3: jax.Array,
    B_w2: jax.Array,
    c: jax.Array,
    w_mod: jax.Array,
):
    del B_x
    return _build()(A_x, A_wqkv, A_wo, B_w1, B_w3, B_w2, c, w_mod)
```

```python
import functools
import math

import jax
import jax.numpy as jnp
import jax.experimental.pallas as pl
import jax.experimental.pallas.tpu as pltpu

S = 2048
D = 1024
F = 3584
H = 32
DH = D // H
WIN = 8
DIL = 2
NC = D // 128
HALO = 16
EPS = 1e-5
NEG = -1000000000.0
SM_SCALE = DH ** -0.5
LOG2E = math.log2(math.e)

TM = 128
NB = S // TM
KV = HALO + TM
RG = 8
LG = 16
NS = 6
NDMA = 27
KP = (0, 256, 512, 1024)
KH = 512

F32 = jnp.float32
BF16 = jnp.bfloat16
U32 = jnp.uint32


def _tree(op, xs):
    xs = list(xs)
    while len(xs) > 1:
        xs = [op(xs[i], xs[i + 1]) if i + 1 < len(xs) else xs[i] for i in range(0, len(xs), 2)]
    return xs[0]


def _add(a, b):
    return a + b


def _fold(op, x):
    while x.shape[0] > 1:
        x = x.reshape(x.shape[0] // 2, 2, *x.shape[1:])
        x = op(x[:, 0], x[:, 1])
    return x[0]


def _lane_gather(x, idx):
    dn = jax.lax.GatherDimensionNumbers(
        offset_dims=(), collapsed_slice_dims=(1,), start_index_map=(1,),
        operand_batching_dims=(0,), start_indices_batching_dims=(0,))
    return jax.lax.gather(x, idx[..., None], dn, (1, 1), mode=jax.lax.GatherScatterMode.PROMISE_IN_BOUNDS)


def _build(TMB=256, FC=512, OCUT=(0, 512, 896, 1024),
           MT=7, NSUB=16, MLAG=8, PR=32, SPREAD=128, SLAG=5,
           P0=1, P1=16, L0=0, L1=0, N0=0, N1=30, PB1=5, TP0=10, TE=3,
           X0=2, X1=3, X2=6, X3=2, A2=7, A3=5, A4=10, A5=11, A6=6, KB=5, F0=10, F1=8,
           E0=14, E1=13, LB=5, WS=54, O0=0, O1=70, G0=134, G1=140, H0=150, H1=182,
           LW=(20, 48, 78, 108, 134, 184), PW=((21, 47), (49, 87), (87, 127), (115, 151), (140, 167)),
           XM=1, MU=80, SKIP_FFN=False):
    NBB = S // TMB
    NQ = len(OCUT) - 1

    def kernel(x_hbm, wqkv_hbm, wo_hbm, w1_hbm, w3_hbm, w2_hbm, c_hbm, wmod_hbm,
               out_hbm,
               x_v, wqkv_v, wtmp, wqkv_p, wo_v, wo_tmp, wo_p, w1_v, w3_v, w2_v,
               wmod_v, wst_v, cb_v, modp_v, modb_v, mod_v,
               h1a, h1b, h1s, part, stats, qka, va, pa, qkb, vb, pb_, qkc, vc, pc,
               oa, ob, oc, sl0, sl1, sl2, sl3, sl4, stat1, stat2,
               y_v, x1n, h2_v, act_v, obuf, c_ref, zs, sem_w, sem_o):
        bufs = {"a": (h1a, qka, va, oa, pa), "b": (h1b, qkb, vb, ob, pb_),
                "c": (None, qkc, vc, oc, pc)}

        free_sl, held = [sl0, sl1, sl2, sl3, sl4], {}

        dmas = {}

        def add_dma(name, src, dst):
            dmas[name] = (src, dst, len(dmas))

        for name, (b0, b1) in (("x0", (0, 2)), ("x23", (2, 4)), ("x45", (4, 6)), ("x6", (6, 7)),
                               ("x1", (7, 9)), ("x2", (9, NB))):
            rows = pl.ds(b0 * TM, (b1 - b0) * TM)
            add_dma(name, x_hbm.at[0, rows, :], x_v.at[rows, :])
        for k in range(3):
            for j, name in enumerate(("sa", "ca")):
                cols = pl.ds(j * D + KP[k], KP[k + 1] - KP[k])
                add_dma(name + str(k), wmod_hbm.at[:, cols], wmod_v.at[:, cols])
            for g in range(3):
                rows, cols = pl.ds(KP[k], KP[k + 1] - KP[k]), pl.ds(g * D, D)
                add_dma("qkv"[g] + str(k), wqkv_hbm.at[rows, cols], wqkv_v.at[rows, cols])
        add_dma("c", c_hbm, c_ref)
        add_dma("wo", wo_hbm, wo_v)
        add_dma("w1", w1_hbm, w1_v)
        assert len(dmas) == NDMA - 3

        def cp_quarter(s):
            i = jnp.minimum(s - NS // 2, 3)
            cps = []
            for k, (src, dst) in enumerate(((w3_hbm, w3_v), (w2_hbm, w2_v))):
                n = src.shape[0] // 4
                rows = pl.ds(pl.multiple_of(i * n, n), n)
                cps.append(pltpu.make_async_copy(src.at[rows, :], dst.at[rows, :], sem_w.at[NDMA - 3 + k]))
            return cps

        def mod_col(s):
            c = jnp.minimum(2 * D + (s - NS // 2) * (MT * 128), 6 * D - MT * 128)
            return pl.multiple_of(c, 128)

        def cp_stage(s):
            return pltpu.make_async_copy(wmod_hbm.at[:, pl.ds(mod_col(s), MT * 128)],
                                         wst_v.at[:, pl.ds(0, MT * 128)], sem_w.at[NDMA - 1])

        def cp(name):
            src, dst, i = dmas[name]
            return pltpu.make_async_copy(src, dst, sem_w.at[i])

        def start(*names):
            for n in names:
                cp(n).start()

        def wait(*names):
            for n in names:
                cp(n).wait()

        def cp_out(j, q):
            rows, cols = pl.ds(j * TMB, TMB), pl.ds(OCUT[q], OCUT[q + 1] - OCUT[q])
            return pltpu.make_async_copy(obuf.at[rows, cols], out_hbm.at[0, rows, cols], sem_o.at[j * NQ + q])

        st = {"z": None, "never": None, "clock": 0, "sched": {}, "tok": None}

        have = set()

        def need(*keys):
            assert all(k in have for k in keys), keys

        def finish():
            assert not st["sched"], "items placed beyond the last unit"

        def begin(sched):
            finish()
            z = zs[0]
            st.update(z=(0, z, 2 * z), never=jnp.full((8, 128), z, jnp.int32) != 0, clock=0, sched=sched, tok=None)

        def gate(val, i, n):
            r = st["tok"]
            if r is None:
                return val
            row = (i * min(SPREAD, r.shape[0]) // n) // 8 * 8
            t = r[row:row + 8, 0:128]
            return jax.lax.select(st["never"], t if val.dtype == F32 else pltpu.bitcast(t, val.dtype), val)

        def place(sched, items, units):
            units = list(units)
            for i, it in enumerate(items):
                sched.setdefault(units[(i * len(units)) // len(items)], []).append(it)

        def matmul(lhs_fn, w_fn, ks, cols, sink, gives=None):
            for n0 in cols:
                r = None
                for k in ks:
                    d = jnp.dot(lhs_fn(k), w_fn(k, n0), preferred_element_type=F32)
                    r = d if r is None else r + d
                    if k == ks[-1]:
                        sink(n0, r)
                    if n0 == cols[-1] and k == ks[-1]:
                        have.add(gives)
                    st["tok"] = r
                    for fn in st["sched"].pop(st["clock"], []):
                        fn()
                    st["tok"] = None
                    st["clock"] += 1

        def lane_iota(rows):
            return jax.lax.broadcasted_iota(jnp.int32, (rows, 128), 1)

        def ld16(ref, r0, n, c0, c1):
            return pltpu.bitcast(ref[r0 // 2:(r0 + n) // 2, c0:c1], BF16)

        def silu_c():
            cf = c_ref[...].astype(F32)
            return (cf * jax.nn.sigmoid(cf)).astype(BF16)

        def mod_mxu(j, k):
            cs = slice(j * D + KP[k], j * D + KP[k + 1])
            lhs = jnp.broadcast_to(silu_c(), (16, D))
            mod_v[:, cs] = jnp.dot(lhs, wmod_v[:, cs], preferred_element_type=F32)[0:8] + float(j == 1)

        def mod(j, c0, c1):
            return (mod_v if j < 2 else modb_v)[:, j * D + c0:j * D + c1]

        def mod_items(col0, ntiles):
            rows = D // NSUB

            def col(t):
                c0 = col0 + t * 128
                return c0 if isinstance(c0, int) else pl.multiple_of(c0, 128)

            def part_sum(t, i):
                src, c0 = (wmod_v, col(t)) if isinstance(col0, int) else (wst_v, t * 128)
                w = src[i * rows:(i + 1) * rows, c0:c0 + 128].astype(F32)
                p = (w * cb_v[i * rows:(i + 1) * rows, :]).reshape(rows // 8, 8, 128)
                modp_v[t, i] = gate(_fold(_add, p), 1, 2)

            def total(t):
                r = gate(_fold(_add, modp_v[t, pl.ds(zrow(0), NSUB)]), 0, 1)
                one = jnp.where((col(t) // D) % 3 == 1, 1.0, 0.0).astype(F32)
                dst = mod_v if isinstance(col0, int) else modb_v
                dst[:, pl.ds(col(t), 128)] = jnp.broadcast_to(jnp.sum(r, axis=0, keepdims=True) + one, (8, 128))
            items = []
            for t in range(ntiles + 1):
                for i in range(NSUB):
                    if t < ntiles:
                        items.append(functools.partial(part_sum, t, i))
                    if t > 0 and i == (MLAG if t < ntiles else 0):
                        items.append(functools.partial(total, t - 1))
            return items

        def perm_mix(g, i, nrows, row0):
            n = nrows // 2
            l = jnp.concatenate([gate(lane_iota(8), h, n) for h in range(0, n, 8)], axis=0)
            w = pltpu.bitcast(wqkv_v[i * nrows:(i + 1) * nrows, g * D:(g + 1) * D], U32)
            vals = [w[:, c * 128:(c + 1) * 128] for c in range(NC)]
            for b in range(3):
                m = (l & (4 << b)) == 0
                for c in range(NC):
                    if c & (1 << b):
                        continue
                    lo, hi = vals[c], vals[c | (1 << b)]
                    vals[c] = jax.lax.select(m, lo, hi)
                    vals[c | (1 << b)] = jax.lax.select(m, hi, lo)
            wtmp[:, pl.ds(pl.multiple_of(zrow(i * n - row0), 8), n), :] = jnp.stack(vals)

        def perm_gather(g, k, j):
            have.add(("w", g, k, j))
            l = lane_iota(8)
            idx = ((((l >> 1) & 3) << 5) | ((((l >> 3) & 7) ^ j) << 2) | ((l >> 6) << 1) | (l & 1))
            n = (KP[k + 1] - KP[k]) // 2
            idx = jnp.concatenate([gate(idx, 0, 1)] * (n // 8), axis=0)
            wqkv_p[KP[k] // 2:KP[k + 1] // 2, g * D + j * 128: g * D + (j + 1) * 128] = _lane_gather(wtmp[j, 0:n], idx)

        def perm_qkv_items(g, k, nrows=PR):
            return ([functools.partial(perm_mix, g, i, nrows, KP[k] // 2) for i in range(KP[k] // nrows, KP[k + 1] // nrows)]
                    + [functools.partial(perm_gather, g, k, j) for j in range(NC)])

        def perm_wo_items():
            sub = jax.lax.broadcasted_iota(jnp.int32, (8, 128), 0)

            def spread(c, h):
                for r in range(h * 256, h * 256 + 256, 8):
                    wo_tmp[c, pl.ds(zrow(r + r // 16), 8), :] = gate(pltpu.bitcast(
                        wo_v[2 * r:2 * r + 16, c * 128:(c + 1) * 128], U32), r % 256, 256)

            def gather(c, h):
                for G in range(h * 32, h * 32 + 32):
                    j, e, ch = G >> 3, (G >> 2) & 1, G & 3
                    dd = (((2 * ch) ^ j) << 1) | e
                    ta = wo_tmp[c, pl.ds(ch * 136 + dd, 8, stride=17), :]
                    tb = wo_tmp[c, pl.ds(ch * 136 + (dd ^ 2), 8, stride=17), :]
                    wo_p[G * 8:G * 8 + 8, c * 128:(c + 1) * 128] = jax.lax.select(gate(sub, G % 32, 32) < 4, ta, tb)
            return [functools.partial(fn, c, h) for fn in (spread, gather) for c in range(NC) for h in range(2)]

        def zrow(row, k=1):
            return row if k == 0 else row + st["z"][k]

        def gate16(v, i, n):
            return jnp.concatenate([gate(v[q:q + 8], i, n) for q in range(0, LG, 8)], axis=0)

        def staged(stages, n, lag):
            items = []
            for t in range(n + lag * (len(stages) - 1)):
                for k in reversed(range(len(stages))):
                    if 0 <= t - k * lag < n:
                        items.append(functools.partial(stages[k], t - k * lag))
            return items

        def ln_stages(load, stat, dst, j_scale, j_shift, cols=(0, KH, D)):
            def chunks(x):
                return [x[:, c * 128:(c + 1) * 128] for c in range(NC)]

            def put(j, r, part, fn):
                m = jnp.sum(part, axis=-1, keepdims=True) * (1.0 / D)
                stat[j, pl.ds(pl.multiple_of(zrow(r), LG), LG), :] = jnp.broadcast_to(fn(m), (LG, 128))

            def s_mean(i):
                part = gate16(_tree(_add, chunks(load(i * LG, 0))), 1, 2)
                if "pull" in st:
                    part = jnp.concatenate([jax.lax.select(st["never"], st.pop("pull"), part[0:8]), part[8:]], axis=0)
                put(0, i * LG, part, lambda m: m)

            def s_var(i):
                r = i * LG
                d = load(r, 1) - jnp.concatenate([gate16(stat[0, r:r + LG, :], 0, 1)] * NC, axis=1)
                put(1, r, _tree(_add, chunks(d * d)), lambda m: jax.lax.rsqrt(m + EPS))

            def s_out(i):
                r = i * LG
                x = load(r, 2)
                for c0, c1 in zip(cols[:-1], cols[1:]):
                    nrep = (c1 - c0) // 128
                    mu = jnp.concatenate([stat[0, r:r + LG, :]] * nrep, axis=1)
                    rs = jnp.concatenate([gate16(stat[1, r:r + LG, :], c0 - cols[0], D)] * nrep, axis=1)
                    y = ((x[:, c0:c1] - mu) * rs).reshape(LG // 8, 8, c1 - c0)
                    y = y * mod(j_scale, c0, c1)[None] + mod(j_shift, c0, c1)[None]
                    dst[r // 2:(r + LG) // 2, c0:c1] = pltpu.bitcast(y.reshape(LG, c1 - c0).astype(BF16), U32)
            return s_mean, s_var, s_out

        def load_x(row0):
            return lambda r, k: x_v[pl.ds(pl.multiple_of(zrow(row0 + r, k), LG), LG), :].astype(F32)

        def ln1_items(row0, buf):
            return staged(ln_stages(load_x(row0), stat1, bufs[buf][0], 1, 0), TM // LG, 1)

        def ln1_start(b, k):
            return ln_stages(load_x(b * TM), stats.at[:, pl.ds(b * TM, TM), :], h1s.at[b] if b < NS else h1a,
                             1, 0, KP[k:k + 2] if b < NS else (k * KH, (k + 1) * KH))

        def stats_items(b, with_out):
            def one(i):
                r = b * TM + i * LG
                rows = pl.ds(r if isinstance(r, int) else pl.multiple_of(r, LG), LG)
                xf = x_v[rows, :].astype(F32)
                part = gate16(_tree(_add, [xf[:, c * 128:(c + 1) * 128] for c in range(NC)]), 0, 1)
                mu = jnp.sum(part, axis=-1, keepdims=True) * (1.0 / D)
                d = xf - mu
                rs = jax.lax.rsqrt(jnp.mean(d * d, axis=-1, keepdims=True) + EPS)
                stats[0, rows, :] = jnp.broadcast_to(mu, (LG, 128))
                stats[1, rows, :] = jnp.broadcast_to(rs, (LG, 128))
                if with_out:
                    have.add(("h", b, 0, i))
                    k1 = KP[1]
                    y = (d[:, :k1] * rs).reshape(LG // 8, 8, k1) * mod(1, 0, k1)[None] + mod(0, 0, k1)[None]
                    h1s[b, i * LG // 2:(i + 1) * LG // 2, 0:k1] = pltpu.bitcast(y.reshape(LG, k1).astype(BF16), U32)
            return [functools.partial(one, i) for i in range(TM // LG)]

        def ln1_out_items(b, k):
            def one(i):
                have.add(("h", b, k, i))
                ln1_start(b, k)[2](i)
            return [functools.partial(one, i) for i in range(TM // LG)]

        def x1_rows(row, n, c0, c1):
            xf = x_v[pl.ds(row, n), c0:c1].astype(F32).reshape(n // 8, 8, c1 - c0)
            y = y_v[pl.ds(row, n), c0:c1].reshape(n // 8, 8, c1 - c0)
            ga = jnp.concatenate([gate(mod(2, c, c + 128), c - c0, 2 * D) for c in range(c0, c1, 128)], axis=1)
            return (xf + ga[None] * y).reshape(n, c1 - c0)

        def post_items(row0):
            def load(r, k):
                if k:
                    return x1n[pl.ds(pl.multiple_of(zrow(r, k), LG), LG), :]
                x1 = x1_rows(row0 + r, LG, 0, D)
                x1n[r:r + LG, :] = x1
                return x1
            return staged(ln_stages(load, stat2, h2_v, 4, 3), TMB // LG, 1)

        def logit_items(buf, first):
            _, qk, _, _, pb = bufs[buf]
            swap = lane_iota(RG) ^ 1
            even = (lane_iota(RG) & 1) == 0

            def s_logit(g):
                need(("q", buf), ("k", buf))
                have.add(("l", buf, g))
                sl = held[buf, g] = free_sl.pop(0)
                r = g * RG
                q = qk[0:NC, HALO + r:HALO + r + RG, :]
                dst = pl.ds(pl.multiple_of(zrow(0), RG), RG)
                for w in range(WIN):
                    k0 = zrow(HALO + r - DIL * w, int(w >= WIN // 2))
                    s = gate(_fold(_add, q * qk[NC:2 * NC, pl.ds(k0, RG), :]), w, WIN)
                    if XM == 2:
                        s = s + _lane_gather(s, swap)
                    s = s + pltpu.roll(s, 64, 1)
                    if XM == 0:
                        s = s + _lane_gather(s, swap)
                    elif XM == 1:
                        s = s + jax.lax.select(even, pltpu.roll(s, 127, 1), pltpu.roll(s, 1, 1))
                    if first and r < DIL * w:
                        pos = r + jax.lax.broadcasted_iota(jnp.int32, (RG, 128), 0)
                        s = jnp.where(pos >= DIL * w, s, NEG * LOG2E)
                    sl[w, dst, :] = s

            def s_soft(g):
                assert ("p", buf, g) not in have
                sl = held.pop((buf, g))
                free_sl.append(sl)
                have.add(("p", buf, g))
                r = g * RG
                s = sl[...]
                e = jnp.exp2(s - gate(_fold(jnp.maximum, s), 0, 1)[None])
                pb[0:WIN, r:r + RG, :] = e
                den = _fold(_add, e)
                inv = pl.reciprocal(den, approx=True)
                pb[WIN, r:r + RG, :] = inv * (2.0 - den * inv)
            return [[functools.partial(fn, g) for g in range(TM // RG)] for fn in (s_logit, s_soft)]

        def logit_plan(items, u0, u1, g0=0, g1=TM // RG, s0=None, s1=None):
            lg, sm = items
            s0, s1 = g0 if s0 is None else s0, g1 if s1 is None else s1
            n = g1 - g0
            pos = [u0 + (i * (u1 - SLAG - u0)) // n for i in range(n)]
            plan = [([sm[g]], [pos[g - g0] + SLAG if g >= g0 else u0]) for g in range(s0, s1)]
            return plan + [([lg[g]], [pos[g - g0]]) for g in range(g0, g1)]

        def pv_items(buf):
            _, _, vp, o, pb = bufs[buf]
            hc = NC // 2

            def one(r, h):
                need(("v", buf), ("p", buf, r // RG), ("p", buf, r // RG + 1))
                if h:
                    have.difference_update({("p", buf, r // RG), ("p", buf, r // RG + 1)})
                    have.update({("o", buf, r // RG), ("o", buf, r // RG + 1)})
                vs = {d: vp[h * hc:(h + 1) * hc, pl.ds(zrow(HALO + r + d, int(d <= -RG)), RG), :]
                      for d in range(RG, -DIL * WIN, -DIL)}
                accs = []
                for q in (0, RG):
                    p = pb[:, pl.ds(pl.multiple_of(zrow(r + q, 1 + h), RG), RG), :]
                    accs.append(_tree(_add, [p[w:w + 1] * vs[q - DIL * w] for w in range(WIN)]) * p[WIN:])
                both = jnp.concatenate([
                    jnp.concatenate([gate(accs[i][c], 2 * c + i, NC) for c in range(hc)], axis=1)
                    for i in range(2)], axis=0)
                o[r // 2:r // 2 + RG, h * KH:(h + 1) * KH] = pltpu.bitcast(both.astype(BF16), U32)
            return [functools.partial(one, r, h) for r in range(0, TM, 2 * RG) for h in range(2)]

        def halo(buf, prev, part):
            c0 = NC if part == 1 else 0
            ref = bufs[buf][part]
            if prev is None:
                val = (jnp.zeros((NC, HALO, 128), F32) if part == 1
                       else jnp.broadcast_to(ref[:, HALO:HALO + 1, :], (NC, HALO, 128)))
            else:
                val = bufs[prev][part][c0:c0 + NC, TM:TM + HALO, :]
                if st["tok"] is not None:
                    val = jnp.stack([gate16(val[c], 1, 2) for c in range(NC)])
            ref[c0:c0 + NC, 0:HALO, :] = val

        def qkv_part(buf, g, sb=None, k=None):
            h1, qk, vp, _, _ = bufs[buf] if buf else (None,) * 5
            if sb is not None:
                h1 = h1s.at[sb]
                need(*[("h", sb, k, i) for i in range(TM // LG)])
            if k in (None, 2):
                for i in range(TM // RG):
                    if g < 2 and ("qk"[g], buf) in have:
                        need(("l", buf, i))
                    if g == 2 and ("v", buf) in have:
                        assert ("p", buf, i) not in have or ("new", buf) in have
                if g == 1:
                    have.difference_update({("l", buf, i) for i in range(TM // RG)})
                    have.add(("new", buf))
                have.discard(("qkv"[g], buf))

            def sink(n0, r):
                for cc in range(r.shape[1] // 128):
                    ch, rc = n0 // 128 + cc, r[:, cc * 128:(cc + 1) * 128]
                    if k in (1, 2):
                        rc = rc + part[sb, ch]
                    if k in (0, 1):
                        part[sb, ch] = rc
                        continue
                    dst, ci = (qk, ch) if ch < 2 * NC else (vp, ch - 2 * NC)
                    dst[ci, HALO:HALO + TM, :] = rc * (SM_SCALE * LOG2E) if ch < NC else rc

            kr = ((0, KH), (KH, D)) if k is None else (KP[k:k + 2],)
            nw = 128 * KH // (kr[0][1] - kr[0][0])

            def weights(kk, n0):
                if k is not None:
                    need(*[("w", g, k, j) for j in range(n0 % D // 128, (n0 % D + nw) // 128)])
                return ld16(wqkv_p, kk[0], kk[1] - kk[0], n0, n0 + nw)
            matmul(lambda kk: ld16(h1, 0, TM, kk[0], kk[1]), weights, kr, range(g * D, (g + 1) * D, nw), sink,
                   ("qkv"[g], buf) if k in (None, 2) else None)
            if g == 2:
                have.discard(("new", buf))

        def wo_mm(buf, row0, m0=0, m1=TM):
            o = bufs[buf][3]
            need(*[("o", buf, i) for i in range(m0 // RG, m1 // RG)])
            have.difference_update({("o", buf, i) for i in range(m0 // RG, m1 // RG)})

            def sink(n0, r):
                y_v[pl.ds(row0 + m0, m1 - m0), n0:n0 + 128] = r
            matmul(lambda k: ld16(o, m0, m1 - m0, k * KH, (k + 1) * KH),
                   lambda k, n0: ld16(wo_p, k * KH, KH, n0, n0 + 128),
                   (0, 1), range(0, D, 128), sink)

        UP = NC * (D // KH)

        def run_now(items):
            for fn in items:
                fn()

        def ffn(j, row0, nxt_row):
            h = ld16(h2_v, 0, TMB, 0, D)
            for f0 in range(0, F, FC):
                g = jnp.dot(h, w1_v[:, f0:f0 + FC], preferred_element_type=F32)
                u = jnp.dot(h, w3_v[:, f0:f0 + FC], preferred_element_type=F32)
                act_v[:, f0:f0 + FC] = pltpu.bitcast((g * jax.nn.sigmoid(g) * u).astype(BF16), U32)
            nk = F // KH
            sched = {}
            place(sched, post_items(nxt_row), range(0, NC * nk - PB1))
            begin(sched)

            def sink(n0, r):
                z = (mod(5, n0, n0 + 128)[None] * r.reshape(TMB // 8, 8, 128)).reshape(TMB, 128)
                obuf[pl.ds(row0, TMB), n0:n0 + 128] = (x1_rows(row0, TMB, n0, n0 + 128) + z).astype(BF16)
                if n0 + 128 in OCUT:
                    cp_out(j, OCUT.index(n0 + 128) - 1).start()
            matmul(lambda k: ld16(act_v, 0, TMB, k * KH, (k + 1) * KH),
                   lambda k, n0: w2_v[k * KH:(k + 1) * KH, n0:n0 + 128],
                   tuple(range(nk)), range(0, D, 128), sink)
            finish()

        def segment(*placements, sparse=()):
            sched = {}
            for items, units in placements:
                place(sched, items, units)
            busy = {u for u, its in sched.items() if any(getattr(i, "func", i).__name__ == "s_logit" for i in its)}
            for items, units in sparse:
                free = [u for u in units if u not in busy]
                free = free if len(free) >= len(items) else list(units)
                for i, it in enumerate(items):
                    u = free[(i * len(free)) // len(items)]
                    sched.setdefault(u, []).append(it)
                    busy.add(u)
            begin(sched)

        def parts(k, *gb):
            for g, b in gb:
                qkv_part(None if k < 2 else sets[b], g, b, k)

        def outs(k, *bs):
            return [it for b in bs for it in ln1_out_items(b, k)]

        def at(u, fn, *args):
            return [functools.partial(fn, *args)], [u]

        sets = "cabcab"
        with jax.named_scope("prologue"):
            zs[0] = 0
            wst_v[0:16, MT * 128:] = jnp.zeros((16, 128), BF16)
            begin({})
            start("c", "x0", "ca0", "q0", "sa0", "x23", "k0", "v0", "x45", "ca1", "sa1", "q1", "k1", "v1",
                  "ca2", "sa2", "q2", "k2", "v2", "x6", "wo", "x1")
            cp_stage(NS // 2).start()
            wait("c")
            cb_v[...] = jnp.broadcast_to(silu_c().astype(F32), (128, D)).T
            wait("x0")

            def stats_body(b, carry):
                run_now(stats_items(b, False))
                return carry
            jax.lax.fori_loop(0, 2, stats_body, 0)
            wait("ca0")
            mod_mxu(1, 0)
            wait("q0")
            run_now(perm_qkv_items(0, 0))
            wait("sa0")
            mod_mxu(0, 0)
            run_now(outs(0, 0))

        with jax.named_scope("pass1"):
            segment((outs(0, 1), range(0, 4)))
            parts(0, (0, 0))
            wait("x23")
            segment((stats_items(2, True), range(0, X0)), (stats_items(3, True), range(X1, X2)))
            parts(0, (0, 1), (0, 2))
            wait("k0")
            segment((perm_qkv_items(1, 0), range(0, X3)))
            parts(0, (0, 3), (1, 0), (1, 1))
            wait("v0")
            segment((perm_qkv_items(2, 0), range(0, A2)))
            parts(0, (1, 2), (1, 3), (2, 0), (2, 1))
            wait("x45")
            segment((stats_items(4, True), range(0, A3)), (stats_items(5, True), range(A3, A4)))
            parts(0, (2, 2), (2, 3), (0, 4), (0, 5))
            wait("ca1", "sa1", "q1")
            segment((mod_items(D + KP[1], 2) + mod_items(KP[1], 2), range(0, A5)),
                    (perm_qkv_items(0, 1), range(A6, 15)),
                    (outs(1, 0), range(A5 + 1, 16)))
            parts(0, (1, 4), (1, 5), (2, 4), (2, 5))
            wait("k1", "v1")
            segment((outs(1, 1), range(0, 3)), (outs(1, 2, 3, 4, 5), range(3, 18)),
                    (perm_qkv_items(1, 1), range(0, 16)),
                    (perm_qkv_items(2, 1), range(16, 34)))
            parts(1, *[(0, b) for b in range(NS)], *[(1, b) for b in range(KB)])
            wait("ca2", "sa2", "q2")
            nu = 4 * (2 * NS - KB)
            segment((mod_items(D + KP[2], 4), range(0, F0)),
                    (mod_items(KP[2], 4), range(F0, 2 * F0)),
                    (perm_qkv_items(0, 2), range(F1, nu - 2)),
                    (outs(2, 0, 1), range(2 * F0 + 1, nu)))
            parts(1, *[(1, b) for b in range(KB, NS)], *[(2, b) for b in range(NS)])

        with jax.named_scope("pass2"):
            wait("k2")
            segment((perm_qkv_items(1, 2), range(0, E0)), (outs(2, 2), range(4, 16)))
            halo("c", None, 1)
            parts(2, (0, 0), (0, 1))
            wait("v2")
            l0 = logit_items("c", True)
            segment((perm_qkv_items(2, 2), range(0, E0)),
                    (outs(2, 3), range(4, 22)),
                    at(8, halo, "a", "c", 1),
                    *logit_plan(l0, E1, 24, 0, LB))
            parts(2, (1, 0), (1, 1), (2, 0))
            halo("c", None, 2)
            halo("a", "c", 2)
            start("x2", "w1")
            wait("x6", "wo")
            plan = [(perm_wo_items(), range(0, WS)), *logit_plan(l0, 0, LW[0], LB),
                    (stats_items(NS, False), range(G0, G1)),
                    ]
            sparse = []
            for b in range(1, NS):
                plan += logit_plan(logit_items(sets[b], False), LW[b - 1] - (SLAG - 1) * (b < NS - 1), LW[b])
            for b in range(NS - 1):
                sparse.append((pv_items(sets[b]), range(*PW[b])))
            for b, u in zip(range(2, NS), (8, 32, 72, 112)):
                plan.append(at(u - 1, halo, sets[b], sets[b - 1], 1))
                plan.append(at(u + 15, halo, sets[b], sets[b - 1], 2))
            sparse += [(outs(2, 4, 5), range(O0, O1)), (ln1_out_items(NS, 0) + ln1_out_items(NS, 1), range(H0, H1))]
            segment(*plan, sparse=sparse)
            parts(2, (2, 1), (0, 2), (1, 2), (2, 2))
            for b in range(3, NS):
                parts(2, (0, b), (1, b), (2, b))
                wo_mm(sets[b - 3], (b - 3) * TM)
            wo_mm(sets[NS - 3], (NS - 3) * TM)
            wo_mm(sets[NS - 2], (NS - 2) * TM)
            finish()
            wait("x1", "x2")


        def half(X, Y, u0, sched, row_ln1, row_wo):
            place(sched, pv_items(Y), range(u0 + P0, u0 + 3 * UP - P1))
            for items, units in logit_plan(logit_items(X, False), u0 + 2 * UP + L0, u0 + 4 * UP - L1):
                place(sched, items, units)
            place(sched, ln1_items(row_ln1, Y), range(u0 + N0, u0 + N1))

            def run():
                halo(X, Y, 1)
                halo(X, Y, 2)
                for g in range(3):
                    qkv_part(X, g)
                wo_mm(Y, row_wo)
            return run

        def a_step(s, carry):
            for c in cp_quarter(s):
                c.start()
            cp_stage(s).wait()

            def refill():
                cp_stage(s + 1).start()
                pad = wst_v[0:16, pl.ds(pl.multiple_of(zrow(MT * 128), 128), 128)]
                st["pull"] = pltpu.bitcast(pad, F32)
            ra = pl.multiple_of(2 * s * TM, TM)
            nxt = pl.multiple_of(jnp.minimum(ra + 2 * TM, S - TM), TM)
            sched = {}
            place(sched, mod_items(mod_col(s), MT), range(0, MU))
            place(sched, [refill], [MU + 1])
            run_a = half("a", "b", 0, sched, ra + TM, ra - TM)
            run_b = half("b", "a", 4 * UP, sched, nxt, ra)
            begin(sched)
            run_a()
            run_b()
            finish()
            assert "pull" not in st
            for c in cp_quarter(s):
                c.wait()
            return carry

        with jax.named_scope("aloop"):
            jax.lax.fori_loop(NS // 2, NB // 2, a_step, 0)
            cp_stage(NB // 2).wait()

        with jax.named_scope("atail"):
            begin({})

            def post0(r):
                x1 = x1_rows(r, LG, 0, D)
                mu = jnp.mean(x1, axis=-1, keepdims=True)
                d = x1 - mu
                rs = jax.lax.rsqrt(jnp.mean(d * d, axis=-1, keepdims=True) + EPS)
                y = (d * rs).reshape(LG // 8, 8, D) * mod(4, 0, D)[None] + mod(3, 0, D)[None]
                h2_v[r // 2:(r + LG) // 2, :] = pltpu.bitcast(y.reshape(LG, D).astype(BF16), U32)
            post = [functools.partial(post0, r) for r in range(0, TMB, LG)]
            pv = pv_items("b")
            run_now(pv[:NC])
            segment((pv[NC:], range(0, UP - 2)), (post, range(TP0, 2 * UP - TE)))
            wo_mm("b", S - TM, 0, TM // 2)
            wo_mm("b", S - TM, TM // 2, TM)
            finish()
            wait("w1")

        def b_step(j, carry):
            row0 = pl.multiple_of(j * TMB, TMB)
            nxt = pl.multiple_of(jnp.minimum(row0 + TMB, S - TMB), TMB)
            if SKIP_FFN:
                obuf[pl.ds(row0, TMB), :] = x1_rows(row0, TMB, 0, D).astype(BF16)
                for q in range(NQ):
                    cp_out(j, q).start()
            else:
                ffn(j, row0, nxt)
            return carry

        with jax.named_scope("bloop"):
            jax.lax.fori_loop(0, NBB, b_step, 0)
        with jax.named_scope("tail"):
            for j in range(NBB):
                for q in range(NQ):
                    cp_out(j, q).wait()

    any_spec = pl.BlockSpec(memory_space=pl.ANY)
    qkv_set = [
        pltpu.VMEM((2 * NC, KV, 128), F32),
        pltpu.VMEM((NC, KV, 128), F32),
        pltpu.VMEM((WIN + 1, TM, 128), F32),
    ]
    scratch = [
        pltpu.VMEM((S, D), BF16),
        pltpu.VMEM((D, 3 * D), BF16),
        pltpu.VMEM((NC, KH // 2, 128), U32),
        pltpu.VMEM((D // 2, 3 * D), U32),
        pltpu.VMEM((D, D), BF16),
        pltpu.VMEM((NC, D // 32 * 17, 128), U32),
        pltpu.VMEM((D // 2, D), U32),
        pltpu.VMEM((D, F), BF16),
        pltpu.VMEM((D, F), BF16),
        pltpu.VMEM((F, D), BF16),
        pltpu.VMEM((D, 2 * D + 128), BF16),
        pltpu.VMEM((D, MT * 128 + 128), BF16),
        pltpu.VMEM((D, 128), F32),
        pltpu.VMEM((MT, NSUB, 8, 128), F32),
        pltpu.VMEM((8, 6 * D), F32),
        pltpu.VMEM((8, 2 * D), F32),
        pltpu.VMEM((TM // 2, D), U32),
        pltpu.VMEM((TM // 2, D), U32),
        pltpu.VMEM((NS, TM // 2, D), U32),
        pltpu.VMEM((NS, 3 * NC, TM, 128), F32),
        pltpu.VMEM((2, (NS + 1) * TM, 128), F32),
        *qkv_set, *qkv_set, *qkv_set,
        *[pltpu.VMEM((TM // 2, D), U32)] * 3,
        *[pltpu.VMEM((WIN, RG, 128), F32)] * 5,
        pltpu.VMEM((2, TM, 128), F32),
        pltpu.VMEM((2, TMB, 128), F32),
        pltpu.VMEM((S, D), F32),
        pltpu.VMEM((TMB, D), F32),
        pltpu.VMEM((TMB // 2, D), U32),
        pltpu.VMEM((TMB // 2, F), U32),
        pltpu.VMEM((S, D), BF16),
        pltpu.VMEM((1, D), BF16),
        pltpu.SMEM((1,), jnp.int32),
        pltpu.SemaphoreType.DMA((NDMA,)),
        pltpu.SemaphoreType.DMA((NBB * NQ,)),
    ]

    def call(A_x, A_wqkv, A_wo, B_w1, B_w3, B_w2, c, w_mod):
        return pl.pallas_call(
            kernel,
            out_shape=jax.ShapeDtypeStruct((1, S, D), BF16),
            in_specs=[any_spec] * 8,
            out_specs=any_spec,
            scratch_shapes=scratch,
            compiler_params=pltpu.CompilerParams(
                vmem_limit_bytes=120 * 1024 * 1024,
                disable_semaphore_checks=True, disable_bounds_checks=True),
        )(A_x, A_wqkv, A_wo, B_w1, B_w3, B_w2, c, w_mod)

    return call


@jax.jit
def pallas_adaLN_cond__sliding_local_dilated__glu_gated_swiglu__prompt_kernel(
    A_x: jax.Array,
    A_wqkv: jax.Array,
    A_wo: jax.Array,
    B_x: jax.Array,
    B_w1: jax.Array,
    B_w3: jax.Array,
    B_w2: jax.Array,
    c: jax.Array,
    w_mod: jax.Array,
):
    del B_x
    return _build()(A_x, A_wqkv, A_wo, B_w1, B_w3, B_w2, c, w_mod)
```

```python
import functools
import math

import jax
import jax.numpy as jnp
import jax.experimental.pallas as pl
import jax.experimental.pallas.tpu as pltpu

S = 2048
D = 1024
F = 3584
H = 32
DH = D // H
WIN = 8
DIL = 2
NC = D // 128
HALO = 16
EPS = 1e-5
NEG = -1000000000.0
SM_SCALE = DH ** -0.5
LOG2E = math.log2(math.e)

TM = 128
NB = S // TM
KV = HALO + TM
RG = 8
LG = 16
NS = 6
NDMA = 27
KP = (0, 256, 512, 1024)
KH = 512

F32 = jnp.float32
BF16 = jnp.bfloat16
U32 = jnp.uint32


def _tree(op, xs):
    xs = list(xs)
    while len(xs) > 1:
        xs = [op(xs[i], xs[i + 1]) if i + 1 < len(xs) else xs[i] for i in range(0, len(xs), 2)]
    return xs[0]


def _add(a, b):
    return a + b


def _fold(op, x):
    n, tail = x.shape[0], x.shape[1:]
    while n > 1:
        n //= 2
        x = x.reshape(n, 2, *tail)
        x = op(x[:, 0:1], x[:, 1:2])
    return x.reshape(tail)


def _lane_gather(x, idx):
    dn = jax.lax.GatherDimensionNumbers(
        offset_dims=(), collapsed_slice_dims=(1,), start_index_map=(1,),
        operand_batching_dims=(0,), start_indices_batching_dims=(0,))
    return jax.lax.gather(x, idx[..., None], dn, (1, 1), mode=jax.lax.GatherScatterMode.PROMISE_IN_BOUNDS)


def _build(TMB=256, FC=512, OCUT=(0, 512, 896, 1024),
           MT=7, NSUB=16, MLAG=8, PR=32, SPREAD=128, SLAG=5,
           P0=1, P1=16, L0=0, L1=0, N0=0, N1=30, PB1=5, TP0=10, TE=3,
           X0=2, X1=3, X2=6, X3=2, A2=7, A3=5, A4=10, A5=11, A6=6, KB=5, F0=10, F1=8,
           E0=14, E1=13, LB=5, WS=54, O0=0, O1=70, G0=134, G1=140, H0=150, H1=182,
           LW=(20, 48, 78, 108, 134, 184), PW=((21, 47), (49, 87), (87, 127), (115, 151), (140, 167)),
           MU=80, SKIP_FFN=False):
    NBB = S // TMB
    NQ = len(OCUT) - 1

    def kernel(x_hbm, wqkv_hbm, wo_hbm, w1_hbm, w3_hbm, w2_hbm, c_hbm, wmod_hbm,
               out_hbm,
               x_v, wqkv_v, wtmp, wqkv_p, wo_v, wo_tmp, wo_p, w1_v, w3_v, w2_v,
               wmod_v, wst_v, cb_v,
               h1a, h1b, h1s, part, stats, qka, va, pa, qkb, vb, pb_, qkc, vc, pc,
               oa, ob, oc, stat1, stat2,
               y_v, x1n, h2_v, act_v, obuf, modp_v, modb_v, mod_v, sl0, sl1, sl2, sl3, sl4, c_ref, zs, sem_w, sem_o):
        bufs = {"a": (h1a, qka, va, oa, pa), "b": (h1b, qkb, vb, ob, pb_),
                "c": (None, qkc, vc, oc, pc)}

        free_sl, held = [sl0, sl1, sl2, sl3, sl4], {}

        dmas = {}

        def add_dma(name, src, dst):
            dmas[name] = (src, dst, len(dmas))

        for name, (b0, b1) in (("x0", (0, 2)), ("x23", (2, 4)), ("x45", (4, 6)), ("x6", (6, 7)),
                               ("x1", (7, 9)), ("x2", (9, NB))):
            rows = pl.ds(b0 * TM, (b1 - b0) * TM)
            add_dma(name, x_hbm.at[0, rows, :], x_v.at[rows, :])
        for k in range(3):
            for j, name in enumerate(("sa", "ca")):
                cols = pl.ds(j * D + KP[k], KP[k + 1] - KP[k])
                add_dma(name + str(k), wmod_hbm.at[:, cols], wmod_v.at[:, cols])
            for g in range(3):
                rows, cols = pl.ds(KP[k], KP[k + 1] - KP[k]), pl.ds(g * D, D)
                add_dma("qkv"[g] + str(k), wqkv_hbm.at[rows, cols], wqkv_v.at[rows, cols])
        add_dma("c", c_hbm, c_ref)
        add_dma("wo", wo_hbm, wo_v)
        add_dma("w1", w1_hbm, w1_v)
        assert len(dmas) == NDMA - 3

        def cp_quarter(s):
            i = jnp.minimum(s - NS // 2, 3)
            cps = []
            for k, (src, dst) in enumerate(((w3_hbm, w3_v), (w2_hbm, w2_v))):
                n = src.shape[0] // 4
                rows = pl.ds(pl.multiple_of(i * n, n), n)
                cps.append(pltpu.make_async_copy(src.at[rows, :], dst.at[rows, :], sem_w.at[NDMA - 3 + k]))
            return cps

        def mod_col(s):
            c = jnp.minimum(2 * D + (s - NS // 2) * (MT * 128), 6 * D - MT * 128)
            return pl.multiple_of(c, 128)

        def cp_stage(s):
            return pltpu.make_async_copy(wmod_hbm.at[:, pl.ds(mod_col(s), MT * 128)],
                                         wst_v.at[:, pl.ds(0, MT * 128)], sem_w.at[NDMA - 1])

        def cp(name):
            src, dst, i = dmas[name]
            return pltpu.make_async_copy(src, dst, sem_w.at[i])

        def start(*names):
            for n in names:
                cp(n).start()

        def wait(*names):
            for n in names:
                cp(n).wait()

        def cp_out(j, q):
            rows, cols = pl.ds(j * TMB, TMB), pl.ds(OCUT[q], OCUT[q + 1] - OCUT[q])
            return pltpu.make_async_copy(obuf.at[rows, cols], out_hbm.at[0, rows, cols], sem_o.at[j * NQ + q])

        st = {"z": None, "never": None, "clock": 0, "sched": {}, "tok": None}

        have = set()

        def need(*keys):
            assert all(k in have for k in keys), keys

        def finish():
            assert not st["sched"], "items placed beyond the last unit"

        def begin(sched):
            finish()
            z = zs[0]
            st.update(z=(0, z, 2 * z), never=jnp.full((8, 128), z, jnp.int32) != 0, clock=0, sched=sched, tok=None)

        def gate(val, i, n):
            r = st["tok"]
            if r is None:
                return val
            row = (i * min(SPREAD, r.shape[0]) // n) // 8 * 8
            key = (row, val.dtype)
            if key not in st["rows"]:
                t = r[row:row + 8, 0:128]
                st["rows"][key] = t if val.dtype == F32 else pltpu.bitcast(t, val.dtype)
            return jax.lax.select(st["never"], st["rows"][key], val)

        def place(sched, items, units):
            units = list(units)
            for i, it in enumerate(items):
                sched.setdefault(units[(i * len(units)) // len(items)], []).append(it)

        def matmul(lhs_fn, w_fn, ks, cols, sink, gives=None):
            for n0 in cols:
                r = None
                for k in ks:
                    d = jnp.dot(lhs_fn(k), w_fn(k, n0), preferred_element_type=F32)
                    r = d if r is None else r + d
                    if k == ks[-1]:
                        sink(n0, r)
                    if n0 == cols[-1] and k == ks[-1]:
                        have.add(gives)
                    st["tok"], st["rows"] = r, {}
                    for fn in st["sched"].pop(st["clock"], []):
                        fn()
                    st["tok"] = None
                    st["clock"] += 1

        def lane_iota(rows):
            return jax.lax.broadcasted_iota(jnp.int32, (rows, 128), 1)

        def ld16(ref, r0, n, c0, c1):
            return pltpu.bitcast(ref[r0 // 2:(r0 + n) // 2, c0:c1], BF16)

        def silu_c():
            cf = c_ref[...].astype(F32)
            return (cf * jax.nn.sigmoid(cf)).astype(BF16)

        def mod_mxu(j, k):
            cs = slice(j * D + KP[k], j * D + KP[k + 1])
            lhs = jnp.broadcast_to(silu_c(), (16, D))
            mod_v[:, cs] = jnp.dot(lhs, wmod_v[:, cs], preferred_element_type=F32)[0:8] + float(j == 1)

        def mod(j, c0, c1):
            return (mod_v if j < 2 else modb_v)[:, j * D + c0:j * D + c1]

        def mod_items(col0, ntiles):
            rows = D // NSUB

            def col(t):
                c0 = col0 + t * 128
                return c0 if isinstance(c0, int) else pl.multiple_of(c0, 128)

            def part_sum(t, i):
                src, c0 = (wmod_v, col(t)) if isinstance(col0, int) else (wst_v, t * 128)
                w = src[i * rows:(i + 1) * rows, c0:c0 + 128].astype(F32)
                p = (w * cb_v[i * rows:(i + 1) * rows, :]).reshape(rows // 8, 8, 128)
                modp_v[t, i] = gate(_fold(_add, p), 1, 2)

            def total(t):
                r = gate(_fold(_add, modp_v[t, pl.ds(zrow(0), NSUB)]), 0, 1)
                one = jnp.where((col(t) // D) % 3 == 1, 1.0, 0.0).astype(F32)
                dst = mod_v if isinstance(col0, int) else modb_v
                dst[:, pl.ds(col(t), 128)] = jnp.broadcast_to(jnp.sum(r, axis=0, keepdims=True) + one, (8, 128))
            items = []
            for t in range(ntiles + 1):
                for i in range(NSUB):
                    if t < ntiles:
                        items.append(functools.partial(part_sum, t, i))
                    if t > 0 and i == (MLAG if t < ntiles else 0):
                        items.append(functools.partial(total, t - 1))
            return items

        def perm_mix(g, i, nrows, row0):
            n = nrows // 2
            l = jnp.concatenate([gate(lane_iota(8), h, n) for h in range(0, n, 8)], axis=0)
            w = pltpu.bitcast(wqkv_v[i * nrows:(i + 1) * nrows, g * D:(g + 1) * D], U32)
            vals = [w[:, c * 128:(c + 1) * 128] for c in range(NC)]
            for b in range(3):
                m = (l & (4 << b)) == 0
                for c in range(NC):
                    if c & (1 << b):
                        continue
                    lo, hi = vals[c], vals[c | (1 << b)]
                    vals[c] = jax.lax.select(m, lo, hi)
                    vals[c | (1 << b)] = jax.lax.select(m, hi, lo)
            wtmp[:, pl.ds(pl.multiple_of(zrow(i * n - row0), 8), n), :] = jnp.stack(vals)

        def perm_gather(g, k, j):
            have.add(("w", g, k, j))
            l = lane_iota(8)
            idx = ((((l >> 1) & 3) << 5) | ((((l >> 3) & 7) ^ j) << 2) | ((l >> 6) << 1) | (l & 1))
            n = (KP[k + 1] - KP[k]) // 2
            idx = jnp.concatenate([gate(idx, 0, 1)] * (n // 8), axis=0)
            wqkv_p[KP[k] // 2:KP[k + 1] // 2, g * D + j * 128: g * D + (j + 1) * 128] = _lane_gather(wtmp[j, 0:n], idx)

        def perm_qkv_items(g, k, nrows=PR):
            return ([functools.partial(perm_mix, g, i, nrows, KP[k] // 2) for i in range(KP[k] // nrows, KP[k + 1] // nrows)]
                    + [functools.partial(perm_gather, g, k, j) for j in range(NC)])

        def perm_wo_items():
            sub = jax.lax.broadcasted_iota(jnp.int32, (8, 128), 0)

            def spread(c, h):
                for r in range(h * 256, h * 256 + 256, 8):
                    wo_tmp[c, pl.ds(zrow(r + r // 16), 8), :] = gate(pltpu.bitcast(
                        wo_v[2 * r:2 * r + 16, c * 128:(c + 1) * 128], U32), r % 256, 256)

            def gather(c, h):
                for G in range(h * 32, h * 32 + 32):
                    j, e, ch = G >> 3, (G >> 2) & 1, G & 3
                    dd = (((2 * ch) ^ j) << 1) | e
                    ta = wo_tmp[c, pl.ds(ch * 136 + dd, 8, stride=17), :]
                    tb = wo_tmp[c, pl.ds(ch * 136 + (dd ^ 2), 8, stride=17), :]
                    wo_p[G * 8:G * 8 + 8, c * 128:(c + 1) * 128] = jax.lax.select(gate(sub, G % 32, 32) < 4, ta, tb)
            return [functools.partial(fn, c, h) for fn in (spread, gather) for c in range(NC) for h in range(2)]

        def zrow(row, k=1):
            return row if k == 0 else row + st["z"][k]

        def gate16(v, i, n):
            return jnp.concatenate([gate(v[q:q + 8], i, n) for q in range(0, LG, 8)], axis=0)

        def staged(stages, n, lag):
            items = []
            for t in range(n + lag * (len(stages) - 1)):
                for k in reversed(range(len(stages))):
                    if 0 <= t - k * lag < n:
                        items.append(functools.partial(stages[k], t - k * lag))
            return items

        def ln_stages(load, stat, dst, j_scale, j_shift, cols=(0, KH, D)):
            def chunks(x):
                return [x[:, c * 128:(c + 1) * 128] for c in range(NC)]

            def put(j, r, part, fn):
                m = jnp.sum(part, axis=-1, keepdims=True) * (1.0 / D)
                stat[j, pl.ds(pl.multiple_of(zrow(r), LG), LG), :] = jnp.broadcast_to(fn(m), (LG, 128))

            def s_mean(i):
                part = gate16(_tree(_add, chunks(load(i * LG, 0))), 1, 2)
                if "pull" in st:
                    part = jnp.concatenate([jax.lax.select(st["never"], st.pop("pull"), part[0:8]), part[8:]], axis=0)
                put(0, i * LG, part, lambda m: m)

            def s_var(i):
                r = i * LG
                d = load(r, 1) - jnp.concatenate([gate16(stat[0, r:r + LG, :], 0, 1)] * NC, axis=1)
                put(1, r, _tree(_add, chunks(d * d)), lambda m: jax.lax.rsqrt(m + EPS))

            def s_out(i):
                r = i * LG
                x = load(r, 2)
                for c0, c1 in zip(cols[:-1], cols[1:]):
                    nrep = (c1 - c0) // 128
                    mu = jnp.concatenate([stat[0, r:r + LG, :]] * nrep, axis=1)
                    rs = jnp.concatenate([gate16(stat[1, r:r + LG, :], c0 - cols[0], D)] * nrep, axis=1)
                    y = ((x[:, c0:c1] - mu) * rs).reshape(LG // 8, 8, c1 - c0)
                    y = y * mod(j_scale, c0, c1)[None] + mod(j_shift, c0, c1)[None]
                    dst[r // 2:(r + LG) // 2, c0:c1] = pltpu.bitcast(y.reshape(LG, c1 - c0).astype(BF16), U32)
            return s_mean, s_var, s_out

        def load_x(row0):
            return lambda r, k: x_v[pl.ds(pl.multiple_of(zrow(row0 + r, k), LG), LG), :].astype(F32)

        def ln1_items(row0, buf):
            return staged(ln_stages(load_x(row0), stat1, bufs[buf][0], 1, 0), TM // LG, 1)

        def ln1_start(b, k):
            return ln_stages(load_x(b * TM), stats.at[:, pl.ds(b * TM, TM), :], h1s.at[b] if b < NS else h1a,
                             1, 0, KP[k:k + 2] if b < NS else (k * KH, (k + 1) * KH))

        def stats_items(b, with_out):
            def one(i):
                r = b * TM + i * LG
                rows = pl.ds(r if isinstance(r, int) else pl.multiple_of(r, LG), LG)
                xf = x_v[rows, :].astype(F32)
                part = gate16(_tree(_add, [xf[:, c * 128:(c + 1) * 128] for c in range(NC)]), 0, 1)
                mu = jnp.sum(part, axis=-1, keepdims=True) * (1.0 / D)
                d = xf - mu
                rs = jax.lax.rsqrt(jnp.mean(d * d, axis=-1, keepdims=True) + EPS)
                stats[0, rows, :] = jnp.broadcast_to(mu, (LG, 128))
                stats[1, rows, :] = jnp.broadcast_to(rs, (LG, 128))
                if with_out:
                    have.add(("h", b, 0, i))
                    k1 = KP[1]
                    y = (d[:, :k1] * rs).reshape(LG // 8, 8, k1) * mod(1, 0, k1)[None] + mod(0, 0, k1)[None]
                    h1s[b, i * LG // 2:(i + 1) * LG // 2, 0:k1] = pltpu.bitcast(y.reshape(LG, k1).astype(BF16), U32)
            return [functools.partial(one, i) for i in range(TM // LG)]

        def ln1_out_items(b, k):
            def one(i):
                have.add(("h", b, k, i))
                ln1_start(b, k)[2](i)
            return [functools.partial(one, i) for i in range(TM // LG)]

        def x1_rows(row, n, c0, c1):
            xf = x_v[pl.ds(row, n), c0:c1].astype(F32).reshape(n // 8, 8, c1 - c0)
            y = y_v[pl.ds(row, n), c0:c1].reshape(n // 8, 8, c1 - c0)
            ga = jnp.concatenate([gate(mod(2, c, c + 128), c - c0, 2 * D) for c in range(c0, c1, 128)], axis=1)
            return (xf + ga[None] * y).reshape(n, c1 - c0)

        def post_items(row0):
            def load(r, k):
                if k:
                    return x1n[pl.ds(pl.multiple_of(zrow(r, k), LG), LG), :]
                x1 = x1_rows(row0 + r, LG, 0, D)
                x1n[r:r + LG, :] = x1
                return x1
            return staged(ln_stages(load, stat2, h2_v, 4, 3), TMB // LG, 1)

        def logit_items(buf, first):
            _, qk, _, _, pb = bufs[buf]
            even = (lane_iota(RG) & 1) == 0

            def s_logit(g):
                need(("q", buf), ("k", buf))
                have.add(("l", buf, g))
                sl = held[buf, g] = free_sl.pop(0)
                r = g * RG
                q = qk[0:NC, HALO + r:HALO + r + RG, :]
                dst = pl.ds(pl.multiple_of(zrow(0), RG), RG)
                for w in range(WIN):
                    k0 = zrow(HALO + r - DIL * w, int(w >= WIN // 2))
                    s = gate(_fold(_add, q * qk[NC:2 * NC, pl.ds(k0, RG), :]), w, WIN)
                    s = s + pltpu.roll(s, 64, 1)
                    s = s + jax.lax.select(even, pltpu.roll(s, 127, 1), pltpu.roll(s, 1, 1))
                    if first and r < DIL * w:
                        pos = r + jax.lax.broadcasted_iota(jnp.int32, (RG, 128), 0)
                        s = jnp.where(pos >= DIL * w, s, NEG * LOG2E)
                    sl[w, dst, :] = s

            def s_soft(g):
                assert ("p", buf, g) not in have
                sl = held.pop((buf, g))
                free_sl.append(sl)
                have.add(("p", buf, g))
                r = g * RG
                s = sl[...]
                e = jnp.exp2(s - gate(_fold(jnp.maximum, s), 0, 1)[None])
                pb[0:WIN, r:r + RG, :] = e
                den = _fold(_add, e)
                inv = pl.reciprocal(den, approx=True)
                pb[WIN, r:r + RG, :] = inv * (2.0 - den * inv)
            return [[functools.partial(fn, g) for g in range(TM // RG)] for fn in (s_logit, s_soft)]

        def logit_plan(items, u0, u1, g0=0, g1=TM // RG, s0=None, s1=None):
            lg, sm = items
            s0, s1 = g0 if s0 is None else s0, g1 if s1 is None else s1
            n = g1 - g0
            pos = [u0 + (i * (u1 - SLAG - u0)) // n for i in range(n)]
            plan = [([sm[g]], [pos[g - g0] + SLAG if g >= g0 else u0]) for g in range(s0, s1)]
            return plan + [([lg[g]], [pos[g - g0]]) for g in range(g0, g1)]

        def pv_items(buf):
            _, _, vp, o, pb = bufs[buf]
            hc = NC // 2

            def one(r, h):
                need(("v", buf), ("p", buf, r // RG), ("p", buf, r // RG + 1))
                if h:
                    have.difference_update({("p", buf, r // RG), ("p", buf, r // RG + 1)})
                    have.update({("o", buf, r // RG), ("o", buf, r // RG + 1)})
                vs = {d: vp[h * hc:(h + 1) * hc, pl.ds(zrow(HALO + r + d, int(d <= -RG)), RG), :]
                      for d in range(RG, -DIL * WIN, -DIL)}
                accs = []
                for q in (0, RG):
                    p = pb[:, pl.ds(pl.multiple_of(zrow(r + q, 1 + h), RG), RG), :]
                    accs.append(_tree(_add, [p[w:w + 1] * vs[q - DIL * w] for w in range(WIN)]) * p[WIN:])
                both = jnp.concatenate([
                    jnp.concatenate([gate(accs[i][c], 2 * c + i, NC) for c in range(hc)], axis=1)
                    for i in range(2)], axis=0)
                o[r // 2:r // 2 + RG, h * KH:(h + 1) * KH] = pltpu.bitcast(both.astype(BF16), U32)
            return [functools.partial(one, r, h) for r in range(0, TM, 2 * RG) for h in range(2)]

        def halo(buf, prev, part):
            c0 = NC if part == 1 else 0
            ref = bufs[buf][part]
            if prev is None:
                val = (jnp.zeros((NC, HALO, 128), F32) if part == 1
                       else jnp.broadcast_to(ref[:, HALO:HALO + 1, :], (NC, HALO, 128)))
            else:
                val = bufs[prev][part][c0:c0 + NC, TM:TM + HALO, :]
                if st["tok"] is not None:
                    val = jnp.stack([gate16(val[c], 1, 2) for c in range(NC)])
            ref[c0:c0 + NC, 0:HALO, :] = val

        def qkv_part(buf, g, sb=None, k=None):
            h1, qk, vp, _, _ = bufs[buf] if buf else (None,) * 5
            if sb is not None:
                h1 = h1s.at[sb]
                need(*[("h", sb, k, i) for i in range(TM // LG)])
            if k in (None, 2):
                for i in range(TM // RG):
                    if g < 2 and ("qk"[g], buf) in have:
                        need(("l", buf, i))
                    if g == 2 and ("v", buf) in have:
                        assert ("p", buf, i) not in have or ("new", buf) in have
                if g == 1:
                    have.difference_update({("l", buf, i) for i in range(TM // RG)})
                    have.add(("new", buf))
                have.discard(("qkv"[g], buf))

            def sink(n0, r):
                for cc in range(r.shape[1] // 128):
                    ch, rc = n0 // 128 + cc, r[:, cc * 128:(cc + 1) * 128]
                    if k in (1, 2):
                        rc = rc + part[sb, ch]
                    if k in (0, 1):
                        part[sb, ch] = rc
                        continue
                    dst, ci = (qk, ch) if ch < 2 * NC else (vp, ch - 2 * NC)
                    dst[ci, HALO:HALO + TM, :] = rc * (SM_SCALE * LOG2E) if ch < NC else rc

            kr = ((0, KH), (KH, D)) if k is None else (KP[k:k + 2],)
            nw = 128 * KH // (kr[0][1] - kr[0][0])

            def weights(kk, n0):
                if k is not None:
                    need(*[("w", g, k, j) for j in range(n0 % D // 128, (n0 % D + nw) // 128)])
                return ld16(wqkv_p, kk[0], kk[1] - kk[0], n0, n0 + nw)
            matmul(lambda kk: ld16(h1, 0, TM, kk[0], kk[1]), weights, kr, range(g * D, (g + 1) * D, nw), sink,
                   ("qkv"[g], buf) if k in (None, 2) else None)
            if g == 2:
                have.discard(("new", buf))

        def wo_mm(buf, row0, m0=0, m1=TM):
            o = bufs[buf][3]
            need(*[("o", buf, i) for i in range(m0 // RG, m1 // RG)])
            have.difference_update({("o", buf, i) for i in range(m0 // RG, m1 // RG)})

            def sink(n0, r):
                y_v[pl.ds(row0 + m0, m1 - m0), n0:n0 + 128] = r
            matmul(lambda k: ld16(o, m0, m1 - m0, k * KH, (k + 1) * KH),
                   lambda k, n0: ld16(wo_p, k * KH, KH, n0, n0 + 128),
                   (0, 1), range(0, D, 128), sink)

        UP = NC * (D // KH)

        def run_now(items):
            for fn in items:
                fn()

        def ffn(j, row0, nxt_row):
            h = ld16(h2_v, 0, TMB, 0, D)
            for f0 in range(0, F, FC):
                g = jnp.dot(h, w1_v[:, f0:f0 + FC], preferred_element_type=F32)
                u = jnp.dot(h, w3_v[:, f0:f0 + FC], preferred_element_type=F32)
                act_v[:, f0:f0 + FC] = pltpu.bitcast((g * jax.nn.sigmoid(g) * u).astype(BF16), U32)
            nk = F // KH
            sched = {}
            place(sched, post_items(nxt_row), range(0, NC * nk - PB1))
            begin(sched)

            def sink(n0, r):
                z = (mod(5, n0, n0 + 128)[None] * r.reshape(TMB // 8, 8, 128)).reshape(TMB, 128)
                obuf[pl.ds(row0, TMB), n0:n0 + 128] = (x1_rows(row0, TMB, n0, n0 + 128) + z).astype(BF16)
                if n0 + 128 in OCUT:
                    cp_out(j, OCUT.index(n0 + 128) - 1).start()
            matmul(lambda k: ld16(act_v, 0, TMB, k * KH, (k + 1) * KH),
                   lambda k, n0: w2_v[k * KH:(k + 1) * KH, n0:n0 + 128],
                   tuple(range(nk)), range(0, D, 128), sink)
            finish()

        def segment(*placements, sparse=()):
            sched = {}
            for items, units in placements:
                place(sched, items, units)
            busy = {u for u, its in sched.items() if any(getattr(i, "func", i).__name__ == "s_logit" for i in its)}
            for items, units in sparse:
                free = [u for u in units if u not in busy]
                free = free if len(free) >= len(items) else list(units)
                for i, it in enumerate(items):
                    u = free[(i * len(free)) // len(items)]
                    sched.setdefault(u, []).append(it)
                    busy.add(u)
            begin(sched)

        def parts(k, *gb):
            for g, b in gb:
                qkv_part(None if k < 2 else sets[b], g, b, k)

        def outs(k, *bs):
            return [it for b in bs for it in ln1_out_items(b, k)]

        def at(u, fn, *args):
            return [functools.partial(fn, *args)], [u]

        sets = "cabcab"
        with jax.named_scope("prologue"):
            zs[0] = 0
            wst_v[0:16, MT * 128:MT * 128 + 128] = jnp.zeros((16, 128), BF16)
            begin({})
            start("c", "x0", "ca0", "q0", "sa0", "x23", "k0", "v0", "x45", "ca1", "sa1", "q1", "k1", "v1",
                  "ca2", "sa2", "q2", "k2", "v2", "x6", "wo", "x1")
            cp_stage(NS // 2).start()
            wait("c")
            cb_v[...] = jnp.broadcast_to(silu_c().astype(F32), (128, D)).T
            wait("x0")

            def stats_body(b, carry):
                run_now(stats_items(b, False))
                return carry
            jax.lax.fori_loop(0, 2, stats_body, 0)
            wait("ca0")
            mod_mxu(1, 0)
            wait("q0")
            run_now(perm_qkv_items(0, 0))
            wait("sa0")
            mod_mxu(0, 0)
            run_now(outs(0, 0))

        with jax.named_scope("pass1"):
            segment((outs(0, 1), range(0, 4)))
            parts(0, (0, 0))
            wait("x23")
            segment((stats_items(2, True), range(0, X0)), (stats_items(3, True), range(X1, X2)))
            parts(0, (0, 1), (0, 2))
            wait("k0")
            segment((perm_qkv_items(1, 0), range(0, X3)))
            parts(0, (0, 3), (1, 0), (1, 1))
            wait("v0")
            segment((perm_qkv_items(2, 0), range(0, A2)))
            parts(0, (1, 2), (1, 3), (2, 0), (2, 1))
            wait("x45")
            segment((stats_items(4, True), range(0, A3)), (stats_items(5, True), range(A3, A4)))
            parts(0, (2, 2), (2, 3), (0, 4), (0, 5))
            wait("ca1", "sa1", "q1")
            segment((mod_items(D + KP[1], 2) + mod_items(KP[1], 2), range(0, A5)),
                    (perm_qkv_items(0, 1), range(A6, 15)),
                    (outs(1, 0), range(A5 + 1, 16)))
            parts(0, (1, 4), (1, 5), (2, 4), (2, 5))
            wait("k1", "v1")
            segment((outs(1, 1), range(0, 3)), (outs(1, 2, 3, 4, 5), range(3, 18)),
                    (perm_qkv_items(1, 1), range(0, 16)),
                    (perm_qkv_items(2, 1), range(16, 34)))
            parts(1, *[(0, b) for b in range(NS)], *[(1, b) for b in range(KB)])
            wait("ca2", "sa2", "q2")
            nu = 4 * (2 * NS - KB)
            segment((mod_items(D + KP[2], 4), range(0, F0)),
                    (mod_items(KP[2], 4), range(F0, 2 * F0)),
                    (perm_qkv_items(0, 2), range(F1, nu - 2)),
                    (outs(2, 0, 1), range(2 * F0 + 1, nu)))
            parts(1, *[(1, b) for b in range(KB, NS)], *[(2, b) for b in range(NS)])

        with jax.named_scope("pass2"):
            wait("k2")
            segment((perm_qkv_items(1, 2), range(0, E0)), (outs(2, 2), range(4, 16)))
            halo("c", None, 1)
            parts(2, (0, 0), (0, 1))
            wait("v2")
            l0 = logit_items("c", True)
            segment((perm_qkv_items(2, 2), range(0, E0)),
                    (outs(2, 3), range(4, 22)),
                    at(8, halo, "a", "c", 1),
                    *logit_plan(l0, E1, 24, 0, LB))
            parts(2, (1, 0), (1, 1), (2, 0))
            halo("c", None, 2)
            halo("a", "c", 2)
            start("x2", "w1")
            wait("x6", "wo")
            plan = [(perm_wo_items(), range(0, WS)), *logit_plan(l0, 0, LW[0], LB),
                    (stats_items(NS, False), range(G0, G1)),
                    ]
            sparse = []
            for b in range(1, NS):
                plan += logit_plan(logit_items(sets[b], False), LW[b - 1] - (SLAG - 1) * (b < NS - 1), LW[b])
            for b in range(NS - 1):
                sparse.append((pv_items(sets[b]), range(*PW[b])))
            for b, u in zip(range(2, NS), (8, 32, 72, 112)):
                plan.append(at(u - 1, halo, sets[b], sets[b - 1], 1))
                plan.append(at(u + 15, halo, sets[b], sets[b - 1], 2))
            sparse += [(outs(2, 4, 5), range(O0, O1)), (ln1_out_items(NS, 0) + ln1_out_items(NS, 1), range(H0, H1))]
            segment(*plan, sparse=sparse)
            parts(2, (2, 1), (0, 2), (1, 2), (2, 2))
            for b in range(3, NS):
                parts(2, (0, b), (1, b), (2, b))
                wo_mm(sets[b - 3], (b - 3) * TM)
            wo_mm(sets[NS - 3], (NS - 3) * TM)
            wo_mm(sets[NS - 2], (NS - 2) * TM)
            finish()
            wait("x1", "x2")


        def half(X, Y, u0, sched, row_ln1, row_wo):
            place(sched, pv_items(Y), range(u0 + P0, u0 + 3 * UP - P1))
            for items, units in logit_plan(logit_items(X, False), u0 + 2 * UP + L0, u0 + 4 * UP - L1):
                place(sched, items, units)
            place(sched, ln1_items(row_ln1, Y), range(u0 + N0, u0 + N1))

            def run():
                halo(X, Y, 1)
                halo(X, Y, 2)
                for g in range(3):
                    qkv_part(X, g)
                wo_mm(Y, row_wo)
            return run

        def a_step(s, carry):
            for c in cp_quarter(s):
                c.start()
            cp_stage(s).wait()

            def refill():
                cp_stage(s + 1).start()
                pad = wst_v[0:16, pl.ds(pl.multiple_of(zrow(MT * 128), 128), 128)]
                st["pull"] = pltpu.bitcast(pad, F32)
            ra = pl.multiple_of(2 * s * TM, TM)
            nxt = pl.multiple_of(jnp.minimum(ra + 2 * TM, S - TM), TM)
            sched = {}
            place(sched, mod_items(mod_col(s), MT), range(0, MU))
            place(sched, [refill], [MU + 1])
            run_a = half("a", "b", 0, sched, ra + TM, ra - TM)
            run_b = half("b", "a", 4 * UP, sched, nxt, ra)
            begin(sched)
            run_a()
            run_b()
            finish()
            assert "pull" not in st
            for c in cp_quarter(s):
                c.wait()
            return carry

        with jax.named_scope("aloop"):
            jax.lax.fori_loop(NS // 2, NB // 2, a_step, 0)
            cp_stage(NB // 2).wait()

        with jax.named_scope("atail"):
            begin({})

            def post0(r):
                x1 = x1_rows(r, LG, 0, D)
                mu = jnp.mean(x1, axis=-1, keepdims=True)
                d = x1 - mu
                rs = jax.lax.rsqrt(jnp.mean(d * d, axis=-1, keepdims=True) + EPS)
                y = (d * rs).reshape(LG // 8, 8, D) * mod(4, 0, D)[None] + mod(3, 0, D)[None]
                h2_v[r // 2:(r + LG) // 2, :] = pltpu.bitcast(y.reshape(LG, D).astype(BF16), U32)
            post = [functools.partial(post0, r) for r in range(0, TMB, LG)]
            pv = pv_items("b")
            run_now(pv[:NC])
            segment((pv[NC:], range(0, UP - 2)), (post, range(TP0, 2 * UP - TE)))
            wo_mm("b", S - TM, 0, TM // 2)
            wo_mm("b", S - TM, TM // 2, TM)
            finish()
            wait("w1")

        def b_step(j, carry):
            row0 = pl.multiple_of(j * TMB, TMB)
            nxt = pl.multiple_of(jnp.minimum(row0 + TMB, S - TMB), TMB)
            if SKIP_FFN:
                obuf[pl.ds(row0, TMB), :] = x1_rows(row0, TMB, 0, D).astype(BF16)
                for q in range(NQ):
                    cp_out(j, q).start()
            else:
                ffn(j, row0, nxt)
            return carry

        with jax.named_scope("bloop"):
            jax.lax.fori_loop(0, NBB, b_step, 0)
        with jax.named_scope("tail"):
            for j in range(NBB):
                for q in range(NQ):
                    cp_out(j, q).wait()

    any_spec = pl.BlockSpec(memory_space=pl.ANY)
    qkv_set = [
        pltpu.VMEM((2 * NC, KV + 8, 128), F32),
        pltpu.VMEM((NC, KV + 8, 128), F32),
        pltpu.VMEM((WIN + 1, TM, 128), F32),
    ]
    scratch = [
        pltpu.VMEM((S, D), BF16),
        pltpu.VMEM((D, 3 * D), BF16),
        pltpu.VMEM((NC, KH // 2, 128), U32),
        pltpu.VMEM((D // 2, 3 * D), U32),
        pltpu.VMEM((D, D), BF16),
        pltpu.VMEM((NC, D // 32 * 17, 128), U32),
        pltpu.VMEM((D // 2, D), U32),
        pltpu.VMEM((D, F), BF16),
        pltpu.VMEM((D, F), BF16),
        pltpu.VMEM((F, D), BF16),
        pltpu.VMEM((D, 2 * D + 128), BF16),
        pltpu.VMEM((D, MT * 128 + 256), BF16),
        pltpu.VMEM((D, 128), F32),
        pltpu.VMEM((TM // 2, D), U32),
        pltpu.VMEM((TM // 2, D), U32),
        pltpu.VMEM((NS, TM // 2, D), U32),
        pltpu.VMEM((NS, 3 * NC, TM, 128), F32),
        pltpu.VMEM((2, (NS + 1) * TM, 128), F32),
        *qkv_set, *qkv_set, *qkv_set,
        *[pltpu.VMEM((TM // 2, D), U32)] * 3,
        pltpu.VMEM((2, TM, 128), F32),
        pltpu.VMEM((2, TMB, 128), F32),
        pltpu.VMEM((S, D), F32),
        pltpu.VMEM((TMB, D), F32),
        pltpu.VMEM((TMB // 2, D), U32),
        pltpu.VMEM((TMB // 2, F), U32),
        pltpu.VMEM((S, D), BF16),
        pltpu.VMEM((MT, NSUB, 8, 128), F32),
        pltpu.VMEM((8, 6 * D), F32),
        pltpu.VMEM((8, 2 * D), F32),
        *[pltpu.VMEM((WIN, RG, 128), F32)] * 5,
        pltpu.VMEM((1, D), BF16),
        pltpu.SMEM((1,), jnp.int32),
        pltpu.SemaphoreType.DMA((NDMA,)),
        pltpu.SemaphoreType.DMA((NBB * NQ,)),
    ]

    def call(A_x, A_wqkv, A_wo, B_w1, B_w3, B_w2, c, w_mod):
        return pl.pallas_call(
            kernel,
            out_shape=jax.ShapeDtypeStruct((1, S, D), BF16),
            in_specs=[any_spec] * 8,
            out_specs=any_spec,
            scratch_shapes=scratch,
            compiler_params=pltpu.CompilerParams(
                vmem_limit_bytes=120 * 1024 * 1024,
                disable_semaphore_checks=True, disable_bounds_checks=True),
        )(A_x, A_wqkv, A_wo, B_w1, B_w3, B_w2, c, w_mod)

    return call


@jax.jit
def pallas_adaLN_cond__sliding_local_dilated__glu_gated_swiglu__prompt_kernel(
    A_x: jax.Array,
    A_wqkv: jax.Array,
    A_wo: jax.Array,
    B_x: jax.Array,
    B_w1: jax.Array,
    B_w3: jax.Array,
    B_w2: jax.Array,
    c: jax.Array,
    w_mod: jax.Array,
):
    del B_x
    return _build()(A_x, A_wqkv, A_wo, B_w1, B_w3, B_w2, c, w_mod)
```
